```python
import jax
import jax.numpy as jnp

def _softmax(x, axis=-1):
    return jax.nn.softmax(x, axis=axis)

def _gelu(x):
    return jax.nn.gelu(x, approximate=True)

def _silu(x):
    return jax.nn.silu(x)

def _sigmoid(x):
    return jax.nn.sigmoid(x)

def _layernorm(x, axis=-1, eps=1e-05):
    m = jnp.mean(x, axis=axis, keepdims=True)
    v = jnp.var(x, axis=axis, keepdims=True)
    return (x - m) / jnp.sqrt(v + eps)

def _scatter_add(tgt, idx, src, axis=0):
    return tgt.at[idx].add(src)

def _segment_sum(src, seg, n):
    return jax.ops.segment_sum(src, seg, n)

class _Rng:

    def __init__(self, key):
        self._k = key

    def _next(self):
        self._k, sub = jax.random.split(self._k)
        return sub

    def normal(self, shape):
        return jax.random.normal(self._next(), shape, dtype=jnp.bfloat16)

    def randint(self, lo, hi, shape):
        return jax.random.randint(self._next(), shape, lo, hi, dtype=jnp.int32)

    def uniform(self, shape, lo=0.0, hi=1.0):
        return jax.random.uniform(self._next(), shape, jnp.bfloat16, lo, hi)

    def permutation(self, n):
        return jax.random.permutation(self._next(), n)
kernel_name = 'adaLN_cond__ssm_conv_h3__mixer_gmlp__prompt'

def setup_inputs():
    _rng = _Rng(jax.random.key(int.from_bytes(__import__("os").urandom(4), "little")))
    _w = lambda a: (lambda t: t.astype(jnp.bfloat16) if jnp.issubdtype(t.dtype, jnp.floating) else t)(jnp.asarray(a))

    def _A_setup():
        B, S, D = (1, 2048, 640)
        ks = 4
        return {'q': _w((lambda *s: _rng.normal(s) * 0.05)(B, S, D)), 'k': _w((lambda *s: _rng.normal(s) * 0.05)(B, S, D)), 'v': _w((lambda *s: _rng.normal(s) * 0.05)(B, S, D)), 'shift_k': _w((lambda *s: _rng.normal(s) * 0.05)(D, ks) * 0.5), 'ssm_k': _w((lambda *s: _rng.normal(s) * 0.05)(D, S) * (1.0 / S ** 0.5)), 'ssm_D': _w((lambda *s: _rng.normal(s) * 0.05)(D))}
    _A_in = _A_setup()

    def _B_setup():
        B, S, D, F = (1, 2048, 640, 1728)
        Fh = F // 2
        return {'x': _w((lambda *s: _rng.normal(s) * 0.05)(B, S, D)), 'w_in': _w((lambda *s: _rng.normal(s) * 0.05)(D, 2 * Fh)), 'w_sp': _w(0.01 * (lambda *s: _rng.normal(s) * 0.05)(S, S)), 'b_sp': _w(1.0 + 0.01 * (lambda *s: _rng.normal(s) * 0.05)(S)), 'w_out': _w((lambda *s: _rng.normal(s) * 0.05)(Fh, D))}
    _B_in = _B_setup()
    return {'A_q': _A_in['q'], 'A_k': _A_in['k'], 'A_v': _A_in['v'], 'A_shift_k': _A_in['shift_k'], 'A_ssm_k': _A_in['ssm_k'], 'A_ssm_D': _A_in['ssm_D'], 'B_x': _B_in['x'], 'B_w_in': _B_in['w_in'], 'B_w_sp': _B_in['w_sp'], 'B_b_sp': _B_in['b_sp'], 'B_w_out': _B_in['w_out'], 'c': _w((lambda *s: _rng.normal(s) * 0.05)(1, 640)), 'w_mod': _w((lambda *s: _rng.normal(s) * 0.05)(640, 6 * 640) * 640 ** (-0.5))}

def reference(A_q, A_k, A_v, A_shift_k, A_ssm_k, A_ssm_D, B_x, B_w_in, B_w_sp, B_b_sp, B_w_out, c, w_mod):

    def _A_ref(q, k, v, shift_k, ssm_k, ssm_D):
        B, S, D = q.shape
        ks = shift_k.shape[-1]
        k_pad = jnp.pad(k, ((0, 0), (ks - 1, 0), (0, 0)))
        k_shift = jnp.zeros_like(k)
        for t in range(ks):
            k_shift = k_shift + k_pad[:, t:t + S, :] * shift_k[:, ks - 1 - t][None, None, :]
        kv = k_shift * v
        L = 2 * S
        kv_pad = jnp.pad(kv, ((0, 0), (0, S), (0, 0)))
        kf_pad = jnp.pad(ssm_k, ((0, 0), (0, S)))
        kv_f = (lambda x, axes=(-2, -1): jnp.fft.rfft2(x.astype(jnp.float32), axes=axes))(kv_pad[:, None, :, :], axes=(1, 2))
        kf_f = (lambda x, axes=(-2, -1): jnp.fft.rfft2(x.astype(jnp.float32), axes=axes))(kf_pad[:, None, :], axes=(1, 2))
        kf_f = (lambda x, *d: x.transpose(*d))(kf_f, 1, 2, 0)
        y_f = kv_f * kf_f[None, :, :, :]
        y = (lambda x, s, axes=(-2, -1): jnp.fft.irfft2(x, s=s, axes=axes).astype(jnp.bfloat16))(y_f, (1, L), axes=(1, 2))[:, 0, :S, :]
        y = y + kv * ssm_D[None, None, :]
        return q * y

    def _B_ref(x, w_in, w_sp, b_sp, w_out):
        B, S, D = x.shape
        F = w_in.shape[-1]
        Fh = F // 2
        z = _gelu(jnp.einsum('bsd,df->bsf', x, w_in))
        z1 = z[..., :Fh].copy()
        z2 = _layernorm(z[..., Fh:], axis=-1)
        g = jnp.einsum('ts,bsf->btf', w_sp, z2) + b_sp[None, :, None]
        return jnp.einsum('bsf,fd->bsd', z1 * g, w_out)
    x = A_q
    mod = (_silu(c) @ w_mod).reshape(c.shape[0], 6, 1, -1)
    sa, ca, ga, sb, cb, gb = (mod[:, 0].copy(), mod[:, 1].copy(), mod[:, 2].copy(), mod[:, 3].copy(), mod[:, 4].copy(), mod[:, 5].copy())
    h = _layernorm(x, axis=-1) * (1 + ca) + sa
    x = x + ga * _A_ref(h, A_k, A_v, A_shift_k, A_ssm_k, A_ssm_D)
    h = _layernorm(x, axis=-1) * (1 + cb) + sb
    x = x + gb * _B_ref(h, B_w_in, B_w_sp, B_b_sp, B_w_out)
    return x
```

```python
import numpy as np

import jax
import jax.numpy as jnp
from jax import lax
import jax.experimental.pallas as pl
import jax.experimental.pallas.tpu as pltpu

S = 2048
D = 640
FH = 864
KS = 4
L = 128
NCT = D // L
C = 512
NCH = S // C
NPOS = 16
TS = 512
TT = 512
EPS = 1e-5
GELU_C0 = float(np.sqrt(2.0 / np.pi))
GELU_C1 = GELU_C0 * 0.044715

F32 = jnp.float32
BF16 = jnp.bfloat16
U32 = jnp.uint32
NT_DIMS = (((1,), (1,)), ((), ()))


def _dft_matrices():
    n_fft = 2 * C
    k1 = np.concatenate([np.arange(0, 128, 2), np.arange(1, 128, 2)]).reshape(NPOS, 8)
    fwd = np.zeros((4, 2 * L, L), np.float64)
    inv = np.zeros((4, L, 2 * L), np.float64)
    col_n1 = (np.arange(L) // 2) + 64 * (np.arange(L) % 2)
    for p in range(4):
        n = 4 * np.arange(L) + p
        phase = ((2 * k1[:, :, None] + 1) * n[None, None, :]) % (2 * n_fft)
        theta = np.pi * phase / n_fft
        f = np.stack([np.cos(theta), -np.sin(theta)], axis=1).reshape(2 * L, L)
        fwd[p] = f[:, col_n1]
        inv[p] = f.T * (2.0 / n_fft)
    return fwd.astype(np.float32).astype(BF16), inv.astype(np.float32).astype(BF16)


_FWD, _INV = _dft_matrices()


def _lo(w):
    return pltpu.unpack_elementwise(w, index=0, packed_dtype=BF16, unpacked_dtype=F32)


def _hi(w):
    return pltpu.unpack_elementwise(w, index=1, packed_dtype=BF16, unpacked_dtype=F32)


def _pack(a, b):
    return pltpu.pack_elementwise([a, b], packed_dtype=BF16)


def _radix4(e, inverse):
    (r0, i0), (r1, i1), (r2, i2), (r3, i3) = e
    sr, si, dr, di = r0 + r2, i0 + i2, r0 - r2, i0 - i2
    tr, ti, ur, ui = r1 + r3, i1 + i3, r1 - r3, i1 - i3
    a = (dr + ui, di - ur)
    b = (dr - ui, di + ur)
    if inverse:
        a, b = b, a
    return [(sr + tr, si + ti), a, (sr - tr, si - ti), b]


def _gelu2(x):
    t = jnp.tanh(x * (x * x * GELU_C1 + GELU_C0))
    return x * t + x


def _kernel(q_hbm, k_hbm, v_hbm, shift_hbm, ssm_hbm, ssmd_hbm, wi_hbm, wsp_hbm, bsp_hbm,
            wo_hbm, c_hbm, wmod_hbm, fwd_hbm, inv_hbm, out_hbm,
            q_v, k_v, v_v, shift_v, ssm_v, ssmd_v, wi_v, wsp_v, bsp_v, wo_v, c_v, wmod_v,
            fwd_v, inv_v, out_v,
            taps_s, ssmd_s, bsp_s, mod_s, phase_s, khat0, khat1, khat2, khat3,
            uhat0, uhat1, uhat2, uhat3, g_s, y_s, x1_s, h_s, z1_s, z2_s, a_s, wot_s, p_s,
            sems, out_sems):
    khat = (khat0, khat1, khat2, khat3)
    uhat = (uhat0, uhat1, uhat2, uhat3)

    copies = {}

    def queue(name, src, dst):
        copies[name] = pltpu.make_async_copy(src, dst, sems.at[len(copies)])
        copies[name].start()

    def rows(ref, i, n):
        return ref.at[pl.ds(i * n, n), :]

    queue("ssm0", rows(ssm_hbm, 0, L), rows(ssm_v, 0, L))
    queue("fwd", fwd_hbm, fwd_v)
    queue("ssmd", ssmd_hbm, ssmd_v)
    queue("shift", shift_hbm, shift_v)
    queue("c", c_hbm, c_v)
    queue("bsp", bsp_hbm, bsp_v)
    for i in range(1, NCT):
        queue(f"ssm{i}", rows(ssm_hbm, i, L), rows(ssm_v, i, L))
    k_v[0:16, :] = jnp.zeros((16, D), BF16)
    for j in range(NCH):
        queue(f"k{j}", rows(k_hbm, j, C), k_v.at[pl.ds(16 + j * C, C), :])
        queue(f"v{j}", rows(v_hbm, j, C), rows(v_v, j, C))
        if j == 0:
            queue("inv", inv_hbm, inv_v)
    queue("wmod", wmod_hbm.at[:, 0:5 * D], wmod_v.at[:, 0:5 * D])
    queue("q0", rows(q_hbm, 0, TS), rows(q_v, 0, TS))
    queue("wi", wi_hbm, wi_v)
    for i in range(1, S // TS):
        queue(f"q{i}", rows(q_hbm, i, TS), rows(q_v, i, TS))
    queue("wgb", wmod_hbm.at[:, 5 * D:6 * D], wmod_v.at[:, 5 * D:6 * D])
    queue("wo", wo_hbm, wo_v)
    for i in range(S // TT):
        queue(f"wsp{i}", rows(wsp_hbm, i, TT), rows(wsp_v, i, TT))

    def wait(name):
        copies[name].wait()

    def lanes(c):
        return pl.ds(pl.multiple_of(c * L, L), L)

    def forward_dft(even, odd):
        phase_s[0] = _pack(even[:L], even[L:])
        phase_s[1] = _pack(odd[:L], odd[L:])
        out = []
        for p in range(4):
            words = phase_s[p % 2, pl.ds(p // 2, L // 2, stride=2), :]
            out.append(jnp.dot(fwd_v[p], pltpu.bitcast(words, BF16), preferred_element_type=F32))
        return out

    def group(x, g):
        return x[16 * g:16 * g + 8], x[16 * g + 8:16 * g + 16]

    def load_group(ref, c, k2, g):
        return ref[c, k2, 16 * g:16 * g + 8, :], ref[c, k2, 16 * g + 8:16 * g + 16, :]

    def store_group(ref, c, k2, g, val):
        ref[c, k2, 16 * g:16 * g + 8, :] = val[0]
        ref[c, k2, 16 * g + 8:16 * g + 16, :] = val[1]

    wait("fwd")
    wait("ssmd")
    wait("shift")
    dvec = ssmd_v[...].astype(F32)
    for i in range(NCT):
        ssmd_s[i] = jnp.broadcast_to(dvec[i:i + 1], (8, L))
    taps = shift_v[...].astype(F32)
    for t in range(KS):
        taps_s[t] = jnp.broadcast_to(taps[t:t + 1], (8, D))

    def filter_spectrum(c, carry):
        for i in range(NCT):
            @pl.when(c == i)
            def _():
                wait(f"ssm{i}")
        prev = None
        for m in range(NCH):
            tile = ssm_v[pl.ds(pl.multiple_of(c * L, L), L), m * C:(m + 1) * C]
            words = pltpu.bitcast(tile.T, U32)
            e = forward_dft(_lo(words), _hi(words))
            cur = []
            for g in range(NPOS):
                pairs = [group(e[p], g) for p in range(4)]
                kk = _radix4(pairs, False)
                cur.append(kk)
                for k2 in range(4):
                    re, im = kk[k2]
                    if m == 0:
                        val = (re + ssmd_s[c], im)
                    elif g < NPOS // 2:
                        val = (re - prev[g][k2][1], im + prev[g][k2][0])
                    else:
                        val = (re + prev[g][k2][1], im - prev[g][k2][0])
                    store_group(khat[m], c, k2, g, val)
            prev = cur
        return carry

    lax.fori_loop(0, NCT, filter_spectrum, 0)

    def signal_spectrum(j, c):
        kw = pltpu.bitcast(k_v[j * C:(j + 1) * C + 16, lanes(c)], U32)
        vw = pltpu.bitcast(v_v[j * C:(j + 1) * C, lanes(c)], U32)
        w0, w1, w2, w3 = [jnp.tile(taps_s[t, :, lanes(c)], (C // 16, 1)) for t in range(KS)]
        cur = kw[8:]
        back1 = pltpu.roll(kw, 1, 0)[8:]
        back2 = pltpu.roll(kw, 2, 0)[8:]
        e0, o0, e1, o1, o2 = _lo(cur), _hi(cur), _lo(back1), _hi(back1), _hi(back2)
        even = (w0 * e0 + w1 * o1 + w2 * e1 + w3 * o2) * _lo(vw)
        odd = (w0 * o0 + w1 * e0 + w2 * o1 + w3 * e1) * _hi(vw)
        e = forward_dft(even, odd)
        for g in range(NPOS):
            uu = _radix4([group(e[p], g) for p in range(4)], False)
            for k2 in range(4):
                store_group(uhat[j], c, k2, g, uu[k2])

    def chunk_product(i, c):
        for g in range(NPOS):
            ys = []
            for k2 in range(4):
                yr = yi = None
                for j in range(i + 1):
                    kr, ki = load_group(khat[i - j], c, k2, g)
                    ur, ui = load_group(uhat[j], c, k2, g)
                    pr, pi = kr * ur - ki * ui, kr * ui + ki * ur
                    yr, yi = (pr, pi) if yr is None else (yr + pr, yi + pi)
                ys.append((yr, yi))
            gg = _radix4(ys, True)
            for p in range(4):
                g_s[i % 2, c, p, 16 * g:16 * g + 16, :] = (
                    jnp.concatenate(gg[p], axis=0).astype(BF16))

    def inverse_dft(i, c):
        y = [jnp.dot(inv_v[p], g_s[i % 2, c, p], preferred_element_type=F32) for p in range(4)]
        base = i * (C // 2)
        y_s[c, pl.ds(base, L, stride=2), :] = _pack(y[0], y[1])
        y_s[c, pl.ds(base + 1, L, stride=2), :] = _pack(y[2], y[3])

    for step in range(NCH + 2):
        if step < NCH:
            wait(f"k{step}")
            wait(f"v{step}")
        if step == 2:
            wait("inv")

        def conv_step(c, carry, step=step):
            if 0 <= step - 2 < NCH:
                inverse_dft(step - 2, c)
            if step < NCH:
                signal_spectrum(step, c)
            if 0 <= step - 1 < NCH:
                chunk_product(step - 1, c)
            return carry

        lax.fori_loop(0, NCT, conv_step, 0)

    wait("c")
    cv = c_v[...].astype(F32)
    act = jnp.broadcast_to(cv * jax.nn.sigmoid(cv), (16, D)).astype(BF16)

    def modulation(i):
        return jnp.dot(act, wmod_v[:, i * D:(i + 1) * D], preferred_element_type=F32)[:8]

    wait("wmod")
    sa, ca, ga, sb, cb = [modulation(i) for i in range(5)]
    mod_s[0] = (1.0 + ca) * ga
    mod_s[1] = sa * ga
    mod_s[2] = 1.0 + cb
    mod_s[3] = sb

    RB = 16

    def layernorm_rows(x):
        d = x - jnp.sum(x, axis=-1, keepdims=True) * (1.0 / D)
        var = jnp.sum(d * d, axis=-1, keepdims=True) * (1.0 / D)
        return d * lax.rsqrt(var + EPS)

    def residual_stage(i):
        ga_scale, ga_shift, b_scale, b_shift = [jnp.tile(mod_s[n], (RB // 8, 1)) for n in range(4)]
        for r in range(TS // RB):
            row = pl.multiple_of(i * TS + r * RB, RB)
            wrow = pl.multiple_of(i * (TS // 2) + r * (RB // 2), RB // 2)
            x = q_v[pl.ds(row, RB), :].astype(F32)
            y = jnp.concatenate(
                [pltpu.bitcast(y_s[c, pl.ds(wrow, RB // 2), :], BF16) for c in range(NCT)],
                axis=1).astype(F32)
            x1 = x + (layernorm_rows(x) * ga_scale + ga_shift) * y
            x1_s[pl.ds(row, RB), :] = x1.astype(BF16)
            h_s[i % 2, r * RB:(r + 1) * RB, :] = (
                layernorm_rows(x1) * b_scale + b_shift).astype(BF16)

    def hidden_stage(i):
        h = h_s[i % 2]
        cols = pl.ds(pl.multiple_of(i * TS, TS), TS)
        a2 = _gelu2(lax.dot_general(wi_v[FH:2 * FH, :], h, NT_DIMS, preferred_element_type=F32))
        d = a2 - jnp.sum(a2, axis=0, keepdims=True) * (1.0 / FH)
        var = jnp.sum(d * d, axis=0, keepdims=True) * (1.0 / FH)
        z2_s[:, cols] = (d * lax.rsqrt(var + 4.0 * EPS)).astype(BF16)
        a1 = _gelu2(lax.dot_general(wi_v[0:FH, :], h, NT_DIMS, preferred_element_type=F32))
        z1_s[:, cols] = a1.astype(BF16)

    wait("q0")
    residual_stage(0)
    wait("wi")
    for i in range(1, S // TS):
        wait(f"q{i}")

    def hidden_step(i, carry):
        hidden_stage(i)
        residual_stage(i + 1)
        return carry

    lax.fori_loop(0, S // TS - 1, hidden_step, 0)
    hidden_stage(S // TS - 1)

    wait("wgb")
    wait("bsp")
    wait("wo")
    mod_s[4] = 0.5 * modulation(5)
    bvec = bsp_v[...].astype(F32)
    for i in range(S // L):
        bsp_s[:, i * L:(i + 1) * L] = jnp.broadcast_to(bvec[i:i + 1], (8, L))
    wot_s[...] = wo_v[...].T

    def out_copy(i):
        row = pl.multiple_of(i * TT, TT)
        return pltpu.make_async_copy(
            out_v.at[pl.ds(row, TT), :], out_hbm.at[pl.ds(row, TT), :], out_sems.at[i])

    def mix_step(i, carry):
        for n in range(S // TT):
            @pl.when(i == n)
            def _():
                wait(f"wsp{n}")
        row = pl.multiple_of(i * TT, TT)
        g = lax.dot_general(z2_s[...], wsp_v[pl.ds(row, TT), :], NT_DIMS,
                            preferred_element_type=F32)
        g = g + bsp_s[0:1, pl.ds(row, TT)]
        p_s[...] = (z1_s[:, pl.ds(row, TT)].astype(F32) * g).astype(BF16)
        o = jnp.dot(wot_s[...], p_s[...], preferred_element_type=F32).T
        res = x1_s[pl.ds(row, TT), :].astype(F32) + mod_s[4, 0:1, :] * o
        out_v[pl.ds(row, TT), :] = res.astype(BF16)
        out_copy(i).start()
        return carry

    lax.fori_loop(0, S // TT, mix_step, 0)
    for i in range(S // TT):
        out_copy(i).wait()


@jax.jit
def pallas_adaLN_cond__ssm_conv_h3__mixer_gmlp__prompt_kernel(
    A_q: jax.Array,
    A_k: jax.Array,
    A_v: jax.Array,
    A_shift_k: jax.Array,
    A_ssm_k: jax.Array,
    A_ssm_D: jax.Array,
    B_x: jax.Array,
    B_w_in: jax.Array,
    B_w_sp: jax.Array,
    B_b_sp: jax.Array,
    B_w_out: jax.Array,
    c: jax.Array,
    w_mod: jax.Array,
):
    del B_x
    operands = (
        A_q.reshape(S, D), A_k.reshape(S, D), A_v.reshape(S, D), A_shift_k.T, A_ssm_k,
        A_ssm_D.reshape(NCT, L), B_w_in.T, B_w_sp, B_b_sp.reshape(S // L, L), B_w_out, c, w_mod,
        _FWD, _INV,
    )
    spectrum = pltpu.VMEM((NCT, 4, 2 * L, L), F32)
    scratch = [
        pltpu.VMEM((S, D), BF16),
        pltpu.VMEM((16 + S, D), BF16),
        pltpu.VMEM((S, D), BF16),
        pltpu.VMEM((KS, D), BF16),
        pltpu.VMEM((D, S), BF16),
        pltpu.VMEM((NCT, L), BF16),
        pltpu.VMEM((2 * FH, D), BF16),
        pltpu.VMEM((S, S), BF16),
        pltpu.VMEM((S // L, L), BF16),
        pltpu.VMEM((FH, D), BF16),
        pltpu.VMEM((1, D), BF16),
        pltpu.VMEM((D, 6 * D), BF16),
        pltpu.VMEM(_FWD.shape, BF16),
        pltpu.VMEM(_INV.shape, BF16),
        pltpu.VMEM((S, D), BF16),
        pltpu.VMEM((KS, 8, D), F32),
        pltpu.VMEM((NCT, 8, L), F32),
        pltpu.VMEM((8, S), F32),
        pltpu.VMEM((5, 8, D), F32),
        pltpu.VMEM((2, L, L), U32),
        *([spectrum] * (2 * NCH)),
        pltpu.VMEM((2, NCT, 4, 2 * L, L), BF16),
        pltpu.VMEM((NCT, S // 2, L), U32),
        pltpu.VMEM((S, D), BF16),
        pltpu.VMEM((2, TS, D), BF16),
        pltpu.VMEM((FH, S), BF16),
        pltpu.VMEM((FH, S), BF16),
        pltpu.VMEM((FH, TS), F32),
        pltpu.VMEM((D, FH), BF16),
        pltpu.VMEM((FH, TT), BF16),
        pltpu.SemaphoreType.DMA((40,)),
        pltpu.SemaphoreType.DMA((S // TT,)),
    ]
    out = pl.pallas_call(
        _kernel,
        out_shape=jax.ShapeDtypeStruct((S, D), BF16),
        in_specs=[pl.BlockSpec(memory_space=pltpu.HBM)] * len(operands),
        out_specs=pl.BlockSpec(memory_space=pltpu.HBM),
        scratch_shapes=scratch,
        compiler_params=pltpu.CompilerParams(vmem_limit_bytes=110 * 1024 * 1024),
    )(*operands)
    return out.reshape(1, S, D)
```

```python
import contextlib
import itertools

import numpy as np

import jax
import jax.numpy as jnp
from jax import lax
import jax.experimental.pallas as pl
import jax.experimental.pallas.tpu as pltpu

S = 2048
D = 640
FH = 864
FQ = FH // 2
KS = 4
L = 128
NCT = D // L
C = 512
NCH = S // C
NPOS = 16
TS = 512
TOKROW = 0
MB = 144
TT = 512
TH = TT // 2
TO = 256
SUMMED = (0, 2, 3, 5, 6)
EPS = 1e-5
GELU_C0 = float(np.sqrt(2.0 / np.pi))
GELU_C1 = GELU_C0 * 0.044715

F32 = jnp.float32
BF16 = jnp.bfloat16
U32 = jnp.uint32
NT_DIMS = (((1,), (1,)), ((), ()))


TRACE_SCOPES = [False]


def _scope(name):
    return jax.named_scope("ph_" + name) if TRACE_SCOPES[0] else contextlib.nullcontext()


def _row_pairs(x):
    bits = x.astype(np.float32).astype(BF16).view(np.uint16).astype(np.uint32)
    return bits[..., 0::2, :] | (bits[..., 1::2, :] << 16)


def _dft_matrices():
    n_fft = 2 * C
    k1 = np.concatenate([np.arange(0, 128, 2), np.arange(1, 128, 2)]).reshape(NPOS, 8)
    fwd = np.zeros((4, 2 * L, L), np.float64)
    inv = np.zeros((4, L, 2 * L), np.float64)
    col_n1 = (np.arange(L) // 2) + 64 * (np.arange(L) % 2)
    for p in range(4):
        n = 4 * np.arange(L) + p
        phase = ((2 * k1[:, :, None] + 1) * n[None, None, :]) % (2 * n_fft)
        theta = np.pi * phase / n_fft
        f = np.stack([np.cos(theta), -np.sin(theta)], axis=1).reshape(2 * L, L)
        fwd[p] = f[:, col_n1]
        inv[p] = np.stack([np.cos(theta), -np.sin(theta)], axis=2).reshape(2 * L, L).T * (2.0 / n_fft)
    return _row_pairs(fwd), _row_pairs(inv)


_FWD, _INV = _dft_matrices()


def _lo(w):
    return pltpu.unpack_elementwise(w, index=0, packed_dtype=BF16, unpacked_dtype=F32)


def _hi(w):
    return pltpu.unpack_elementwise(w, index=1, packed_dtype=BF16, unpacked_dtype=F32)


def _pack(a, b):
    return pltpu.pack_elementwise([a, b], packed_dtype=BF16)


def _bf16(words):
    return pltpu.bitcast(words, BF16)


def _words(x):
    return pltpu.bitcast(x.astype(BF16), U32)


def _interleave(streams):
    steps = sorted(((k + 0.5) / n, i) for i, (_, n) in enumerate(streams) for k in range(n))
    for _, i in steps:
        next(streams[i][0], None)
    for stream, _ in streams:
        for _ in stream:
            pass


def _radix4(e, inverse):
    (r0, i0), (r1, i1), (r2, i2), (r3, i3) = e
    sr, si, dr, di = r0 + r2, i0 + i2, r0 - r2, i0 - i2
    tr, ti, ur, ui = r1 + r3, i1 + i3, r1 - r3, i1 - i3
    a = (dr + ui, di - ur)
    b = (dr - ui, di + ur)
    if inverse:
        a, b = b, a
    return [(sr + tr, si + ti), a, (sr - tr, si - ti), b]


def _strassen_lhs(a11, a12, a21, a22):
    return [a11 + a22, a21 + a22, a11, a22, a11 + a12, a21 - a11, a12 - a22]


def _strassen_rhs(b11, b12, b21, b22):
    return [b11 + b22, b11, b12 - b22, b21 - b11, b22, b11 + b12, b21 + b22]


def _strassen_product(product):
    m3, m5 = product(2), product(4)
    c12 = m3 + m5
    m2, m4 = product(1), product(3)
    c21 = m2 + m4
    c11, c22 = m4 - m5, m3 - m2
    m1 = product(0)
    c11, c22 = c11 + m1, c22 + m1
    return c11 + product(6), c12, c21, c22 + product(5)


def _gelu2(x):
    t = jnp.tanh(x * (x * x * GELU_C1 + GELU_C0))
    return x * t + x


def _kernel(q_hbm, k_hbm, v_hbm, shift_hbm, ssm_hbm, ssmd_hbm, wi_hbm, wsp_hbm, bsp_hbm,
            wo_hbm, c_hbm, wmod_hbm, fwd_hbm, inv_hbm, out_hbm,
            q_v, k_v, v_v, shift_v, ssm_v, ssmd_v, wi_v, wsp_v, bsp_v, wo_v, c_v, wmod_v,
            fwd_v, inv_v, out_v,
            taps_s, ssmd_s, bsp_s, mod_s, phase_s, khat,
            uhat, kv_s, g_s, y_s, x1_s, h_s, z1_s, z2_s, wb_s, a_s, wot_s, p_s,
            sems, out_sems):

    copies = {}

    def queue(name, src, dst):
        copies[name] = pltpu.make_async_copy(src, dst, sems.at[len(copies)])
        copies[name].start()

    def rows(ref, i, n):
        return ref.at[pl.ds(i * n, n), :]

    queue("ssm0", rows(ssm_hbm, 0, L), rows(ssm_v, 0, L))
    queue("fwd", fwd_hbm, fwd_v)
    queue("ssmd", ssmd_hbm, ssmd_v)
    queue("shift", shift_hbm, shift_v)
    queue("c", c_hbm, c_v)
    queue("bsp", bsp_hbm, bsp_v)
    for i in range(1, NCT):
        queue(f"ssm{i}", rows(ssm_hbm, i, L), rows(ssm_v, i, L))
    k_v[0:8, :] = jnp.zeros((8, D), U32)
    for j in range(NCH):
        queue(f"k{j}", rows(k_hbm, j, C), k_v.at[pl.ds(8 + j * C // 2, C // 2), :].bitcast(BF16))
        queue(f"v{j}", rows(v_hbm, j, C), rows(v_v, j, C // 2).bitcast(BF16))
        if j == 0:
            queue("inv", inv_hbm, inv_v)
    queue("wmod", wmod_hbm.at[:, 0:5 * D], wmod_v.at[:, 0:5 * D])
    queue("q0", rows(q_hbm, 0, TS), rows(q_v, 0, TS // 2).bitcast(BF16))
    queue("wi", wi_hbm, wi_v.bitcast(BF16))
    for i in range(1, S // TS):
        queue(f"q{i}", rows(q_hbm, i, TS), rows(q_v, i, TS // 2).bitcast(BF16))
    queue("wgb", wmod_hbm.at[:, 5 * D:6 * D], wmod_v.at[:, 5 * D:6 * D])
    queue("wo", wo_hbm, wo_v)
    for i in range(S // TT):
        queue(f"wsp{i}", rows(wsp_hbm, i, TT), rows(wsp_v, i, TH).bitcast(BF16))

    def wait(name):
        copies[name].wait()

    def lanes(c):
        return pl.ds(pl.multiple_of(c * L, L), L)

    def forward_dft(even, odd):
        phase_s[0] = _pack(even[:L], even[L:])
        phase_s[1] = _pack(odd[:L], odd[L:])
        out = []
        for p in range(4):
            words = phase_s[p % 2, pl.ds(p // 2, L // 2, stride=2), :]
            out.append(jnp.dot(_bf16(fwd_v[p]), pltpu.bitcast(words, BF16), preferred_element_type=F32))
        return out

    def group(x, g):
        return x[16 * g:16 * g + 8], x[16 * g + 8:16 * g + 16]

    def load_group(ref, c, k2, g):
        return ref[c, k2, 16 * g:16 * g + 8, :], ref[c, k2, 16 * g + 8:16 * g + 16, :]

    def store_group(ref, c, k2, g, val):
        ref[c, k2, 16 * g:16 * g + 8, :] = val[0]
        ref[c, k2, 16 * g + 8:16 * g + 16, :] = val[1]

    wait("fwd")
    wait("ssmd")
    wait("shift")
    dvec = ssmd_v[...].astype(F32)
    for i in range(NCT):
        ssmd_s[i] = jnp.broadcast_to(dvec[i:i + 1], (8, L))
    taps = shift_v[...].astype(F32)
    for t in range(KS):
        taps_s[t] = jnp.broadcast_to(taps[t:t + 1], (8, D))

    def filter_spectrum(c, carry):
        for i in range(NCT):
            @pl.when(c == i)
            def _():
                wait(f"ssm{i}")
        prev = None
        for m in range(NCH):
            tile = ssm_v[pl.ds(pl.multiple_of(c * L, L), L), m * C:(m + 1) * C]
            words = pltpu.bitcast(tile.T, U32)
            e = forward_dft(_lo(words), _hi(words))
            cur = []
            for g in range(NPOS):
                pairs = [group(e[p], g) for p in range(4)]
                kk = _radix4(pairs, False)
                cur.append(kk)
                for k2 in range(4):
                    re, im = kk[k2]
                    if m == 0:
                        val = (re + ssmd_s[c], im)
                    elif g < NPOS // 2:
                        val = (re - prev[g][k2][1], im + prev[g][k2][0])
                    else:
                        val = (re + prev[g][k2][1], im - prev[g][k2][0])
                    store_group(khat[m], c, k2, g, val)
            prev = cur
        return carry

    with _scope("filter"):
        lax.fori_loop(0, NCT, filter_spectrum, 0)

    def short_conv(j, c):
        w0, w1, w2, w3 = [taps_s[t, :, lanes(c)] for t in range(KS)]
        for u in range(L // 8):
            halves = []
            for h in range(2):
                r0 = j * (C // 2) + h * L + 8 * u
                kw = k_v[r0:r0 + 16, lanes(c)]
                vw = v_v[r0:r0 + 8, lanes(c)]
                cur, back1, back2 = kw[8:], pltpu.roll(kw, 1, 0)[8:], pltpu.roll(kw, 2, 0)[8:]
                e0, o0, e1, o1, o2 = _lo(cur), _hi(cur), _lo(back1), _hi(back1), _hi(back2)
                halves.append((((w0 * e0 + w1 * o1) + (w2 * e1 + w3 * o2)) * _lo(vw),
                               ((w0 * o0 + w1 * e0) + (w2 * o1 + w3 * e1)) * _hi(vw)))
            for s in range(2):
                kv_s[j % 2][c, s, 8 * u:8 * u + 8, :] = _pack(halves[0][s], halves[1][s])

    def chunk_product(i, c):
        e = [jnp.dot(_bf16(fwd_v[p]),
                     _bf16(kv_s[i % 2][c, p % 2, pl.ds(p // 2, L // 2, stride=2), :]),
                     preferred_element_type=F32) for p in range(4)]
        for g in range(NPOS):
            uu = _radix4([group(x, g) for x in e], False)
            ys = []
            for k2 in range(4):
                if i < NCH - 1:
                    store_group(uhat[i], c, k2, g, uu[k2])
                yr = yi = None
                for j in range(i, -1, -1):
                    kr, ki = load_group(khat[i - j], c, k2, g)
                    ur, ui = uu[k2] if j == i else load_group(uhat[j], c, k2, g)
                    pr, pi = kr * ur - ki * ui, kr * ui + ki * ur
                    yr, yi = (pr, pi) if yr is None else (yr + pr, yi + pi)
                ys.append((yr, yi))
            gg = _radix4(ys, True)
            for p in range(4):
                g_s[i % 2][c, p, 8 * g:8 * g + 8, :] = _pack(*gg[p])

    def inverse_dft(i, c):
        y = [jnp.dot(_bf16(inv_v[p]), _bf16(g_s[i % 2][c, p]), preferred_element_type=F32) for p in range(4)]
        base = i * (C // 2)
        y_s[c, pl.ds(base, L, stride=2), :] = _pack(y[0], y[1])
        y_s[c, pl.ds(base + 1, L, stride=2), :] = _pack(y[2], y[3])

    for step in range(-1, NCH + 1):
        if step + 1 < NCH:
            wait(f"k{step + 1}")
            wait(f"v{step + 1}")
        if step == 1:
            wait("inv")

        def conv_step(c, carry, step=step):
            if 0 <= step < NCH:
                chunk_product(step, c)
            if step + 1 < NCH:
                short_conv(step + 1, c)
            if step >= 1:
                inverse_dft(step - 1, c)
            return carry

        with _scope(f"conv{step}"):
            lax.fori_loop(0, NCT, conv_step, 0)

    wait("c")
    cv = c_v[...].astype(F32)
    act = jnp.broadcast_to(cv * jax.nn.sigmoid(cv), (16, D)).astype(BF16)

    def modulation(i):
        return jnp.dot(act, wmod_v[:, i * D:(i + 1) * D], preferred_element_type=F32)[:8]

    wait("wmod")
    with _scope("mod"):
        sa, ca, ga, sb, cb = [modulation(i) for i in range(5)]
        mod_s[0] = (1.0 + ca) * ga
        mod_s[1] = sa * ga
        mod_s[2] = 1.0 + cb
        mod_s[3] = sb

    never = jnp.tile(fwd_v[0, 0:8, :], (1, TS // L)) == 0x12345678

    def after(first, value):
        return jnp.where(never, first, value)

    def layernorm_rows(x):
        d = x - jnp.sum(x, axis=-1, keepdims=True) * (1.0 / D)
        var = jnp.sum(d * d, axis=-1, keepdims=True) * (1.0 / D)
        return d * lax.rsqrt(var + EPS)

    def residual_stage(i, h_ref):
        for r in range(TS // 16):
            wrow = pl.ds(pl.multiple_of(i * (TS // 2) + r * 8, 8), 8)
            xw = q_v[wrow, :]
            yw = jnp.concatenate([y_s[c, wrow, :] for c in range(NCT)], axis=1)
            x1, h = [], []
            for half in (_lo, _hi):
                x = half(xw)
                x1.append(x + (layernorm_rows(x) * mod_s[0] + mod_s[1]) * half(yw))
                h.append(layernorm_rows(x1[-1]) * mod_s[2] + mod_s[3])
            x1_s[wrow, :] = _pack(*x1)
            h_ref[r * 8:(r + 1) * 8, :] = _pack(*h)
            yield

    def hidden_stage(i, h_ref):
        cols = pl.ds(pl.multiple_of(i * TS, TS), TS)
        half_cols = pl.ds(pl.multiple_of(i * (TS // 2), TS // 2), TS // 2)

        def preact(r0):
            return lax.dot_general(_bf16(wi_v[r0 // 2:(r0 + MB) // 2, :]), _bf16(h_ref[...]),
                                   NT_DIMS, preferred_element_type=F32)

        def tiles(x):
            return x.reshape(x.shape[0] // 8, 8, TS)

        def column_mean(acc):
            return jnp.broadcast_to(jnp.sum(acc, axis=0, keepdims=True) * (1.0 / FH), (8, TS))

        acc = jnp.zeros((8, TS), F32)
        for r0 in range(0, FH, MB):
            a = _gelu2(preact(FH + r0))
            a_s[r0:r0 + MB, :] = a
            acc = acc + tiles(a).sum(axis=0)
            yield
        mean = column_mean(acc)

        n = FH // MB
        n_var = n // 2
        acc = jnp.zeros((8, TS), F32)
        prev = None
        for k in range(n):
            z = _gelu2(preact(k * MB))
            z1_s[k * MB:(k + 1) * MB, cols] = z.astype(BF16)
            m = mean if prev is None else after(prev, mean)
            if k < n_var:
                lo, hi = k * FH // n_var, (k + 1) * FH // n_var
                d = tiles(a_s[lo:hi, :]) - m
                acc = acc + (d * d).sum(axis=0)
                if k == n_var - 1:
                    rstd = lax.rsqrt(column_mean(acc) + 4.0 * EPS)
            else:
                lo, hi = (k - n_var) * FQ // (n - n_var), (k - n_var + 1) * FQ // (n - n_var)
                top, bot = [((tiles(a_s[o + lo:o + hi, :]) - m) * rstd).reshape(hi - lo, TS)
                            for o in (0, FQ)]
                ops = _strassen_lhs(top[:, :TS // 2], top[:, TS // 2:],
                                    bot[:, :TS // 2], bot[:, TS // 2:])
                for q in range(7):
                    z2_s[q, lo:hi, half_cols] = ops[q].astype(BF16)
            prev = z[TOKROW:TOKROW + 8]
            yield

    wait("q0")
    with _scope("res0"):
        _interleave([(residual_stage(0, h_s.at[0]), 1)])
    wait("wi")
    for i in range(1, S // TS):
        wait(f"q{i}")

    def hidden_step(i, carry):
        _interleave([(hidden_stage(i, h_s.at[i % 2]), 2 * FH // MB),
                     (residual_stage(i + 1, h_s.at[(i + 1) % 2]), TS // 16)])
        return carry

    with _scope("hidden"):
        lax.fori_loop(0, S // TS - 1, hidden_step, 0)
    def mixer_operands(i):
        for r in range(TH // 16):
            top = pl.ds(pl.multiple_of(i * TH + r * 8, 8), 8)
            bot = pl.ds(pl.multiple_of(i * TH + TH // 2 + r * 8, 8), 8)
            for n in range(S // TS):
                left, right = slice(n * TS, n * TS + TS // 2), slice(n * TS + TS // 2, (n + 1) * TS)
                w = [wsp_v[top, left], wsp_v[bot, left], wsp_v[top, right], wsp_v[bot, right]]
                lo, hi = _strassen_rhs(*[_lo(x) for x in w]), _strassen_rhs(*[_hi(x) for x in w])
                for slot, q in enumerate(SUMMED):
                    wb_s[i % 2, slot, r * 8:(r + 1) * 8, n * TS // 2:(n + 1) * TS // 2] = (
                        _pack(lo[q], hi[q]))
            yield

    for i in range(2):
        wait(f"wsp{i}")
    with _scope("hidden_last"):
        _interleave([(hidden_stage(S // TS - 1, h_s.at[1]), 2 * FH // MB),
                     (mixer_operands(0), TH // 16)])

    wait("wgb")
    wait("bsp")
    wait("wo")
    mod_s[4] = 0.5 * modulation(5)
    bvec = bsp_v[...].astype(F32)
    for i in range(S // L):
        bsp_s[:, i * L:(i + 1) * L] = jnp.broadcast_to(bvec[i:i + 1], (8, L))
    wot_s[...] = wo_v[...].T

    def out_copy(i):
        return pltpu.make_async_copy(
            out_v.at[pl.ds(pl.multiple_of(i * TH, TH), TH), :].bitcast(BF16),
            out_hbm.at[pl.ds(pl.multiple_of(i * TT, TT), TT), :], out_sems.at[i])

    def mix_stage(i):
        def product(q):
            if q in SUMMED:
                w = wb_s[i % 2, SUMMED.index(q)]
            else:
                o = 0 if q == 1 else 1
                row = pl.ds(pl.multiple_of(i * TH + o * (TH // 2), TH // 2), TH // 2)
                w = jnp.concatenate(
                    [wsp_v[row, n * TS + o * TS // 2:n * TS + (o + 1) * TS // 2]
                     for n in range(S // TS)], axis=1)
            return lax.dot_general(z2_s[q], _bf16(w), NT_DIMS, preferred_element_type=F32)

        for n, g in enumerate(_strassen_product(product)):
            f = slice((n // 2) * FQ, (n // 2 + 1) * FQ)
            t = pl.ds(pl.multiple_of(i * TT + (n % 2) * TH, TH), TH)
            g = (g.reshape(FQ // 8, 8, TH) + bsp_s[:, t]).reshape(FQ, TH)
            p_s[f, (n % 2) * TH:(n % 2 + 1) * TH] = (z1_s[f, t].astype(F32) * g).astype(BF16)
        yield
        for n in range(TT // TO):
            o = jnp.dot(wot_s[...], p_s[:, n * TO:(n + 1) * TO], preferred_element_type=F32).T
            row = pl.ds(pl.multiple_of(i * TH + n * (TO // 2), TO // 2), TO // 2)
            res = _bf16(x1_s[row, :]).astype(F32).reshape(TO // 8, 8, D) + mod_s[4] * o.reshape(TO // 8, 8, D)
            out_v.bitcast(BF16)[pl.ds(pl.multiple_of(i * TT + n * TO, TO), TO), :] = res.reshape(TO, D).astype(BF16)
            yield

    n_steps = S // TT

    def mix_step(i, carry):
        for n in range(1, n_steps - 1):
            @pl.when(i == n)
            def _():
                wait(f"wsp{n + 1}")
        _interleave([(mix_stage(i), 1 + TT // TO), (mixer_operands(i + 1), TH // 16)])
        out_copy(i).start()
        return carry

    with _scope("mix"):
        lax.fori_loop(0, n_steps - 1, mix_step, 0)
    with _scope("mix_last"):
        _interleave([(mix_stage(n_steps - 1), 1)])
    out_copy(n_steps - 1).start()
    for i in range(n_steps):
        out_copy(i).wait()


@jax.jit
def pallas_adaLN_cond__ssm_conv_h3__mixer_gmlp__prompt_kernel(
    A_q: jax.Array,
    A_k: jax.Array,
    A_v: jax.Array,
    A_shift_k: jax.Array,
    A_ssm_k: jax.Array,
    A_ssm_D: jax.Array,
    B_x: jax.Array,
    B_w_in: jax.Array,
    B_w_sp: jax.Array,
    B_b_sp: jax.Array,
    B_w_out: jax.Array,
    c: jax.Array,
    w_mod: jax.Array,
):
    del B_x
    operands = (
        A_q.reshape(S, D), A_k.reshape(S, D), A_v.reshape(S, D), A_shift_k.T, A_ssm_k,
        A_ssm_D.reshape(NCT, L), B_w_in.T, B_w_sp, B_b_sp.reshape(S // L, L), B_w_out, c, w_mod,
        _FWD, _INV,
    )
    spectrum = pltpu.VMEM((NCT, 4, 2 * L, L), F32)
    scratch = [
        pltpu.VMEM((S // 2, D), U32),
        pltpu.VMEM((8 + S // 2, D), U32),
        pltpu.VMEM((S // 2, D), U32),
        pltpu.VMEM((KS, D), BF16),
        pltpu.VMEM((D, S), BF16),
        pltpu.VMEM((NCT, L), BF16),
        pltpu.VMEM((FH, D), U32),
        pltpu.VMEM((S // 2, S), U32),
        pltpu.VMEM((S // L, L), BF16),
        pltpu.VMEM((FH, D), BF16),
        pltpu.VMEM((1, D), BF16),
        pltpu.VMEM((D, 6 * D), BF16),
        pltpu.VMEM(_FWD.shape, U32),
        pltpu.VMEM(_INV.shape, U32),
        pltpu.VMEM((S // 2, D), U32),
        pltpu.VMEM((KS, 8, D), F32),
        pltpu.VMEM((NCT, 8, L), F32),
        pltpu.VMEM((8, S), F32),
        pltpu.VMEM((5, 8, D), F32),
        pltpu.VMEM((2, L, L), U32),
        [spectrum] * NCH,
        [spectrum] * (NCH - 1),
        [pltpu.VMEM((NCT, 2, L, L), U32)] * 2,
        [pltpu.VMEM((NCT, 4, L, L), U32)] * 2,
        pltpu.VMEM((NCT, S // 2, L), U32),
        pltpu.VMEM((S // 2, D), U32),
        pltpu.VMEM((2, TS // 2, D), U32),
        pltpu.VMEM((FH, S), BF16),
        pltpu.VMEM((7, FQ, S // 2), BF16),
        pltpu.VMEM((2, 5, TH // 2, S // 2), U32),
        pltpu.VMEM((FH, TS), F32),
        pltpu.VMEM((D, FH), BF16),
        pltpu.VMEM((FH, TT), BF16),
        pltpu.SemaphoreType.DMA((40,)),
        pltpu.SemaphoreType.DMA((S // TT,)),
    ]
    out = pl.pallas_call(
        _kernel,
        out_shape=jax.ShapeDtypeStruct((S, D), BF16),
        in_specs=[pl.BlockSpec(memory_space=pltpu.HBM)] * len(operands),
        out_specs=pl.BlockSpec(memory_space=pltpu.HBM),
        scratch_shapes=scratch,
        compiler_params=pltpu.CompilerParams(vmem_limit_bytes=110 * 1024 * 1024),
    )(*operands)
    return out.reshape(1, S, D)
```

```python
import contextlib
import itertools

import numpy as np

import jax
import jax.numpy as jnp
from jax import lax
import jax.experimental.pallas as pl
import jax.experimental.pallas.tpu as pltpu

S = 2048
D = 640
FH = 864
FQ = FH // 2
KS = 4
L = 128
NCT = D // L
C = 512
CH = C // 2
NCH = S // C
NPOS = 16
TICKS = 3
FILL = 0.93
MB = 144
DEPTH = 4
SPLIT = 4
TO = 256
CONV_MATMULS = "D2 K0 K1 K2 D3 B0 K3 B1 D0 B2 D1 B3".split()
CONV_VECTOR = "T0 T1 T2 C3 A0 T3 A1 C0 A2 C1 A3 C2".split()
CONV_BUDGET = 66
CONV_LEAD = 4
CARRIED = ("D2", "C3", "D3")
SUMMED = (0, 2, 3, 5, 6)
NEVER = 0x12345678
EPS = 1e-5
GELU_C0 = float(np.sqrt(2.0 / np.pi))
GELU_C1 = GELU_C0 * 0.044715

F32 = jnp.float32
BF16 = jnp.bfloat16
U32 = jnp.uint32
NT_DIMS = (((1,), (1,)), ((), ()))

TRACE_SCOPES = [False]


def _scope(name):
    return jax.named_scope("ph_" + name) if TRACE_SCOPES[0] else contextlib.nullcontext()


def _row_pairs(x):
    bits = x.astype(np.float32).astype(BF16).view(np.uint16).astype(np.uint32)
    return bits[..., 0::2, :] | (bits[..., 1::2, :] << 16)


def _dft_matrices():
    n_fft = 2 * C
    k1 = np.concatenate([np.arange(0, 128, 2), np.arange(1, 128, 2)]).reshape(NPOS, 8)
    fwd = np.zeros((4, 2 * L, L), np.float64)
    inv = np.zeros((4, L, 2 * L), np.float64)
    col_n1 = (np.arange(L) // 2) + 64 * (np.arange(L) % 2)
    for p in range(4):
        n = 4 * np.arange(L) + p
        phase = ((2 * k1[:, :, None] + 1) * n[None, None, :]) % (2 * n_fft)
        theta = np.pi * phase / n_fft
        parts = [np.cos(theta), -np.sin(theta)]
        fwd[p] = np.stack(parts, axis=1).reshape(2 * L, L)[:, col_n1]
        inv[p] = np.stack(parts, axis=2).reshape(2 * L, L).T * (2.0 / n_fft)
    return _row_pairs(fwd), _row_pairs(inv)


_FWD, _INV = _dft_matrices()


def _lo(w):
    return pltpu.unpack_elementwise(w, index=0, packed_dtype=BF16, unpacked_dtype=F32)


def _hi(w):
    return pltpu.unpack_elementwise(w, index=1, packed_dtype=BF16, unpacked_dtype=F32)


def _pack(a, b):
    return pltpu.pack_elementwise([a, b], packed_dtype=BF16)


def _bf16(words):
    return pltpu.bitcast(words, BF16)


def _dot(a, b):
    return jnp.dot(a, b, preferred_element_type=F32)


def _dot_nt(a, b):
    return lax.dot_general(a, b, NT_DIMS, preferred_element_type=F32)


def _tiles(x):
    return x.reshape(x.shape[0] // 8, 8, x.shape[1])


def _interleave(*streams):
    steps = sorted(((k + 0.5) / n * (FILL if i else 1.0), i)
                   for i, (_, n) in enumerate(streams) for k in range(n))
    for _, i in steps:
        next(streams[i][0], None)
    for stream, _ in streams:
        for _ in stream:
            pass


def _conv_schedule():
    steps = dict(T=8, A=16, C=4 * NPOS)
    cost = dict(T0=24, T1=24, T2=24, T3=24, A0=46, A1=46, A2=46, A3=46, C0=12, C1=20, C2=28, C3=36,
                K0=17, K1=28, K2=24, K3=24, B0=16, B1=16, B2=16, B3=16, D0=6, D1=6, D2=6, D3=6)
    vector = [(x, k) for x in CONV_VECTOR for k in range(steps[x[0]])]
    matmul = [(x, k) for x in CONV_MATMULS for k in range(NPOS)]
    order, done, budget = [], set(), 0
    for n, (x, k) in enumerate(matmul):
        for ahead, _ in matmul[n:n + CONV_LEAD + 1]:
            need = dict(K="T", B="A", D="C")[ahead[0]] + ahead[1]
            while ahead != "D2" and any(v == need for v, _ in vector):
                order.append(vector.pop(0)[0])
                budget -= cost[order[-1]]
        order.append(x)
        done.add((x, k))
        budget = min(budget + CONV_BUDGET - cost[x], CONV_BUDGET)
        while vector and budget > 0:
            v, j = vector[0]
            if v[0] == "C" and v != "C3" and not {("K" + v[1], j // 4), ("B" + v[1], j // 4)} <= done:
                break
            order.append(vector.pop(0)[0])
            budget -= cost[v]
    return order + [v for v, _ in vector]


def _radix4(e, inverse):
    (r0, i0), (r1, i1), (r2, i2), (r3, i3) = e
    sr, si, dr, di = r0 + r2, i0 + i2, r0 - r2, i0 - i2
    tr, ti, ur, ui = r1 + r3, i1 + i3, r1 - r3, i1 - i3
    a = (dr + ui, di - ur)
    b = (dr - ui, di + ur)
    if inverse:
        a, b = b, a
    return [(sr + tr, si + ti), a, (sr - tr, si - ti), b]


def _strassen_lhs(a11, a12, a21, a22):
    return [a11 + a22, a21 + a22, a11, a22, a11 + a12, a21 - a11, a12 - a22]


def _strassen_rhs(b11, b12, b21, b22):
    return [b11 + b22, b11, b12 - b22, b21 - b11, b22, b11 + b12, b21 + b22]


def _strassen_product(product):
    m3, m5 = product(2), product(4)
    c12 = m3 + m5
    m2, m4 = product(1), product(3)
    c21 = m2 + m4
    c11, c22 = m4 - m5, m3 - m2
    m1 = product(0)
    c11, c22 = c11 + m1, c22 + m1
    return c11 + product(6), c12, c21, c22 + product(5)


def _gelu2(x):
    t = jnp.tanh(x * (x * x * GELU_C1 + GELU_C0))
    return x * t + x


def _layernorm_rows(x):
    d = x - jnp.sum(x, axis=-1, keepdims=True) * (1.0 / D)
    var = jnp.sum(d * d, axis=-1, keepdims=True) * (1.0 / D)
    return d * lax.rsqrt(var + EPS)


def _kernel(q_hbm, k_hbm, v_hbm, shift_hbm, ssm_hbm, ssmd_hbm, wi_hbm, wsp_hbm, bsp_hbm,
            wo_hbm, c_hbm, wmod_hbm, fwd_hbm, inv_hbm, out_hbm,
            q_v, k_v, v_v, shift_v, ssm_v, ssmd_v, wi_v, wsp_v, bsp_v, wo_v, c_v, wmod_v,
            fwd_v, inv_v, out_v,
            chan_s, bsp_s, mod_s, fstage, ktile, utile, kraw, khat, uhat, g_s, y_s, x1_s, xn_s, h_s,
            a_s, z1_s, z2_s, wb_s, m_s, wot_s, p_s, sems, out_sems):
    copies = {}

    def queue(name, src, dst):
        group = copies.setdefault(name, [])
        group.append(pltpu.make_async_copy(src, dst, sems.at[list(copies).index(name)]))
        group[-1].start()

    def wait(*names):
        for name in names:
            for copy in copies[name]:
                copy.wait()

    def rows(ref, r0, n):
        return ref.at[pl.ds(r0, n), :]

    def queue_pairs(name, src, dst, r0, n):
        queue(name, rows(src, r0, n), rows(dst, r0 // 2, n // 2).bitcast(BF16))

    def queue_wmod(name, i0, i1):
        queue(name, wmod_hbm.at[:, i0 * D:i1 * D], wmod_v.at[:, i0 * D:i1 * D])

    queue("small", fwd_hbm, fwd_v)
    queue("small", inv_hbm, inv_v)
    for src, dst in ((ssmd_hbm, ssmd_v), (shift_hbm, shift_v), (c_hbm, c_v), (bsp_hbm, bsp_v)):
        queue("small", src, dst)
    n = S // SPLIT
    for c in range(NCT):
        queue(f"tile{c}", rows(ssm_hbm, c * L, L), rows(ssm_v, c * L, L))
        for h in range(SPLIT):
            for src, dst, pad in ((k_hbm, k_v, 8), (v_hbm, v_v, 0)):
                queue(f"tile{c}", src.at[pl.ds(h * n, n), pl.ds(c * L, L)],
                      dst.at[c, pl.ds(pad + h * n // 2, n // 2), :].bitcast(BF16))
    queue_pairs("first", q_hbm, q_v, 0, C)
    queue_wmod("first", 0, 3)
    queue_wmod("second", 3, 5)
    wi_groups = {FH: 2 * MB, FH + 2 * MB: FH - 2 * MB, 0: FH}
    for r0, n in wi_groups.items():
        queue_pairs(f"wi{r0}", wi_hbm, wi_v, r0, n)
    for i in range(NCH):
        cols = pl.ds(i * C, C)
        queue(f"chunk{i}", wsp_hbm.at[:, cols], wsp_v.at[:, cols].bitcast(BF16))
        if i + 1 < NCH:
            queue_pairs(f"chunk{i}", q_hbm, q_v, (i + 1) * C, C)
    queue_wmod(f"chunk{NCH - 1}", 5, 6)
    queue(f"chunk{NCH - 1}", wo_hbm, wo_v)

    def wait_step(i, names_of, steps):
        for n in steps:
            @pl.when(i == n)
            def _():
                wait(*names_of(n))

    def span(start, size):
        return pl.ds(start if isinstance(start, int) else pl.multiple_of(start, size), size)

    latest = [None]

    def paced(x):
        if latest[0] is None:
            return x
        n = x.shape[1] // L
        never = jnp.tile(fwd_v[0, 0:8, :], (1, n)) == NEVER
        return jnp.where(never, pltpu.bitcast(jnp.tile(latest[0], (1, n)), x.dtype), x)

    def load_group(ref, k2, g):
        return ref[k2 + zero, 16 * g:16 * g + 8, :], ref[k2 + zero, 16 * g + 8:16 * g + 16, :]

    def store_group(ref, k2, g, val):
        ref[k2, 16 * g:16 * g + 8, :] = val[0]
        ref[k2, 16 * g + 8:16 * g + 16, :] = val[1]

    def spectrum_groups(tiles):
        e = [_dot(_bf16(fwd_v[p]), _bf16(tiles[p + zero])) for p in range(4)]
        for g in range(NPOS):
            latest[0] = e[0][16 * g:16 * g + 8]
            yield _radix4([(x[16 * g:16 * g + 8], x[16 * g + 8:16 * g + 16]) for x in e], False)

    def filter_tiles(c, m):
        fstage[m][...] = pltpu.bitcast(ssm_v[span(c * L, L), m * C:(m + 1) * C].T, U32)
        for u in range(L // 16):
            for s in range(2):
                a = paced(fstage[m][pl.ds(16 * u + s, 8, stride=2), :])
                b = fstage[m][pl.ds(L + 16 * u + s, 8, stride=2), :]
                ktile[m][2 * s, 8 * u:8 * u + 8, :] = _pack(_lo(a), _lo(b))
                ktile[m][2 * s + 1, 8 * u:8 * u + 8, :] = _pack(_hi(a), _hi(b))
            yield

    def signal_tiles(c, j):
        w1, w2, w3 = [chan_s[c, t] for t in range(1, KS)]
        for u in range(L // 16):
            halves = []
            for h in range(2):
                w0 = paced(chan_s[c, 0])
                r0 = j * CH + h * L + 16 * u
                kw = [k_v[c, pl.ds(8 + r0 + o, 8, stride=2), :] for o in range(-2, 2)]
                vw = [v_v[c, pl.ds(r0 + o, 8, stride=2), :] for o in range(2)]
                ks = [_hi(kw[0])] + [f(x) for x in kw[1:] for f in (_lo, _hi)]
                vs = [f(x) for x in vw for f in (_lo, _hi)]
                halves.append([((w0 * ks[p + 3] + w1 * ks[p + 2]) + (w2 * ks[p + 1] + w3 * ks[p]))
                               * vs[p] for p in range(4)])
                if h == 1:
                    for p in range(4):
                        utile[j][p, 8 * u:8 * u + 8, :] = _pack(halves[0][p], halves[1][p])
                yield

    def filter_spectrum(c, m):
        for g, kk in enumerate(spectrum_groups(ktile[m])):
            for k2 in range(4):
                re, im = kk[k2]
                if m == 0:
                    knew = (re + chan_s[c, KS], im)
                else:
                    if m == 1:
                        pre, pim = load_group(khat[0].at[c % 2], k2, g)
                        pre = pre - chan_s[c, KS]
                    else:
                        pre, pim = load_group(kraw[m % 2], k2, g)
                    knew = (re - pim, im + pre) if g < NPOS // 2 else (re + pim, im - pre)
                if 0 < m < NCH - 1:
                    store_group(kraw[(m + 1) % 2], k2, g, kk[k2])
                store_group(khat[m].at[c % 2], k2, g, knew)
            yield

    def signal_spectrum(c, j):
        for g, uu in enumerate(spectrum_groups(utile[j])):
            for k2 in range(4):
                store_group(uhat[j], k2, g, uu[k2])
            yield

    def chunk_product(c, i):
        for g in range(NPOS):
            ys = []
            for k2 in range(4):
                yr = yi = None
                for j in range(i + 1):
                    kr, ki = load_group(khat[i - j].at[c % 2], k2, g)
                    ur, ui = load_group(uhat[j], k2, g)
                    if j == 0:
                        kr = paced(kr)
                    pr, pi = kr * ur - ki * ui, kr * ui + ki * ur
                    yr, yi = (pr, pi) if yr is None else (yr + pr, yi + pi)
                ys.append((yr, yi))
                if k2 == 3:
                    for p, pair in enumerate(_radix4(ys, True)):
                        g_s[i][p, 8 * g:8 * g + 8, :] = _pack(*pair)
                yield

    def inverse_dft(c, i):
        y = None
        for k0 in range(0, 2 * L, L):
            part = [_dot(_bf16(inv_v[p, :, k0:k0 + L]), _bf16(g_s[i][p + zero, k0 // 2:(k0 + L) // 2, :]))
                    for p in range(4)]
            for r in range(0, L, 16):
                latest[0] = part[0][r:r + 8]
                if y is not None:
                    for o in (r, r + 8):
                        full = [a[o:o + 8] + b[o:o + 8] for a, b in zip(y, part)]
                        for s in range(2):
                            y_s[c, pl.ds(i * CH + 2 * o + s, 8, stride=2), :] = (
                                _pack(full[2 * s], full[2 * s + 1]))
                yield
            y = part

    for ref in [x.at[0] for x in khat] + uhat + [g_s[NCH - 2]]:
        ref[...] = jnp.zeros(ref.shape, ref.dtype)
    k_v[:, 0:8, :] = jnp.zeros((NCT, 8, L), U32)
    wait("small")
    probe = pltpu.bitcast(fwd_v[0, 0:8, :], jnp.int32)[0, 0]
    zero = (probe == NEVER).astype(jnp.int32)
    n_blocks = itertools.count()

    def block(name, *streams):
        latest[0] = None

        @pl.when(probe != NEVER + next(n_blocks))
        def _():
            with _scope(name):
                _interleave(*streams)

        latest[0] = None

    dvec = ssmd_v[...].astype(F32)
    taps = shift_v[...].astype(F32)
    for i in range(NCT):
        chan_s[i, KS] = jnp.broadcast_to(dvec[i:i + 1], (8, L))
        for t in range(KS):
            chan_s[i, t] = jnp.broadcast_to(taps[t:t + 1, i * L:(i + 1) * L], (8, L))

    stages = dict(T=filter_tiles, A=signal_tiles, K=filter_spectrum, B=signal_spectrum,
                  C=chunk_product, D=inverse_dft)

    def conv_step(c, carry):
        wait_step(c, lambda n: [f"tile{n}"], range(NCT))
        before = jnp.maximum(c - 1, 0)
        streams = {x: stages[x[0]](before if x in CARRIED else c, int(x[1]))
                   for x in CONV_MATMULS + CONV_VECTOR}
        latest[0] = None
        for x in _conv_schedule():
            next(streams[x])
        latest[0] = None
        return carry

    with _scope("conv"):
        lax.fori_loop(0, NCT, conv_step, 0)

    def residual_stage(i):
        for r in range(CH // 8):
            at = span(i * CH + 8 * r, 8)
            xw = q_v[at, :]
            yw = jnp.concatenate([y_s[c, at, :] for c in range(NCT)], axis=1)
            xw = jnp.concatenate([paced(xw[:, :L]), xw[:, L:]], axis=1)
            x1, h = [], []
            for half in (_lo, _hi):
                x = half(xw)
                x1.append(x + (_layernorm_rows(x) * mod_s[0] + mod_s[1]) * half(yw))
                h.append(_layernorm_rows(x1[-1]) * mod_s[2] + mod_s[3])
            x1_s[at, :] = _pack(*x1)
            h_s[8 * r:8 * r + 8, :] = _pack(*h)
            yield

    cv = c_v[...].astype(F32)
    act = jnp.broadcast_to(cv * jax.nn.sigmoid(cv), (16, D)).astype(BF16)

    def modulation(i):
        return _dot(act, wmod_v[:, i * D:(i + 1) * D])[:8]

    def first_gate():
        sa, ca, ga = [modulation(i) for i in range(3)]
        mod_s[0] = (1.0 + ca) * ga
        mod_s[1] = sa * ga
        latest[0] = ga[:, :L]
        yield

    def first_norm():
        for r in range(0, CH, 8):
            xw = q_v[r:r + 8, :]
            xw = jnp.concatenate([paced(xw[:, :L]), xw[:, L:]], axis=1)
            for s, half in enumerate((_lo, _hi)):
                xn_s[s, r:r + 8, :] = _layernorm_rows(half(xw))
            yield

    def first_residual():
        done = []
        for r in range(0, CH, 8):
            latest[0] = done[-DEPTH] if len(done) >= DEPTH else None
            yw = jnp.concatenate([paced(y_s[0, r:r + 8, :])]
                                 + [y_s[c, r:r + 8, :] for c in range(1, NCT)], axis=1)
            x1 = [half(q_v[r:r + 8, :]) + (xn_s[s, r:r + 8, :] * mod_s[0] + mod_s[1]) * half(yw)
                  for s, half in enumerate((_lo, _hi))]
            x1_s[r:r + 8, :] = _pack(*x1)
            for s in range(2):
                xn = _layernorm_rows(x1[s])
                xn_s[s, r:r + 8, :] = xn
            done.append(xn[:, :L])
            yield

    def first_modulate():
        wait("second")
        shift, scale = modulation(3), 1.0 + modulation(4)
        mod_s[2] = scale
        mod_s[3] = shift
        for r in range(0, CH, 8):
            h_s[r:r + 8, :] = _pack(*[xn_s[s, r:r + 8, :] * scale + shift for s in range(2)])
        yield

    wait("first")
    block("drain",
          (itertools.chain(inverse_dft(NCT - 1, 2), first_gate(), range(24),
                           inverse_dft(NCT - 1, 3)), 2 * NPOS + 25),
          (itertools.chain(chunk_product(NCT - 1, 3), range(32)), 4 * NPOS + 32),
          (first_norm(), CH // 8))
    block("res0", (first_residual(), 1))
    block("mod", (first_modulate(), 1))

    def hidden_stage(i, first=False, extra=None):
        def preact(r0):
            if first and r0 in wi_groups:
                wait(f"wi{r0}")
            z = None
            for k0 in range(0, D, L):
                part = _dot_nt(_bf16(wi_v[r0 // 2:(r0 + MB) // 2, k0:k0 + L]),
                               _bf16(h_s[:, k0:k0 + L]))
                z = part if z is None else z + part
                for r in range(0, MB, MB // TICKS):
                    latest[0] = part[r:r + 8, 0:L]
                    yield
            return z

        def column_mean(acc):
            return jnp.broadcast_to(jnp.sum(acc, axis=0, keepdims=True) * (1.0 / FH), (8, C))

        total = [jnp.zeros((8, C), F32)]

        def activate():
            for r0 in range(0, FH, MB):
                z = yield from preact(FH + r0)
                for r in range(0, MB, 16):
                    a = _gelu2(z[r:r + 16])
                    a_s[r0 + r:r0 + r + 16, :] = a
                    total[0] = total[0] + (a[:8] + a[8:])

        ticks = TICKS * NCT * FH // MB
        _interleave((activate(), ticks), *([extra] if extra else []))
        mean = column_mean(total[0])

        def layernorm():
            acc = jnp.zeros((8, C), F32)
            for r in range(0, FH, 32):
                d = _tiles(a_s[r:r + 32, :]) - paced(mean)
                acc = acc + (d * d).sum(axis=0)
                yield
            rstd = lax.rsqrt(column_mean(acc) + 4.0 * EPS)
            means = [mean[:, c0:c0 + L] for c0 in range(0, C, L)]
            for r in range(0, FQ, 16):
                for c0 in range(0, CH, L):
                    blocks = []
                    for o in (0, FQ):
                        for cols in (slice(c0, c0 + L), slice(CH + c0, CH + c0 + L)):
                            m = means[cols.start // L]
                            if (o == 0) == (cols.start == c0):
                                m = paced(m)
                            d = (_tiles(a_s[o + r:o + r + 16, cols]) - m) * rstd[:, cols]
                            blocks.append(d.reshape(16, L))
                    for q, op in enumerate(_strassen_lhs(*blocks)):
                        z2_s[q, r:r + 16, c0:c0 + L] = op.astype(BF16)
                    yield

        def gate():
            for r0 in range(0, FH, MB):
                z = yield from preact(r0)
                for r in range(0, MB, 16):
                    z1_s[r0 + r:r0 + r + 16, span(i * C, C)] = _gelu2(z[r:r + 16]).astype(BF16)

        _interleave((gate(), ticks), (layernorm(), FH // 32 + FQ // 8))
        yield

    def mixer_sums(i):
        left, right = span(i * C, CH), span(i * C + CH, CH)
        for n in range(NCH):
            for r in range(0, CH // 2, 8):
                top = slice(n * CH + r, n * CH + r + 8)
                bot = slice(n * CH + CH // 2 + r, n * CH + CH // 2 + r + 8)
                w = [paced(wsp_v[top, left]), wsp_v[bot, left],
                     wsp_v[top, right], paced(wsp_v[bot, right])]
                lo, hi = _strassen_rhs(*[_lo(x) for x in w]), _strassen_rhs(*[_hi(x) for x in w])
                for slot, q in enumerate(SUMMED):
                    wb_s[slot, n * CH // 2 + r:n * CH // 2 + r + 8, :] = _pack(lo[q], hi[q])
                yield

    def mixer_operand(i, q, n):
        if q in SUMMED:
            return wb_s[SUMMED.index(q), span(n * (CH // 2), CH // 2), :]
        o = 0 if q == 1 else 1
        return wsp_v[span(n * CH + o * (CH // 2), CH // 2), span(i * C + o * CH, CH)]

    def mixer_partial(i, products):
        for n in range(0, NCH, 2):
            for q in products:
                w = jnp.concatenate([mixer_operand(i, q, n), mixer_operand(i, q, n + 1)], axis=0)
                cols = slice(n * CH, (n + 2) * CH)
                for r0 in range(0, FQ, MB):
                    m = _dot_nt(z2_s[q, r0:r0 + MB, :], _bf16(w))
                    for r in range(0, MB, 8):
                        at = (q, slice(r0 + r, r0 + r + 8), cols)
                        m_s[at] = jnp.where(i > 0, m_s[at], 0.0) + m[r:r + 8]
                    for r in range(0, MB, MB // TICKS):
                        latest[0] = m[r:r + 8, 0:L]
                        yield

    def partial_stage(i):
        ticks = TICKS * 2 * FQ // MB
        _interleave((mixer_partial(i, (1, 4)), 2 * ticks), (mixer_sums(i), NCH * CH // 16))
        _interleave((mixer_partial(i, SUMMED), 5 * ticks), (residual_stage(i + 1), CH // 8))
        yield

    block("hidden0", (hidden_stage(0, first=True), 1))

    def chunk_step(i, carry):
        wait_step(i, lambda n: [f"chunk{n}"], range(NCH - 1))
        block("partial", (partial_stage(i), 1))

        @pl.when(i < NCH - 2)
        def _():
            block("hidden", (hidden_stage(i + 1), 1))

        return carry

    lax.fori_loop(0, NCH - 1, chunk_step, 0)

    def output_operands():
        bvec = bsp_v[...].astype(F32)
        for i in range(S // L):
            bsp_s[:, i * L:(i + 1) * L] = jnp.broadcast_to(bvec[i:i + 1], (8, L))
        wot_s[...] = wo_v[...].T
        yield from mixer_sums(NCH - 1)
        mod_s[4] = 0.5 * modulation(5)

    wait(f"chunk{NCH - 1}")
    block("hidden_last", (hidden_stage(NCH - 1, extra=(output_operands(), NCH * CH // 16)), 1))

    def out_copy(n):
        return pltpu.make_async_copy(
            out_v.at[span(n * C, C), :], out_hbm.at[span(n * C, C), :], out_sems.at[n])

    def output_step(n, carry):
        def product(q):
            return (m_s[q, :, span(n * CH, CH)]
                    + _dot_nt(z2_s[q], _bf16(mixer_operand(NCH - 1, q, n))))

        for b, g in enumerate(_strassen_product(product)):
            f = slice((b // 2) * FQ, (b // 2 + 1) * FQ)
            t = span(n * C + (b % 2) * CH, CH)
            g = (_tiles(g) + bsp_s[:, t]).reshape(FQ, CH)
            p_s[f, (b % 2) * CH:(b % 2 + 1) * CH] = (z1_s[f, t].astype(F32) * g).astype(BF16)
        for b in range(C // TO):
            o = _dot(wot_s[...], p_s[:, b * TO:(b + 1) * TO]).T
            x1 = _bf16(x1_s[span(n * CH + b * (TO // 2), TO // 2), :]).astype(F32)
            res = _tiles(x1) + mod_s[4] * _tiles(o)
            out_v[span(n * C + b * TO, TO), :] = res.reshape(TO, D).astype(BF16)
        out_copy(n).start()
        return carry

    with _scope("output"):
        lax.fori_loop(0, NCH, output_step, 0)
    for n in range(NCH):
        out_copy(n).wait()


@jax.jit
def pallas_adaLN_cond__ssm_conv_h3__mixer_gmlp__prompt_kernel(
    A_q: jax.Array,
    A_k: jax.Array,
    A_v: jax.Array,
    A_shift_k: jax.Array,
    A_ssm_k: jax.Array,
    A_ssm_D: jax.Array,
    B_x: jax.Array,
    B_w_in: jax.Array,
    B_w_sp: jax.Array,
    B_b_sp: jax.Array,
    B_w_out: jax.Array,
    c: jax.Array,
    w_mod: jax.Array,
):
    del B_x
    operands = (
        A_q.reshape(S, D), A_k.reshape(S, D), A_v.reshape(S, D), A_shift_k.T, A_ssm_k,
        A_ssm_D.reshape(NCT, L), B_w_in.T, B_w_sp, B_b_sp.reshape(S // L, L), B_w_out, c, w_mod,
        _FWD, _INV,
    )
    spectrum = pltpu.VMEM((4, 2 * L, L), F32)
    scratch = [
        pltpu.VMEM((S // 2, D), U32),
        pltpu.VMEM((NCT, 8 + S // 2, L), U32),
        pltpu.VMEM((NCT, S // 2, L), U32),
        pltpu.VMEM((KS, D), BF16),
        pltpu.VMEM((D, S), BF16),
        pltpu.VMEM((NCT, L), BF16),
        pltpu.VMEM((FH, D), U32),
        pltpu.VMEM((S // 2, S), U32),
        pltpu.VMEM((S // L, L), BF16),
        pltpu.VMEM((FH, D), BF16),
        pltpu.VMEM((1, D), BF16),
        pltpu.VMEM((D, 6 * D), BF16),
        pltpu.VMEM(_FWD.shape, U32),
        pltpu.VMEM(_INV.shape, U32),
        pltpu.VMEM((S, D), BF16),
        pltpu.VMEM((NCT, KS + 1, 8, L), F32),
        pltpu.VMEM((8, S), F32),
        pltpu.VMEM((5, 8, D), F32),
        [pltpu.VMEM((CH, L), U32)] * NCH,
        [pltpu.VMEM((4, L // 2, L), U32)] * NCH,
        [pltpu.VMEM((4, L // 2, L), U32)] * NCH,
        [spectrum] * 2,
        [pltpu.VMEM((2, 4, 2 * L, L), F32)] * NCH,
        [spectrum] * NCH,
        [pltpu.VMEM((4, L, L), U32)] * NCH,
        pltpu.VMEM((NCT, S // 2, L), U32),
        pltpu.VMEM((S // 2, D), U32),
        pltpu.VMEM((2, CH, D), F32),
        pltpu.VMEM((CH, D), U32),
        pltpu.VMEM((FH, C), F32),
        pltpu.VMEM((FH, S), BF16),
        pltpu.VMEM((7, FQ, CH), BF16),
        pltpu.VMEM((5, S // 4, CH), U32),
        pltpu.VMEM((7, FQ, S // 2), F32),
        pltpu.VMEM((D, FH), BF16),
        pltpu.VMEM((FH, C), BF16),
        pltpu.SemaphoreType.DMA((15,)),
        pltpu.SemaphoreType.DMA((NCH,)),
    ]
    out = pl.pallas_call(
        _kernel,
        out_shape=jax.ShapeDtypeStruct((S, D), BF16),
        in_specs=[pl.BlockSpec(memory_space=pltpu.HBM)] * len(operands),
        out_specs=pl.BlockSpec(memory_space=pltpu.HBM),
        scratch_shapes=scratch,
        compiler_params=pltpu.CompilerParams(vmem_limit_bytes=120 * 1024 * 1024),
    )(*operands)
    return out.reshape(1, S, D)
```

```python
import contextlib
import itertools

import numpy as np

import jax
import jax.numpy as jnp
from jax import lax
import jax.experimental.pallas as pl
import jax.experimental.pallas.tpu as pltpu

S = 2048
D = 640
FH = 864
FQ = FH // 2
KS = 4
L = 128
NCT = D // L
C = 512
CH = C // 2
NCH = S // C
NPOS = 16
TICK = 48
TICKS = 3
FILL = 0.93
MB = 144
DEPTH = 12
SPLIT = 4
DH = D // 2
FM = 384
GATE_ROWS = ((0, 128), (128, 256), (256, FQ))
CONV_MATMULS = "D2 K0 K1 K2 D3 B0 K3 B1 D0 B2 D1 B3".split()
CONV_VECTOR = "T0 T1 T2 C3 A0 T3 A1 C0 A2 C1 A3 C2".split()
CONV_BUDGET = 66
CONV_LEAD = 4
CARRIED = ("D2", "C3", "D3")
DM = 256
SUMMED_LHS = (0, 1, 4, 5, 6)
SUMMED = (0, 2, 3, 5, 6)
NEVER = 0x12345678
EPS = 1e-5
GELU_C0 = float(np.sqrt(2.0 / np.pi))
GELU_C1 = GELU_C0 * 0.044715

F32 = jnp.float32
BF16 = jnp.bfloat16
U32 = jnp.uint32
NT_DIMS = (((1,), (1,)), ((), ()))

TRACE_SCOPES = [False]


def _scope(name):
    return jax.named_scope("ph_" + name) if TRACE_SCOPES[0] else contextlib.nullcontext()


def _row_pairs(x):
    bits = x.astype(np.float32).astype(BF16).view(np.uint16).astype(np.uint32)
    return bits[..., 0::2, :] | (bits[..., 1::2, :] << 16)


def _dft_matrices():
    n_fft = 2 * C
    k1 = np.concatenate([np.arange(0, 128, 2), np.arange(1, 128, 2)]).reshape(NPOS, 8)
    fwd = np.zeros((4, 2 * L, L), np.float64)
    inv = np.zeros((4, L, 2 * L), np.float64)
    col_n1 = (np.arange(L) // 2) + 64 * (np.arange(L) % 2)
    for p in range(4):
        n = 4 * np.arange(L) + p
        phase = ((2 * k1[:, :, None] + 1) * n[None, None, :]) % (2 * n_fft)
        theta = np.pi * phase / n_fft
        parts = [np.cos(theta), -np.sin(theta)]
        fwd[p] = np.stack(parts, axis=1).reshape(2 * L, L)[:, col_n1]
        inv[p] = np.stack(parts, axis=2).reshape(2 * L, L).T * (2.0 / n_fft)
    return _row_pairs(fwd), _row_pairs(inv)


_FWD, _INV = _dft_matrices()


def _lo(w):
    return pltpu.unpack_elementwise(w, index=0, packed_dtype=BF16, unpacked_dtype=F32)


def _hi(w):
    return pltpu.unpack_elementwise(w, index=1, packed_dtype=BF16, unpacked_dtype=F32)


def _pack(a, b):
    return pltpu.pack_elementwise([a, b], packed_dtype=BF16)


def _bf16(words):
    return pltpu.bitcast(words, BF16)


def _dot(a, b):
    return jnp.dot(a, b, preferred_element_type=F32)


def _dot_nt(a, b):
    return lax.dot_general(a, b, NT_DIMS, preferred_element_type=F32)


def _tiles(x):
    return x.reshape(x.shape[0] // 8, 8, x.shape[1])


def _interleave(*streams):
    steps = sorted(((k + 0.5) / n * (FILL if i else 1.0), i)
                   for i, (_, n) in enumerate(streams) for k in range(n))
    for _, i in steps:
        next(streams[i][0], None)
    for stream, _ in streams:
        for _ in stream:
            pass


def _conv_schedule():
    steps = dict(T=8, A=16, C=4 * NPOS)
    cost = dict(T0=24, T1=24, T2=24, T3=24, A0=46, A1=46, A2=46, A3=46, C0=12, C1=20, C2=28, C3=36,
                K0=17, K1=28, K2=24, K3=24, B0=16, B1=16, B2=16, B3=16, D0=6, D1=6, D2=6, D3=6)
    vector = [(x, k) for x in CONV_VECTOR for k in range(steps[x[0]])]
    matmul = [(x, k) for x in CONV_MATMULS for k in range(NPOS)]
    order, done, budget = [], set(), 0
    for n, (x, k) in enumerate(matmul):
        for ahead, _ in matmul[n:n + CONV_LEAD + 1]:
            need = dict(K="T", B="A", D="C")[ahead[0]] + ahead[1]
            while ahead != "D2" and any(v == need for v, _ in vector):
                order.append(vector.pop(0)[0])
                budget -= cost[order[-1]]
        order.append(x)
        done.add((x, k))
        budget = min(budget + CONV_BUDGET - cost[x], CONV_BUDGET)
        while vector and budget > 0:
            v, j = vector[0]
            if v[0] == "C" and v != "C3" and not {("K" + v[1], j // 4), ("B" + v[1], j // 4)} <= done:
                break
            order.append(vector.pop(0)[0])
            budget -= cost[v]
    return order + [v for v, _ in vector]


def _radix4(e, inverse):
    (r0, i0), (r1, i1), (r2, i2), (r3, i3) = e
    sr, si, dr, di = r0 + r2, i0 + i2, r0 - r2, i0 - i2
    tr, ti, ur, ui = r1 + r3, i1 + i3, r1 - r3, i1 - i3
    a = (dr + ui, di - ur)
    b = (dr - ui, di + ur)
    if inverse:
        a, b = b, a
    return [(sr + tr, si + ti), a, (sr - tr, si - ti), b]


def _strassen_lhs(a11, a12, a21, a22):
    return [a11 + a22, a21 + a22, a11, a22, a11 + a12, a21 - a11, a12 - a22]


def _strassen_rhs(b11, b12, b21, b22):
    return [b11 + b22, b11, b12 - b22, b21 - b11, b22, b11 + b12, b21 + b22]


def _strassen_product(product):
    m3 = yield from product(2)
    m4 = yield from product(3)
    m5 = yield from product(4)
    m2 = yield from product(1)
    m1 = yield from product(0)
    m7 = yield from product(6)
    m6 = yield from product(5)
    return [lambda r: (m4[r] - m5[r]) + m1[r] + m7[r], lambda r: m3[r] + m5[r],
            lambda r: m2[r] + m4[r], lambda r: (m3[r] - m2[r]) + m1[r] + m6[r]]


def _gelu2(x):
    t = jnp.tanh(x * (x * x * GELU_C1 + GELU_C0))
    return x * t + x


def _layernorm_rows(x):
    d = x - jnp.sum(x, axis=-1, keepdims=True) * (1.0 / D)
    var = jnp.sum(d * d, axis=-1, keepdims=True) * (1.0 / D)
    return d * lax.rsqrt(var + EPS)


def _kernel(q_hbm, k_hbm, v_hbm, shift_hbm, ssm_hbm, ssmd_hbm, wi_hbm, wsp_hbm, bsp_hbm,
            wo_hbm, c_hbm, wmod_hbm, fwd_hbm, inv_hbm, out_hbm,
            q_v, k_v, v_v, shift_v, ssm_v, ssmd_v, wi_v, wsp_v, bsp_v, wo_v, c_v, wmod_v,
            fwd_v, inv_v, out_v,
            chan_s, bsp_s, mod_s, fstage, ktile, utile, kraw, khat, uhat, g_s, y_s, x1_s, xn_s, hq_s, hr_s, wq_s,
            a_s, z1_s, z2_s, wb_s, m_s, wot_s, wor_s, woq_s, pq_s, pr_s, o_s, sems, out_sems):
    copies = {}

    def queue(name, src, dst):
        group = copies.setdefault(name, [])
        group.append(pltpu.make_async_copy(src, dst, sems.at[list(copies).index(name)]))
        group[-1].start()

    def wait(*names):
        for name in names:
            for copy in copies[name]:
                copy.wait()

    def rows(ref, r0, n):
        return ref.at[pl.ds(r0, n), :]

    def queue_pairs(name, src, dst, r0, n):
        queue(name, rows(src, r0, n), rows(dst, r0 // 2, n // 2).bitcast(BF16))

    def queue_wmod(name, i0, i1):
        queue(name, wmod_hbm.at[:, i0 * D:i1 * D], wmod_v.at[:, i0 * D:i1 * D])

    queue("small", fwd_hbm, fwd_v)
    queue("small", inv_hbm, inv_v)
    for src, dst in ((ssmd_hbm, ssmd_v), (shift_hbm, shift_v), (c_hbm, c_v), (bsp_hbm, bsp_v)):
        queue("small", src, dst)
    n = S // SPLIT
    for c in range(NCT):
        queue(f"tile{c}", rows(ssm_hbm, c * L, L), rows(ssm_v, c * L, L))
        for h in range(SPLIT):
            for src, dst, pad in ((k_hbm, k_v, 8), (v_hbm, v_v, 0)):
                queue(f"tile{c}", src.at[pl.ds(h * n, n), pl.ds(c * L, L)],
                      dst.at[c, pl.ds(pad + h * n // 2, n // 2), :].bitcast(BF16))
    queue_pairs("first", q_hbm, q_v, 0, C)
    queue_wmod("first", 0, 3)
    queue_wmod("second", 3, 5)
    wi_groups = {FH: MB, FH + MB: FQ - MB, 0: FQ}
    for r0, n in wi_groups.items():
        for o in (0, FQ):
            queue_pairs(f"wi{r0}", wi_hbm, wi_v, r0 + o, n)
    for i in range(NCH):
        cols = pl.ds(i * C, C)
        queue(f"chunk{i}", wsp_hbm.at[:, cols], wsp_v.at[:, cols].bitcast(BF16))
        if i + 1 < NCH:
            queue_pairs(f"chunk{i}", q_hbm, q_v, (i + 1) * C, C)
    queue_wmod(f"chunk{NCH - 1}", 5, 6)
    queue(f"chunk{NCH - 1}", wo_hbm, wo_v)

    def wait_step(i, names_of, steps):
        for n in steps:
            @pl.when(i == n)
            def _():
                wait(*names_of(n))

    def span(start, size):
        return pl.ds(start if isinstance(start, int) else pl.multiple_of(start, size), size)

    latest = [None]

    def paced(x):
        if latest[0] is None:
            return x
        n = x.shape[1] // L
        never = jnp.tile(fwd_v[0, 0:8, :], (1, n)) == NEVER
        return jnp.where(never, pltpu.bitcast(jnp.tile(latest[0], (1, n)), x.dtype), x)

    def ticks(m):
        for r in range(0, m.shape[0], TICK):
            latest[0] = m[r:r + 8, 0:L]
            yield
        return m

    def load_group(ref, k2, g):
        return ref[k2 + zero, 16 * g:16 * g + 8, :], ref[k2 + zero, 16 * g + 8:16 * g + 16, :]

    def store_group(ref, k2, g, val):
        ref[k2, 16 * g:16 * g + 8, :] = val[0]
        ref[k2, 16 * g + 8:16 * g + 16, :] = val[1]

    def spectrum_groups(tiles):
        e = [_dot(_bf16(fwd_v[p]), _bf16(tiles[p + zero])) for p in range(4)]
        for g in range(NPOS):
            latest[0] = e[0][16 * g:16 * g + 8]
            yield _radix4([(x[16 * g:16 * g + 8], x[16 * g + 8:16 * g + 16]) for x in e], False)

    def filter_tiles(c, m):
        fstage[m][...] = pltpu.bitcast(ssm_v[span(c * L, L), m * C:(m + 1) * C].T, U32)
        for u in range(L // 16):
            for s in range(2):
                a = paced(fstage[m][pl.ds(16 * u + s, 8, stride=2), :])
                b = fstage[m][pl.ds(L + 16 * u + s, 8, stride=2), :]
                ktile[m][2 * s, 8 * u:8 * u + 8, :] = _pack(_lo(a), _lo(b))
                ktile[m][2 * s + 1, 8 * u:8 * u + 8, :] = _pack(_hi(a), _hi(b))
            yield

    def signal_tiles(c, j):
        w1, w2, w3 = [chan_s[c, t] for t in range(1, KS)]
        for u in range(L // 16):
            halves = []
            for h in range(2):
                w0 = paced(chan_s[c, 0])
                r0 = j * CH + h * L + 16 * u
                kw = [k_v[c, pl.ds(8 + r0 + o, 8, stride=2), :] for o in range(-2, 2)]
                vw = [v_v[c, pl.ds(r0 + o, 8, stride=2), :] for o in range(2)]
                ks = [_hi(kw[0])] + [f(x) for x in kw[1:] for f in (_lo, _hi)]
                vs = [f(x) for x in vw for f in (_lo, _hi)]
                halves.append([((w0 * ks[p + 3] + w1 * ks[p + 2]) + (w2 * ks[p + 1] + w3 * ks[p]))
                               * vs[p] for p in range(4)])
                if h == 1:
                    for p in range(4):
                        utile[j][p, 8 * u:8 * u + 8, :] = _pack(halves[0][p], halves[1][p])
                yield

    def filter_spectrum(c, m):
        for g, kk in enumerate(spectrum_groups(ktile[m])):
            for k2 in range(4):
                re, im = kk[k2]
                if m == 0:
                    knew = (re + chan_s[c, KS], im)
                else:
                    if m == 1:
                        pre, pim = load_group(khat[0].at[c % 2], k2, g)
                        pre = pre - chan_s[c, KS]
                    else:
                        pre, pim = load_group(kraw[m % 2], k2, g)
                    knew = (re - pim, im + pre) if g < NPOS // 2 else (re + pim, im - pre)
                if 0 < m < NCH - 1:
                    store_group(kraw[(m + 1) % 2], k2, g, kk[k2])
                store_group(khat[m].at[c % 2], k2, g, knew)
            yield

    def signal_spectrum(c, j):
        for g, uu in enumerate(spectrum_groups(utile[j])):
            for k2 in range(4):
                store_group(uhat[j], k2, g, uu[k2])
            yield

    def chunk_product(c, i):
        for g in range(NPOS):
            ys = []
            for k2 in range(4):
                yr = yi = None
                for j in range(i + 1):
                    kr, ki = load_group(khat[i - j].at[c % 2], k2, g)
                    ur, ui = load_group(uhat[j], k2, g)
                    if j == 0:
                        kr = paced(kr)
                    pr, pi = kr * ur - ki * ui, kr * ui + ki * ur
                    yr, yi = (pr, pi) if yr is None else (yr + pr, yi + pi)
                ys.append((yr, yi))
                if k2 == 3:
                    for p, pair in enumerate(_radix4(ys, True)):
                        g_s[i][p, 8 * g:8 * g + 8, :] = _pack(*pair)
                yield

    def inverse_dft(c, i):
        y = None
        for k0 in range(0, 2 * L, L):
            part = [_dot(_bf16(inv_v[p, :, k0:k0 + L]), _bf16(g_s[i][p + zero, k0 // 2:(k0 + L) // 2, :]))
                    for p in range(4)]
            for r in range(0, L, 16):
                latest[0] = part[0][r:r + 8]
                if y is not None:
                    for o in (r, r + 8):
                        full = [a[o:o + 8] + b[o:o + 8] for a, b in zip(y, part)]
                        for s in range(2):
                            y_s[c, pl.ds(i * CH + 2 * o + s, 8, stride=2), :] = (
                                _pack(full[2 * s], full[2 * s + 1]))
                yield
            y = part

    for ref in [x.at[0] for x in khat] + uhat + [g_s[NCH - 2]]:
        ref[...] = jnp.zeros(ref.shape, ref.dtype)
    k_v[:, 0:8, :] = jnp.zeros((NCT, 8, L), U32)
    wait("small")
    probe = pltpu.bitcast(fwd_v[0, 0:8, :], jnp.int32)[0, 0]
    zero = (probe == NEVER).astype(jnp.int32)
    n_blocks = itertools.count()

    def block(name, *streams):
        latest[0] = None

        @pl.when(probe != NEVER + next(n_blocks))
        def _():
            with _scope(name):
                _interleave(*streams)

        latest[0] = None

    dvec = ssmd_v[...].astype(F32)
    taps = shift_v[...].astype(F32)
    for i in range(NCT):
        chan_s[i, KS] = jnp.broadcast_to(dvec[i:i + 1], (8, L))
        for t in range(KS):
            chan_s[i, t] = jnp.broadcast_to(taps[t:t + 1, i * L:(i + 1) * L], (8, L))

    stages = dict(T=filter_tiles, A=signal_tiles, K=filter_spectrum, B=signal_spectrum,
                  C=chunk_product, D=inverse_dft)

    def conv_step(c, carry):
        wait_step(c, lambda n: [f"tile{n}"], range(NCT))
        before = jnp.maximum(c - 1, 0)
        streams = {x: stages[x[0]](before if x in CARRIED else c, int(x[1]))
                   for x in CONV_MATMULS + CONV_VECTOR}
        latest[0] = None
        for x in _conv_schedule():
            next(streams[x])
        latest[0] = None
        return carry

    with _scope("conv"):
        lax.fori_loop(0, NCT, conv_step, 0)

    def store_modulated(r, h):
        ops = [_strassen_rhs(h[0][s][:, :DM], h[1][s][:, :DM],
                             h[0][s][:, DM:2 * DM], h[1][s][:, DM:2 * DM]) for s in range(2)]
        for q in range(7):
            hq_s[q, r:r + 8, :] = _pack(ops[0][q], ops[1][q])
        for a in range(2):
            hr_s[a * L + r:a * L + r + 8, :] = _pack(h[a][0][:, 2 * DM:], h[a][1][:, 2 * DM:])

    def residual_stage(i):
        for r in range(0, L, 8):
            h = []
            for a in range(2):
                at = span(i * CH + a * L + r, 8)
                xw = q_v[at, :]
                yw = jnp.concatenate([y_s[c, at, :] for c in range(NCT)], axis=1)
                xw = jnp.concatenate([paced(xw[:, :L]), xw[:, L:]], axis=1)
                x1 = [half(xw) + (_layernorm_rows(half(xw)) * mod_s[0] + mod_s[1]) * half(yw)
                      for half in (_lo, _hi)]
                x1_s[at, :] = _pack(*x1)
                h.append([_layernorm_rows(x) * mod_s[2] + mod_s[3] for x in x1])
                if a == 1:
                    store_modulated(r, h)
                yield

    cv = c_v[...].astype(F32)
    act = jnp.broadcast_to(cv * jax.nn.sigmoid(cv), (16, D)).astype(BF16)

    def modulation(i):
        return _dot(act, wmod_v[:, i * D:(i + 1) * D])[:8]

    def first_gate():
        sa, ca, ga = [modulation(i) for i in range(3)]
        mod_s[0] = (1.0 + ca) * ga
        mod_s[1] = sa * ga
        latest[0] = ga[:, :L]
        yield

    def first_norm():
        for r in range(0, CH, 8):
            xw = q_v[r:r + 8, :]
            xw = jnp.concatenate([paced(xw[:, :L]), xw[:, L:]], axis=1)
            for s, half in enumerate((_lo, _hi)):
                xn_s[s, r:r + 8, :] = _layernorm_rows(half(xw))
            yield

    def first_residual():
        done = []
        for r in range(0, CH, 8):
            latest[0] = done[-DEPTH] if len(done) >= DEPTH else None
            yw = jnp.concatenate([paced(y_s[0, r:r + 8, :])]
                                 + [y_s[c, r:r + 8, :] for c in range(1, NCT)], axis=1)
            x1 = [half(q_v[r:r + 8, :]) + (xn_s[s, r:r + 8, :] * mod_s[0] + mod_s[1]) * half(yw)
                  for s, half in enumerate((_lo, _hi))]
            x1_s[r:r + 8, :] = _pack(*x1)
            for s in range(2):
                xn = _layernorm_rows(x1[s])
                xn_s[s, r:r + 8, :] = xn
            done.append(xn[:, :L])
            yield

    def first_modulate():
        wait("second")
        shift, scale = modulation(3), 1.0 + modulation(4)
        mod_s[2] = scale
        mod_s[3] = shift
        for r in range(0, L, 8):
            store_modulated(r, [[xn_s[s, a * L + r:a * L + r + 8, :] * scale + shift
                                 for s in range(2)] for a in range(2)])
        yield

    wait("first")
    block("drain",
          (itertools.chain(inverse_dft(NCT - 1, 2), first_gate(), range(24),
                           inverse_dft(NCT - 1, 3)), 2 * NPOS + 25),
          (itertools.chain(chunk_product(NCT - 1, 3), range(32)), 4 * NPOS + 32),
          (first_norm(), CH // 8))
    block("res0", (first_residual(), 1))
    block("mod", (first_modulate(), 1))

    def hidden_stage(i, first=False, extra=None):
        def weight_sums(r0):
            for r in range(r0 // 2, (r0 + MB) // 2, 8):
                top, bot = slice(r, r + 8), slice(r + FQ // 2, r + FQ // 2 + 8)
                w = [paced(wi_v[top, :DM]), wi_v[top, DM:2 * DM],
                     wi_v[bot, :DM], paced(wi_v[bot, DM:2 * DM])]
                lo, hi = _strassen_lhs(*[_lo(x) for x in w]), _strassen_lhs(*[_hi(x) for x in w])
                for slot, q in enumerate(SUMMED_LHS):
                    wq_s[slot, top, :] = _pack(lo[q], hi[q])
                yield

        def preact(r0):
            top = slice(r0 // 2, (r0 + MB) // 2)
            bot = slice((r0 + FQ) // 2, (r0 + FQ + MB) // 2)
            if first and r0 in wi_groups:
                wait(f"wi{r0}")
            sums = weight_sums(r0) if first else iter(())

            def product(q):
                w = (wi_v[top, :DM] if q == 2 else wi_v[bot, DM:2 * DM] if q == 3
                     else wq_s[SUMMED_LHS.index(q), top, :])
                m = _dot_nt(_bf16(w), _bf16(hq_s[q]))
                for _ in ticks(m):
                    next(sums, None)
                    yield
                return m

            rest = []
            for part in (top, bot):
                rest.append(_dot_nt(_bf16(wi_v[part, 2 * DM:]), _bf16(hr_s[...])))
                for _ in ticks(rest[-1]):
                    next(sums, None)
                    yield
            z = yield from _strassen_product(product)
            return lambda b, r: z[b](r) + rest[b // 2][r, (b % 2) * CH:(b % 2 + 1) * CH]

        def column_mean(acc):
            return jnp.broadcast_to(jnp.sum(acc, axis=0, keepdims=True) * (1.0 / FH), (8, C))

        total = [jnp.zeros((8, CH), F32)] * 2

        def activate():
            for r0 in range(0, FQ, MB):
                z = yield from preact(FH + r0)
                for b in (1, 2, 0, 3):
                    for r in range(0, MB, 16):
                        a = _gelu2(z(b, slice(r, r + 16)))
                        f = (b // 2) * FQ + r0 + r
                        a_s[f:f + 16, (b % 2) * CH:(b % 2 + 1) * CH] = a
                        total[b % 2] = total[b % 2] + (a[:8] + a[8:])

        n_ticks = 9 * FQ // TICK
        _interleave((activate(), n_ticks), *([extra] if extra else []))
        mean = column_mean(jnp.concatenate(total, axis=1))

        def layernorm():
            acc = jnp.zeros((8, C), F32)
            for r in range(0, FH, 32):
                d = _tiles(a_s[r:r + 32, :]) - paced(mean)
                acc = acc + (d * d).sum(axis=0)
                yield
            rstd = lax.rsqrt(column_mean(acc) + 4.0 * EPS)
            means = [mean[:, c0:c0 + L] for c0 in range(0, C, L)]
            for r in range(0, FQ, 16):
                for c0 in range(0, CH, L):
                    blocks = []
                    for o in (0, FQ):
                        for cols in (slice(c0, c0 + L), slice(CH + c0, CH + c0 + L)):
                            m = means[cols.start // L]
                            if (o == 0) == (cols.start == c0):
                                m = paced(m)
                            d = (_tiles(a_s[o + r:o + r + 16, cols]) - m) * rstd[:, cols]
                            blocks.append(d.reshape(16, L))
                    for q, op in enumerate(_strassen_lhs(*blocks)):
                        z2_s[q, r:r + 16, c0:c0 + L] = op.astype(BF16)
                    yield

        def gate():
            for r0 in range(0, FQ, MB):
                z = yield from preact(r0)
                for b in (1, 2, 0, 3):
                    for r in range(0, MB, 16):
                        f = (b // 2) * FQ + r0 + r
                        z1_s[f:f + 16, span(i * C + (b % 2) * CH, CH)] = (
                            z(b, slice(r, r + 16)).astype(BF16))

        _interleave((gate(), n_ticks), (layernorm(), FH // 32 + FQ // 8))
        yield

    def mixer_sums(i):
        left, right = span(i * C, CH), span(i * C + CH, CH)
        for n in range(NCH):
            for r in range(0, CH // 2, 8):
                top = slice(n * CH + r, n * CH + r + 8)
                bot = slice(n * CH + CH // 2 + r, n * CH + CH // 2 + r + 8)
                w = [paced(wsp_v[top, left]), wsp_v[bot, left],
                     wsp_v[top, right], paced(wsp_v[bot, right])]
                lo, hi = _strassen_rhs(*[_lo(x) for x in w]), _strassen_rhs(*[_hi(x) for x in w])
                for slot, q in enumerate(SUMMED):
                    wb_s[slot, n * CH // 2 + r:n * CH // 2 + r + 8, :] = _pack(lo[q], hi[q])
                yield

    def mixer_operand(i, q, n):
        if q in SUMMED:
            return wb_s[SUMMED.index(q), span(n * (CH // 2), CH // 2), :]
        o = 0 if q == 1 else 1
        return wsp_v[span(n * CH + o * (CH // 2), CH // 2), span(i * C + o * CH, CH)]

    def mixer_partial(i, products):
        for n in range(0, NCH, 2):
            for q in products:
                w = jnp.concatenate([mixer_operand(i, q, n), mixer_operand(i, q, n + 1)], axis=0)
                cols = slice(n * CH, (n + 2) * CH)
                for r0 in range(0, FQ, MB):
                    m = _dot_nt(z2_s[q, r0:r0 + MB, :], _bf16(w))
                    for r in range(0, MB, 8):
                        at = (q, slice(r0 + r, r0 + r + 8), cols)
                        m_s[at] = jnp.where(i > 0, m_s[at], 0.0) + m[r:r + 8]
                    for r in range(0, MB, MB // TICKS):
                        latest[0] = m[r:r + 8, 0:L]
                        yield

    def partial_stage(i):
        ticks = TICKS * 2 * FQ // MB
        _interleave((mixer_partial(i, (1, 4)), 2 * ticks), (mixer_sums(i), NCH * CH // 16))
        _interleave((mixer_partial(i, SUMMED), 5 * ticks), (residual_stage(i + 1), CH // 8))
        yield

    block("hidden0", (hidden_stage(0, first=True), 1))

    def chunk_step(i, carry):
        wait_step(i, lambda n: [f"chunk{n}"], range(NCH - 1))
        block("partial", (partial_stage(i), 1))

        @pl.when(i < NCH - 2)
        def _():
            block("hidden", (hidden_stage(i + 1), 1))

        return carry

    lax.fori_loop(0, NCH - 1, chunk_step, 0)

    def output_operands():
        bvec = bsp_v[...].astype(F32)
        for i in range(S // L):
            bsp_s[:, i * L:(i + 1) * L] = jnp.broadcast_to(bvec[i:i + 1], (8, L))
        wot_s[0] = wo_v[0:FM, :].T
        wot_s[1] = wo_v[FQ:FQ + FM, :].T
        wor_s[...] = jnp.concatenate([wo_v[FM:FQ, :], wo_v[FQ + FM:FH, :]], axis=0).T
        yield from mixer_sums(NCH - 1)
        for r in range(0, DH, 16):
            for c0 in range(0, FM, L):
                blocks = [wot_s[b % 2, r + (b // 2) * DH:r + (b // 2) * DH + 16, c0:c0 + L]
                          for b in range(4)]
                blocks = [x.astype(F32) for x in blocks]
                for b in (0, 3):
                    blocks[b] = jnp.concatenate([paced(blocks[b][:8]), blocks[b][8:]], axis=0)
                for q, op in enumerate(_strassen_lhs(*blocks)):
                    woq_s[q, r:r + 16, c0:c0 + L] = op.astype(BF16)
            yield
        mod_s[4] = 0.5 * modulation(5)

    wait(f"chunk{NCH - 1}")
    block("hidden_last",
          (hidden_stage(NCH - 1, extra=(output_operands(), NCH * CH // 16 + DH // 16)), 1))

    def gated_product(n):
        for r0, r1 in GATE_ROWS:
            def product(q):
                m = yield from ticks(_dot_nt(z2_s[q, r0:r1, :], _bf16(mixer_operand(NCH - 1, q, n))))
                return m_s[q, r0:r1, span(n * CH, CH)] + m

            g = yield from _strassen_product(product)
            for r in range(r0, r1, 16):
                p = []
                for b in range(4):
                    t = span(n * C + (b % 2) * CH, CH)
                    f = (b // 2) * FQ + r
                    gb = _tiles(g[b](slice(r - r0, r - r0 + 16))) + bsp_s[:, t]
                    p.append(_gelu2(z1_s[f:f + 16, t].astype(F32)) * gb.reshape(16, CH))
                if r < FM:
                    for q, op in enumerate(_strassen_rhs(*p)):
                        pq_s[q, r:r + 16, :] = op.astype(BF16)
                else:
                    for b in range(4):
                        f = (b // 2) * (FQ - FM) + r - FM
                        pr_s[f:f + 16, (b % 2) * CH:(b % 2 + 1) * CH] = p[b].astype(BF16)

    def project():
        rest = yield from ticks(_dot(wor_s[...], pr_s[...]))
        o = yield from _strassen_product(lambda q: ticks(_dot(woq_s[q], pq_s[q])))
        for b in (1, 2, 0, 3):
            for r in range(0, DH, 8):
                d = (b // 2) * DH + r
                o_s[b % 2, d:d + 8, :] = (o[b](slice(r, r + 8))
                                          + rest[d:d + 8, (b % 2) * CH:(b % 2 + 1) * CH])

    def out_copy(n, h):
        at = span(n * C + h * CH, CH)
        return pltpu.make_async_copy(out_v.at[at, :], out_hbm.at[at, :], out_sems.at[0])

    def finish(n):
        for h in range(2):
            for t0 in range(0, CH, L):
                for c in range(NCT):
                    cols = slice(c * L, (c + 1) * L)
                    o = o_s[h, cols, t0:t0 + L].T
                    x1 = _bf16(x1_s[span(n * CH + (h * CH + t0) // 2, L // 2), cols]).astype(F32)
                    res = _tiles(x1) + mod_s[4, :, cols] * _tiles(o)
                    out_v[span(n * C + h * CH + t0, L), cols] = res.reshape(L, L).astype(BF16)
                    yield
            out_copy(n, h).start()

    gate_ticks = 7 * sum(-(-(r1 - r0) // TICK) for r0, r1 in GATE_ROWS)
    block("gate0", (gated_product(0), 1))

    def output_step(n, carry):
        latest[0] = None
        _interleave((project(), 1))
        _interleave((gated_product(n + 1), gate_ticks), (finish(n), 8 * NCT))
        return carry

    with _scope("output"):
        lax.fori_loop(0, NCH - 1, output_step, 0)
    block("output_last", (itertools.chain(project(), finish(NCH - 1)), 1))
    for n in range(NCH):
        for h in range(2):
            out_copy(n, h).wait()


@jax.jit
def pallas_adaLN_cond__ssm_conv_h3__mixer_gmlp__prompt_kernel(
    A_q: jax.Array,
    A_k: jax.Array,
    A_v: jax.Array,
    A_shift_k: jax.Array,
    A_ssm_k: jax.Array,
    A_ssm_D: jax.Array,
    B_x: jax.Array,
    B_w_in: jax.Array,
    B_w_sp: jax.Array,
    B_b_sp: jax.Array,
    B_w_out: jax.Array,
    c: jax.Array,
    w_mod: jax.Array,
):
    del B_x
    operands = (
        A_q.reshape(S, D), A_k.reshape(S, D), A_v.reshape(S, D), A_shift_k.T, A_ssm_k,
        A_ssm_D.reshape(NCT, L), B_w_in.T, B_w_sp, B_b_sp.reshape(S // L, L), B_w_out, c, w_mod,
        _FWD, _INV,
    )
    spectrum = pltpu.VMEM((4, 2 * L, L), F32)
    scratch = [
        pltpu.VMEM((S // 2, D), U32),
        pltpu.VMEM((NCT, 8 + S // 2, L), U32),
        pltpu.VMEM((NCT, S // 2, L), U32),
        pltpu.VMEM((KS, D), BF16),
        pltpu.VMEM((D, S), BF16),
        pltpu.VMEM((NCT, L), BF16),
        pltpu.VMEM((FH, D), U32),
        pltpu.VMEM((S // 2, S), U32),
        pltpu.VMEM((S // L, L), BF16),
        pltpu.VMEM((FH, D), BF16),
        pltpu.VMEM((1, D), BF16),
        pltpu.VMEM((D, 6 * D), BF16),
        pltpu.VMEM(_FWD.shape, U32),
        pltpu.VMEM(_INV.shape, U32),
        pltpu.VMEM((S, D), BF16),
        pltpu.VMEM((NCT, KS + 1, 8, L), F32),
        pltpu.VMEM((8, S), F32),
        pltpu.VMEM((5, 8, D), F32),
        [pltpu.VMEM((CH, L), U32)] * NCH,
        [pltpu.VMEM((4, L // 2, L), U32)] * NCH,
        [pltpu.VMEM((4, L // 2, L), U32)] * NCH,
        [spectrum] * 2,
        [pltpu.VMEM((2, 4, 2 * L, L), F32)] * NCH,
        [spectrum] * NCH,
        [pltpu.VMEM((4, L, L), U32)] * NCH,
        pltpu.VMEM((NCT, S // 2, L), U32),
        pltpu.VMEM((S // 2, D), U32),
        pltpu.VMEM((2, CH, D), F32),
        pltpu.VMEM((7, L, DM), U32),
        pltpu.VMEM((CH, D - 2 * DM), U32),
        pltpu.VMEM((5, FH, DM), U32),
        pltpu.VMEM((FH, C), F32),
        pltpu.VMEM((FH, S), BF16),
        pltpu.VMEM((7, FQ, CH), BF16),
        pltpu.VMEM((5, S // 4, CH), U32),
        pltpu.VMEM((7, FQ, S // 2), F32),
        pltpu.VMEM((2, D, FM), BF16),
        pltpu.VMEM((D, FH - 2 * FM), BF16),
        pltpu.VMEM((7, DH, FM), BF16),
        pltpu.VMEM((7, FM, CH), BF16),
        pltpu.VMEM((FH - 2 * FM, C), BF16),
        pltpu.VMEM((2, D, CH), F32),
        pltpu.SemaphoreType.DMA((15,)),
        pltpu.SemaphoreType.DMA((1,)),
    ]
    out = pl.pallas_call(
        _kernel,
        out_shape=jax.ShapeDtypeStruct((S, D), BF16),
        in_specs=[pl.BlockSpec(memory_space=pltpu.HBM)] * len(operands),
        out_specs=pl.BlockSpec(memory_space=pltpu.HBM),
        scratch_shapes=scratch,
        compiler_params=pltpu.CompilerParams(vmem_limit_bytes=120 * 1024 * 1024),
    )(*operands)
    return out.reshape(1, S, D)
```

```python
import contextlib
import itertools

import numpy as np

import jax
import jax.numpy as jnp
from jax import lax
import jax.experimental.pallas as pl
import jax.experimental.pallas.tpu as pltpu

S = 2048
D = 640
FH = 864
FQ = FH // 2
KS = 4
L = 128
NCT = D // L
C = 512
CH = C // 2
NCH = S // C
NPOS = 16
TICK = 48
TICKS = 3
FINISH_END = 0.9
FILL = 0.97
MB = 144
DEPTH = 12
SPLIT = 4
DH = D // 2
FM = 384
GATE_ROWS = ((0, 128), (128, 256), (256, FQ))
CONV_MATMULS = "D2 K0 K1 K2 D3 B0 K3 B1 D0 B2 D1 B3".split()
CONV_VECTOR = "T0 T1 T2 C3 A0 T3 A1 C0 A2 C1 A3 C2".split()
CONV_BUDGET = 66
CONV_LEAD = 4
CARRIED = ("D2", "C3", "D3")
DM = 256
SUMMED_LHS = (0, 1, 4, 5, 6)
SUMMED = (0, 2, 3, 5, 6)
NEVER = 0x12345678
EPS = 1e-5
GELU_C0 = float(np.sqrt(2.0 / np.pi))
GELU_C1 = GELU_C0 * 0.044715

F32 = jnp.float32
BF16 = jnp.bfloat16
U32 = jnp.uint32
NT_DIMS = (((1,), (1,)), ((), ()))

TRACE_SCOPES = [False]


def _scope(name):
    return jax.named_scope("ph_" + name) if TRACE_SCOPES[0] else contextlib.nullcontext()


def _row_pairs(x):
    bits = x.astype(np.float32).astype(BF16).view(np.uint16).astype(np.uint32)
    return bits[..., 0::2, :] | (bits[..., 1::2, :] << 16)


def _dft_matrices():
    n_fft = 2 * C
    k1 = np.concatenate([np.arange(0, 128, 2), np.arange(1, 128, 2)]).reshape(NPOS, 8)
    fwd = np.zeros((4, 2 * L, L), np.float64)
    inv = np.zeros((4, L, 2 * L), np.float64)
    col_n1 = (np.arange(L) // 2) + 64 * (np.arange(L) % 2)
    for p in range(4):
        n = 4 * np.arange(L) + p
        phase = ((2 * k1[:, :, None] + 1) * n[None, None, :]) % (2 * n_fft)
        theta = np.pi * phase / n_fft
        parts = [np.cos(theta), -np.sin(theta)]
        fwd[p] = np.stack(parts, axis=1).reshape(2 * L, L)[:, col_n1]
        inv[p] = np.stack(parts, axis=2).reshape(2 * L, L).T * (2.0 / n_fft)
    return _row_pairs(fwd), _row_pairs(inv)


_FWD, _INV = _dft_matrices()


def _lo(w):
    return pltpu.unpack_elementwise(w, index=0, packed_dtype=BF16, unpacked_dtype=F32)


def _hi(w):
    return pltpu.unpack_elementwise(w, index=1, packed_dtype=BF16, unpacked_dtype=F32)


def _pack(a, b):
    return pltpu.pack_elementwise([a, b], packed_dtype=BF16)


def _bf16(words):
    return pltpu.bitcast(words, BF16)


def _dot(a, b):
    return jnp.dot(a, b, preferred_element_type=F32)


def _dot_nt(a, b):
    return lax.dot_general(a, b, NT_DIMS, preferred_element_type=F32)


def _tiles(x):
    return x.reshape(x.shape[0] // 8, 8, x.shape[1])


def _interleave(*streams):
    steps = sorted(((k + 0.5) / n, i) for i, (_, n) in enumerate(streams) for k in range(n))
    for _, i in steps:
        next(streams[i][0], None)
    for stream, _ in streams:
        for _ in stream:
            pass


def _spread(stream, n, start, end):
    per_unit = n / (end - start)
    return itertools.chain(range(round(start * per_unit)), stream), round(per_unit)


def _conv_schedule():
    steps = dict(T=8, A=16, C=4 * NPOS)
    cost = dict(T0=24, T1=24, T2=24, T3=24, A0=46, A1=46, A2=46, A3=46, C0=12, C1=20, C2=28, C3=36,
                K0=17, K1=28, K2=24, K3=24, B0=16, B1=16, B2=16, B3=16, D0=6, D1=6, D2=6, D3=6)
    vector = [(x, k) for x in CONV_VECTOR for k in range(steps[x[0]])]
    matmul = [(x, k) for x in CONV_MATMULS for k in range(NPOS)]
    order, done, budget = [], set(), 0
    for n, (x, k) in enumerate(matmul):
        for ahead, _ in matmul[n:n + CONV_LEAD + 1]:
            need = dict(K="T", B="A", D="C")[ahead[0]] + ahead[1]
            while ahead != "D2" and any(v == need for v, _ in vector):
                order.append(vector.pop(0)[0])
                budget -= cost[order[-1]]
        order.append(x)
        done.add((x, k))
        budget = min(budget + CONV_BUDGET - cost[x], CONV_BUDGET)
        while vector and budget > 0:
            v, j = vector[0]
            if v[0] == "C" and v != "C3" and not {("K" + v[1], j // 4), ("B" + v[1], j // 4)} <= done:
                break
            order.append(vector.pop(0)[0])
            budget -= cost[v]
    return order + [v for v, _ in vector]


def _radix4(e, inverse):
    (r0, i0), (r1, i1), (r2, i2), (r3, i3) = e
    sr, si, dr, di = r0 + r2, i0 + i2, r0 - r2, i0 - i2
    tr, ti, ur, ui = r1 + r3, i1 + i3, r1 - r3, i1 - i3
    a = (dr + ui, di - ur)
    b = (dr - ui, di + ur)
    if inverse:
        a, b = b, a
    return [(sr + tr, si + ti), a, (sr - tr, si - ti), b]


def _strassen_lhs(a11, a12, a21, a22):
    return [a11 + a22, a21 + a22, a11, a22, a11 + a12, a21 - a11, a12 - a22]


def _strassen_rhs(b11, b12, b21, b22):
    return [b11 + b22, b11, b12 - b22, b21 - b11, b22, b11 + b12, b21 + b22]


def _strassen_product(product):
    m3 = yield from product(2)
    m4 = yield from product(3)
    m5 = yield from product(4)
    m2 = yield from product(1)
    m1 = yield from product(0)
    m7 = yield from product(6)
    m6 = yield from product(5)
    return [lambda r: (m4[r] - m5[r]) + m1[r] + m7[r], lambda r: m3[r] + m5[r],
            lambda r: m2[r] + m4[r], lambda r: (m3[r] - m2[r]) + m1[r] + m6[r]]


def _gelu2(x):
    t = jnp.tanh(x * (x * x * GELU_C1 + GELU_C0))
    return x * t + x


def _layernorm_rows(x):
    d = x - jnp.sum(x, axis=-1, keepdims=True) * (1.0 / D)
    var = jnp.sum(d * d, axis=-1, keepdims=True) * (1.0 / D)
    return d * lax.rsqrt(var + EPS)


def _kernel(q_hbm, k_hbm, v_hbm, shift_hbm, ssm_hbm, ssmd_hbm, wi_hbm, wsp_hbm, bsp_hbm,
            wo_hbm, c_hbm, wmod_hbm, fwd_hbm, inv_hbm, out_hbm,
            q_v, k_v, v_v, shift_v, ssm_v, ssmd_v, wi_v, wsp_v, bsp_v, wo_v, c_v, wmod_v,
            fwd_v, inv_v, out_v,
            chan_s, bsp_s, mod_s, fstage, ktile, utile, kraw, khat, uhat, g_s, y_s, x1_s, xn_s, hq_s, hr_s, wq_s,
            a_s, z1_s, z2_s, wb_s, m_s, wot_s, wor_s, woq_s, pq_s, pr_s, o_s, sems, out_sem):
    copies = {}

    def queue(name, src, dst):
        group = copies.setdefault(name, [])
        group.append(pltpu.make_async_copy(src, dst, sems.at[list(copies).index(name)]))
        group[-1].start()

    def wait(*names):
        for name in names:
            for copy in copies[name]:
                copy.wait()

    def rows(ref, r0, n):
        return ref.at[pl.ds(r0, n), :]

    def queue_pairs(name, src, dst, r0, n):
        queue(name, rows(src, r0, n), rows(dst, r0 // 2, n // 2).bitcast(BF16))

    def queue_wmod(name, i0, i1):
        queue(name, wmod_hbm.at[:, i0 * D:i1 * D], wmod_v.at[:, i0 * D:i1 * D])

    queue("small", fwd_hbm, fwd_v)
    queue("small", inv_hbm, inv_v)
    for src, dst in ((ssmd_hbm, ssmd_v), (shift_hbm, shift_v), (c_hbm, c_v), (bsp_hbm, bsp_v)):
        queue("small", src, dst)
    n = S // SPLIT
    for c in range(NCT):
        queue(f"tile{c}", rows(ssm_hbm, c * L, L), rows(ssm_v, c * L, L))
        for h in range(SPLIT):
            for src, dst, pad in ((k_hbm, k_v, 8), (v_hbm, v_v, 0)):
                queue(f"tile{c}", src.at[pl.ds(h * n, n), pl.ds(c * L, L)],
                      dst.at[c, pl.ds(pad + h * n // 2, n // 2), :].bitcast(BF16))
    queue_pairs("first", q_hbm, q_v, 0, C)
    queue_wmod("first", 0, 3)
    queue_wmod("second", 3, 5)
    wi_groups = {FH: MB, FH + MB: FQ - MB, 0: FQ}
    for r0, n in wi_groups.items():
        for o in (0, FQ):
            queue_pairs(f"wi{r0}", wi_hbm, wi_v, r0 + o, n)
    for i in range(NCH):
        cols = pl.ds(i * C, C)
        queue(f"chunk{i}", wsp_hbm.at[:, cols], wsp_v.at[:, cols].bitcast(BF16))
        if i + 1 < NCH:
            queue_pairs(f"chunk{i}", q_hbm, q_v, (i + 1) * C, C)
            for o in (0, FQ):
                queue(f"chunk{i}", rows(wo_hbm, o + i * L, L), rows(wo_v, o + i * L, L))
    queue_wmod(f"chunk{NCH - 1}", 5, 6)
    for o in (0, FQ):
        queue(f"chunk{NCH - 1}", rows(wo_hbm, o + FM, FQ - FM), rows(wo_v, o + FM, FQ - FM))

    def wait_step(i, names_of, steps):
        for n in steps:
            @pl.when(i == n)
            def _():
                wait(*names_of(n))

    def span(start, size):
        return pl.ds(start if isinstance(start, int) else pl.multiple_of(start, size), size)

    latest = [None]

    def paced(x):
        if latest[0] is None:
            return x
        n = x.shape[1] // L
        never = jnp.tile(fwd_v[0, 0:8, :], (1, n)) == NEVER
        return jnp.where(never, pltpu.bitcast(jnp.tile(latest[0], (1, n)), x.dtype), x)

    def ticks(m):
        for r in range(0, m.shape[0], TICK):
            latest[0] = m[r:r + 8, 0:L]
            yield
        return m

    def load_group(ref, k2, g):
        return ref[k2 + zero, 16 * g:16 * g + 8, :], ref[k2 + zero, 16 * g + 8:16 * g + 16, :]

    def store_group(ref, k2, g, val):
        ref[k2, 16 * g:16 * g + 8, :] = val[0]
        ref[k2, 16 * g + 8:16 * g + 16, :] = val[1]

    def spectrum_groups(tiles):
        e = [_dot(_bf16(fwd_v[p]), _bf16(tiles[p + zero])) for p in range(4)]
        for g in range(NPOS):
            latest[0] = e[0][16 * g:16 * g + 8]
            yield _radix4([(x[16 * g:16 * g + 8], x[16 * g + 8:16 * g + 16]) for x in e], False)

    def filter_tiles(c, m):
        fstage[m][...] = pltpu.bitcast(ssm_v[span(c * L, L), m * C:(m + 1) * C].T, U32)
        for u in range(L // 16):
            for s in range(2):
                a = paced(fstage[m][pl.ds(16 * u + s, 8, stride=2), :])
                b = fstage[m][pl.ds(L + 16 * u + s, 8, stride=2), :]
                ktile[m][2 * s, 8 * u:8 * u + 8, :] = _pack(_lo(a), _lo(b))
                ktile[m][2 * s + 1, 8 * u:8 * u + 8, :] = _pack(_hi(a), _hi(b))
            yield

    def signal_tiles(c, j):
        w1, w2, w3 = [chan_s[c, t] for t in range(1, KS)]
        for u in range(L // 16):
            halves = []
            for h in range(2):
                w0 = paced(chan_s[c, 0])
                r0 = j * CH + h * L + 16 * u
                kw = [k_v[c, pl.ds(8 + r0 + o, 8, stride=2), :] for o in range(-2, 2)]
                vw = [v_v[c, pl.ds(r0 + o, 8, stride=2), :] for o in range(2)]
                ks = [_hi(kw[0])] + [f(x) for x in kw[1:] for f in (_lo, _hi)]
                vs = [f(x) for x in vw for f in (_lo, _hi)]
                halves.append([((w0 * ks[p + 3] + w1 * ks[p + 2]) + (w2 * ks[p + 1] + w3 * ks[p]))
                               * vs[p] for p in range(4)])
                if h == 1:
                    for p in range(4):
                        utile[j][p, 8 * u:8 * u + 8, :] = _pack(halves[0][p], halves[1][p])
                yield

    def filter_spectrum(c, m):
        for g, kk in enumerate(spectrum_groups(ktile[m])):
            for k2 in range(4):
                re, im = kk[k2]
                if m == 0:
                    knew = (re + chan_s[c, KS], im)
                else:
                    if m == 1:
                        pre, pim = load_group(khat[0].at[c % 2], k2, g)
                        pre = pre - chan_s[c, KS]
                    else:
                        pre, pim = load_group(kraw[m % 2], k2, g)
                    knew = (re - pim, im + pre) if g < NPOS // 2 else (re + pim, im - pre)
                if 0 < m < NCH - 1:
                    store_group(kraw[(m + 1) % 2], k2, g, kk[k2])
                store_group(khat[m].at[c % 2], k2, g, knew)
            yield

    def signal_spectrum(c, j):
        for g, uu in enumerate(spectrum_groups(utile[j])):
            for k2 in range(4):
                store_group(uhat[j], k2, g, uu[k2])
            yield

    def chunk_product(c, i):
        for g in range(NPOS):
            ys = []
            for k2 in range(4):
                yr = yi = None
                for j in range(i + 1):
                    kr, ki = load_group(khat[i - j].at[c % 2], k2, g)
                    ur, ui = load_group(uhat[j], k2, g)
                    if j == 0:
                        kr = paced(kr)
                    pr, pi = kr * ur - ki * ui, kr * ui + ki * ur
                    yr, yi = (pr, pi) if yr is None else (yr + pr, yi + pi)
                ys.append((yr, yi))
                if k2 == 3:
                    for p, pair in enumerate(_radix4(ys, True)):
                        g_s[i][p, 8 * g:8 * g + 8, :] = _pack(*pair)
                yield

    def inverse_dft(c, i):
        y = None
        for k0 in range(0, 2 * L, L):
            part = [_dot(_bf16(inv_v[p, :, k0:k0 + L]), _bf16(g_s[i][p + zero, k0 // 2:(k0 + L) // 2, :]))
                    for p in range(4)]
            for r in range(0, L, 16):
                latest[0] = part[0][r:r + 8]
                if y is not None:
                    for o in (r, r + 8):
                        full = [a[o:o + 8] + b[o:o + 8] for a, b in zip(y, part)]
                        for s in range(2):
                            y_s[c, pl.ds(i * CH + 2 * o + s, 8, stride=2), :] = (
                                _pack(full[2 * s], full[2 * s + 1]))
                yield
            y = part

    for ref in [x.at[0] for x in khat] + uhat + [g_s[NCH - 2]]:
        ref[...] = jnp.zeros(ref.shape, ref.dtype)
    k_v[:, 0:8, :] = jnp.zeros((NCT, 8, L), U32)
    wait("small")
    probe = pltpu.bitcast(fwd_v[0, 0:8, :], jnp.int32)[0, 0]
    zero = (probe == NEVER).astype(jnp.int32)
    n_blocks = itertools.count()

    def block(name, *streams):
        latest[0] = None

        @pl.when(probe != NEVER + next(n_blocks))
        def _():
            with _scope(name):
                _interleave(*streams)

        latest[0] = None

    dvec = ssmd_v[...].astype(F32)
    taps = shift_v[...].astype(F32)
    for i in range(NCT):
        chan_s[i, KS] = jnp.broadcast_to(dvec[i:i + 1], (8, L))
        for t in range(KS):
            chan_s[i, t] = jnp.broadcast_to(taps[t:t + 1, i * L:(i + 1) * L], (8, L))

    stages = dict(T=filter_tiles, A=signal_tiles, K=filter_spectrum, B=signal_spectrum,
                  C=chunk_product, D=inverse_dft)

    def conv_step(c, carry):
        wait_step(c, lambda n: [f"tile{n}"], range(NCT))
        before = jnp.maximum(c - 1, 0)
        streams = {x: stages[x[0]](before if x in CARRIED else c, int(x[1]))
                   for x in CONV_MATMULS + CONV_VECTOR}
        latest[0] = None
        for x in _conv_schedule():
            next(streams[x])
        latest[0] = None
        return carry

    with _scope("conv"):
        lax.fori_loop(0, NCT, conv_step, 0)

    def store_modulated(r, h):
        ops = [_strassen_rhs(h[0][s][:, :DM], h[1][s][:, :DM],
                             h[0][s][:, DM:2 * DM], h[1][s][:, DM:2 * DM]) for s in range(2)]
        for q in range(7):
            hq_s[q, r:r + 8, :] = _pack(ops[0][q], ops[1][q])
        for a in range(2):
            hr_s[a * L + r:a * L + r + 8, :] = _pack(h[a][0][:, 2 * DM:], h[a][1][:, 2 * DM:])

    def residual_stage(i):
        for r in range(0, L, 8):
            h = []
            for a in range(2):
                at = span(i * CH + a * L + r, 8)
                xw = q_v[at, :]
                yw = jnp.concatenate([y_s[c, at, :] for c in range(NCT)], axis=1)
                xw = jnp.concatenate([paced(xw[:, :L]), xw[:, L:]], axis=1)
                x1 = [half(xw) + (_layernorm_rows(half(xw)) * mod_s[0] + mod_s[1]) * half(yw)
                      for half in (_lo, _hi)]
                x1_s[at, :] = _pack(*x1)
                h.append([_layernorm_rows(x) * mod_s[2] + mod_s[3] for x in x1])
                if a == 1:
                    store_modulated(r, h)
                yield

    cv = c_v[...].astype(F32)
    act = jnp.broadcast_to(cv * jax.nn.sigmoid(cv), (16, D)).astype(BF16)

    def modulation(i):
        return _dot(act, wmod_v[:, i * D:(i + 1) * D])[:8]

    def first_gate():
        sa, ca, ga = [modulation(i) for i in range(3)]
        mod_s[0] = (1.0 + ca) * ga
        mod_s[1] = sa * ga
        latest[0] = ga[:, :L]
        yield

    def first_norm():
        for r in range(0, CH, 8):
            xw = q_v[r:r + 8, :]
            xw = jnp.concatenate([paced(xw[:, :L]), xw[:, L:]], axis=1)
            for s, half in enumerate((_lo, _hi)):
                xn_s[s, r:r + 8, :] = _layernorm_rows(half(xw))
            yield

    def first_residual():
        done = []
        for r in range(0, CH, 8):
            latest[0] = done[-DEPTH] if len(done) >= DEPTH else None
            yw = jnp.concatenate([paced(y_s[0, r:r + 8, :])]
                                 + [y_s[c, r:r + 8, :] for c in range(1, NCT)], axis=1)
            x1 = [half(q_v[r:r + 8, :]) + (xn_s[s, r:r + 8, :] * mod_s[0] + mod_s[1]) * half(yw)
                  for s, half in enumerate((_lo, _hi))]
            x1_s[r:r + 8, :] = _pack(*x1)
            for s in range(2):
                xn = _layernorm_rows(x1[s])
                xn_s[s, r:r + 8, :] = xn
            done.append(xn[:, :L])
            yield

    def first_modulate():
        wait("second")
        shift, scale = modulation(3), 1.0 + modulation(4)
        mod_s[2] = scale
        mod_s[3] = shift
        for r in range(0, L, 8):
            store_modulated(r, [[xn_s[s, a * L + r:a * L + r + 8, :] * scale + shift
                                 for s in range(2)] for a in range(2)])
        yield

    wait("first")
    block("drain",
          (itertools.chain(inverse_dft(NCT - 1, 2), first_gate(), range(24),
                           inverse_dft(NCT - 1, 3)), 2 * NPOS + 25),
          _spread(chunk_product(NCT - 1, 3), 4 * NPOS, 0.0, 0.65),
          _spread(first_norm(), CH // 8, 0.0, FILL))
    block("res0", (first_residual(), 1))
    block("mod", (first_modulate(), 1))

    def hidden_stage(i, first=False):
        def weight_sums(r0):
            for r in range(r0 // 2, (r0 + MB) // 2, 8):
                top, bot = slice(r, r + 8), slice(r + FQ // 2, r + FQ // 2 + 8)
                w = [paced(wi_v[top, :DM]), wi_v[top, DM:2 * DM],
                     wi_v[bot, :DM], paced(wi_v[bot, DM:2 * DM])]
                lo, hi = _strassen_lhs(*[_lo(x) for x in w]), _strassen_lhs(*[_hi(x) for x in w])
                for slot, q in enumerate(SUMMED_LHS):
                    wq_s[slot, top, :] = _pack(lo[q], hi[q])
                yield

        def preact(r0):
            top = slice(r0 // 2, (r0 + MB) // 2)
            bot = slice((r0 + FQ) // 2, (r0 + FQ + MB) // 2)
            if first and r0 in wi_groups:
                wait(f"wi{r0}")
            sums = weight_sums(r0) if first else iter(())

            def product(q):
                w = (wi_v[top, :DM] if q == 2 else wi_v[bot, DM:2 * DM] if q == 3
                     else wq_s[SUMMED_LHS.index(q), top, :])
                m = _dot_nt(_bf16(w), _bf16(hq_s[q]))
                for _ in ticks(m):
                    next(sums, None)
                    yield
                return m

            rest = []
            for part in (top, bot):
                rest.append(_dot_nt(_bf16(wi_v[part, 2 * DM:]), _bf16(hr_s[...])))
                for _ in ticks(rest[-1]):
                    next(sums, None)
                    yield
            z = yield from _strassen_product(product)
            return lambda b, r: z[b](r) + rest[b // 2][r, (b % 2) * CH:(b % 2 + 1) * CH]

        def column_mean(acc):
            return jnp.broadcast_to(jnp.sum(acc, axis=0, keepdims=True) * (1.0 / FH), (8, C))

        total = [jnp.zeros((8, CH), F32)] * 2

        def activate():
            for r0 in range(0, FQ, MB):
                z = yield from preact(FH + r0)
                for b in (1, 2, 0, 3):
                    for r in range(0, MB, 16):
                        a = _gelu2(z(b, slice(r, r + 16)))
                        f = (b // 2) * FQ + r0 + r
                        a_s[f:f + 16, (b % 2) * CH:(b % 2 + 1) * CH] = a
                        total[b % 2] = total[b % 2] + (a[:8] + a[8:])

        def layernorm():
            mean = column_mean(jnp.concatenate(total, axis=1))
            acc = jnp.zeros((8, C), F32)
            for r in range(0, FH, 32):
                d = _tiles(a_s[r:r + 32, :]) - paced(mean)
                acc = acc + (d * d).sum(axis=0)
                yield
            rstd = lax.rsqrt(column_mean(acc) + 4.0 * EPS)
            means = [mean[:, c0:c0 + L] for c0 in range(0, C, L)]
            for r in range(0, FQ, 16):
                for c0 in range(0, CH, L):
                    blocks = []
                    for o in (0, FQ):
                        for cols in (slice(c0, c0 + L), slice(CH + c0, CH + c0 + L)):
                            m = means[cols.start // L]
                            if (o == 0) == (cols.start == c0):
                                m = paced(m)
                            d = (_tiles(a_s[o + r:o + r + 16, cols]) - m) * rstd[:, cols]
                            blocks.append(d.reshape(16, L))
                    for q, op in enumerate(_strassen_lhs(*blocks)):
                        z2_s[q, r:r + 16, c0:c0 + L] = op.astype(BF16)
                    yield

        def gate():
            for r0 in range(0, FQ, MB):
                z = yield from preact(r0)
                for b in (1, 2, 0, 3):
                    for r in range(0, MB, 16):
                        f = (b // 2) * FQ + r0 + r
                        z1_s[f:f + 16, span(i * C + (b % 2) * CH, CH)] = (
                            z(b, slice(r, r + 16)).astype(BF16))

        return ((itertools.chain(activate(), gate()), 18 * FQ // TICK),
                _spread(layernorm(), FH // 32 + FQ // 8, 0.51, FILL))

    def mixer_sums(i, n):
        left, right = span(i * C, CH), span(i * C + CH, CH)
        for r in range(0, L, 8):
            top, bot = span(n * CH + r, 8), span(n * CH + L + r, 8)
            w = [paced(wsp_v[top, left]), wsp_v[bot, left],
                 wsp_v[top, right], paced(wsp_v[bot, right])]
            lo, hi = _strassen_rhs(*[_lo(x) for x in w]), _strassen_rhs(*[_hi(x) for x in w])
            for slot, q in enumerate(SUMMED):
                wb_s[slot, span(n * L + r, 8), :] = _pack(lo[q], hi[q])
            yield

    def mixer_operand(i, q, n):
        if q in SUMMED:
            return wb_s[SUMMED.index(q), span(n * L, L), :]
        o = 0 if q == 1 else 1
        return wsp_v[span(n * CH + o * L, L), span(i * C + o * CH, CH)]

    def mixer_partial(i):
        for products in ((1, 4), SUMMED):
            for n in range(0, NCH, 2):
                for q in products:
                    w = jnp.concatenate([mixer_operand(i, q, n + o) for o in range(2)], axis=0)
                    for r0 in range(0, FQ, MB):
                        m = _dot_nt(z2_s[q, r0:r0 + MB, :], _bf16(w))
                        for r in range(0, MB, 8):
                            at = (q, slice(r0 + r, r0 + r + 8), slice(n * CH, (n + 2) * CH))
                            m_s[at] = jnp.where(i > 0, m_s[at], 0.0) + m[r:r + 8]
                        yield from ticks(m)

    def output_operands(i):
        for a in range(2):
            wot_s[a] = wo_v[pl.ds(pl.multiple_of(a * FQ + i * L, 16), L), :].T
        for r in range(0, DH, 16):
            blocks = [wot_s[b % 2, r + (b // 2) * DH:r + (b // 2) * DH + 16, :].astype(F32)
                      for b in range(4)]
            for b in (0, 3):
                blocks[b] = jnp.concatenate([paced(blocks[b][:8]), blocks[b][8:]], axis=0)
            for q, op in enumerate(_strassen_lhs(*blocks)):
                woq_s[q, r:r + 16, span(i * L, L)] = op.astype(BF16)
            yield

    block("hidden0", *hidden_stage(0, first=True))

    def chunk_step(i, carry):
        wait_step(i, lambda n: [f"chunk{n}"], range(NCH - 1))
        block("partial", (mixer_partial(i), 14 * FQ // TICK),
              _spread(itertools.chain(*[mixer_sums(i, n) for n in range(NCH)]),
                      NCH * L // 8, 0.0, 0.3),
              _spread(residual_stage(i + 1), CH // 8, 0.25, 0.85),
              _spread(output_operands(i), DH // 16, 0.8, FILL))
        block("hidden", *hidden_stage(i + 1))
        return carry

    lax.fori_loop(0, NCH - 1, chunk_step, 0)

    def gated_product(n):
        for r0, r1 in GATE_ROWS:
            def product(q):
                m = yield from ticks(_dot_nt(z2_s[q, r0:r1, :], _bf16(mixer_operand(NCH - 1, q, n))))
                return m_s[q, r0:r1, span(n * CH, CH)] + m

            g = yield from _strassen_product(product)
            for r in range(r0, r1, 16):
                p = []
                for b in range(4):
                    t = span(n * C + (b % 2) * CH, CH)
                    f = (b // 2) * FQ + r
                    gb = _tiles(g[b](slice(r - r0, r - r0 + 16))) + bsp_s[:, t]
                    p.append(_gelu2(z1_s[f:f + 16, t].astype(F32)) * gb.reshape(16, CH))
                if r < FM:
                    for q, op in enumerate(_strassen_rhs(*p)):
                        pq_s[q, r:r + 16, :] = op.astype(BF16)
                else:
                    for b in range(4):
                        f = (b // 2) * (FQ - FM) + r - FM
                        pr_s[f:f + 16, (b % 2) * CH:(b % 2 + 1) * CH] = p[b].astype(BF16)

    def project():
        rest = yield from ticks(_dot(wor_s[...], pr_s[...]))
        o = yield from _strassen_product(lambda q: ticks(_dot(woq_s[q], pq_s[q])))
        for b in (1, 2, 0, 3):
            for r in range(0, DH, 8):
                d = (b // 2) * DH + r
                o_s[b % 2, d:d + 8, :] = (o[b](slice(r, r + 8))
                                          + rest[d:d + 8, (b % 2) * CH:(b % 2 + 1) * CH])

    def out_copy(row, n):
        return pltpu.make_async_copy(
            out_v.at[span(row, n), :], out_hbm.at[span(row, n), :], out_sem.at[0])

    def finish(n, h, t0):
        for c in range(NCT):
            cols = slice(c * L, (c + 1) * L)
            o = o_s[h, cols, t0:t0 + L].T
            x1 = _bf16(x1_s[span(n * CH + (h * CH + t0) // 2, L // 2), cols]).astype(F32)
            gate = paced(mod_s[4, :, cols])
            res = _tiles(x1) + gate * _tiles(o)
            out_v[span(n * C + h * CH + t0, L), cols] = res.reshape(L, L).astype(BF16)
            yield

    quarters = [(h, t0) for h in range(2) for t0 in range(0, CH, L)]
    wait(f"chunk{NCH - 1}")
    bvec = bsp_v[...].astype(F32)
    for i in range(S // L):
        bsp_s[:, i * L:(i + 1) * L] = jnp.broadcast_to(bvec[i:i + 1], (8, L))
    wor_s[...] = jnp.concatenate([wo_v[FM:FQ, :], wo_v[FQ + FM:FH, :]], axis=0).T
    mod_s[4] = 0.5 * modulation(5)
    _interleave((mixer_sums(NCH - 1, 0), 1))

    _interleave((gated_product(0), 1))

    def output_step(n, carry):
        latest[0] = None
        _interleave((project(), -(-D // TICK) + 7 * -(-DH // TICK)),
                    _spread(mixer_sums(NCH - 1, n + 1), L // 8, 0.0, 0.7))
        _interleave((gated_product(n + 1), 7 * sum(-(-(b - a) // TICK) for a, b in GATE_ROWS)),
                    _spread(itertools.chain(*[finish(n, *x) for x in quarters]),
                            4 * NCT, 0.0, FINISH_END))
        out_copy(n * C, C).start()
        return carry

    with _scope("output"):
        lax.fori_loop(0, NCH - 1, output_step, 0)
    _interleave((project(), 1))
    latest[0] = None
    for h in range(2):
        _interleave(*[(finish(NCH - 1, h, t0), NCT) for t0 in range(0, CH, L)])
        out_copy((NCH - 1) * C + h * CH, CH).start()
    for n in range(NCH - 1):
        out_copy(n * C, C).wait()
    for h in range(2):
        out_copy((NCH - 1) * C + h * CH, CH).wait()


@jax.jit
def pallas_adaLN_cond__ssm_conv_h3__mixer_gmlp__prompt_kernel(
    A_q: jax.Array,
    A_k: jax.Array,
    A_v: jax.Array,
    A_shift_k: jax.Array,
    A_ssm_k: jax.Array,
    A_ssm_D: jax.Array,
    B_x: jax.Array,
    B_w_in: jax.Array,
    B_w_sp: jax.Array,
    B_b_sp: jax.Array,
    B_w_out: jax.Array,
    c: jax.Array,
    w_mod: jax.Array,
):
    del B_x
    operands = (
        A_q.reshape(S, D), A_k.reshape(S, D), A_v.reshape(S, D), A_shift_k.T, A_ssm_k,
        A_ssm_D.reshape(NCT, L), B_w_in.T, B_w_sp, B_b_sp.reshape(S // L, L), B_w_out, c, w_mod,
        _FWD, _INV,
    )
    spectrum = pltpu.VMEM((4, 2 * L, L), F32)
    scratch = [
        pltpu.VMEM((S // 2, D), U32),
        pltpu.VMEM((NCT, 8 + S // 2, L), U32),
        pltpu.VMEM((NCT, S // 2, L), U32),
        pltpu.VMEM((KS, D), BF16),
        pltpu.VMEM((D, S), BF16),
        pltpu.VMEM((NCT, L), BF16),
        pltpu.VMEM((FH, D), U32),
        pltpu.VMEM((S // 2, S), U32),
        pltpu.VMEM((S // L, L), BF16),
        pltpu.VMEM((FH, D), BF16),
        pltpu.VMEM((1, D), BF16),
        pltpu.VMEM((D, 6 * D), BF16),
        pltpu.VMEM(_FWD.shape, U32),
        pltpu.VMEM(_INV.shape, U32),
        pltpu.VMEM((S, D), BF16),
        pltpu.VMEM((NCT, KS + 1, 8, L), F32),
        pltpu.VMEM((8, S), F32),
        pltpu.VMEM((5, 8, D), F32),
        [pltpu.VMEM((CH, L), U32)] * NCH,
        [pltpu.VMEM((4, L // 2, L), U32)] * NCH,
        [pltpu.VMEM((4, L // 2, L), U32)] * NCH,
        [spectrum] * 2,
        [pltpu.VMEM((2, 4, 2 * L, L), F32)] * NCH,
        [spectrum] * NCH,
        [pltpu.VMEM((4, L, L), U32)] * NCH,
        pltpu.VMEM((NCT, S // 2, L), U32),
        pltpu.VMEM((S // 2, D), U32),
        pltpu.VMEM((2, CH, D), F32),
        pltpu.VMEM((7, L, DM), U32),
        pltpu.VMEM((CH, D - 2 * DM), U32),
        pltpu.VMEM((5, FH, DM), U32),
        pltpu.VMEM((FH, C), F32),
        pltpu.VMEM((FH, S), BF16),
        pltpu.VMEM((7, FQ, CH), BF16),
        pltpu.VMEM((5, S // 4, CH), U32),
        pltpu.VMEM((7, FQ, S // 2), F32),
        pltpu.VMEM((2, D, L), BF16),
        pltpu.VMEM((D, FH - 2 * FM), BF16),
        pltpu.VMEM((7, DH, FM), BF16),
        pltpu.VMEM((7, FM, CH), BF16),
        pltpu.VMEM((FH - 2 * FM, C), BF16),
        pltpu.VMEM((2, D, CH), F32),
        pltpu.SemaphoreType.DMA((15,)),
        pltpu.SemaphoreType.DMA((1,)),
    ]
    out = pl.pallas_call(
        _kernel,
        out_shape=jax.ShapeDtypeStruct((S, D), BF16),
        in_specs=[pl.BlockSpec(memory_space=pltpu.HBM)] * len(operands),
        out_specs=pl.BlockSpec(memory_space=pltpu.HBM),
        scratch_shapes=scratch,
        compiler_params=pltpu.CompilerParams(vmem_limit_bytes=120 * 1024 * 1024),
    )(*operands)
    return out.reshape(1, S, D)
```

```python
import contextlib
import itertools

import numpy as np

import jax
import jax.numpy as jnp
from jax import lax
import jax.experimental.pallas as pl
import jax.experimental.pallas.tpu as pltpu

S = 2048
D = 640
FH = 864
FQ = FH // 2
KS = 4
L = 128
NCT = D // L
C = 512
CH = C // 2
NCH = S // C
NPOS = 16
TICK = 24
TICKS = 3
FINISH_END = 0.9
RES_START = 0.3
RES_END = 0.9
GATE_ORDER = (1, 4, 2, 3, 0, 5, 6)
MP = 144
SUMS_END = 0.3
LATE = 2
FILL = 0.97
MB = 144
DEPTH = 12
SPLIT = 4
DH = D // 2
FM = 384
GATE_ROWS = ((0, 144), (144, 288), (288, FQ))
CONV_MATMULS = "K3 D3 B0 B1 D0 B2 D1 B3 D2 K0 K1 K2".split()
CONV_VECTOR = "A0 T2 A1 A3 T3 C0 A2 C1 C2 T1 T0 C3".split()
CONV_AHEAD = "T0 T1 T2 T3 K0 K1 K2".split()
CONV_PACE = 4
CONV_LAG = 0
CONV_DEBT = 1000
CONV_BUDGET = 71
CONV_LEAD = 4
DM = 256
SUMMED_LHS = (0, 1, 4, 5, 6)
SUMMED = (0, 2, 3, 5, 6)
NEVER = 0x7F7F7F7F
EPS = 1e-5
GELU_C0 = float(np.sqrt(2.0 / np.pi))
GELU_C1 = GELU_C0 * 0.044715

F32 = jnp.float32
BF16 = jnp.bfloat16
U32 = jnp.uint32
NT_DIMS = (((1,), (1,)), ((), ()))

TRACE_SCOPES = [False]


def _scope(name):
    return jax.named_scope("ph_" + name) if TRACE_SCOPES[0] else contextlib.nullcontext()


def _lo(w):
    return pltpu.unpack_elementwise(w, index=0, packed_dtype=BF16, unpacked_dtype=F32)


def _hi(w):
    return pltpu.unpack_elementwise(w, index=1, packed_dtype=BF16, unpacked_dtype=F32)


def _pack(a, b):
    return pltpu.pack_elementwise([a, b], packed_dtype=BF16)


def _bf16(words):
    return pltpu.bitcast(words, BF16)


def _riffle(x):
    return _pack(x[:8], x[8:])


def _dot(a, b):
    return jnp.dot(a, b, preferred_element_type=F32)


def _dot_nt(a, b):
    return lax.dot_general(a, b, NT_DIMS, preferred_element_type=F32)


def _tiles(x):
    return x.reshape(x.shape[0] // 8, 8, x.shape[1])


def _interleave(*streams):
    steps = sorted(((k + 0.5) / n, i) for i, (_, n) in enumerate(streams) for k in range(n))
    for _, i in steps:
        next(streams[i][0], None)
    for stream, _ in streams:
        for _ in stream:
            pass


def _spread(stream, n, start, end):
    per_unit = n / (end - start)
    return itertools.chain(range(round(start * per_unit)), stream), round(per_unit)


def _conv_schedule():
    steps = dict(T=8, A=16, C=4 * NPOS)
    cost = dict(T0=24, T1=24, T2=24, T3=24, A0=46, A1=46, A2=46, A3=46, C0=12, C1=20, C2=28, C3=36,
                K0=17, K1=28, K2=24, K3=24, B0=16, B1=16, B2=16, B3=16, D0=6, D1=6, D2=6, D3=6)
    vector = [(x, k) for x in CONV_VECTOR for k in range(steps[x[0]])]
    matmul = [(x, k) for x in CONV_MATMULS for k in range(NPOS)]
    order, done, budget = [], set(), 0
    for n, (x, k) in enumerate(matmul):
        for ahead, _ in matmul[n:n + CONV_LEAD + 1]:
            need = dict(K="T", B="A", D="C")[ahead[0]] + ahead[1]
            while ahead not in ("K3", "D3") and any(v == need for v, _ in vector):
                order.append(vector.pop(0)[0])
                budget -= cost[order[-1]]
        order.append(x)
        done.add((x, k))
        budget = min(max(budget, -CONV_DEBT) + CONV_BUDGET - cost[x], CONV_BUDGET)
        while vector and budget > 0:
            v, j = vector[0]
            if v[0] == "C" and ("B" + v[1], min(j // 4 + CONV_LAG, NPOS - 1)) not in done:
                break
            order.append(vector.pop(0)[0])
            budget -= cost[v]
    return order + [v for v, _ in vector]


def _radix4(e, inverse):
    (r0, i0), (r1, i1), (r2, i2), (r3, i3) = e
    sr, si, dr, di = r0 + r2, i0 + i2, r0 - r2, i0 - i2
    tr, ti, ur, ui = r1 + r3, i1 + i3, r1 - r3, i1 - i3
    a = (dr + ui, di - ur)
    b = (dr - ui, di + ur)
    if inverse:
        a, b = b, a
    return [(sr + tr, si + ti), a, (sr - tr, si - ti), b]


def _strassen_lhs(a11, a12, a21, a22):
    return [a11 + a22, a21 + a22, a11, a22, a11 + a12, a21 - a11, a12 - a22]


STRASSEN_RHS_NEEDS = ((0, 3), (0,), (1, 3), (0, 2), (3,), (0, 1), (2, 3))


def _strassen_rhs(b11, b12, b21, b22):
    return [b11 + b22, b11, b12 - b22, b21 - b11, b22, b11 + b12, b21 + b22]


STRASSEN_USES = ({0: 1, 3: 1}, {2: 1, 3: -1}, {1: 1, 3: 1}, {0: 1, 2: 1}, {0: -1, 1: 1}, {3: 1}, {0: 1})


def _pieces(x):
    return [x[r:r + 16] for r in range(0, x.shape[0], 16)]


def _strassen_product(product, order, blocks, complete):
    blocks = list(blocks)
    for n, q in enumerate(order):
        m = _pieces((yield from product(q)))
        for b, sign in STRASSEN_USES[q].items():
            if blocks[b] is None:
                blocks[b] = m if sign > 0 else [-x for x in m]
            else:
                blocks[b] = [x + y if sign > 0 else x - y for x, y in zip(blocks[b], m)]
            if not any(b in STRASSEN_USES[later] for later in order[n + 1:]):
                complete(b, blocks[b])


def _gelu2(x):
    t = jnp.tanh(x * (x * x * GELU_C1 + GELU_C0))
    return x * t + x


def _layernorm_rows(x):
    d = x - jnp.sum(x, axis=-1, keepdims=True) * (1.0 / D)
    var = jnp.sum(d * d, axis=-1, keepdims=True) * (1.0 / D)
    return d * lax.rsqrt(var + EPS)


def _kernel(q_hbm, k_hbm, v_hbm, shift_hbm, ssm_hbm, ssmd_hbm, wi_hbm, wsp_hbm, bsp_hbm,
            wo_hbm, c_hbm, wmod_hbm, out_hbm,
            q_v, k_v, v_v, shift_v, ssm_v, ssmd_v, wi_v, wsp_v, bsp_v, wo_v, c_v, wmod_v,
            fwd_v, inv_v, out_v,
            chan_s, bsp_s, mod_s, fstage, ktile, utile, kraw, khat, uhat, g_s, y_s, x1_s, xn_s, hq_s, hr_s, wq_s,
            a_s, z1_s, z2_s, wb_s, m_s, wot_s, wor_s, woq_s, pq_s, pr_s, o_s, sems, out_sem):
    copies = {}

    def queue(name, src, dst):
        group = copies.setdefault(name, [])
        group.append(pltpu.make_async_copy(src, dst, sems.at[list(copies).index(name)]))
        group[-1].start()

    def wait(*names):
        for name in names:
            for copy in copies[name]:
                copy.wait()

    def rows(ref, r0, n):
        return ref.at[pl.ds(r0, n), :]

    def queue_pairs(name, src, dst, r0, n):
        queue(name, rows(src, r0, n), rows(dst, r0 // 2, n // 2).bitcast(BF16))

    def queue_wmod(name, i0, i1):
        queue(name, wmod_hbm.at[:, i0 * D:i1 * D], wmod_v.at[:, i0 * D:i1 * D])

    queue("small", rows(ssm_hbm, 0, L), rows(ssm_v, 0, L))
    for src, dst in ((ssmd_hbm, ssmd_v), (shift_hbm, shift_v), (c_hbm, c_v), (bsp_hbm, bsp_v)):
        queue("small", src, dst)
    n = S // SPLIT
    for c in range(NCT):
        for h in range(SPLIT):
            for src, dst, pad in ((k_hbm, k_v, 8), (v_hbm, v_v, 0)):
                queue(f"tile{c}", src.at[pl.ds(h * n, n), pl.ds(c * L, L)],
                      dst.at[c, pl.ds(pad + h * n // 2, n // 2), :].bitcast(BF16))
        if c + 1 < NCT:
            queue(f"tile{c}", rows(ssm_hbm, (c + 1) * L, L), rows(ssm_v, (c + 1) * L, L))
    queue_pairs("first", q_hbm, q_v, 0, C)
    queue_wmod("first", 0, 3)
    queue_wmod("second", 3, 5)
    wi_groups = {FH: MB, FH + MB: FQ - MB, 0: FQ}
    for r0, n in wi_groups.items():
        for o in (0, FQ):
            queue_pairs(f"wi{r0}", wi_hbm, wi_v, r0 + o, n)
    for i in range(NCH):
        cols = pl.ds(i * C, C)
        queue(f"chunk{i}", wsp_hbm.at[:, cols], wsp_v.at[:, cols].bitcast(BF16))
        if i + 1 < NCH:
            queue_pairs(f"chunk{i}", q_hbm, q_v, (i + 1) * C, C)
        if i == 1:
            queue("chunk1", wo_hbm, wo_v)
    queue_wmod(f"chunk{NCH - 1}", 5, 6)

    def wait_step(i, names_of, steps):
        for n in steps:
            @pl.when(i == n)
            def _():
                wait(*names_of(n))

    def span(start, size):
        return pl.ds(start if isinstance(start, int) else pl.multiple_of(start, size), size)

    latest = [None]

    def paced(x):
        if latest[0] is None:
            return x
        n = x.shape[1] // L
        never = jnp.tile(fwd_v[0, 0:8, :], (1, n)) == NEVER
        return jnp.where(never, pltpu.bitcast(jnp.tile(latest[0], (1, n)), x.dtype), x)

    overdue = []

    def hurried(words):
        head = words[:8, :L]
        while len(overdue) > LATE:
            head = jnp.where(fwd_v[0, 0:8, :] == NEVER, overdue.pop(0), head)
        head = jnp.concatenate([head, words[:8, L:]], axis=1)
        return jnp.concatenate([head, words[8:]], axis=0)

    def ticks(m):
        for r in range(0, m.shape[0], TICK):
            latest[0] = m[r:r + 8, 0:L]
            yield
        return m

    def load_group(ref, k2, g):
        return ref[k2 + zero, 16 * g:16 * g + 8, :], ref[k2 + zero, 16 * g + 8:16 * g + 16, :]

    def store_group(ref, k2, g, val):
        ref[k2, 16 * g:16 * g + 8, :] = val[0]
        ref[k2, 16 * g + 8:16 * g + 16, :] = val[1]

    def spectrum_groups(tiles):
        e = [_dot(_bf16(fwd_v[p]), _bf16(tiles[p + zero])) for p in range(4)]
        for g in range(NPOS):
            latest[0] = e[0][16 * g:16 * g + 8]
            yield _radix4([(x[16 * g:16 * g + 8], x[16 * g + 8:16 * g + 16]) for x in e], False)

    def dft_matrices():
        sub = lax.broadcasted_iota(jnp.int32, (8, L), 0)
        lane = lax.broadcasted_iota(jnp.int32, (8, L), 1)

        def unit(turns):
            angle = (((turns + 2 * C) & (4 * C - 1)) - 2 * C).astype(F32) * (np.pi / (2 * C))
            return jnp.cos(angle), -jnp.sin(angle)

        def times(a, b):
            return a[0] * b[0] - a[1] * b[1], a[0] * b[1] + a[1] * b[0]

        for p in range(4):
            n = 4 * ((lane >> 1) + (L // 2) * (lane & 1)) + p
            fwd, fwd1, fwd16 = unit((4 * sub + 1) * n), unit(2 * n), unit(32 * n)
            n = 4 * lane + p
            inv = unit((4 * (sub >> 1) + 1) * n + C * (sub & 1))
            inv1, inv8 = unit(2 * n), unit(16 * n)
            for parity in range(2):
                w = times(fwd, fwd1) if parity else fwd
                for g in range(NPOS // 2):
                    fwd_v.bitcast(BF16)[p, pl.ds(L * parity + 16 * g, 16), :] = (
                        jnp.concatenate(w, axis=0).astype(BF16))
                    w = times(w, fwd16)
                w = times(inv, inv1) if parity else inv
                rows_t = []
                for g in range(NPOS):
                    rows_t.append(w[0] * (1.0 / C))
                    w = times(w, inv8)
                inv_v.bitcast(BF16)[p, :, parity * L:(parity + 1) * L] = (
                    jnp.concatenate(rows_t, axis=0).T.astype(BF16))

    def last_tile(c):
        return c if isinstance(c, int) else jnp.minimum(c, NCT - 1)

    def filter_tiles(c, m):
        fstage[m][...] = pltpu.bitcast(ssm_v[span(last_tile(c) * L, L), m * C:(m + 1) * C].T, U32)
        for u in range(L // 16):
            for s in range(2):
                a = paced(fstage[m][pl.ds(16 * u + s, 8, stride=2), :])
                b = fstage[m][pl.ds(L + 16 * u + s, 8, stride=2), :]
                ktile[m][2 * s, 8 * u:8 * u + 8, :] = _pack(_lo(a), _lo(b))
                ktile[m][2 * s + 1, 8 * u:8 * u + 8, :] = _pack(_hi(a), _hi(b))
            yield

    def signal_tiles(c, j):
        w1, w2, w3 = [chan_s[c, t] for t in range(1, KS)]
        for u in range(L // 16):
            halves = []
            for h in range(2):
                w0 = paced(chan_s[c, 0])
                r0 = j * CH + h * L + 16 * u
                kw = [k_v[c, pl.ds(8 + r0 + o, 8, stride=2), :] for o in range(-2, 2)]
                vw = [v_v[c, pl.ds(r0 + o, 8, stride=2), :] for o in range(2)]
                ks = [_hi(kw[0])] + [f(x) for x in kw[1:] for f in (_lo, _hi)]
                vs = [f(x) for x in vw for f in (_lo, _hi)]
                halves.append([((w0 * ks[p + 3] + w1 * ks[p + 2]) + (w2 * ks[p + 1] + w3 * ks[p]))
                               * vs[p] for p in range(4)])
                if h == 1:
                    for p in range(4):
                        utile[j][p, 8 * u:8 * u + 8, :] = _pack(halves[0][p], halves[1][p])
                yield

    def filter_spectrum(c, m):
        for g, kk in enumerate(spectrum_groups(ktile[m])):
            for k2 in range(4):
                re, im = kk[k2]
                if m == 0:
                    knew = (re + chan_s[last_tile(c), KS], im)
                else:
                    if m == 1:
                        pre, pim = load_group(khat[0].at[c % 2], k2, g)
                        pre = pre - chan_s[last_tile(c), KS]
                    else:
                        pre, pim = load_group(kraw[m % 2], k2, g)
                    knew = (re - pim, im + pre) if g < NPOS // 2 else (re + pim, im - pre)
                if 0 < m < NCH - 1:
                    store_group(kraw[(m + 1) % 2], k2, g, kk[k2])
                store_group(khat[m].at[c % 2], k2, g, knew)
            yield

    def signal_spectrum(c, j):
        for g, uu in enumerate(spectrum_groups(utile[j])):
            for k2 in range(4):
                store_group(uhat[j], k2, g, uu[k2])
            yield

    def chunk_product(c, i):
        for g in range(NPOS):
            ys = []
            for k2 in range(4):
                yr = yi = None
                for j in range(i + 1):
                    kr, ki = load_group(khat[i - j].at[c % 2], k2, g)
                    ur, ui = load_group(uhat[j], k2, g)
                    if j == 0 and k2 % CONV_PACE == 0:
                        kr = paced(kr)
                    pr, pi = kr * ur - ki * ui, kr * ui + ki * ur
                    yr, yi = (pr, pi) if yr is None else (yr + pr, yi + pi)
                ys.append((yr, yi))
                if k2 == 3:
                    for p, pair in enumerate(_radix4(ys, True)):
                        g_s[i][p, 8 * g:8 * g + 8, :] = _pack(*pair)
                yield

    def inverse_dft(c, i):
        y = None
        for k0 in range(0, 2 * L, L):
            part = [_dot(_bf16(inv_v[p, :, k0:k0 + L]), _bf16(g_s[i][p + zero, k0 // 2:(k0 + L) // 2, :]))
                    for p in range(4)]
            for r in range(0, L, 16):
                latest[0] = part[0][r:r + 8]
                if y is not None:
                    for o in (r, r + 8):
                        full = [a[o:o + 8] + b[o:o + 8] for a, b in zip(y, part)]
                        for s in range(2):
                            y_s[c, pl.ds(i * CH + 2 * o + s, 8, stride=2), :] = (
                                _pack(full[2 * s], full[2 * s + 1]))
                yield
            y = part

    dft_matrices()
    g_s[NCH - 1][...] = jnp.zeros(g_s[NCH - 1].shape, U32)
    k_v[:, 0:8, :] = jnp.zeros((NCT, 8, L), U32)
    wait("small")
    probe = pltpu.bitcast(fwd_v[0, 0:8, :], jnp.int32)[0, 0]
    zero = (probe == NEVER).astype(jnp.int32)
    n_blocks = itertools.count()

    def block(name, *streams):
        latest[0] = None
        overdue.clear()

        @pl.when(probe != NEVER + next(n_blocks))
        def _():
            with _scope(name):
                _interleave(*streams)

        latest[0] = None

    dvec = ssmd_v[...].astype(F32)
    taps = shift_v[...].astype(F32)
    for i in range(NCT):
        chan_s[i, KS] = jnp.broadcast_to(dvec[i:i + 1], (8, L))
        for t in range(KS):
            chan_s[i, t] = jnp.broadcast_to(taps[t:t + 1, i * L:(i + 1) * L], (8, L))

    stages = dict(T=filter_tiles, A=signal_tiles, K=filter_spectrum, B=signal_spectrum,
                  C=chunk_product, D=inverse_dft)

    def conv_step(c, carry):
        wait_step(c, lambda n: [f"tile{n}"], range(NCT))
        tile = dict(D3=jnp.maximum(c - 1, 0), **{x: c + 1 for x in CONV_AHEAD})
        streams = {x: stages[x[0]](tile.get(x, c), int(x[1])) for x in CONV_MATMULS + CONV_VECTOR}
        latest[0] = None
        for x in _conv_schedule():
            next(streams[x])
        latest[0] = None
        return carry

    block("fill", (itertools.chain(*[stages[x[0]](0, int(x[1])) for x in CONV_AHEAD]), 1))
    with _scope("conv"):
        lax.fori_loop(0, NCT, conv_step, 0)

    def store_modulated(r, h):
        ops = [_strassen_rhs(h[0][s][:, :DM], h[1][s][:, :DM],
                             h[0][s][:, DM:2 * DM], h[1][s][:, DM:2 * DM]) for s in range(2)]
        for q in range(7):
            words = _pack(ops[0][q], ops[1][q])
            hq_s[q, r:r + 8, :] = words
            if q == 0:
                overdue.append(words[:, :L])
        for a in range(2):
            hr_s[a * L + r:a * L + r + 8, :] = _pack(h[a][0][:, 2 * DM:], h[a][1][:, 2 * DM:])

    def residual_stage(i):
        for r in range(0, L, 8):
            h = []
            for a in range(2):
                at = span(i * CH + a * L + r, 8)
                xw = q_v[at, :]
                yw = jnp.concatenate([y_s[c, at, :] for c in range(NCT)], axis=1)
                xw = jnp.concatenate([paced(xw[:, :L]), xw[:, L:]], axis=1)
                x1 = [half(xw) + (_layernorm_rows(half(xw)) * mod_s[0] + mod_s[1]) * half(yw)
                      for half in (_lo, _hi)]
                x1_s[at, :] = _pack(*x1)
                h.append([_layernorm_rows(x) * mod_s[2] + mod_s[3] for x in x1])
                if a == 1:
                    store_modulated(r, h)
                yield

    cv = c_v[...].astype(F32)
    act = jnp.broadcast_to(cv * jax.nn.sigmoid(cv), (16, D)).astype(BF16)

    def modulation(i):
        return _dot(act, wmod_v[:, i * D:(i + 1) * D])[:8]

    def first_gate():
        sa, ca, ga = [modulation(i) for i in range(3)]
        mod_s[0] = (1.0 + ca) * ga
        mod_s[1] = sa * ga
        latest[0] = ga[:, :L]
        yield

    def first_norm():
        for r in range(0, CH, 8):
            xw = q_v[r:r + 8, :]
            xw = jnp.concatenate([paced(xw[:, :L]), xw[:, L:]], axis=1)
            for s, half in enumerate((_lo, _hi)):
                xn_s[s, r:r + 8, :] = _layernorm_rows(half(xw))
            yield

    def first_residual():
        done = []
        for r in range(0, CH, 8):
            latest[0] = done[-DEPTH] if len(done) >= DEPTH else None
            yw = jnp.concatenate([paced(y_s[0, r:r + 8, :])]
                                 + [y_s[c, r:r + 8, :] for c in range(1, NCT)], axis=1)
            x1 = [half(q_v[r:r + 8, :]) + (xn_s[s, r:r + 8, :] * mod_s[0] + mod_s[1]) * half(yw)
                  for s, half in enumerate((_lo, _hi))]
            x1_s[r:r + 8, :] = _pack(*x1)
            for s in range(2):
                xn = _layernorm_rows(x1[s])
                xn_s[s, r:r + 8, :] = xn
            done.append(xn[:, :L])
            yield

    def first_modulate():
        wait("second")
        shift, scale = modulation(3), 1.0 + modulation(4)
        mod_s[2] = scale
        mod_s[3] = shift
        for r in range(0, L, 8):
            store_modulated(r, [[xn_s[s, a * L + r:a * L + r + 8, :] * scale + shift
                                 for s in range(2)] for a in range(2)])
        yield

    wait("first")
    block("drain", (itertools.chain(inverse_dft(NCT - 1, NCH - 1), first_gate()), NPOS + 1),
          _spread(first_norm(), CH // 8, 0.0, 0.5))
    block("res0", (first_residual(), 1))
    block("mod", (first_modulate(), 1))

    def hidden_stage(i, first=False):
        def weight_sums(r0):
            for r in range(r0 // 2, (r0 + MB) // 2, 8):
                top, bot = slice(r, r + 8), slice(r + FQ // 2, r + FQ // 2 + 8)
                w = [paced(wi_v[top, :DM]), wi_v[top, DM:2 * DM],
                     wi_v[bot, :DM], paced(wi_v[bot, DM:2 * DM])]
                lo, hi = _strassen_lhs(*[_lo(x) for x in w]), _strassen_lhs(*[_hi(x) for x in w])
                for slot, q in enumerate(SUMMED_LHS):
                    wq_s[slot, top, :] = _pack(lo[q], hi[q])
                yield

        def preact(r0, complete):
            top = slice(r0 // 2, (r0 + MB) // 2)
            bot = slice((r0 + FQ) // 2, (r0 + FQ + MB) // 2)
            if first and r0 in wi_groups:
                wait(f"wi{r0}")
            sums = weight_sums(r0) if first else iter(())

            def product(q):
                w = (wi_v[top, :DM] if q == 2 else wi_v[bot, DM:2 * DM] if q == 3
                     else wq_s[SUMMED_LHS.index(q), top, :])
                m = _dot_nt(_bf16(w), _bf16(hq_s[q]))
                for _ in ticks(m):
                    next(sums, None)
                    yield
                return m

            rest = []
            for part in (top, bot):
                rest.append(_dot_nt(_bf16(wi_v[part, 2 * DM:]), _bf16(hr_s[...])))
                for _ in ticks(rest[-1]):
                    next(sums, None)
                    yield
            yield from _strassen_product(
                product, (2, 3, 4, 1, 0, 6, 5),
                [_pieces(rest[b // 2][:, (b % 2) * CH:(b % 2 + 1) * CH]) for b in range(4)], complete)

        def column_mean(acc):
            return jnp.broadcast_to(jnp.sum(acc, axis=0, keepdims=True) * (1.0 / FH), (8, C))

        total = [jnp.zeros((8, CH), F32)] * 2

        def activate():
            for r0 in range(0, FQ, MB):
                def complete(b, z):
                    for n, x in enumerate(z):
                        a = _gelu2(x)
                        f = (b // 2) * FQ + r0 + 16 * n
                        a_s[f:f + 16, (b % 2) * CH:(b % 2 + 1) * CH] = a
                        total[b % 2] = total[b % 2] + (a[:8] + a[8:])

                yield from preact(FH + r0, complete)

        def layernorm():
            mean = column_mean(jnp.concatenate(total, axis=1))
            acc = jnp.zeros((8, C), F32)
            for r in range(0, FH, 32):
                d = _tiles(a_s[r:r + 32, :]) - paced(mean)
                acc = acc + (d * d).sum(axis=0)
                yield
            rstd = lax.rsqrt(column_mean(acc) + 4.0 * EPS)
            means = [mean[:, c0:c0 + L] for c0 in range(0, C, L)]
            for r in range(0, FQ, 16):
                for c0 in range(0, CH, L):
                    blocks = []
                    for o in (0, FQ):
                        for cols in (slice(c0, c0 + L), slice(CH + c0, CH + c0 + L)):
                            m = means[cols.start // L]
                            if (o == 0) == (cols.start == c0):
                                m = paced(m)
                            d = (_tiles(a_s[o + r:o + r + 16, cols]) - m) * rstd[:, cols]
                            blocks.append(d.reshape(16, L))
                    for q, op in enumerate(_strassen_lhs(*blocks)):
                        z2_s[q, r // 2:r // 2 + 8, c0:c0 + L] = _riffle(op)
                    yield

        def gate():
            for r0 in range(0, FQ, MB):
                def complete(b, z):
                    for n, x in enumerate(z):
                        f = ((b // 2) * FQ + r0) // 2 + 8 * n
                        z1_s[f:f + 8, span(i * C + (b % 2) * CH, CH)] = _riffle(_gelu2(x))

                yield from preact(r0, complete)

        return ((itertools.chain(activate(), gate()), 18 * FQ // TICK),
                _spread(layernorm(), FH // 32 + FQ // 8, 0.51, FILL))

    def mixer_sums(i, n):
        left, right = span(i * C, CH), span(i * C + CH, CH)
        for r in range(0, L, 8):
            top, bot = span(n * CH + r, 8), span(n * CH + L + r, 8)
            w = [paced(wsp_v[top, left]), wsp_v[bot, left],
                 wsp_v[top, right], paced(wsp_v[bot, right])]
            lo, hi = _strassen_rhs(*[_lo(x) for x in w]), _strassen_rhs(*[_hi(x) for x in w])
            for slot, q in enumerate(SUMMED):
                wb_s[slot, span(n * L + r, 8), :] = _pack(lo[q], hi[q])
            yield

    def mixer_operand(i, q, n):
        if q in SUMMED:
            return wb_s[SUMMED.index(q), span(n * L, L), :]
        o = 0 if q == 1 else 1
        return wsp_v[span(n * CH + o * L, L), span(i * C + o * CH, CH)]

    def mixer_partial(i):
        for products in ((1, 4), SUMMED):
            for n in range(0, NCH, 2):
                for q in products:
                    w = jnp.concatenate([mixer_operand(i, q, n + o) for o in range(2)], axis=0)
                    for r0 in range(0, FQ, MP):
                        m = _dot_nt(_bf16(hurried(z2_s[q, r0 // 2:(r0 + MP) // 2, :])), _bf16(w))
                        for r in range(0, MP, 8):
                            at = (q, slice(r0 + r, r0 + r + 8), slice(n * CH, (n + 2) * CH))
                            m_s[at] = jnp.where(i > 0, m_s[at], 0.0) + m[r:r + 8]
                        yield from ticks(m)

    def output_columns(starts):
        def group(f):
            x = wo_v[pl.ds(f if isinstance(f, int) else pl.multiple_of(f, 16), 16), :]
            for _ in range(2):
                x = _bf16(_riffle(x.astype(F32)))
            return x

        return jnp.concatenate([group(f) for f in starts], axis=0).T

    def output_operands(i):
        for a in range(2):
            wot_s[a] = output_columns([a * FQ + i * L + r for r in range(0, L, 16)])
        for r in range(0, DH, 16):
            w = [pltpu.bitcast(wot_s[b % 2, r + (b // 2) * DH:r + (b // 2) * DH + 16, :], U32)
                 for b in range(4)]
            w[0], w[3] = paced(w[0]), paced(w[3])
            lo, hi = _strassen_lhs(*[_lo(x) for x in w]), _strassen_lhs(*[_hi(x) for x in w])
            for q in range(7):
                woq_s[q, r // 2:r // 2 + 8, span(i * L, L)] = _pack(lo[q], hi[q])
            yield

    block("hidden0", *hidden_stage(0, first=True))

    wait("chunk0")

    def chunk_step(i, carry):
        block("partial", (mixer_partial(i), 14 * FQ // TICK),
              _spread(itertools.chain(*[mixer_sums(i, n) for n in range(NCH)]),
                      NCH * L // 8, 0.0, SUMS_END),
              _spread(residual_stage(i + 1), CH // 8, RES_START, RES_END))
        wait_step(i, lambda n: [f"chunk{n + 1}"], range(NCH - 1))
        block("hidden", *hidden_stage(i + 1), _spread(output_operands(i), DH // 16, 0.1, 0.45))
        return carry

    lax.fori_loop(0, NCH - 1, chunk_step, 0)

    def gated_product(n):
        for r0, r1 in GATE_ROWS:
            def product(q):
                m = yield from ticks(_dot_nt(_bf16(z2_s[q, r0 // 2:r1 // 2, :]),
                                             _bf16(mixer_operand(NCH - 1, q, n))))
                return m_s[q, r0:r1, span(n * CH, CH)] + m

            p = {}

            def complete(b, g):
                t = span(n * C + (b % 2) * CH, CH)
                p[b] = []
                for k, x in enumerate(g):
                    r = r0 + 16 * k
                    f = ((b // 2) * FQ + r) // 2
                    z1 = _bf16(z1_s[f:f + 8, t]).astype(F32)
                    p[b].append(z1 * (_tiles(x) + bsp_s[:, t]).reshape(16, CH))
                    if r >= FM:
                        f = ((b // 2) * (FQ - FM) + r - FM) // 2
                        pr_s[f:f + 8, (b % 2) * CH:(b % 2 + 1) * CH] = _riffle(p[b][k])
                        continue
                    ops = _strassen_rhs(*[p[a][k] if a in p else x for a in range(4)])
                    for q, needs in enumerate(STRASSEN_RHS_NEEDS):
                        if b in needs and all(a in p for a in needs):
                            pq_s[q, r // 2:r // 2 + 8, :] = _riffle(ops[q])

            yield from _strassen_product(product, GATE_ORDER, [None] * 4, complete)

    def project():
        rest = yield from ticks(_dot(wor_s[...], _bf16(pr_s[...])))

        def complete(b, o):
            for k, x in enumerate(o):
                d = (b // 2) * DH + 16 * k
                o_s[b % 2, d:d + 16, :] = x

        yield from _strassen_product(
            lambda q: ticks(_dot(_bf16(woq_s[q]), _bf16(pq_s[q]))), (1, 3, 4, 0, 6, 2, 5),
            [_pieces(rest[(b // 2) * DH:(b // 2 + 1) * DH, (b % 2) * CH:(b % 2 + 1) * CH])
             for b in range(4)], complete)

    def out_copy(row, n, c0=0, c1=NCT):
        at = (span(row, n), slice(c0 * L, c1 * L))
        return pltpu.make_async_copy(out_v.at[at], out_hbm.at[at], out_sem.at[0])

    def finish(n, h, c0=0, c1=NCT):
        for c in reversed(range(c0, c1)):
            for t0 in range(0, CH, L):
                cols = slice(c * L, (c + 1) * L)
                o = o_s[h, cols, t0:t0 + L].T
                x1 = _bf16(x1_s[span(n * CH + (h * CH + t0) // 2, L // 2), cols]).astype(F32)
                res = _tiles(x1) + mod_s[4, :, cols] * _tiles(o)
                out_v[span(n * C + h * CH + t0, L), cols] = res.reshape(L, L).astype(BF16)
                yield

    bvec = bsp_v[...].astype(F32)
    for i in range(S // L):
        bsp_s[:, i * L:(i + 1) * L] = jnp.broadcast_to(bvec[i:i + 1], (8, L))
    wor_s[...] = output_columns([a * FQ + r for a in range(2) for r in range(FM, FQ, 16)])
    gate_ticks = 7 * sum(-(-(b - a) // TICK) for a, b in GATE_ROWS)
    _interleave((gated_product(0), gate_ticks), (mixer_sums(NCH - 1, 0), 10 * L // 8 + 8))
    mod_s[4] = 0.5 * modulation(5)

    def output_step(n, carry):
        latest[0] = None
        _interleave((project(), -(-D // TICK) + 7 * -(-DH // TICK)),
                    _spread(mixer_sums(NCH - 1, n + 1), L // 8, 0.0, 0.7))
        _interleave((gated_product(n + 1), gate_ticks),
                    _spread(itertools.chain(finish(n, 0), finish(n, 1)),
                            4 * NCT, 0.0, FINISH_END))
        out_copy(n * C, C).start()
        return carry

    with _scope("output"):
        lax.fori_loop(0, NCH - 1, output_step, 0)
    _interleave((project(), 1))
    latest[0] = None
    last_parts = ((0, 0, NCT), (1, 0, DH // L), (1, DH // L, NCT))
    for h, c0, c1 in last_parts:
        _interleave((finish(NCH - 1, h, c0, c1), 1))
        out_copy((NCH - 1) * C + h * CH, CH, c0, c1).start()
    for n in range(NCH - 1):
        out_copy(n * C, C).wait()
    for h, c0, c1 in last_parts:
        out_copy((NCH - 1) * C + h * CH, CH, c0, c1).wait()


@jax.jit
def pallas_adaLN_cond__ssm_conv_h3__mixer_gmlp__prompt_kernel(
    A_q: jax.Array,
    A_k: jax.Array,
    A_v: jax.Array,
    A_shift_k: jax.Array,
    A_ssm_k: jax.Array,
    A_ssm_D: jax.Array,
    B_x: jax.Array,
    B_w_in: jax.Array,
    B_w_sp: jax.Array,
    B_b_sp: jax.Array,
    B_w_out: jax.Array,
    c: jax.Array,
    w_mod: jax.Array,
):
    del B_x
    operands = (
        A_q.reshape(S, D), A_k.reshape(S, D), A_v.reshape(S, D), A_shift_k.T, A_ssm_k,
        A_ssm_D.reshape(NCT, L), B_w_in.T, B_w_sp, B_b_sp.reshape(S // L, L), B_w_out, c, w_mod,
    )
    spectrum = pltpu.VMEM((4, 2 * L, L), F32)
    scratch = [
        pltpu.VMEM((S // 2, D), U32),
        pltpu.VMEM((NCT, 8 + S // 2, L), U32),
        pltpu.VMEM((NCT, S // 2, L), U32),
        pltpu.VMEM((KS, D), BF16),
        pltpu.VMEM((D, S), BF16),
        pltpu.VMEM((NCT, L), BF16),
        pltpu.VMEM((FH, D), U32),
        pltpu.VMEM((S // 2, S), U32),
        pltpu.VMEM((S // L, L), BF16),
        pltpu.VMEM((FH, D), BF16),
        pltpu.VMEM((1, D), BF16),
        pltpu.VMEM((D, 6 * D), BF16),
        pltpu.VMEM((4, L, L), U32),
        pltpu.VMEM((4, L // 2, 2 * L), U32),
        pltpu.VMEM((S, D), BF16),
        pltpu.VMEM((NCT, KS + 1, 8, L), F32),
        pltpu.VMEM((8, S), F32),
        pltpu.VMEM((5, 8, D), F32),
        [pltpu.VMEM((CH, L), U32)] * NCH,
        [pltpu.VMEM((4, L // 2, L), U32)] * NCH,
        [pltpu.VMEM((4, L // 2, L), U32)] * NCH,
        [spectrum] * 2,
        [pltpu.VMEM((2, 4, 2 * L, L), F32)] * NCH,
        [spectrum] * NCH,
        [pltpu.VMEM((4, L, L), U32)] * NCH,
        pltpu.VMEM((NCT, S // 2, L), U32),
        pltpu.VMEM((S // 2, D), U32),
        pltpu.VMEM((2, CH, D), F32),
        pltpu.VMEM((7, L, DM), U32),
        pltpu.VMEM((CH, D - 2 * DM), U32),
        pltpu.VMEM((5, FH, DM), U32),
        pltpu.VMEM((FH, C), F32),
        pltpu.VMEM((FQ, S), U32),
        pltpu.VMEM((7, FQ // 2, CH), U32),
        pltpu.VMEM((5, S // 4, CH), U32),
        pltpu.VMEM((7, FQ, S // 2), F32),
        pltpu.VMEM((2, D, L), BF16),
        pltpu.VMEM((D, FH - 2 * FM), BF16),
        pltpu.VMEM((7, DH // 2, FM), U32),
        pltpu.VMEM((7, FM // 2, CH), U32),
        pltpu.VMEM((FQ - FM, C), U32),
        pltpu.VMEM((2, D, CH), F32),
        pltpu.SemaphoreType.DMA((15,)),
        pltpu.SemaphoreType.DMA((1,)),
    ]
    out = pl.pallas_call(
        _kernel,
        out_shape=jax.ShapeDtypeStruct((S, D), BF16),
        in_specs=[pl.BlockSpec(memory_space=pltpu.HBM)] * len(operands),
        out_specs=pl.BlockSpec(memory_space=pltpu.HBM),
        scratch_shapes=scratch,
        compiler_params=pltpu.CompilerParams(vmem_limit_bytes=120 * 1024 * 1024),
    )(*operands)
    return out.reshape(1, S, D)
```

```python
import contextlib
import itertools

import numpy as np

import jax
import jax.numpy as jnp
from jax import lax
import jax.experimental.pallas as pl
import jax.experimental.pallas.tpu as pltpu

S = 2048
D = 640
FH = 864
FQ = FH // 2
KS = 4
L = 128
NCT = D // L
C = 512
CH = C // 2
NCH = S // C
NPOS = 16
TICK = 24
TICKS = 3
FINISH_END = 0.9
RES_START = 0.3
RES_END = 0.9
GATE_ORDER = (1, 4, 2, 3, 0, 5, 6)
MP = 144
SUMS_END = 0.3
LATE = 2
WAIT_AT = 6
FILL = 0.97
MB = 144
DEPTH = 12
SPLIT = 4
DH = D // 2
FM = 384
GATE_ROWS = ((0, 144), (144, 288), (288, FQ))
CONV_MATMULS = "K3 D3 B0 B1 D0 B2 D1 B3 D2 K0 K1 K2".split()
CONV_VECTOR = "A0 T2 A1 A3 T3 C0 A2 C1 C2 T1 T0 C3".split()
CONV_AHEAD = "T0 T1 T2 T3 K0 K1 K2".split()
CONV_PACE = 4
CONV_LAG = 0
CONV_DEBT = 1000
CONV_BUDGET = 71
CONV_LEAD = 4
DM = 256
SUMMED_LHS = (0, 1, 4, 5, 6)
SUMMED = (0, 2, 3, 5, 6)
NEVER = 0x7F7F7F7F
EPS = 1e-5
GELU_C0 = float(np.sqrt(2.0 / np.pi))
GELU_C1 = GELU_C0 * 0.044715

F32 = jnp.float32
BF16 = jnp.bfloat16
U32 = jnp.uint32
NT_DIMS = (((1,), (1,)), ((), ()))

TRACE_SCOPES = [False]


def _scope(name):
    return jax.named_scope("ph_" + name) if TRACE_SCOPES[0] else contextlib.nullcontext()


def _lo(w):
    return pltpu.unpack_elementwise(w, index=0, packed_dtype=BF16, unpacked_dtype=F32)


def _hi(w):
    return pltpu.unpack_elementwise(w, index=1, packed_dtype=BF16, unpacked_dtype=F32)


def _pack(a, b):
    return pltpu.pack_elementwise([a, b], packed_dtype=BF16)


def _bf16(words):
    return pltpu.bitcast(words, BF16)


def _riffle(x):
    return _pack(x[:8], x[8:])


def _dot(a, b):
    return jnp.dot(a, b, preferred_element_type=F32)


def _dot_nt(a, b):
    return lax.dot_general(a, b, NT_DIMS, preferred_element_type=F32)


def _tiles(x):
    return x.reshape(x.shape[0] // 8, 8, x.shape[1])


def _interleave(*streams):
    steps = sorted(((k + 0.5) / n, i) for i, (_, n) in enumerate(streams) for k in range(n))
    for _, i in steps:
        next(streams[i][0], None)
    for stream, _ in streams:
        for _ in stream:
            pass


def _spread(stream, n, start, end):
    per_unit = n / (end - start)
    return itertools.chain(range(round(start * per_unit)), stream), round(per_unit)


def _conv_schedule():
    steps = dict(T=8, A=16, C=4 * NPOS)
    cost = dict(T0=24, T1=24, T2=24, T3=24, A0=46, A1=46, A2=46, A3=46, C0=12, C1=20, C2=28, C3=36,
                K0=17, K1=28, K2=24, K3=24, B0=16, B1=16, B2=16, B3=16, D0=6, D1=6, D2=6, D3=6)
    vector = [(x, k) for x in CONV_VECTOR for k in range(steps[x[0]])]
    matmul = [(x, k) for x in CONV_MATMULS for k in range(NPOS)]
    order, done, budget = [], set(), 0
    for n, (x, k) in enumerate(matmul):
        for ahead, _ in matmul[n:n + CONV_LEAD + 1]:
            need = dict(K="T", B="A", D="C")[ahead[0]] + ahead[1]
            while ahead not in ("K3", "D3") and any(v == need for v, _ in vector):
                order.append(vector.pop(0)[0])
                budget -= cost[order[-1]]
        order.append(x)
        done.add((x, k))
        budget = min(max(budget, -CONV_DEBT) + CONV_BUDGET - cost[x], CONV_BUDGET)
        while vector and budget > 0:
            v, j = vector[0]
            if v[0] == "C" and ("B" + v[1], min(j // 4 + CONV_LAG, NPOS - 1)) not in done:
                break
            order.append(vector.pop(0)[0])
            budget -= cost[v]
    return order + [v for v, _ in vector]


def _radix4(e, inverse):
    (r0, i0), (r1, i1), (r2, i2), (r3, i3) = e
    sr, si, dr, di = r0 + r2, i0 + i2, r0 - r2, i0 - i2
    tr, ti, ur, ui = r1 + r3, i1 + i3, r1 - r3, i1 - i3
    a = (dr + ui, di - ur)
    b = (dr - ui, di + ur)
    if inverse:
        a, b = b, a
    return [(sr + tr, si + ti), a, (sr - tr, si - ti), b]


def _strassen_lhs(a11, a12, a21, a22):
    return [a11 + a22, a21 + a22, a11, a22, a11 + a12, a21 - a11, a12 - a22]


STRASSEN_RHS_NEEDS = ((0, 3), (0,), (1, 3), (0, 2), (3,), (0, 1), (2, 3))


def _strassen_rhs(b11, b12, b21, b22):
    return [b11 + b22, b11, b12 - b22, b21 - b11, b22, b11 + b12, b21 + b22]


STRASSEN_USES = ({0: 1, 3: 1}, {2: 1, 3: -1}, {1: 1, 3: 1}, {0: 1, 2: 1}, {0: -1, 1: 1}, {3: 1}, {0: 1})


def _pieces(x):
    return [x[r:r + 16] for r in range(0, x.shape[0], 16)]


def _strassen_product(product, order, blocks, complete):
    blocks = list(blocks)
    for n, q in enumerate(order):
        m = _pieces((yield from product(q)))
        for b, sign in STRASSEN_USES[q].items():
            if blocks[b] is None:
                blocks[b] = m if sign > 0 else [-x for x in m]
            else:
                blocks[b] = [x + y if sign > 0 else x - y for x, y in zip(blocks[b], m)]
            if not any(b in STRASSEN_USES[later] for later in order[n + 1:]):
                complete(b, blocks[b])


def _gelu2(x):
    t = jnp.tanh(x * (x * x * GELU_C1 + GELU_C0))
    return x * t + x


def _layernorm_rows(x):
    d = x - jnp.sum(x, axis=-1, keepdims=True) * (1.0 / D)
    var = jnp.sum(d * d, axis=-1, keepdims=True) * (1.0 / D)
    return d * lax.rsqrt(var + EPS)


def _kernel(q_hbm, k_hbm, v_hbm, shift_hbm, ssm_hbm, ssmd_hbm, wi_hbm, wsp_hbm, bsp_hbm,
            wo_hbm, c_hbm, wmod_hbm, out_hbm,
            q_v, k_v, v_v, shift_v, ssm_v, ssmd_v, wi_v, wsp_v, bsp_v, wo_v, c_v, wmod_v,
            fwd_v, inv_v, out_v,
            chan_s, bsp_s, mod_s, fstage, ktile, utile, kraw, khat, uhat, g_s, y_s, x1_s, xn_s, hq_s, hr_s, wq_s,
            a_s, z1_s, z2_s, wb_s, m_s, wot_s, wor_s, woq_s, pq_s, pr_s, o_s, sems, out_sem):
    copies = {}

    def queue(name, src, dst):
        group = copies.setdefault(name, [])
        group.append(pltpu.make_async_copy(src, dst, sems.at[list(copies).index(name)]))
        group[-1].start()

    def wait(*names):
        for name in names:
            for copy in copies[name]:
                copy.wait()

    def rows(ref, r0, n):
        return ref.at[pl.ds(r0, n), :]

    def queue_pairs(name, src, dst, r0, n):
        queue(name, rows(src, r0, n), rows(dst, r0 // 2, n // 2).bitcast(BF16))

    def queue_wmod(name, i0, i1):
        queue(name, wmod_hbm.at[:, i0 * D:i1 * D], wmod_v.at[:, i0 * D:i1 * D])

    queue("small", rows(ssm_hbm, 0, L), rows(ssm_v, 0, L))
    for src, dst in ((ssmd_hbm, ssmd_v), (shift_hbm, shift_v), (c_hbm, c_v), (bsp_hbm, bsp_v)):
        queue("small", src, dst)
    n = S // SPLIT
    for c in range(NCT):
        for h in range(SPLIT):
            for src, dst, pad in ((k_hbm, k_v, 8), (v_hbm, v_v, 0)):
                queue(f"tile{c}", src.at[pl.ds(h * n, n), pl.ds(c * L, L)],
                      dst.at[c, pl.ds(pad + h * n // 2, n // 2), :].bitcast(BF16))
        if c + 1 < NCT:
            queue(f"tile{c}", rows(ssm_hbm, (c + 1) * L, L), rows(ssm_v, (c + 1) * L, L))
    queue_pairs("first", q_hbm, q_v, 0, C)
    queue_wmod("first", 0, 3)
    queue_wmod("second", 3, 5)
    wi_groups = {FH: MB, FH + MB: FQ - MB, 0: FQ}
    for r0, n in wi_groups.items():
        for o in (0, FQ):
            queue_pairs(f"wi{r0}", wi_hbm, wi_v, r0 + o, n)
    for i in range(NCH):
        cols = pl.ds(i * C, C)
        queue(f"chunk{i}", wsp_hbm.at[:, cols], wsp_v.at[:, cols].bitcast(BF16))
        if i + 1 < NCH:
            queue_pairs(f"chunk{i}", q_hbm, q_v, (i + 1) * C, C)
        if i == 1:
            queue("chunk1", wo_hbm, wo_v)
    queue_wmod(f"chunk{NCH - 1}", 5, 6)

    def wait_step(i, names_of, steps):
        for n in steps:
            @pl.when(i == n)
            def _():
                wait(*names_of(n))

    def span(start, size):
        return pl.ds(start if isinstance(start, int) else pl.multiple_of(start, size), size)

    latest = [None]

    def paced(x):
        if latest[0] is None:
            return x
        n = x.shape[1] // L
        never = jnp.tile(fwd_v[0, 0:8, :], (1, n)) == NEVER
        return jnp.where(never, pltpu.bitcast(jnp.tile(latest[0], (1, n)), x.dtype), x)

    overdue = []

    def hurried(words):
        head = words[:8, :L]
        while len(overdue) > LATE:
            head = jnp.where(fwd_v[0, 0:8, :] == NEVER, overdue.pop(0), head)
        head = jnp.concatenate([head, words[:8, L:]], axis=1)
        return jnp.concatenate([head, words[8:]], axis=0)

    def ticks(m):
        for r in range(0, m.shape[0], TICK):
            latest[0] = m[r:r + 8, 0:L]
            yield
        return m

    def load_group(ref, k2, g):
        return ref[k2 + zero, 16 * g:16 * g + 8, :], ref[k2 + zero, 16 * g + 8:16 * g + 16, :]

    def store_group(ref, k2, g, val):
        ref[k2, 16 * g:16 * g + 8, :] = val[0]
        ref[k2, 16 * g + 8:16 * g + 16, :] = val[1]

    def spectrum_groups(tiles):
        e = [_dot(_bf16(fwd_v[p]), _bf16(tiles[p + zero])) for p in range(4)]
        for g in range(NPOS):
            latest[0] = e[0][16 * g:16 * g + 8]
            yield _radix4([(x[16 * g:16 * g + 8], x[16 * g + 8:16 * g + 16]) for x in e], False)

    def dft_matrices():
        sub = lax.broadcasted_iota(jnp.int32, (8, L), 0)
        lane = lax.broadcasted_iota(jnp.int32, (8, L), 1)

        def unit(turns):
            angle = (((turns + 2 * C) & (4 * C - 1)) - 2 * C).astype(F32) * (np.pi / (2 * C))
            return jnp.cos(angle), -jnp.sin(angle)

        def times(a, b):
            return a[0] * b[0] - a[1] * b[1], a[0] * b[1] + a[1] * b[0]

        for p in range(4):
            n = 4 * ((lane >> 1) + (L // 2) * (lane & 1)) + p
            fwd, fwd1, fwd16 = unit((4 * sub + 1) * n), unit(2 * n), unit(32 * n)
            n = 4 * lane + p
            inv = unit((4 * (sub >> 1) + 1) * n + C * (sub & 1))
            inv1, inv8 = unit(2 * n), unit(16 * n)
            for parity in range(2):
                w = times(fwd, fwd1) if parity else fwd
                for g in range(NPOS // 2):
                    fwd_v.bitcast(BF16)[p, pl.ds(L * parity + 16 * g, 16), :] = (
                        jnp.concatenate(w, axis=0).astype(BF16))
                    w = times(w, fwd16)
                w = times(inv, inv1) if parity else inv
                rows_t = []
                for g in range(NPOS):
                    rows_t.append(w[0] * (1.0 / C))
                    w = times(w, inv8)
                inv_v.bitcast(BF16)[p, :, parity * L:(parity + 1) * L] = (
                    jnp.concatenate(rows_t, axis=0).T.astype(BF16))

    def last_tile(c):
        return c if isinstance(c, int) else jnp.minimum(c, NCT - 1)

    def filter_tiles(c, m):
        fstage[m][...] = pltpu.bitcast(ssm_v[span(last_tile(c) * L, L), m * C:(m + 1) * C].T, U32)
        for u in range(L // 16):
            for s in range(2):
                a = paced(fstage[m][pl.ds(16 * u + s, 8, stride=2), :])
                b = fstage[m][pl.ds(L + 16 * u + s, 8, stride=2), :]
                ktile[m][2 * s, 8 * u:8 * u + 8, :] = _pack(_lo(a), _lo(b))
                ktile[m][2 * s + 1, 8 * u:8 * u + 8, :] = _pack(_hi(a), _hi(b))
            yield

    def signal_tiles(c, j):
        w1, w2, w3 = [chan_s[c, t] for t in range(1, KS)]
        for u in range(L // 16):
            halves = []
            for h in range(2):
                w0 = paced(chan_s[c, 0])
                r0 = j * CH + h * L + 16 * u
                kw = [k_v[c, pl.ds(8 + r0 + o, 8, stride=2), :] for o in range(-2, 2)]
                vw = [v_v[c, pl.ds(r0 + o, 8, stride=2), :] for o in range(2)]
                ks = [_hi(kw[0])] + [f(x) for x in kw[1:] for f in (_lo, _hi)]
                vs = [f(x) for x in vw for f in (_lo, _hi)]
                halves.append([((w0 * ks[p + 3] + w1 * ks[p + 2]) + (w2 * ks[p + 1] + w3 * ks[p]))
                               * vs[p] for p in range(4)])
                if h == 1:
                    for p in range(4):
                        utile[j][p, 8 * u:8 * u + 8, :] = _pack(halves[0][p], halves[1][p])
                yield

    def filter_spectrum(c, m):
        for g, kk in enumerate(spectrum_groups(ktile[m])):
            for k2 in range(4):
                re, im = kk[k2]
                if m == 0:
                    knew = (re + chan_s[last_tile(c), KS], im)
                else:
                    if m == 1:
                        pre, pim = load_group(khat[0].at[c % 2], k2, g)
                        pre = pre - chan_s[last_tile(c), KS]
                    else:
                        pre, pim = load_group(kraw[m % 2], k2, g)
                    knew = (re - pim, im + pre) if g < NPOS // 2 else (re + pim, im - pre)
                if 0 < m < NCH - 1:
                    store_group(kraw[(m + 1) % 2], k2, g, kk[k2])
                store_group(khat[m].at[c % 2], k2, g, knew)
            yield

    def signal_spectrum(c, j):
        for g, uu in enumerate(spectrum_groups(utile[j])):
            for k2 in range(4):
                store_group(uhat[j], k2, g, uu[k2])
            yield

    def chunk_product(c, i):
        for g in range(NPOS):
            ys = []
            for k2 in range(4):
                yr = yi = None
                for j in range(i + 1):
                    kr, ki = load_group(khat[i - j].at[c % 2], k2, g)
                    ur, ui = load_group(uhat[j], k2, g)
                    if j == 0 and k2 % CONV_PACE == 0:
                        kr = paced(kr)
                    pr, pi = kr * ur - ki * ui, kr * ui + ki * ur
                    yr, yi = (pr, pi) if yr is None else (yr + pr, yi + pi)
                ys.append((yr, yi))
                if k2 == 3:
                    for p, pair in enumerate(_radix4(ys, True)):
                        g_s[i][p, 8 * g:8 * g + 8, :] = _pack(*pair)
                yield

    def inverse_dft(c, i):
        y = None
        for k0 in range(0, 2 * L, L):
            part = [_dot(_bf16(inv_v[p, :, k0:k0 + L]), _bf16(g_s[i][p + zero, k0 // 2:(k0 + L) // 2, :]))
                    for p in range(4)]
            for r in range(0, L, 16):
                latest[0] = part[0][r:r + 8]
                if y is not None:
                    for o in (r, r + 8):
                        full = [a[o:o + 8] + b[o:o + 8] for a, b in zip(y, part)]
                        for s in range(2):
                            y_s[c, pl.ds(i * CH + 2 * o + s, 8, stride=2), :] = (
                                _pack(full[2 * s], full[2 * s + 1]))
                yield
            y = part

    dft_matrices()
    g_s[NCH - 1][...] = jnp.zeros(g_s[NCH - 1].shape, U32)
    k_v[:, 0:8, :] = jnp.zeros((NCT, 8, L), U32)
    wait("small")
    probe = pltpu.bitcast(fwd_v[0, 0:8, :], jnp.int32)[0, 0]
    zero = (probe == NEVER).astype(jnp.int32)
    n_blocks = itertools.count()

    def block(name, *streams):
        latest[0] = None
        overdue.clear()

        @pl.when(probe != NEVER + next(n_blocks))
        def _():
            with _scope(name):
                _interleave(*streams)

        latest[0] = None

    dvec = ssmd_v[...].astype(F32)
    taps = shift_v[...].astype(F32)
    for i in range(NCT):
        chan_s[i, KS] = jnp.broadcast_to(dvec[i:i + 1], (8, L))
        for t in range(KS):
            chan_s[i, t] = jnp.broadcast_to(taps[t:t + 1, i * L:(i + 1) * L], (8, L))

    stages = dict(T=filter_tiles, A=signal_tiles, K=filter_spectrum, B=signal_spectrum,
                  C=chunk_product, D=inverse_dft)

    def conv_step(c, carry):
        wait_step(c, lambda n: [f"tile{n}"], range(NCT))
        tile = dict(D3=jnp.maximum(c - 1, 0), **{x: c + 1 for x in CONV_AHEAD})
        streams = {x: stages[x[0]](tile.get(x, c), int(x[1])) for x in CONV_MATMULS + CONV_VECTOR}
        latest[0] = None
        for x in _conv_schedule():
            next(streams[x])
        latest[0] = None
        return carry

    block("fill", (itertools.chain(*[stages[x[0]](0, int(x[1])) for x in CONV_AHEAD]), 1))
    with _scope("conv"):
        lax.fori_loop(0, NCT, conv_step, 0)

    def store_modulated(r, h):
        ops = [_strassen_rhs(h[0][s][:, :DM], h[1][s][:, :DM],
                             h[0][s][:, DM:2 * DM], h[1][s][:, DM:2 * DM]) for s in range(2)]
        for q in range(7):
            words = _pack(ops[0][q], ops[1][q])
            hq_s[q, r:r + 8, :] = words
            if q == 0:
                overdue.append(words[:, :L])
        for a in range(2):
            hr_s[a * L + r:a * L + r + 8, :] = _pack(h[a][0][:, 2 * DM:], h[a][1][:, 2 * DM:])

    def residual_stage(i):
        for r in range(0, L, 8):
            h = []
            for a in range(2):
                at = span(i * CH + a * L + r, 8)
                xw = q_v[at, :]
                yw = jnp.concatenate([y_s[c, at, :] for c in range(NCT)], axis=1)
                xw = jnp.concatenate([paced(xw[:, :L]), xw[:, L:]], axis=1)
                x1 = [half(xw) + (_layernorm_rows(half(xw)) * mod_s[0] + mod_s[1]) * half(yw)
                      for half in (_lo, _hi)]
                x1_s[at, :] = _pack(*x1)
                h.append([_layernorm_rows(x) * mod_s[2] + mod_s[3] for x in x1])
                if a == 1:
                    store_modulated(r, h)
                yield

    cv = c_v[...].astype(F32)
    act = jnp.broadcast_to(cv * jax.nn.sigmoid(cv), (16, D)).astype(BF16)

    def modulation(i):
        return _dot(act, wmod_v[:, i * D:(i + 1) * D])[:8]

    def first_gate():
        sa, ca, ga = [modulation(i) for i in range(3)]
        mod_s[0] = (1.0 + ca) * ga
        mod_s[1] = sa * ga
        latest[0] = ga[:, :L]
        yield

    def first_norm():
        for r in range(0, CH, 8):
            xw = q_v[r:r + 8, :]
            xw = jnp.concatenate([paced(xw[:, :L]), xw[:, L:]], axis=1)
            for s, half in enumerate((_lo, _hi)):
                xn_s[s, r:r + 8, :] = _layernorm_rows(half(xw))
            yield

    def first_residual():
        done = []
        for r in range(0, CH, 8):
            latest[0] = done[-DEPTH] if len(done) >= DEPTH else None
            yw = jnp.concatenate([paced(y_s[0, r:r + 8, :])]
                                 + [y_s[c, r:r + 8, :] for c in range(1, NCT)], axis=1)
            x1 = [half(q_v[r:r + 8, :]) + (xn_s[s, r:r + 8, :] * mod_s[0] + mod_s[1]) * half(yw)
                  for s, half in enumerate((_lo, _hi))]
            x1_s[r:r + 8, :] = _pack(*x1)
            for s in range(2):
                xn = _layernorm_rows(x1[s])
                xn_s[s, r:r + 8, :] = xn
            done.append(xn[:, :L])
            yield

    def first_modulate():
        wait("second")
        shift, scale = modulation(3), 1.0 + modulation(4)
        mod_s[2] = scale
        mod_s[3] = shift
        for r in range(0, L, 8):
            store_modulated(r, [[xn_s[s, a * L + r:a * L + r + 8, :] * scale + shift
                                 for s in range(2)] for a in range(2)])
        yield

    wait("first")
    block("drain", (itertools.chain(inverse_dft(NCT - 1, NCH - 1), first_gate()), NPOS + 1),
          _spread(first_norm(), CH // 8, 0.0, 0.5))
    block("res0", (first_residual(), 1))
    block("mod", (first_modulate(), 1))

    def hidden_stage(i, first=False):
        def weight_sums(r0):
            for r in range(r0 // 2, (r0 + MB) // 2, 8):
                top, bot = slice(r, r + 8), slice(r + FQ // 2, r + FQ // 2 + 8)
                w = [paced(wi_v[top, :DM]), wi_v[top, DM:2 * DM],
                     wi_v[bot, :DM], paced(wi_v[bot, DM:2 * DM])]
                lo, hi = _strassen_lhs(*[_lo(x) for x in w]), _strassen_lhs(*[_hi(x) for x in w])
                for slot, q in enumerate(SUMMED_LHS):
                    wq_s[slot, top, :] = _pack(lo[q], hi[q])
                yield

        def preact(r0, complete):
            top = slice(r0 // 2, (r0 + MB) // 2)
            bot = slice((r0 + FQ) // 2, (r0 + FQ + MB) // 2)
            following = 0 if r0 + MB == FH + FQ else r0 + MB
            sums = weight_sums(r0) if first else iter(())

            def product(q):
                if first and q == WAIT_AT and following in wi_groups:
                    wait(f"wi{following}")
                w = (wi_v[top, :DM] if q == 2 else wi_v[bot, DM:2 * DM] if q == 3
                     else wq_s[SUMMED_LHS.index(q), top, :])
                m = _dot_nt(_bf16(w), _bf16(hq_s[q]))
                for _ in ticks(m):
                    next(sums, None)
                    yield
                return m

            rest = []
            for part in (top, bot):
                rest.append(_dot_nt(_bf16(wi_v[part, 2 * DM:]), _bf16(hr_s[...])))
                for _ in ticks(rest[-1]):
                    next(sums, None)
                    yield
            yield from _strassen_product(
                product, (2, 3, 4, 1, 0, 6, 5),
                [_pieces(rest[b // 2][:, (b % 2) * CH:(b % 2 + 1) * CH]) for b in range(4)], complete)

        def column_mean(acc):
            return jnp.broadcast_to(jnp.sum(acc, axis=0, keepdims=True) * (1.0 / FH), (8, C))

        total = [jnp.zeros((8, CH), F32)] * 2

        def activate():
            for r0 in range(0, FQ, MB):
                def complete(b, z):
                    for n, x in enumerate(z):
                        a = _gelu2(x)
                        f = (b // 2) * FQ + r0 + 16 * n
                        a_s[f:f + 16, (b % 2) * CH:(b % 2 + 1) * CH] = a
                        total[b % 2] = total[b % 2] + (a[:8] + a[8:])

                yield from preact(FH + r0, complete)

        def layernorm():
            mean = column_mean(jnp.concatenate(total, axis=1))
            acc = jnp.zeros((8, C), F32)
            for r in range(0, FH, 32):
                d = _tiles(a_s[r:r + 32, :]) - paced(mean)
                acc = acc + (d * d).sum(axis=0)
                yield
            rstd = lax.rsqrt(column_mean(acc) + 4.0 * EPS)
            means = [mean[:, c0:c0 + L] for c0 in range(0, C, L)]
            for r in range(0, FQ, 16):
                for c0 in range(0, CH, L):
                    blocks = []
                    for o in (0, FQ):
                        for cols in (slice(c0, c0 + L), slice(CH + c0, CH + c0 + L)):
                            m = means[cols.start // L]
                            if (o == 0) == (cols.start == c0):
                                m = paced(m)
                            d = (_tiles(a_s[o + r:o + r + 16, cols]) - m) * rstd[:, cols]
                            blocks.append(d.reshape(16, L))
                    for q, op in enumerate(_strassen_lhs(*blocks)):
                        z2_s[q, r // 2:r // 2 + 8, c0:c0 + L] = _riffle(op)
                    yield

        def gate():
            for r0 in range(0, FQ, MB):
                def complete(b, z):
                    for n, x in enumerate(z):
                        f = ((b // 2) * FQ + r0) // 2 + 8 * n
                        z1_s[f:f + 8, span(i * C + (b % 2) * CH, CH)] = _riffle(_gelu2(x))

                yield from preact(r0, complete)

        return ((itertools.chain(activate(), gate()), 18 * FQ // TICK),
                _spread(layernorm(), FH // 32 + FQ // 8, 0.51, FILL))

    def mixer_sums(i, n):
        left, right = span(i * C, CH), span(i * C + CH, CH)
        for r in range(0, L, 8):
            top, bot = span(n * CH + r, 8), span(n * CH + L + r, 8)
            w = [paced(wsp_v[top, left]), wsp_v[bot, left],
                 wsp_v[top, right], paced(wsp_v[bot, right])]
            lo, hi = _strassen_rhs(*[_lo(x) for x in w]), _strassen_rhs(*[_hi(x) for x in w])
            for slot, q in enumerate(SUMMED):
                wb_s[slot, span(n * L + r, 8), :] = _pack(lo[q], hi[q])
            yield

    def mixer_operand(i, q, n):
        if q in SUMMED:
            return wb_s[SUMMED.index(q), span(n * L, L), :]
        o = 0 if q == 1 else 1
        return wsp_v[span(n * CH + o * L, L), span(i * C + o * CH, CH)]

    def mixer_partial(i):
        for products in ((1, 4), SUMMED):
            for n in range(0, NCH, 2):
                for q in products:
                    w = jnp.concatenate([mixer_operand(i, q, n + o) for o in range(2)], axis=0)
                    for r0 in range(0, FQ, MP):
                        m = _dot_nt(_bf16(hurried(z2_s[q, r0 // 2:(r0 + MP) // 2, :])), _bf16(w))
                        for r in range(0, MP, 8):
                            at = (q, slice(r0 + r, r0 + r + 8), slice(n * CH, (n + 2) * CH))
                            m_s[at] = jnp.where(i > 0, m_s[at], 0.0) + m[r:r + 8]
                        yield from ticks(m)

    def output_columns(starts):
        def group(f):
            x = wo_v[pl.ds(f if isinstance(f, int) else pl.multiple_of(f, 16), 16), :]
            for _ in range(2):
                x = _bf16(_riffle(x.astype(F32)))
            return x

        return jnp.concatenate([group(f) for f in starts], axis=0).T

    def output_operands(i):
        for a in range(2):
            wot_s[a] = output_columns([a * FQ + i * L + r for r in range(0, L, 16)])
        for r in range(0, DH, 16):
            w = [pltpu.bitcast(wot_s[b % 2, r + (b // 2) * DH:r + (b // 2) * DH + 16, :], U32)
                 for b in range(4)]
            w[0], w[3] = paced(w[0]), paced(w[3])
            lo, hi = _strassen_lhs(*[_lo(x) for x in w]), _strassen_lhs(*[_hi(x) for x in w])
            for q in range(7):
                woq_s[q, r // 2:r // 2 + 8, span(i * L, L)] = _pack(lo[q], hi[q])
            yield

    wait(f"wi{FH}")
    block("hidden0", *hidden_stage(0, first=True))

    wait("chunk0")

    def chunk_step(i, carry):
        block("partial", (mixer_partial(i), 14 * FQ // TICK),
              _spread(itertools.chain(*[mixer_sums(i, n) for n in range(NCH)]),
                      NCH * L // 8, 0.0, SUMS_END),
              _spread(residual_stage(i + 1), CH // 8, RES_START, RES_END))
        wait_step(i, lambda n: [f"chunk{n + 1}"], range(NCH - 1))
        block("hidden", *hidden_stage(i + 1), _spread(output_operands(i), DH // 16, 0.1, 0.45))
        return carry

    lax.fori_loop(0, NCH - 1, chunk_step, 0)

    def gated_product(n):
        for r0, r1 in GATE_ROWS:
            def product(q):
                m = yield from ticks(_dot_nt(_bf16(z2_s[q, r0 // 2:r1 // 2, :]),
                                             _bf16(mixer_operand(NCH - 1, q, n))))
                return m_s[q, r0:r1, span(n * CH, CH)] + m

            p = {}

            def complete(b, g):
                t = span(n * C + (b % 2) * CH, CH)
                p[b] = []
                for k, x in enumerate(g):
                    r = r0 + 16 * k
                    f = ((b // 2) * FQ + r) // 2
                    z1 = _bf16(z1_s[f:f + 8, t]).astype(F32)
                    p[b].append(z1 * (_tiles(x) + bsp_s[:, t]).reshape(16, CH))
                    if r >= FM:
                        f = ((b // 2) * (FQ - FM) + r - FM) // 2
                        pr_s[f:f + 8, (b % 2) * CH:(b % 2 + 1) * CH] = _riffle(p[b][k])
                        continue
                    ops = _strassen_rhs(*[p[a][k] if a in p else x for a in range(4)])
                    for q, needs in enumerate(STRASSEN_RHS_NEEDS):
                        if b in needs and all(a in p for a in needs):
                            pq_s[q, r // 2:r // 2 + 8, :] = _riffle(ops[q])

            yield from _strassen_product(product, GATE_ORDER, [None] * 4, complete)

    def project():
        rest = yield from ticks(_dot(wor_s[...], _bf16(pr_s[...])))

        def complete(b, o):
            for k, x in enumerate(o):
                d = (b // 2) * DH + 16 * k
                o_s[b % 2, d:d + 16, :] = x

        yield from _strassen_product(
            lambda q: ticks(_dot(_bf16(woq_s[q]), _bf16(pq_s[q]))), (1, 3, 4, 0, 6, 2, 5),
            [_pieces(rest[(b // 2) * DH:(b // 2 + 1) * DH, (b % 2) * CH:(b % 2 + 1) * CH])
             for b in range(4)], complete)

    def out_copy(row, n, c0=0, c1=NCT):
        at = (span(row, n), slice(c0 * L, c1 * L))
        return pltpu.make_async_copy(out_v.at[at], out_hbm.at[at], out_sem.at[0])

    def finish(n, h, c0=0, c1=NCT):
        for c in reversed(range(c0, c1)):
            for t0 in range(0, CH, L):
                cols = slice(c * L, (c + 1) * L)
                o = o_s[h, cols, t0:t0 + L].T
                x1 = _bf16(x1_s[span(n * CH + (h * CH + t0) // 2, L // 2), cols]).astype(F32)
                res = _tiles(x1) + mod_s[4, :, cols] * _tiles(o)
                out_v[span(n * C + h * CH + t0, L), cols] = res.reshape(L, L).astype(BF16)
                yield

    bvec = bsp_v[...].astype(F32)
    for i in range(S // L):
        bsp_s[:, i * L:(i + 1) * L] = jnp.broadcast_to(bvec[i:i + 1], (8, L))
    wor_s[...] = output_columns([a * FQ + r for a in range(2) for r in range(FM, FQ, 16)])
    gate_ticks = 7 * sum(-(-(b - a) // TICK) for a, b in GATE_ROWS)
    _interleave((gated_product(0), gate_ticks), (mixer_sums(NCH - 1, 0), 10 * L // 8 + 8))
    mod_s[4] = 0.5 * modulation(5)

    def output_step(n, carry):
        latest[0] = None
        _interleave((project(), -(-D // TICK) + 7 * -(-DH // TICK)),
                    _spread(mixer_sums(NCH - 1, n + 1), L // 8, 0.0, 0.7))
        _interleave((gated_product(n + 1), gate_ticks),
                    _spread(itertools.chain(finish(n, 0), finish(n, 1)),
                            4 * NCT, 0.0, FINISH_END))
        out_copy(n * C, C).start()
        return carry

    with _scope("output"):
        lax.fori_loop(0, NCH - 1, output_step, 0)
    _interleave((project(), 1))
    latest[0] = None
    last_parts = ((0, 0, NCT), (1, 0, DH // L), (1, DH // L, NCT))
    for h, c0, c1 in last_parts:
        _interleave((finish(NCH - 1, h, c0, c1), 1))
        out_copy((NCH - 1) * C + h * CH, CH, c0, c1).start()
    for n in range(NCH - 1):
        out_copy(n * C, C).wait()
    for h, c0, c1 in last_parts:
        out_copy((NCH - 1) * C + h * CH, CH, c0, c1).wait()


@jax.jit
def pallas_adaLN_cond__ssm_conv_h3__mixer_gmlp__prompt_kernel(
    A_q: jax.Array,
    A_k: jax.Array,
    A_v: jax.Array,
    A_shift_k: jax.Array,
    A_ssm_k: jax.Array,
    A_ssm_D: jax.Array,
    B_x: jax.Array,
    B_w_in: jax.Array,
    B_w_sp: jax.Array,
    B_b_sp: jax.Array,
    B_w_out: jax.Array,
    c: jax.Array,
    w_mod: jax.Array,
):
    del B_x
    operands = (
        A_q.reshape(S, D), A_k.reshape(S, D), A_v.reshape(S, D), A_shift_k.T, A_ssm_k,
        A_ssm_D.reshape(NCT, L), B_w_in.T, B_w_sp, B_b_sp.reshape(S // L, L), B_w_out, c, w_mod,
    )
    spectrum = pltpu.VMEM((4, 2 * L, L), F32)
    scratch = [
        pltpu.VMEM((S // 2, D), U32),
        pltpu.VMEM((NCT, 8 + S // 2, L), U32),
        pltpu.VMEM((NCT, S // 2, L), U32),
        pltpu.VMEM((KS, D), BF16),
        pltpu.VMEM((D, S), BF16),
        pltpu.VMEM((NCT, L), BF16),
        pltpu.VMEM((FH, D), U32),
        pltpu.VMEM((S // 2, S), U32),
        pltpu.VMEM((S // L, L), BF16),
        pltpu.VMEM((FH, D), BF16),
        pltpu.VMEM((1, D), BF16),
        pltpu.VMEM((D, 6 * D), BF16),
        pltpu.VMEM((4, L, L), U32),
        pltpu.VMEM((4, L // 2, 2 * L), U32),
        pltpu.VMEM((S, D), BF16),
        pltpu.VMEM((NCT, KS + 1, 8, L), F32),
        pltpu.VMEM((8, S), F32),
        pltpu.VMEM((5, 8, D), F32),
        [pltpu.VMEM((CH, L), U32)] * NCH,
        [pltpu.VMEM((4, L // 2, L), U32)] * NCH,
        [pltpu.VMEM((4, L // 2, L), U32)] * NCH,
        [spectrum] * 2,
        [pltpu.VMEM((2, 4, 2 * L, L), F32)] * NCH,
        [spectrum] * NCH,
        [pltpu.VMEM((4, L, L), U32)] * NCH,
        pltpu.VMEM((NCT, S // 2, L), U32),
        pltpu.VMEM((S // 2, D), U32),
        pltpu.VMEM((2, CH, D), F32),
        pltpu.VMEM((7, L, DM), U32),
        pltpu.VMEM((CH, D - 2 * DM), U32),
        pltpu.VMEM((5, FH, DM), U32),
        pltpu.VMEM((FH, C), F32),
        pltpu.VMEM((FQ, S), U32),
        pltpu.VMEM((7, FQ // 2, CH), U32),
        pltpu.VMEM((5, S // 4, CH), U32),
        pltpu.VMEM((7, FQ, S // 2), F32),
        pltpu.VMEM((2, D, L), BF16),
        pltpu.VMEM((D, FH - 2 * FM), BF16),
        pltpu.VMEM((7, DH // 2, FM), U32),
        pltpu.VMEM((7, FM // 2, CH), U32),
        pltpu.VMEM((FQ - FM, C), U32),
        pltpu.VMEM((2, D, CH), F32),
        pltpu.SemaphoreType.DMA((15,)),
        pltpu.SemaphoreType.DMA((1,)),
    ]
    out = pl.pallas_call(
        _kernel,
        out_shape=jax.ShapeDtypeStruct((S, D), BF16),
        in_specs=[pl.BlockSpec(memory_space=pltpu.HBM)] * len(operands),
        out_specs=pl.BlockSpec(memory_space=pltpu.HBM),
        scratch_shapes=scratch,
        compiler_params=pltpu.CompilerParams(vmem_limit_bytes=120 * 1024 * 1024),
    )(*operands)
    return out.reshape(1, S, D)
```

```python
import contextlib
import itertools

import numpy as np

import jax
import jax.numpy as jnp
from jax import lax
import jax.experimental.pallas as pl
import jax.experimental.pallas.tpu as pltpu

S = 2048
D = 640
FH = 864
FQ = FH // 2
KS = 4
L = 128
NCT = D // L
C = 512
CH = C // 2
NCH = S // C
NPOS = 16
TICK = 24
TICKS = 3
FINISH_END = 0.9
RES_START = 0.3
RES_END = 0.9
GATE_ORDER = (1, 4, 2, 3, 0, 5, 6)
MP = 144
SUMS_END = 0.3
LATE = 2
WAIT_AT = 6
FILL = 0.97
MB = 144
DEPTH = 12
DH = D // 2
FM = 384
GATE_ROWS = ((0, 144), (144, 288), (288, FQ))
CONV_STEP = ("K3 D3 B0 B1 D0 B2 D1 B3 D2 K0 K1 K2", "A0 T2 A1 A3 T3 C0 A2 C1 C2 T1 T0 C3", 71)
CONV_AHEAD = "T0 T1 T2 T3 K0 K1 K2".split()
CONV_LAST = ("K3 D3 B0 B1 D0 B2 D1 B3 D2", "A0 A1 A2 C0 A3 C1 C2 C3", 71)
CONV_LEAD = 4
DM = 256
SUMMED_LHS = (0, 1, 4, 5, 6)
SUMMED = (0, 2, 3, 5, 6)
NEVER = 0x7F7F7F7F
EPS = 1e-5
GELU_C0 = float(np.sqrt(2.0 / np.pi))
GELU_C1 = GELU_C0 * 0.044715

F32 = jnp.float32
BF16 = jnp.bfloat16
U32 = jnp.uint32
NT_DIMS = (((1,), (1,)), ((), ()))

TRACE_SCOPES = [False]


def _scope(name):
    return jax.named_scope("ph_" + name) if TRACE_SCOPES[0] else contextlib.nullcontext()


def _lo(w):
    return pltpu.unpack_elementwise(w, index=0, packed_dtype=BF16, unpacked_dtype=F32)


def _hi(w):
    return pltpu.unpack_elementwise(w, index=1, packed_dtype=BF16, unpacked_dtype=F32)


def _pack(a, b):
    return pltpu.pack_elementwise([a, b], packed_dtype=BF16)


def _bf16(words):
    return pltpu.bitcast(words, BF16)


def _riffle(x):
    return _pack(x[:8], x[8:])


def _dot(a, b):
    return jnp.dot(a, b, preferred_element_type=F32)


def _dot_nt(a, b):
    return lax.dot_general(a, b, NT_DIMS, preferred_element_type=F32)


def _tiles(x):
    return x.reshape(x.shape[0] // 8, 8, x.shape[1])


def _interleave(*streams):
    steps = sorted(((k + 0.5) / n, i) for i, (_, n) in enumerate(streams) for k in range(n))
    for _, i in steps:
        next(streams[i][0], None)
    for stream, _ in streams:
        for _ in stream:
            pass


def _spread(stream, n, start, end):
    per_unit = n / (end - start)
    return itertools.chain(range(round(start * per_unit)), stream), round(per_unit)


def _conv_schedule(matmuls, vector, per_step):
    steps = dict(T=8, A=16, C=4 * NPOS)
    cost = dict(T=(24,) * 4, A=(46,) * 4, C=(12, 20, 28, 36), K=(17, 28, 24, 24),
                B=(16,) * 4, D=(6,) * 4)
    vector = [(x, k) for x in vector.split() for k in range(steps[x[0]])]
    matmul = [(x, k) for x in matmuls.split() for k in range(NPOS)]
    order, done, budget = [], set(), 0
    for n, (x, k) in enumerate(matmul):
        for ahead, _ in matmul[n:n + CONV_LEAD + 1]:
            need = dict(K="T", B="A", D="C")[ahead[0]] + ahead[1]
            while ahead not in ("K3", "D3") and any(v == need for v, _ in vector):
                order.append(vector.pop(0)[0])
                budget -= cost[order[-1][0]][int(order[-1][1])]
        order.append(x)
        done.add((x, k))
        budget = min(budget + per_step - cost[x[0]][int(x[1])], per_step)
        while vector and budget > 0:
            v, j = vector[0]
            if v[0] == "C" and ("B" + v[1], j // 4) not in done:
                break
            order.append(vector.pop(0)[0])
            budget -= cost[v[0]][int(v[1])]
    return order + [v for v, _ in vector]


def _radix4(e, inverse):
    (r0, i0), (r1, i1), (r2, i2), (r3, i3) = e
    sr, si, dr, di = r0 + r2, i0 + i2, r0 - r2, i0 - i2
    tr, ti, ur, ui = r1 + r3, i1 + i3, r1 - r3, i1 - i3
    a = (dr + ui, di - ur)
    b = (dr - ui, di + ur)
    if inverse:
        a, b = b, a
    return [(sr + tr, si + ti), a, (sr - tr, si - ti), b]


def _strassen_lhs(a11, a12, a21, a22):
    return [a11 + a22, a21 + a22, a11, a22, a11 + a12, a21 - a11, a12 - a22]


STRASSEN_RHS_NEEDS = ((0, 3), (0,), (1, 3), (0, 2), (3,), (0, 1), (2, 3))


def _strassen_rhs(b11, b12, b21, b22):
    return [b11 + b22, b11, b12 - b22, b21 - b11, b22, b11 + b12, b21 + b22]


STRASSEN_USES = ({0: 1, 3: 1}, {2: 1, 3: -1}, {1: 1, 3: 1}, {0: 1, 2: 1}, {0: -1, 1: 1}, {3: 1}, {0: 1})


def _pieces(x):
    return [x[r:r + 16] for r in range(0, x.shape[0], 16)]


def _strassen_product(product, order, blocks, complete):
    blocks = list(blocks)
    for n, q in enumerate(order):
        m = _pieces((yield from product(q)))
        for b, sign in STRASSEN_USES[q].items():
            if blocks[b] is None:
                blocks[b] = m if sign > 0 else [-x for x in m]
            else:
                blocks[b] = [x + y if sign > 0 else x - y for x, y in zip(blocks[b], m)]
            if not any(b in STRASSEN_USES[later] for later in order[n + 1:]):
                complete(b, blocks[b])


def _gelu2(x):
    t = jnp.tanh(x * (x * x * GELU_C1 + GELU_C0))
    return x * t + x


def _layernorm_rows(x):
    d = x - jnp.sum(x, axis=-1, keepdims=True) * (1.0 / D)
    var = jnp.sum(d * d, axis=-1, keepdims=True) * (1.0 / D)
    return d * lax.rsqrt(var + EPS)


def _kernel(q_hbm, k_hbm, v_hbm, shift_hbm, ssm_hbm, ssmd_hbm, wi_hbm, wsp_hbm, bsp_hbm,
            wo_hbm, c_hbm, wmod_hbm, out_hbm,
            q_v, k_v, v_v, shift_v, ssm_v, ssmd_v, wi_v, wsp_v, bsp_v, wo_v, c_v, wmod_v,
            fwd_v, inv_v, out_v,
            chan_s, bsp_s, mod_s, fstage, ktile, utile, kraw, khat, uhat, g_s, y_s, x1_s, xn_s, hq_s, hr_s, wq_s,
            a_s, z1_s, z2_s, wb_s, m_s, wot_s, wor_s, woq_s, pq_s, pr_s, o_s, sems, out_sem):
    copies = {}

    def queue(name, src, dst):
        group = copies.setdefault(name, [])
        group.append(pltpu.make_async_copy(src, dst, sems.at[list(copies).index(name)]))
        group[-1].start()

    def wait(*names):
        for name in names:
            for copy in copies[name]:
                copy.wait()

    def rows(ref, r0, n):
        return ref.at[pl.ds(r0, n), :]

    def queue_pairs(name, src, dst, r0, n):
        queue(name, rows(src, r0, n), rows(dst, r0 // 2, n // 2).bitcast(BF16))

    def queue_wmod(name, i0, i1):
        queue(name, wmod_hbm.at[:, i0 * D:i1 * D], wmod_v.at[:, i0 * D:i1 * D].bitcast(BF16))

    queue("small", rows(ssm_hbm, 0, L), rows(ssm_v, 0, L))
    for src, dst in ((ssmd_hbm, ssmd_v), (shift_hbm, shift_v), (c_hbm, c_v), (bsp_hbm, bsp_v)):
        queue("small", src, dst)
    n = C
    for c in range(NCT):
        for h in range(NCH):
            for src, dst, pad in ((k_hbm, k_v, 8), (v_hbm, v_v, 0)):
                queue(f"tile{c}", src.at[pl.ds(h * n, n), pl.ds(c * L, L)],
                      dst.at[c, pl.ds(pad + h * n // 2, n // 2), :].bitcast(BF16))
        if c + 1 < NCT:
            queue(f"tile{c}", rows(ssm_hbm, (c + 1) * L, L), rows(ssm_v, (c + 1) * L, L))
    queue_pairs(f"tile{NCT - 1}", q_hbm, q_v, 0, C)
    queue_wmod("first", 0, 3)
    queue_wmod("second", 3, 5)
    wi_groups = {FH: MB, FH + MB: FQ - MB, 0: FQ}
    for r0, n in wi_groups.items():
        for o in (0, FQ):
            queue_pairs(f"wi{r0}", wi_hbm, wi_v, r0 + o, n)
    for i in range(NCH):
        cols = pl.ds(i * C, C)
        queue(f"chunk{i}", wsp_hbm.at[:, cols], wsp_v.at[:, cols].bitcast(BF16))
        if i + 1 < NCH:
            queue_pairs(f"chunk{i}", q_hbm, q_v, (i + 1) * C, C)
        if i == 1:
            queue("chunk1", wo_hbm, wo_v)
    queue_wmod(f"chunk{NCH - 1}", 5, 6)

    def wait_step(i, names_of, steps):
        for n in steps:
            @pl.when(i == n)
            def _():
                wait(*names_of(n))

    def span(start, size):
        return pl.ds(start if isinstance(start, int) else pl.multiple_of(start, size), size)

    latest = [None]

    def paced(x):
        if latest[0] is None:
            return x
        n = x.shape[1] // L
        never = jnp.tile(fwd_v[0, 0:8, :], (1, n)) == NEVER
        return jnp.where(never, pltpu.bitcast(jnp.tile(latest[0], (1, n)), x.dtype), x)

    overdue = []

    def hurried(words):
        head = words[:8, :L]
        while len(overdue) > LATE:
            head = jnp.where(fwd_v[0, 0:8, :] == NEVER, overdue.pop(0), head)
        head = jnp.concatenate([head, words[:8, L:]], axis=1)
        return jnp.concatenate([head, words[8:]], axis=0)

    def ticks(m):
        for r in range(0, m.shape[0], TICK):
            latest[0] = m[r:r + 8, 0:L]
            yield
        return m

    def load_group(ref, k2, g):
        return ref[k2 + zero, 16 * g:16 * g + 8, :], ref[k2 + zero, 16 * g + 8:16 * g + 16, :]

    def store_group(ref, k2, g, val):
        ref[k2, 16 * g:16 * g + 8, :] = val[0]
        ref[k2, 16 * g + 8:16 * g + 16, :] = val[1]

    def spectrum_groups(tiles):
        e = [_dot(_bf16(fwd_v[p]), _bf16(tiles[p + zero])) for p in range(4)]
        for g in range(NPOS):
            latest[0] = e[0][16 * g:16 * g + 8]
            yield _radix4([(x[16 * g:16 * g + 8], x[16 * g + 8:16 * g + 16]) for x in e], False)

    def dft_matrices():
        sub = lax.broadcasted_iota(jnp.int32, (8, L), 0)
        lane = lax.broadcasted_iota(jnp.int32, (8, L), 1)

        def unit(turns):
            angle = (((turns + 2 * C) & (4 * C - 1)) - 2 * C).astype(F32) * (np.pi / (2 * C))
            return jnp.cos(angle), -jnp.sin(angle)

        def times(a, b):
            return a[0] * b[0] - a[1] * b[1], a[0] * b[1] + a[1] * b[0]

        for p in range(4):
            n = 4 * ((lane >> 1) + (L // 2) * (lane & 1)) + p
            fwd, fwd1, fwd16 = unit((4 * sub + 1) * n), unit(2 * n), unit(32 * n)
            n = 4 * lane + p
            inv = unit((4 * (sub >> 1) + 1) * n + C * (sub & 1))
            inv1, inv8 = unit(2 * n), unit(16 * n)
            for parity in range(2):
                w = times(fwd, fwd1) if parity else fwd
                for g in range(NPOS // 2):
                    fwd_v.bitcast(BF16)[p, pl.ds(L * parity + 16 * g, 16), :] = (
                        jnp.concatenate(w, axis=0).astype(BF16))
                    w = times(w, fwd16)
                w = times(inv, inv1) if parity else inv
                rows_t = []
                for g in range(NPOS):
                    rows_t.append(w[0] * (1.0 / C))
                    w = times(w, inv8)
                inv_v.bitcast(BF16)[p, :, parity * L:(parity + 1) * L] = (
                    jnp.concatenate(rows_t, axis=0).T.astype(BF16))

    def filter_tiles(c, m):
        fstage[m][...] = pltpu.bitcast(ssm_v[span(c * L, L), m * C:(m + 1) * C].T, U32)
        for u in range(L // 16):
            for s in range(2):
                a = paced(fstage[m][pl.ds(16 * u + s, 8, stride=2), :])
                b = fstage[m][pl.ds(L + 16 * u + s, 8, stride=2), :]
                ktile[m][2 * s, 8 * u:8 * u + 8, :] = _pack(_lo(a), _lo(b))
                ktile[m][2 * s + 1, 8 * u:8 * u + 8, :] = _pack(_hi(a), _hi(b))
            yield

    def signal_tiles(c, j):
        w1, w2, w3 = [chan_s[c, t] for t in range(1, KS)]
        for u in range(L // 16):
            halves = []
            for h in range(2):
                w0 = paced(chan_s[c, 0])
                r0 = j * CH + h * L + 16 * u
                kw = [k_v[c, pl.ds(8 + r0 + o, 8, stride=2), :] for o in range(-2, 2)]
                vw = [v_v[c, pl.ds(r0 + o, 8, stride=2), :] for o in range(2)]
                ks = [_hi(kw[0])] + [f(x) for x in kw[1:] for f in (_lo, _hi)]
                vs = [f(x) for x in vw for f in (_lo, _hi)]
                halves.append([((w0 * ks[p + 3] + w1 * ks[p + 2]) + (w2 * ks[p + 1] + w3 * ks[p]))
                               * vs[p] for p in range(4)])
                if h == 1:
                    for p in range(4):
                        utile[j][p, 8 * u:8 * u + 8, :] = _pack(halves[0][p], halves[1][p])
                yield

    def filter_spectrum(c, m):
        for g, kk in enumerate(spectrum_groups(ktile[m])):
            for k2 in range(4):
                re, im = kk[k2]
                if m == 0:
                    knew = (re + chan_s[c, KS], im)
                else:
                    if m == 1:
                        pre, pim = load_group(khat[0].at[c % 2], k2, g)
                        pre = pre - chan_s[c, KS]
                    else:
                        pre, pim = load_group(kraw[m % 2], k2, g)
                    knew = (re - pim, im + pre) if g < NPOS // 2 else (re + pim, im - pre)
                if 0 < m < NCH - 1:
                    store_group(kraw[(m + 1) % 2], k2, g, kk[k2])
                store_group(khat[m].at[c % 2], k2, g, knew)
            yield

    def signal_spectrum(c, j):
        for g, uu in enumerate(spectrum_groups(utile[j])):
            for k2 in range(4):
                store_group(uhat[j], k2, g, uu[k2])
            yield

    def chunk_product(c, i):
        for g in range(NPOS):
            ys = []
            for k2 in range(4):
                yr = yi = None
                for j in range(i + 1):
                    kr, ki = load_group(khat[i - j].at[c % 2], k2, g)
                    ur, ui = load_group(uhat[j], k2, g)
                    if j == 0 and k2 == 0:
                        kr = paced(kr)
                    pr, pi = kr * ur - ki * ui, kr * ui + ki * ur
                    yr, yi = (pr, pi) if yr is None else (yr + pr, yi + pi)
                ys.append((yr, yi))
                if k2 == 3:
                    for p, pair in enumerate(_radix4(ys, True)):
                        g_s[i][p, 8 * g:8 * g + 8, :] = _pack(*pair)
                yield

    def inverse_dft(c, i):
        y = None
        for k0 in range(0, 2 * L, L):
            part = [_dot(_bf16(inv_v[p, :, k0:k0 + L]), _bf16(g_s[i][p + zero, k0 // 2:(k0 + L) // 2, :]))
                    for p in range(4)]
            for r in range(0, L, 16):
                latest[0] = part[0][r:r + 8]
                if y is not None:
                    for o in (r, r + 8):
                        full = [a[o:o + 8] + b[o:o + 8] for a, b in zip(y, part)]
                        for s in range(2):
                            y_s[c, pl.ds(i * CH + 2 * o + s, 8, stride=2), :] = (
                                _pack(full[2 * s], full[2 * s + 1]))
                yield
            y = part

    dft_matrices()
    g_s[NCH - 1][...] = jnp.zeros(g_s[NCH - 1].shape, U32)
    k_v[:, 0:8, :] = jnp.zeros((NCT, 8, L), U32)
    wait("small")
    probe = pltpu.bitcast(fwd_v[0, 0:8, :], jnp.int32)[0, 0]
    zero = (probe == NEVER).astype(jnp.int32)
    n_blocks = itertools.count()

    def block(name, *streams):
        latest[0] = None
        overdue.clear()

        @pl.when(probe != NEVER + next(n_blocks))
        def _():
            with _scope(name):
                _interleave(*streams)

        latest[0] = None

    dvec = ssmd_v[...].astype(F32)
    taps = shift_v[...].astype(F32)
    for i in range(NCT):
        chan_s[i, KS] = jnp.broadcast_to(dvec[i:i + 1], (8, L))
        for t in range(KS):
            chan_s[i, t] = jnp.broadcast_to(taps[t:t + 1, i * L:(i + 1) * L], (8, L))

    stages = dict(T=filter_tiles, A=signal_tiles, K=filter_spectrum, B=signal_spectrum,
                  C=chunk_product, D=inverse_dft)

    def conv_stages(c, plan):
        def stage(x):
            tile = c + 1 if x in CONV_AHEAD else jnp.maximum(c - 1, 0) if x == "D3" else c
            return stages[x[0]](tile, int(x[1]))

        streams = {x: stage(x) for x in plan[0].split() + plan[1].split()}
        latest[0] = None
        for x in _conv_schedule(*plan):
            next(streams[x])
        latest[0] = None
        yield

    def conv_step(c, carry):
        wait_step(c, lambda n: [f"tile{n}"], range(NCT - 1))
        _interleave((conv_stages(c, CONV_STEP), 1))
        return carry

    block("fill", (itertools.chain(*[stages[x[0]](0, int(x[1])) for x in CONV_AHEAD]), 1))
    with _scope("conv"):
        lax.fori_loop(0, NCT - 1, conv_step, 0)

    def store_modulated(r, h):
        ops = [_strassen_rhs(h[0][s][:, :DM], h[1][s][:, :DM],
                             h[0][s][:, DM:2 * DM], h[1][s][:, DM:2 * DM]) for s in range(2)]
        for q in range(7):
            words = _pack(ops[0][q], ops[1][q])
            hq_s[q, r:r + 8, :] = words
            if q == 0:
                overdue.append(words[:, :L])
        for a in range(2):
            hr_s[a * L + r:a * L + r + 8, :] = _pack(h[a][0][:, 2 * DM:], h[a][1][:, 2 * DM:])

    def residual_stage(i):
        for r in range(0, L, 8):
            h = []
            for a in range(2):
                at = span(i * CH + a * L + r, 8)
                xw = q_v[at, :]
                yw = jnp.concatenate([y_s[c, at, :] for c in range(NCT)], axis=1)
                xw = jnp.concatenate([paced(xw[:, :L]), xw[:, L:]], axis=1)
                x1 = [half(xw) + (_layernorm_rows(half(xw)) * mod_s[0] + mod_s[1]) * half(yw)
                      for half in (_lo, _hi)]
                x1_s[at, :] = _pack(*x1)
                h.append([_layernorm_rows(x) * mod_s[2] + mod_s[3] for x in x1])
                if a == 1:
                    store_modulated(r, h)
                yield

    cv = c_v[...].astype(F32)
    act = jnp.broadcast_to(cv * jax.nn.sigmoid(cv), (16, D)).astype(BF16)

    def modulation(i):
        return _dot(act, _bf16(wmod_v[:, i * D:(i + 1) * D]))[:8]

    def first_gate():
        sa, ca, ga = [modulation(i) for i in range(3)]
        mod_s[0] = (1.0 + ca) * ga
        mod_s[1] = sa * ga
        latest[0] = ga[:, :L]
        yield

    def first_norm():
        for r in range(0, CH, 8):
            xw = q_v[r:r + 8, :]
            xw = jnp.concatenate([paced(xw[:, :L]), xw[:, L:]], axis=1)
            for s, half in enumerate((_lo, _hi)):
                xn_s[s, r:r + 8, :] = _layernorm_rows(half(xw))
            yield

    def first_residual():
        done = []
        for r in range(0, CH, 8):
            latest[0] = done[-DEPTH] if len(done) >= DEPTH else None
            yw = jnp.concatenate([paced(y_s[0, r:r + 8, :])]
                                 + [y_s[c, r:r + 8, :] for c in range(1, NCT)], axis=1)
            x1 = [half(q_v[r:r + 8, :]) + (xn_s[s, r:r + 8, :] * mod_s[0] + mod_s[1]) * half(yw)
                  for s, half in enumerate((_lo, _hi))]
            x1_s[r:r + 8, :] = _pack(*x1)
            for s in range(2):
                xn = _layernorm_rows(x1[s])
                xn_s[s, r:r + 8, :] = xn
            done.append(xn[:, :L])
            yield

    def first_modulate():
        wait("second")
        shift, scale = modulation(3), 1.0 + modulation(4)
        mod_s[2] = scale
        mod_s[3] = shift
        for r in range(0, L, 8):
            store_modulated(r, [[xn_s[s, a * L + r:a * L + r + 8, :] * scale + shift
                                 for s in range(2)] for a in range(2)])
        yield

    wait(f"tile{NCT - 1}")
    block("conv_last", (conv_stages(NCT - 1, CONV_LAST), 1))
    wait("first")
    block("norm0", (itertools.chain(inverse_dft(NCT - 1, 3), first_gate()), 2 * NPOS),
          _spread(first_norm(), CH // 8, 0.0, 0.5))
    block("res0", (first_residual(), 1))
    block("mod", (first_modulate(), 1))

    def hidden_stage(i, first=False):
        def weight_sums(r0):
            for r in range(r0 // 2, (r0 + MB) // 2, 8):
                top, bot = slice(r, r + 8), slice(r + FQ // 2, r + FQ // 2 + 8)
                w = [paced(wi_v[top, :DM]), wi_v[top, DM:2 * DM],
                     wi_v[bot, :DM], paced(wi_v[bot, DM:2 * DM])]
                lo, hi = _strassen_lhs(*[_lo(x) for x in w]), _strassen_lhs(*[_hi(x) for x in w])
                for slot, q in enumerate(SUMMED_LHS):
                    wq_s[slot, top, :] = _pack(lo[q], hi[q])
                yield

        def preact(r0, complete):
            top = slice(r0 // 2, (r0 + MB) // 2)
            bot = slice((r0 + FQ) // 2, (r0 + FQ + MB) // 2)
            following = 0 if r0 + MB == FH + FQ else r0 + MB
            sums = weight_sums(r0) if first else iter(())

            def product(q):
                if first and q == WAIT_AT and following in wi_groups:
                    wait(f"wi{following}")
                w = (wi_v[top, :DM] if q == 2 else wi_v[bot, DM:2 * DM] if q == 3
                     else wq_s[SUMMED_LHS.index(q), top, :])
                m = _dot_nt(_bf16(w), _bf16(hq_s[q]))
                for _ in ticks(m):
                    next(sums, None)
                    yield
                return m

            rest = []
            for part in (top, bot):
                rest.append(_dot_nt(_bf16(wi_v[part, 2 * DM:]), _bf16(hr_s[...])))
                for _ in ticks(rest[-1]):
                    next(sums, None)
                    yield
            yield from _strassen_product(
                product, (2, 3, 4, 1, 0, 6, 5),
                [_pieces(rest[b // 2][:, (b % 2) * CH:(b % 2 + 1) * CH]) for b in range(4)], complete)

        def column_mean(acc):
            return jnp.broadcast_to(jnp.sum(acc, axis=0, keepdims=True) * (1.0 / FH), (8, C))

        total = [jnp.zeros((8, CH), F32)] * 2

        def activate():
            for r0 in range(0, FQ, MB):
                def complete(b, z):
                    for n, x in enumerate(z):
                        a = _gelu2(x)
                        f = (b // 2) * FQ + r0 + 16 * n
                        a_s[f:f + 16, (b % 2) * CH:(b % 2 + 1) * CH] = a
                        total[b % 2] = total[b % 2] + (a[:8] + a[8:])

                yield from preact(FH + r0, complete)

        def layernorm():
            mean = column_mean(jnp.concatenate(total, axis=1))
            acc = jnp.zeros((8, C), F32)
            for r in range(0, FH, 32):
                d = _tiles(a_s[r:r + 32, :]) - paced(mean)
                acc = acc + (d * d).sum(axis=0)
                yield
            rstd = lax.rsqrt(column_mean(acc) + 4.0 * EPS)
            means = [mean[:, c0:c0 + L] for c0 in range(0, C, L)]
            for r in range(0, FQ, 16):
                for c0 in range(0, CH, L):
                    blocks = []
                    for o in (0, FQ):
                        for cols in (slice(c0, c0 + L), slice(CH + c0, CH + c0 + L)):
                            m = means[cols.start // L]
                            if (o == 0) == (cols.start == c0):
                                m = paced(m)
                            d = (_tiles(a_s[o + r:o + r + 16, cols]) - m) * rstd[:, cols]
                            blocks.append(d.reshape(16, L))
                    for q, op in enumerate(_strassen_lhs(*blocks)):
                        z2_s[q, r // 2:r // 2 + 8, c0:c0 + L] = _riffle(op)
                    yield

        def gate():
            for r0 in range(0, FQ, MB):
                def complete(b, z):
                    for n, x in enumerate(z):
                        f = ((b // 2) * FQ + r0) // 2 + 8 * n
                        z1_s[f:f + 8, span(i * C + (b % 2) * CH, CH)] = _riffle(_gelu2(x))

                yield from preact(r0, complete)

        return ((itertools.chain(activate(), gate()), 18 * FQ // TICK),
                _spread(layernorm(), FH // 32 + FQ // 8, 0.51, FILL))

    def mixer_sums(i, n):
        left, right = span(i * C, CH), span(i * C + CH, CH)
        for r in range(0, L, 8):
            top, bot = span(n * CH + r, 8), span(n * CH + L + r, 8)
            w = [paced(wsp_v[top, left]), wsp_v[bot, left],
                 wsp_v[top, right], paced(wsp_v[bot, right])]
            lo, hi = _strassen_rhs(*[_lo(x) for x in w]), _strassen_rhs(*[_hi(x) for x in w])
            for slot, q in enumerate(SUMMED):
                wb_s[slot, span(n * L + r, 8), :] = _pack(lo[q], hi[q])
            yield

    def mixer_operand(i, q, n):
        if q in SUMMED:
            return wb_s[SUMMED.index(q), span(n * L, L), :]
        o = 0 if q == 1 else 1
        return wsp_v[span(n * CH + o * L, L), span(i * C + o * CH, CH)]

    def mixer_partial(i):
        for products in ((1, 4), SUMMED):
            for n in range(0, NCH, 2):
                for q in products:
                    w = jnp.concatenate([mixer_operand(i, q, n + o) for o in range(2)], axis=0)
                    for r0 in range(0, FQ, MP):
                        m = _dot_nt(_bf16(hurried(z2_s[q, r0 // 2:(r0 + MP) // 2, :])), _bf16(w))
                        for r in range(0, MP, 8):
                            at = (q, slice(r0 + r, r0 + r + 8), slice(n * CH, (n + 2) * CH))
                            m_s[at] = jnp.where(i > 0, m_s[at], 0.0) + m[r:r + 8]
                        yield from ticks(m)

    def output_columns(starts):
        def group(f):
            x = wo_v[pl.ds(f if isinstance(f, int) else pl.multiple_of(f, 16), 16), :]
            for _ in range(2):
                x = _bf16(_riffle(x.astype(F32)))
            return x

        return jnp.concatenate([group(f) for f in starts], axis=0).T

    def output_operands(i):
        for a in range(2):
            wot_s[a] = output_columns([a * FQ + i * L + r for r in range(0, L, 16)])
        for r in range(0, DH, 16):
            w = [pltpu.bitcast(wot_s[b % 2, r + (b // 2) * DH:r + (b // 2) * DH + 16, :], U32)
                 for b in range(4)]
            w[0], w[3] = paced(w[0]), paced(w[3])
            lo, hi = _strassen_lhs(*[_lo(x) for x in w]), _strassen_lhs(*[_hi(x) for x in w])
            for q in range(7):
                woq_s[q, r // 2:r // 2 + 8, span(i * L, L)] = _pack(lo[q], hi[q])
            yield

    wait(f"wi{FH}")
    block("hidden0", *hidden_stage(0, first=True))

    wait("chunk0")

    def chunk_step(i, carry):
        block("partial", (mixer_partial(i), 14 * FQ // TICK),
              _spread(itertools.chain(*[mixer_sums(i, n) for n in range(NCH)]),
                      NCH * L // 8, 0.0, SUMS_END),
              _spread(residual_stage(i + 1), CH // 8, RES_START, RES_END))
        wait_step(i, lambda n: [f"chunk{n + 1}"], range(NCH - 1))
        block("hidden", *hidden_stage(i + 1), _spread(output_operands(i), DH // 16, 0.1, 0.45))
        return carry

    lax.fori_loop(0, NCH - 1, chunk_step, 0)

    def gated_product(n):
        for r0, r1 in GATE_ROWS:
            def product(q):
                m = yield from ticks(_dot_nt(_bf16(z2_s[q, r0 // 2:r1 // 2, :]),
                                             _bf16(mixer_operand(NCH - 1, q, n))))
                return m_s[q, r0:r1, span(n * CH, CH)] + m

            p = {}

            def complete(b, g):
                t = span(n * C + (b % 2) * CH, CH)
                p[b] = []
                for k, x in enumerate(g):
                    r = r0 + 16 * k
                    f = ((b // 2) * FQ + r) // 2
                    z1 = _bf16(z1_s[f:f + 8, t]).astype(F32)
                    p[b].append(z1 * (_tiles(x) + bsp_s[:, t]).reshape(16, CH))
                    if r >= FM:
                        f = ((b // 2) * (FQ - FM) + r - FM) // 2
                        pr_s[f:f + 8, (b % 2) * CH:(b % 2 + 1) * CH] = _riffle(p[b][k])
                        continue
                    ops = _strassen_rhs(*[p[a][k] if a in p else x for a in range(4)])
                    for q, needs in enumerate(STRASSEN_RHS_NEEDS):
                        if b in needs and all(a in p for a in needs):
                            pq_s[q, r // 2:r // 2 + 8, :] = _riffle(ops[q])

            yield from _strassen_product(product, GATE_ORDER, [None] * 4, complete)

    def project():
        rest = yield from ticks(_dot(wor_s[...], _bf16(pr_s[...])))

        def complete(b, o):
            for k, x in enumerate(o):
                d = (b // 2) * DH + 16 * k
                o_s[b % 2, d:d + 16, :] = x

        yield from _strassen_product(
            lambda q: ticks(_dot(_bf16(woq_s[q]), _bf16(pq_s[q]))), (1, 3, 4, 0, 6, 2, 5),
            [_pieces(rest[(b // 2) * DH:(b // 2 + 1) * DH, (b % 2) * CH:(b % 2 + 1) * CH])
             for b in range(4)], complete)

    def out_copy(row, n, c0=0, c1=NCT):
        at = (span(row, n), slice(c0 * L, c1 * L))
        return pltpu.make_async_copy(out_v.at[at], out_hbm.at[at], out_sem.at[0])

    def finish(n, h, c0=0, c1=NCT):
        for c in reversed(range(c0, c1)):
            for t0 in range(0, CH, L):
                cols = slice(c * L, (c + 1) * L)
                o = o_s[h, cols, t0:t0 + L].T
                x1 = _bf16(x1_s[span(n * CH + (h * CH + t0) // 2, L // 2), cols]).astype(F32)
                res = _tiles(x1) + mod_s[4, :, cols] * _tiles(o)
                out_v[span(n * C + h * CH + t0, L), cols] = res.reshape(L, L).astype(BF16)
                yield

    bvec = bsp_v[...].astype(F32)
    for i in range(S // L):
        bsp_s[:, i * L:(i + 1) * L] = jnp.broadcast_to(bvec[i:i + 1], (8, L))
    wor_s[...] = output_columns([a * FQ + r for a in range(2) for r in range(FM, FQ, 16)])
    gate_ticks = 7 * sum(-(-(b - a) // TICK) for a, b in GATE_ROWS)
    _interleave((gated_product(0), gate_ticks), (mixer_sums(NCH - 1, 0), 10 * L // 8 + 8))
    mod_s[4] = 0.5 * modulation(5)

    def output_step(n, carry):
        @pl.when(n > 0)
        def _():
            out_copy((n - 1) * C, C).start()

        latest[0] = None
        _interleave((project(), -(-D // TICK) + 7 * -(-DH // TICK)),
                    _spread(mixer_sums(NCH - 1, n + 1), L // 8, 0.0, 0.7))
        _interleave((gated_product(n + 1), gate_ticks),
                    _spread(itertools.chain(finish(n, 0), finish(n, 1)),
                            4 * NCT, 0.0, FINISH_END))
        return carry

    with _scope("output"):
        lax.fori_loop(0, NCH - 1, output_step, 0)
    out_copy((NCH - 2) * C, C).start()
    _interleave((project(), 1))
    latest[0] = None
    last_parts = ((0, 0, NCT), (1, 0, DH // L), (1, DH // L, NCT))
    for h, c0, c1 in last_parts:
        _interleave((finish(NCH - 1, h, c0, c1), 1))
        out_copy((NCH - 1) * C + h * CH, CH, c0, c1).start()
    for n in range(NCH - 1):
        out_copy(n * C, C).wait()
    for h, c0, c1 in last_parts:
        out_copy((NCH - 1) * C + h * CH, CH, c0, c1).wait()


@jax.jit
def pallas_adaLN_cond__ssm_conv_h3__mixer_gmlp__prompt_kernel(
    A_q: jax.Array,
    A_k: jax.Array,
    A_v: jax.Array,
    A_shift_k: jax.Array,
    A_ssm_k: jax.Array,
    A_ssm_D: jax.Array,
    B_x: jax.Array,
    B_w_in: jax.Array,
    B_w_sp: jax.Array,
    B_b_sp: jax.Array,
    B_w_out: jax.Array,
    c: jax.Array,
    w_mod: jax.Array,
):
    del B_x
    operands = (
        A_q.reshape(S, D), A_k.reshape(S, D), A_v.reshape(S, D), A_shift_k.T, A_ssm_k,
        A_ssm_D.reshape(NCT, L), B_w_in.T, B_w_sp, B_b_sp.reshape(S // L, L), B_w_out, c, w_mod,
    )
    spectrum = pltpu.VMEM((4, 2 * L, L), F32)
    scratch = [
        pltpu.VMEM((S // 2, D), U32),
        pltpu.VMEM((NCT, 8 + S // 2, L), U32),
        pltpu.VMEM((NCT, S // 2, L), U32),
        pltpu.VMEM((KS, D), BF16),
        pltpu.VMEM((D, S), BF16),
        pltpu.VMEM((NCT, L), BF16),
        pltpu.VMEM((FH, D), U32),
        pltpu.VMEM((S // 2, S), U32),
        pltpu.VMEM((S // L, L), BF16),
        pltpu.VMEM((FH, D), BF16),
        pltpu.VMEM((1, D), BF16),
        pltpu.VMEM((DH, 6 * D), U32),
        pltpu.VMEM((4, L, L), U32),
        pltpu.VMEM((4, L // 2, 2 * L), U32),
        pltpu.VMEM((S, D), BF16),
        pltpu.VMEM((NCT, KS + 1, 8, L), F32),
        pltpu.VMEM((8, S), F32),
        pltpu.VMEM((5, 8, D), F32),
        [pltpu.VMEM((CH, L), U32)] * NCH,
        [pltpu.VMEM((4, L // 2, L), U32)] * NCH,
        [pltpu.VMEM((4, L // 2, L), U32)] * NCH,
        [spectrum] * 2,
        [pltpu.VMEM((2, 4, 2 * L, L), F32)] * NCH,
        [spectrum] * NCH,
        [pltpu.VMEM((4, L, L), U32)] * NCH,
        pltpu.VMEM((NCT, S // 2, L), U32),
        pltpu.VMEM((S // 2, D), U32),
        pltpu.VMEM((2, CH, D), F32),
        pltpu.VMEM((7, L, DM), U32),
        pltpu.VMEM((CH, D - 2 * DM), U32),
        pltpu.VMEM((5, FH, DM), U32),
        pltpu.VMEM((FH, C), F32),
        pltpu.VMEM((FQ, S), U32),
        pltpu.VMEM((7, FQ // 2, CH), U32),
        pltpu.VMEM((5, S // 4, CH), U32),
        pltpu.VMEM((7, FQ, S // 2), F32),
        pltpu.VMEM((2, D, L), BF16),
        pltpu.VMEM((D, FH - 2 * FM), BF16),
        pltpu.VMEM((7, DH // 2, FM), U32),
        pltpu.VMEM((7, FM // 2, CH), U32),
        pltpu.VMEM((FQ - FM, C), U32),
        pltpu.VMEM((2, D, CH), F32),
        pltpu.SemaphoreType.DMA((15,)),
        pltpu.SemaphoreType.DMA((1,)),
    ]
    out = pl.pallas_call(
        _kernel,
        out_shape=jax.ShapeDtypeStruct((S, D), BF16),
        in_specs=[pl.BlockSpec(memory_space=pltpu.HBM)] * len(operands),
        out_specs=pl.BlockSpec(memory_space=pltpu.HBM),
        scratch_shapes=scratch,
        compiler_params=pltpu.CompilerParams(vmem_limit_bytes=120 * 1024 * 1024),
    )(*operands)
    return out.reshape(1, S, D)
```

```python
import contextlib
import itertools

import numpy as np

import jax
import jax.numpy as jnp
from jax import lax
import jax.experimental.pallas as pl
import jax.experimental.pallas.tpu as pltpu

S = 2048
D = 640
FH = 864
FQ = FH // 2
KS = 4
L = 128
NCT = D // L
C = 512
CH = C // 2
NCH = S // C
NPOS = 16
TICK = 24
TICKS = 3
FINISH_END = 0.9
RES_START = 0.35
RES_END = 0.9
GATE_ORDER = (1, 4, 2, 3, 0, 5, 6)
MP = 144
SUMS_END = 0.3
WAIT_AT = 6
FILL = 0.97
MB = 144
DEPTH = 12
DH = D // 2
FM = 384
GATE_ROWS = ((0, 144), (144, 288), (288, FQ))
CONV_STEP = ("K3 D3 B0 B1 D0 B2 D1 B3 D2 K0 K1 K2", "A0 A1 T3 T2 A3 C0 A2 C1 T0 C2 T1 C3", 71)
CONV_AHEAD = "T0 T1 T2 T3 K0 K1 K2".split()
CONV_LAST = ("K3 D3 B0 B1 D0 B2 D1 B3 D2", "A0 A1 A2 C0 A3 C1 C2 C3", 71)
CONV_LEAD = 4
DM = 256
SUMMED_LHS = (0, 1, 4, 5, 6)
SUMMED = (0, 2, 3, 5, 6)
NEVER = 0x7F7F7F7F
EPS = 1e-5
GELU_C0 = float(np.sqrt(2.0 / np.pi))
GELU_C1 = GELU_C0 * 0.044715

F32 = jnp.float32
BF16 = jnp.bfloat16
U32 = jnp.uint32
NT_DIMS = (((1,), (1,)), ((), ()))

TRACE_SCOPES = [False]


def _scope(name):
    return jax.named_scope("ph_" + name) if TRACE_SCOPES[0] else contextlib.nullcontext()


def _lo(w):
    return lax.bitcast_convert_type(w << 16, F32)


def _hi(w):
    return lax.bitcast_convert_type(w & np.uint32(0xFFFF0000), F32)


def _bf16(words):
    return pltpu.bitcast(words, BF16)


def _f32(words):
    return _bf16(words).astype(F32)


def _put(ref, lead, first, rows, x):
    for n in range(x.shape[1] // L):
        ref[(*lead, first + n, rows)] = x[:, n * L:(n + 1) * L].astype(BF16)


def _get(ref, lead, first, count, word_rows=slice(None)):
    return jnp.concatenate(
        [ref.bitcast(U32)[(*lead, first + n, word_rows)] for n in range(count)], axis=1)


def _dot(a, b):
    return jnp.dot(a, b, preferred_element_type=F32)


def _dot_nt(a, b):
    return lax.dot_general(a, b, NT_DIMS, preferred_element_type=F32)


def _tiles(x):
    return x.reshape(x.shape[0] // 8, 8, x.shape[1])


def _interleave(*streams):
    steps = sorted(((k + 0.5) / n, i) for i, (_, n) in enumerate(streams) for k in range(n))
    for _, i in steps:
        next(streams[i][0], None)
    for stream, _ in streams:
        for _ in stream:
            pass


def _spread(stream, n, start, end):
    per_unit = n / (end - start)
    return itertools.chain(range(round(start * per_unit)), stream), round(per_unit)


def _conv_schedule(matmuls, vector, per_step):
    steps = dict(T=8, A=16, C=4 * NPOS)
    cost = dict(T=(24,) * 4, A=(46,) * 4, C=(12, 20, 28, 36), K=(17, 25, 25, 25),
                B=(16,) * 4, D=(6,) * 4)
    vector = [(x, k) for x in vector.split() for k in range(steps[x[0]])]
    matmul = [(x, k) for x in matmuls.split() for k in range(NPOS)]
    order, done, budget = [], set(), 0
    for n, (x, k) in enumerate(matmul):
        for ahead, _ in matmul[n:n + CONV_LEAD + 1]:
            need = dict(K="T", B="A", D="C")[ahead[0]] + ahead[1]
            while ahead not in ("K3", "D3") and any(v == need for v, _ in vector):
                order.append(vector.pop(0)[0])
                budget -= cost[order[-1][0]][int(order[-1][1])]
        order.append(x)
        done.add((x, k))
        budget = min(budget + per_step - cost[x[0]][int(x[1])], per_step)
        while vector and budget > 0:
            v, j = vector[0]
            if v[0] == "C" and ("B" + v[1], j // 4) not in done:
                break
            order.append(vector.pop(0)[0])
            budget -= cost[v[0]][int(v[1])]
    return order + [v for v, _ in vector]


def _radix4(e, inverse):
    (r0, i0), (r1, i1), (r2, i2), (r3, i3) = e
    sr, si, dr, di = r0 + r2, i0 + i2, r0 - r2, i0 - i2
    tr, ti, ur, ui = r1 + r3, i1 + i3, r1 - r3, i1 - i3
    a = (dr + ui, di - ur)
    b = (dr - ui, di + ur)
    if inverse:
        a, b = b, a
    return [(sr + tr, si + ti), a, (sr - tr, si - ti), b]


def _strassen_lhs(a11, a12, a21, a22):
    return [a11 + a22, a21 + a22, a11, a22, a11 + a12, a21 - a11, a12 - a22]


STRASSEN_RHS_NEEDS = ((0, 3), (0,), (1, 3), (0, 2), (3,), (0, 1), (2, 3))


def _strassen_rhs(b11, b12, b21, b22):
    return [b11 + b22, b11, b12 - b22, b21 - b11, b22, b11 + b12, b21 + b22]


STRASSEN_USES = ({0: 1, 3: 1}, {2: 1, 3: -1}, {1: 1, 3: 1}, {0: 1, 2: 1}, {0: -1, 1: 1}, {3: 1}, {0: 1})


def _pieces(x):
    return [x[r:r + 16] for r in range(0, x.shape[0], 16)]


def _strassen_product(product, order, blocks, complete):
    blocks = list(blocks)
    for n, q in enumerate(order):
        m = _pieces((yield from product(q)))
        for b, sign in STRASSEN_USES[q].items():
            if blocks[b] is None:
                blocks[b] = m if sign > 0 else [-x for x in m]
            else:
                blocks[b] = [x + y if sign > 0 else x - y for x, y in zip(blocks[b], m)]
            if not any(b in STRASSEN_USES[later] for later in order[n + 1:]):
                complete(b, blocks[b])


def _gelu2(x):
    t = jnp.tanh(x * (x * x * GELU_C1 + GELU_C0))
    return x * t + x


def _layernorm_rows(x):
    d = x - jnp.sum(x, axis=-1, keepdims=True) * (1.0 / D)
    var = jnp.sum(d * d, axis=-1, keepdims=True) * (1.0 / D)
    return d * lax.rsqrt(var + EPS)


def _kernel(q_hbm, k_hbm, v_hbm, shift_hbm, ssm_hbm, ssmd_hbm, wi_hbm, wsp_hbm, bsp_hbm,
            wo_hbm, c_hbm, wmod_hbm, out_hbm,
            q_v, k_v, v_v, shift_v, ssm_v, ssmd_v, wi_v, wsp_v, bsp_v, wo_v, c_v, wmod_v,
            fwd_v, inv_v, out_v,
            mark_s, chan_s, bsp_s, mod_s, fstage, ktile, utile, kraw, khat, uhat, g_s, y_s, x1_s, xn_s, hq_s, hr_s, wq_s,
            a_s, z1_s, z2_s, wb_s, m_s, wot_s, wor_s, woq_s, pq_s, pr_s, o_s, sems, out_sem):
    copies = {}

    def queue(name, src, dst):
        group = copies.setdefault(name, [])
        group.append(pltpu.make_async_copy(src, dst, sems.at[list(copies).index(name)]))
        group[-1].start()

    def wait(*names):
        for name in names:
            for copy in copies[name]:
                copy.wait()

    def rows(ref, r0, n):
        return ref.at[pl.ds(r0, n), :]

    def queue_pairs(name, src, dst, r0, n):
        queue(name, rows(src, r0, n), rows(dst, r0 // 2, n // 2).bitcast(BF16))

    def queue_wmod(name, i0, i1):
        queue(name, wmod_hbm.at[:, i0 * D:i1 * D], wmod_v.at[:, i0 * D:i1 * D].bitcast(BF16))

    queue_pairs("small", ssm_hbm, ssm_v, 0, L)
    for src, dst in ((ssmd_hbm, ssmd_v), (shift_hbm, shift_v), (c_hbm, c_v), (bsp_hbm, bsp_v)):
        queue("small", src, dst)
    n = C
    for c in range(NCT):
        for h in range(NCH):
            for src, dst, pad in ((k_hbm, k_v, 8), (v_hbm, v_v, 0)):
                queue(f"tile{c}", src.at[pl.ds(h * n, n), pl.ds(c * L, L)],
                      dst.at[c, pl.ds(pad + h * n // 2, n // 2), :].bitcast(BF16))
        if c + 1 < NCT:
            queue_pairs(f"tile{c}", ssm_hbm, ssm_v, (c + 1) * L, L)
    queue_pairs(f"tile{NCT - 1}", q_hbm, q_v, 0, C)
    queue_wmod("first", 0, 3)
    queue_wmod("second", 3, 5)
    wi_groups = {FH: MB, FH + MB: FQ - MB, 0: FQ}
    for r0, n in wi_groups.items():
        for o in (0, FQ):
            queue_pairs(f"wi{r0}", wi_hbm, wi_v, r0 + o, n)
    for i in range(NCH):
        cols = pl.ds(i * C, C)
        queue(f"chunk{i}", wsp_hbm.at[:, cols], wsp_v.at[:, cols].bitcast(BF16))
        if i + 1 < NCH:
            queue_pairs(f"chunk{i}", q_hbm, q_v, (i + 1) * C, C)
        if i == 1:
            queue("chunk1", wo_hbm, wo_v)
    queue_wmod(f"chunk{NCH - 1}", 5, 6)

    def wait_step(i, names_of, steps):
        for n in steps:
            @pl.when(i == n)
            def _():
                wait(*names_of(n))

    def span(start, size):
        return pl.ds(start if isinstance(start, int) else pl.multiple_of(start, size), size)

    latest = [None]

    def paced(x):
        if latest[0] is None:
            return x
        n = x.shape[1] // L
        if x.shape[0] > 8:
            return jnp.concatenate([paced(x[:8]), x[8:]], axis=0)
        never = jnp.tile(mark_s[...], (1, n)) == NEVER
        return jnp.where(never, lax.bitcast_convert_type(jnp.tile(latest[0], (1, n)), x.dtype), x)

    def ticks(m):
        for r in range(0, m.shape[0], TICK):
            latest[0] = m[r:r + 8, 0:L]
            yield
        return m

    def load_group(ref, k2, g):
        return ref[k2 + zero, 16 * g:16 * g + 8, :], ref[k2 + zero, 16 * g + 8:16 * g + 16, :]

    def store_group(ref, k2, g, val):
        ref[k2, 16 * g:16 * g + 8, :] = val[0]
        ref[k2, 16 * g + 8:16 * g + 16, :] = val[1]

    def spectrum_groups(tiles, adjust=lambda g, pair: pair):
        e = [_dot(_bf16(_get(fwd_v, (), p, 1)), _bf16(_get(tiles, (), p + zero, 1)))
             for p in range(4)]
        for g in range(NPOS):
            latest[0] = e[0][16 * g:16 * g + 8]
            pairs = [(x[16 * g:16 * g + 8], x[16 * g + 8:16 * g + 16]) for x in e]
            yield _radix4([adjust(g, pairs[0])] + pairs[1:], False)

    def dft_matrices():
        sub = lax.broadcasted_iota(jnp.int32, (8, L), 0)
        lane = lax.broadcasted_iota(jnp.int32, (8, L), 1)

        def unit(turns):
            angle = (((turns + 2 * C) & (4 * C - 1)) - 2 * C).astype(F32) * (np.pi / (2 * C))
            return jnp.cos(angle), -jnp.sin(angle)

        def times(a, b):
            return a[0] * b[0] - a[1] * b[1], a[0] * b[1] + a[1] * b[0]

        for p in range(4):
            for inverse in (False, True):
                n1 = lane if inverse else 8 * (lane >> 4) + (lane & 7) + 8 * (lane & 8)
                n = 4 * n1 + p
                even, one, sixteen = unit((4 * sub + 1) * n), unit(2 * n), unit(32 * n)
                for parity in range(2):
                    w, parts = times(even, one) if parity else even, []
                    for _ in range(NPOS // 2):
                        parts += w
                        w = times(w, sixteen)
                    half = jnp.concatenate(parts, axis=0)
                    if inverse:
                        _put(inv_v, (p,), parity, slice(None), (half * (1.0 / C)).T)
                    else:
                        _put(fwd_v, (), p, slice(parity * L, (parity + 1) * L), half)

    def filter_tiles(c, m):
        fstage[m][0:CH, :] = pltpu.bitcast(
            _bf16(ssm_v[span(c * (L // 2), L // 2), m * C:(m + 1) * C]).T, U32)
        for u in range(L // 16):
            for s in range(2):
                a = paced(fstage[m][pl.ds(16 * u + s, 8, stride=2), :])
                b = fstage[m][pl.ds(L + 16 * u + s, 8, stride=2), :]
                for o, half in enumerate((_lo, _hi)):
                    _put(ktile[m], (), 2 * s + o, slice(16 * u, 16 * u + 16),
                         jnp.concatenate([half(a), half(b)], axis=0))
            yield

    def signal_tiles(c, j):
        w1, w2, w3 = [chan_s[c, t] for t in range(1, KS)]
        for u in range(L // 16):
            halves = []
            for h in range(2):
                w0 = paced(chan_s[c, 0])
                r0 = j * CH + h * L + 16 * u
                kw = [k_v[c, pl.ds(8 + r0 + o, 8, stride=2), :] for o in range(-2, 2)]
                vw = [v_v[c, pl.ds(r0 + o, 8, stride=2), :] for o in range(2)]
                ks = [_hi(kw[0])] + [f(x) for x in kw[1:] for f in (_lo, _hi)]
                vs = [f(x) for x in vw for f in (_lo, _hi)]
                halves.append([((w0 * ks[p + 3] + w1 * ks[p + 2]) + (w2 * ks[p + 1] + w3 * ks[p]))
                               * vs[p] for p in range(4)])
                if h == 1:
                    for p in range(4):
                        _put(utile[j], (), p, slice(16 * u, 16 * u + 16),
                             jnp.concatenate([halves[0][p], halves[1][p]], axis=0))
                yield

    def filter_spectrum(c, m):
        def skip(g, pair):
            re, im = pair
            d = chan_s[c, KS]
            if m % 2 == 0:
                return (re - d if m else re + d), im
            return re, (im - d if (m == 1) == (g < NPOS // 2) else im + d)

        before = None if m == 0 else khat[0].at[c % 2] if m == 1 else kraw[m % 2]
        for g, kk in enumerate(spectrum_groups(ktile[m], skip)):
            for k2 in range(4):
                re, im = kk[k2]
                if 0 < m < NCH - 1:
                    store_group(kraw[(m + 1) % 2], k2, g, kk[k2])
                if m > 0:
                    pre, pim = load_group(before, k2, g)
                    re, im = (re - pim, im + pre) if g < NPOS // 2 else (re + pim, im - pre)
                store_group(khat[m].at[c % 2], k2, g, (re, im))
            yield

    def signal_spectrum(c, j):
        for g, uu in enumerate(spectrum_groups(utile[j])):
            for k2 in range(4):
                store_group(uhat[j], k2, g, uu[k2])
            yield

    def chunk_product(c, i):
        for g in range(NPOS):
            ys = []
            for k2 in range(4):
                yr = yi = None
                for j in range(i + 1):
                    kr, ki = load_group(khat[i - j].at[c % 2], k2, g)
                    ur, ui = load_group(uhat[j], k2, g)
                    if j == 0 and k2 == 0:
                        kr = paced(kr)
                    pr, pi = kr * ur - ki * ui, kr * ui + ki * ur
                    yr, yi = (pr, pi) if yr is None else (yr + pr, yi + pi)
                ys.append((yr, yi))
                if k2 == 3:
                    for p, pair in enumerate(_radix4(ys, True)):
                        _put(g_s[i], (), p, slice(16 * g, 16 * g + 16), jnp.concatenate(pair, axis=0))
                yield

    def inverse_dft(c, i):
        y = None
        for n in range(2):
            part = [_dot(_bf16(_get(inv_v, (p,), n, 1)),
                         _bf16(_get(g_s[i], (), p + zero, 1, slice(n * L // 2, (n + 1) * L // 2))))
                    for p in range(4)]
            for r in range(0, L, 16):
                latest[0] = part[0][r:r + 8]
                if y is not None:
                    for o in (r, r + 8):
                        for p in range(4):
                            y_s[c, pl.ds(i * C + 4 * o + p, 8, stride=4), :] = (
                                y[p][o:o + 8] + part[p][o:o + 8])
                yield
            y = part

    dft_matrices()
    mark_s[...] = _get(fwd_v, (), 0, 1, slice(0, 8))
    g_s[NCH - 1][...] = jnp.zeros(g_s[NCH - 1].shape, BF16)
    k_v[:, 0:8, :] = jnp.zeros((NCT, 8, L), U32)
    wait("small")
    probe = lax.bitcast_convert_type(mark_s[...], jnp.int32)[0, 0]
    zero = (probe == NEVER).astype(jnp.int32)
    n_blocks = itertools.count()

    def block(name, *streams):
        latest[0] = None

        @pl.when(probe != NEVER + next(n_blocks))
        def _():
            with _scope(name):
                _interleave(*streams)

        latest[0] = None

    dvec = ssmd_v[...].astype(F32)
    taps = shift_v[...].astype(F32)
    for i in range(NCT):
        chan_s[i, KS] = jnp.broadcast_to(dvec[i:i + 1], (8, L))
        for t in range(KS):
            chan_s[i, t] = jnp.broadcast_to(taps[t:t + 1, i * L:(i + 1) * L], (8, L))

    stages = dict(T=filter_tiles, A=signal_tiles, K=filter_spectrum, B=signal_spectrum,
                  C=chunk_product, D=inverse_dft)

    def conv_stages(c, plan):
        def stage(x):
            tile = c + 1 if x in CONV_AHEAD else jnp.maximum(c - 1, 0) if x == "D3" else c
            return stages[x[0]](tile, int(x[1]))

        streams = {x: stage(x) for x in plan[0].split() + plan[1].split()}
        latest[0] = None
        for x in _conv_schedule(*plan):
            next(streams[x])
        latest[0] = None
        yield

    def conv_step(c, carry):
        wait_step(c, lambda n: [f"tile{n}"], range(NCT - 1))
        _interleave((conv_stages(c, CONV_STEP), 1))
        return carry

    block("fill", (itertools.chain(*[stages[x[0]](0, int(x[1])) for x in CONV_AHEAD]), 1))
    with _scope("conv"):
        lax.fori_loop(0, NCT - 1, conv_step, 0)

    def gated_residual(i, r, x, y0, normed=None):
        y = jnp.concatenate([y0] + [y_s[c, span(i * C + r, 16), :] for c in range(1, NCT)], axis=1)
        x1 = []
        for rows8 in (slice(0, 8), slice(8, 16)):
            xn = _layernorm_rows(x[rows8]) if normed is None else normed[rows8]
            x1.append(x[rows8] + (xn * mod_s[0] + mod_s[1]) * y[rows8])
        _put(x1_s, (i,), 0, slice(r, r + 16), jnp.concatenate(x1, axis=0))
        return [_layernorm_rows(x) for x in x1]

    def store_modulated(r, h):
        ops = [_strassen_rhs(h[0][s][:, :DM], h[1][s][:, :DM],
                             h[0][s][:, DM:2 * DM], h[1][s][:, DM:2 * DM]) for s in range(2)]
        for q in range(7):
            _put(hq_s, (q,), 0, slice(r, r + 16), jnp.concatenate([ops[0][q], ops[1][q]], axis=0))
        for a in range(2):
            _put(hr_s, (), 0, slice(a * CH + r, a * CH + r + 16),
                 jnp.concatenate(h[a], axis=0)[:, 2 * DM:])

    def paced_rows(words):
        words = jnp.concatenate([paced(words[:, :L]), words[:, L:]], axis=1)
        return _f32(words)

    def residual_stage(i):
        for r in range(0, CH, 16):
            normed = []
            for a in range(2):
                row = a * CH + r
                x = paced_rows(q_v[span(i * CH + row // 2, 8), :])
                normed.append([xn * mod_s[2] + mod_s[3] for xn in gated_residual(
                    i, row, x, y_s[0, span(i * C + row, 16), :])])
                if a == 1:
                    store_modulated(r, normed)
                yield

    cv = c_v[...].astype(F32)
    act = jnp.broadcast_to(cv * jax.nn.sigmoid(cv), (16, D)).astype(BF16)

    def modulation(i):
        return _dot(act, _bf16(wmod_v[:, i * D:(i + 1) * D]))[:8]

    def first_gate():
        sa, ca, ga = [modulation(i) for i in range(3)]
        mod_s[0] = (1.0 + ca) * ga
        mod_s[1] = sa * ga
        latest[0] = ga[:, :L]
        yield

    def first_norm():
        for r in range(0, C, 16):
            xn_s[r:r + 16, :] = _layernorm_rows(paced_rows(q_v[r // 2:r // 2 + 8, :]))
            yield

    def first_residual():
        done = []
        for r in range(0, C, 16):
            latest[0] = done[-DEPTH] if len(done) >= DEPTH else None
            xn = gated_residual(0, r, _f32(q_v[r // 2:r // 2 + 8, :]), paced(y_s[0, r:r + 16, :]),
                                xn_s[r:r + 16, :])
            xn_s[r:r + 16, :] = jnp.concatenate(xn, axis=0)
            done.append(xn[1][:, :L])
            yield

    def first_modulate():
        wait("second")
        shift, scale = modulation(3), 1.0 + modulation(4)
        mod_s[2] = scale
        mod_s[3] = shift
        for r in range(0, CH, 16):
            store_modulated(r, [[xn_s[pl.ds(a * CH + r + 8 * s, 8), :] * scale + shift
                                 for s in range(2)] for a in range(2)])
        yield

    wait(f"tile{NCT - 1}")
    block("conv_last", (conv_stages(NCT - 1, CONV_LAST), 1))
    wait("first")
    block("norm0", (itertools.chain(inverse_dft(NCT - 1, 3), first_gate()), 2 * NPOS),
          _spread(first_norm(), CH // 8, 0.0, 0.5))
    block("res0", (first_residual(), 1))
    block("mod", (first_modulate(), 1))

    def hidden_stage(i, first=False):
        def weight_sums(r0):
            for r in range(r0 // 2, (r0 + MB) // 2, 8):
                top, bot = slice(r, r + 8), slice(r + FQ // 2, r + FQ // 2 + 8)
                w = [paced(wi_v[top, :DM]), wi_v[top, DM:2 * DM],
                     wi_v[bot, :DM], paced(wi_v[bot, DM:2 * DM])]
                ops = _strassen_lhs(*[_f32(x) for x in w])
                for slot, q in enumerate(SUMMED_LHS):
                    _put(wq_s, (slot,), 0, slice(2 * r, 2 * r + 16), ops[q])
                yield

        def preact(r0, complete):
            top = slice(r0 // 2, (r0 + MB) // 2)
            bot = slice((r0 + FQ) // 2, (r0 + FQ + MB) // 2)
            following = 0 if r0 + MB == FH + FQ else r0 + MB
            sums = weight_sums(r0) if first else iter(())

            def product(q):
                if first and q == WAIT_AT and following in wi_groups:
                    wait(f"wi{following}")
                w = (wi_v[top, :DM] if q == 2 else wi_v[bot, DM:2 * DM] if q == 3
                     else _get(wq_s, (SUMMED_LHS.index(q),), 0, DM // L, top))
                m = _dot_nt(_bf16(w), _bf16(_get(hq_s, (q,), 0, DM // L)))
                for _ in ticks(m):
                    next(sums, None)
                    yield
                return m

            rest = []
            for part in (top, bot):
                rest.append(_dot_nt(_bf16(wi_v[part, 2 * DM:]), _bf16(_get(hr_s, (), 0, 1))))
                for _ in ticks(rest[-1]):
                    next(sums, None)
                    yield
            yield from _strassen_product(
                product, (2, 3, 4, 1, 0, 6, 5),
                [_pieces(rest[b // 2][:, (b % 2) * CH:(b % 2 + 1) * CH]) for b in range(4)], complete)

        def column_mean(acc):
            return jnp.broadcast_to(jnp.sum(acc, axis=0, keepdims=True) * (1.0 / FH), (8, C))

        total = [jnp.zeros((8, CH), F32)] * 2

        def activate():
            for r0 in range(0, FQ, MB):
                def complete(b, z):
                    for n, x in enumerate(z):
                        a = _gelu2(x)
                        f = (b // 2) * FQ + r0 + 16 * n
                        a_s[f:f + 16, (b % 2) * CH:(b % 2 + 1) * CH] = a
                        total[b % 2] = total[b % 2] + (a[:8] + a[8:])

                yield from preact(FH + r0, complete)

        def layernorm():
            mean = column_mean(jnp.concatenate(total, axis=1))
            acc = jnp.zeros((8, C), F32)
            for r in range(0, FH, 32):
                d = _tiles(a_s[r:r + 32, :]) - paced(mean)
                acc = acc + (d * d).sum(axis=0)
                yield
            rstd = lax.rsqrt(column_mean(acc) + 4.0 * EPS)
            means = [mean[:, c0:c0 + L] for c0 in range(0, C, L)]
            for r in range(0, FQ, 16):
                for c0 in range(0, CH, L):
                    blocks = []
                    for o in (0, FQ):
                        for cols in (slice(c0, c0 + L), slice(CH + c0, CH + c0 + L)):
                            m = means[cols.start // L]
                            if (o == 0) == (cols.start == c0):
                                m = paced(m)
                            d = (_tiles(a_s[o + r:o + r + 16, cols]) - m) * rstd[:, cols]
                            blocks.append(d.reshape(16, L))
                    for q, op in enumerate(_strassen_lhs(*blocks)):
                        _put(z2_s, (q,), c0 // L, slice(r, r + 16), op)
                    yield

        def gate():
            for r0 in range(0, FQ, MB):
                def complete(b, z):
                    for n, x in enumerate(z):
                        f = (b // 2) * FQ + r0 + 16 * n
                        _put(z1_s, (i,), 2 * (b % 2), slice(f, f + 16), _gelu2(x))

                yield from preact(r0, complete)

        return ((itertools.chain(activate(), gate()), 18 * FQ // TICK),
                _spread(layernorm(), FH // 32 + FQ // 8, 0.51, FILL))

    def mixer_sums(i, n):
        left, right = span(i * C, CH), span(i * C + CH, CH)
        for r in range(0, L, 8):
            top, bot = span(n * CH + r, 8), span(n * CH + L + r, 8)
            w = [paced(wsp_v[top, left]), wsp_v[bot, left],
                 wsp_v[top, right], paced(wsp_v[bot, right])]
            ops = _strassen_rhs(*[_f32(x) for x in w])
            for slot, q in enumerate(SUMMED):
                _put(wb_s, (slot, n), 0, slice(2 * r, 2 * r + 16), ops[q])
            yield

    def mixer_operand(i, q, n):
        if q in SUMMED:
            return _get(wb_s, (SUMMED.index(q), n), 0, 2)
        o = 0 if q == 1 else 1
        return wsp_v[span(n * CH + o * L, L), span(i * C + o * CH, CH)]

    def mixer_partial(i):
        for products in ((1, 4), SUMMED):
            for n in range(0, NCH, 2):
                for q in products:
                    w = jnp.concatenate([mixer_operand(i, q, n + o) for o in range(2)], axis=0)
                    for r0 in range(0, FQ, MP):
                        z = _get(z2_s, (q,), 0, 2, slice(r0 // 2, (r0 + MP) // 2))
                        m = _dot_nt(_bf16(z), _bf16(w))
                        for r in range(0, MP, 8):
                            at = (q, slice(r0 + r, r0 + r + 8), slice(n * CH, (n + 2) * CH))
                            m_s[at] = jnp.where(i > 0, m_s[at], 0.0) + m[r:r + 8]
                        yield from ticks(m)

    def output_operands(i):
        for a in range(2):
            f = pl.multiple_of(a * FQ + i * L, 16)
            wot_s[a] = wo_v[pl.ds(f, L), :].T
        for r in range(0, DH, 16):
            w = [_get(wot_s, (), b % 2, 1, pl.ds((r + (b // 2) * DH) // 2, 8)) for b in range(4)]
            w[0], w[3] = paced(w[0]), paced(w[3])
            for q, op in enumerate(_strassen_lhs(*[_f32(x) for x in w])):
                _put(woq_s, (q,), i, slice(r, r + 16), op)
            yield

    wait(f"wi{FH}")
    block("hidden0", *hidden_stage(0, first=True))

    wait("chunk0")

    def chunk_step(i, carry):
        block("partial", (mixer_partial(i), 14 * FQ // TICK),
              _spread(itertools.chain(*[mixer_sums(i, n) for n in range(NCH)]),
                      NCH * L // 8, 0.0, SUMS_END),
              _spread(residual_stage(i + 1), CH // 8, RES_START, RES_END))
        wait_step(i, lambda n: [f"chunk{n + 1}"], range(NCH - 1))
        block("hidden", *hidden_stage(i + 1), _spread(output_operands(i), DH // 16, 0.1, 0.45))
        return carry

    lax.fori_loop(0, NCH - 1, chunk_step, 0)

    def gated_product(n):
        for r0, r1 in GATE_ROWS:
            def product(q):
                m = yield from ticks(_dot_nt(_bf16(_get(z2_s, (q,), 0, 2, slice(r0 // 2, r1 // 2))),
                                             _bf16(mixer_operand(NCH - 1, q, n))))
                return m_s[q, r0:r1, span(n * CH, CH)] + m

            p = {}

            def complete(b, g):
                t = span(n * C + (b % 2) * CH, CH)
                p[b] = []
                for k, x in enumerate(g):
                    r = r0 + 16 * k
                    f = ((b // 2) * FQ + r) // 2
                    z1 = _f32(_get(z1_s, (n,), 2 * (b % 2), 2, slice(f, f + 8)))
                    p[b].append(z1 * (_tiles(x) + bsp_s[:, t]).reshape(16, CH))
                    if r >= FM:
                        f = (b // 2) * (FQ - FM) + r - FM
                        _put(pr_s, (), 2 * (b % 2), slice(f, f + 16), p[b][k])
                        continue
                    ops = _strassen_rhs(*[p[a][k] if a in p else x for a in range(4)])
                    for q, needs in enumerate(STRASSEN_RHS_NEEDS):
                        if b in needs and all(a in p for a in needs):
                            _put(pq_s, (q,), 0, slice(r, r + 16), ops[q])

            yield from _strassen_product(product, GATE_ORDER, [None] * 4, complete)

    def project():
        rest = yield from ticks(_dot(wor_s[...], _bf16(_get(pr_s, (), 0, C // L))))

        def complete(b, o):
            for k, x in enumerate(o):
                d = (b // 2) * DH + 16 * k
                o_s[b % 2, d:d + 16, :] = x

        yield from _strassen_product(
            lambda q: ticks(_dot(_bf16(_get(woq_s, (q,), 0, FM // L)),
                                 _bf16(_get(pq_s, (q,), 0, 2)))), (1, 3, 4, 0, 6, 2, 5),
            [_pieces(rest[(b // 2) * DH:(b // 2 + 1) * DH, (b % 2) * CH:(b % 2 + 1) * CH])
             for b in range(4)], complete)

    def out_copy(row, n, c0=0, c1=NCT):
        at = (span(row, n), slice(c0 * L, c1 * L))
        return pltpu.make_async_copy(out_v.at[at], out_hbm.at[at], out_sem.at[0])

    def finish(n, h, c0=0, c1=NCT):
        for c in reversed(range(c0, c1)):
            for t0 in range(0, CH, L):
                cols = slice(c * L, (c + 1) * L)
                o = o_s[h, cols, t0:t0 + L].T
                x1 = _f32(_get(x1_s, (n,), c, 1, pl.ds((h * CH + t0) // 2, L // 2)))
                res = _tiles(x1) + mod_s[4, :, cols] * _tiles(o)
                out_v[span(n * C + h * CH + t0, L), cols] = res.reshape(L, L).astype(BF16)
                yield

    bvec = bsp_v[...].astype(F32)
    for i in range(S // L):
        bsp_s[:, i * L:(i + 1) * L] = jnp.broadcast_to(bvec[i:i + 1], (8, L))
    wor_s[...] = jnp.concatenate([wo_v[FM:FQ, :], wo_v[FQ + FM:FH, :]], axis=0).T
    gate_ticks = 7 * sum(-(-(b - a) // TICK) for a, b in GATE_ROWS)
    _interleave((gated_product(0), gate_ticks), (mixer_sums(NCH - 1, 0), 10 * L // 8 + 8))
    mod_s[4] = 0.5 * modulation(5)

    def output_step(n, carry):
        @pl.when(n > 0)
        def _():
            out_copy((n - 1) * C, C).start()

        latest[0] = None
        _interleave((project(), -(-D // TICK) + 7 * -(-DH // TICK)),
                    _spread(mixer_sums(NCH - 1, n + 1), L // 8, 0.0, 0.7))
        _interleave((gated_product(n + 1), gate_ticks),
                    _spread(itertools.chain(finish(n, 0), finish(n, 1)),
                            4 * NCT, 0.0, FINISH_END))
        return carry

    with _scope("output"):
        lax.fori_loop(0, NCH - 1, output_step, 0)
    out_copy((NCH - 2) * C, C).start()
    _interleave((project(), 1))
    latest[0] = None
    last_parts = ((0, 0, NCT), (1, 0, DH // L), (1, DH // L, NCT))
    for h, c0, c1 in last_parts:
        _interleave((finish(NCH - 1, h, c0, c1), 1))
        out_copy((NCH - 1) * C + h * CH, CH, c0, c1).start()
    for n in range(NCH - 1):
        out_copy(n * C, C).wait()
    for h, c0, c1 in last_parts:
        out_copy((NCH - 1) * C + h * CH, CH, c0, c1).wait()


@jax.jit
def pallas_adaLN_cond__ssm_conv_h3__mixer_gmlp__prompt_kernel(
    A_q: jax.Array,
    A_k: jax.Array,
    A_v: jax.Array,
    A_shift_k: jax.Array,
    A_ssm_k: jax.Array,
    A_ssm_D: jax.Array,
    B_x: jax.Array,
    B_w_in: jax.Array,
    B_w_sp: jax.Array,
    B_b_sp: jax.Array,
    B_w_out: jax.Array,
    c: jax.Array,
    w_mod: jax.Array,
):
    del B_x
    operands = (
        A_q.reshape(S, D), A_k.reshape(S, D), A_v.reshape(S, D), A_shift_k.T, A_ssm_k,
        A_ssm_D.reshape(NCT, L), B_w_in.T, B_w_sp, B_b_sp.reshape(S // L, L), B_w_out, c, w_mod,
    )
    def planes(*shape):
        return pltpu.VMEM((*shape, L), BF16)

    spectrum = pltpu.VMEM((4, 2 * L, L), F32)
    scratch = [
        pltpu.VMEM((S // 2, D), U32),
        pltpu.VMEM((NCT, 16 + S // 2, L), U32),
        pltpu.VMEM((NCT, 8 + S // 2, L), U32),
        pltpu.VMEM((KS, D), BF16),
        pltpu.VMEM((DH, S), U32),
        pltpu.VMEM((NCT, L), BF16),
        pltpu.VMEM((FH, D), U32),
        pltpu.VMEM((S // 2, S), U32),
        pltpu.VMEM((S // L, L), BF16),
        pltpu.VMEM((FH, D), BF16),
        pltpu.VMEM((1, D), BF16),
        pltpu.VMEM((DH, 6 * D), U32),
        planes(4, 2 * L),
        planes(4, 2, L),
        pltpu.VMEM((S, D), BF16),
        pltpu.VMEM((8, L), U32),
        pltpu.VMEM((NCT, KS + 1, 8, L), F32),
        pltpu.VMEM((8, S), F32),
        pltpu.VMEM((5, 8, D), F32),
        [pltpu.VMEM((CH + 8, L), U32)] * NCH,
        [planes(4, L)] * NCH,
        [planes(4, L)] * NCH,
        [spectrum] * 2,
        [pltpu.VMEM((2, 4, 2 * L, L), F32)] * NCH,
        [spectrum] * NCH,
        [planes(4, 2 * L)] * NCH,
        pltpu.VMEM((NCT, S + 8, L), F32),
        planes(NCH, NCT, C),
        pltpu.VMEM((C, D), F32),
        planes(7, DM // L, CH),
        planes(1, C),
        planes(5, DM // L, 2 * FH),
        pltpu.VMEM((FH, C), F32),
        planes(NCH, C // L, FH),
        planes(7, 2, FQ),
        planes(5, NCH, 2, CH),
        pltpu.VMEM((7, FQ, S // 2), F32),
        planes(2, D),
        pltpu.VMEM((D, FH - 2 * FM), BF16),
        planes(7, FM // L, DH),
        planes(7, 2, FM),
        planes(C // L, FH - 2 * FM),
        pltpu.VMEM((2, D, CH), F32),
        pltpu.SemaphoreType.DMA((15,)),
        pltpu.SemaphoreType.DMA((1,)),
    ]
    out = pl.pallas_call(
        _kernel,
        out_shape=jax.ShapeDtypeStruct((S, D), BF16),
        in_specs=[pl.BlockSpec(memory_space=pltpu.HBM)] * len(operands),
        out_specs=pl.BlockSpec(memory_space=pltpu.HBM),
        scratch_shapes=scratch,
        compiler_params=pltpu.CompilerParams(
            vmem_limit_bytes=120 * 1024 * 1024,
            flags={"XLA_TPU_EVENLY_DISTRIBUTE_CRITICAL_NODES": True}),
    )(*operands)
    return out.reshape(1, S, D)
```

```python
import contextlib
import itertools

import numpy as np

import jax
import jax.numpy as jnp
from jax import lax
import jax.experimental.pallas as pl
import jax.experimental.pallas.tpu as pltpu

S = 2048
D = 640
FH = 864
FQ = FH // 2
KS = 4
L = 128
NCT = D // L
C = 512
CH = C // 2
NCH = S // C
NPOS = 16
TICK = 24
TICKS = 3
FINISH_END = 0.9
RES_START = 0.352
RES_END = 0.882
GATE_ORDER = (1, 4, 2, 0, 5, 3, 6)
MP = 432
SUMS_END = 0.269
WAIT_AT = 6
FILL = 0.97
MB = 144
DEPTH = 11
DH = D // 2
FM = 384
GATE_ROWS = ((0, 176), (176, 320), (320, FQ))
CONV_STEP = ("K3 D3 B0 B1 D0 B2 D1 B3 D2 K0 K1 K2", "A0 A1 T3 T2 A3 C0 A2 C1 T0 C2 T1 C3", 71)
CONV_AHEAD = "T0 T1 T2 T3 K0 K1 K2".split()
CONV_LAST = ("K3 D3 B0 B1 D0 B2 D1 B3 D2", "A0 A1 A2 C0 A3 C1 C2 C3", 71)
CONV_LEAD = 4
DM = 256
SUMMED_LHS = (0, 1, 4, 5, 6)
SUMMED = (0, 2, 3, 5, 6)
NEVER = 0x7F7F7F7F
EPS = 1e-5
GELU_C0 = float(np.sqrt(2.0 / np.pi))
GELU_C1 = GELU_C0 * 0.044715

F32 = jnp.float32
BF16 = jnp.bfloat16
U32 = jnp.uint32
NT_DIMS = (((1,), (1,)), ((), ()))

TRACE_SCOPES = [False]


def _scope(name):
    return jax.named_scope("ph_" + name) if TRACE_SCOPES[0] else contextlib.nullcontext()


def _lo(w):
    return lax.bitcast_convert_type(w << 16, F32)


def _hi(w):
    return lax.bitcast_convert_type(w & np.uint32(0xFFFF0000), F32)


def _bf16(words):
    return pltpu.bitcast(words, BF16)


def _f32(words):
    return _bf16(words).astype(F32)


def _put(ref, lead, first, rows, x):
    for n in range(x.shape[1] // L):
        ref[(*lead, first + n, rows)] = x[:, n * L:(n + 1) * L].astype(BF16)


def _get(ref, lead, first, count, word_rows=slice(None)):
    return jnp.concatenate(
        [ref.bitcast(U32)[(*lead, first + n, word_rows)] for n in range(count)], axis=1)


def _dot(a, b):
    return jnp.dot(a, b, preferred_element_type=F32)


def _dot_nt(a, b):
    return lax.dot_general(a, b, NT_DIMS, preferred_element_type=F32)


def _tiles(x):
    return x.reshape(x.shape[0] // 8, 8, x.shape[1])


def _interleave(*streams):
    steps = sorted(((k + 0.5) / n, i) for i, (_, n) in enumerate(streams) for k in range(n))
    for _, i in steps:
        next(streams[i][0], None)
    for stream, _ in streams:
        for _ in stream:
            pass


def _spread(stream, n, start, end):
    per_unit = n / (end - start)
    return itertools.chain(range(round(start * per_unit)), stream), round(per_unit)


def _conv_schedule(matmuls, vector, per_step):
    steps = dict(T=8, A=16, C=4 * NPOS)
    cost = dict(T=(24,) * 4, A=(46,) * 4, C=(12, 20, 28, 36), K=(17, 25, 25, 25),
                B=(16,) * 4, D=(6,) * 4)
    vector = [(x, k) for x in vector.split() for k in range(steps[x[0]])]
    matmul = [(x, k) for x in matmuls.split() for k in range(NPOS)]
    order, done, budget = [], set(), 0
    for n, (x, k) in enumerate(matmul):
        for ahead, _ in matmul[n:n + CONV_LEAD + 1]:
            need = dict(K="T", B="A", D="C")[ahead[0]] + ahead[1]
            while ahead not in ("K3", "D3") and any(v == need for v, _ in vector):
                order.append(vector.pop(0)[0])
                budget -= cost[order[-1][0]][int(order[-1][1])]
        order.append(x)
        done.add((x, k))
        budget = min(budget + per_step - cost[x[0]][int(x[1])], per_step)
        while vector and budget > 0:
            v, j = vector[0]
            if v[0] == "C" and ("B" + v[1], j // 4) not in done:
                break
            order.append(vector.pop(0)[0])
            budget -= cost[v[0]][int(v[1])]
    return order + [v for v, _ in vector]


def _radix4(e, inverse):
    (r0, i0), (r1, i1), (r2, i2), (r3, i3) = e
    sr, si, dr, di = r0 + r2, i0 + i2, r0 - r2, i0 - i2
    tr, ti, ur, ui = r1 + r3, i1 + i3, r1 - r3, i1 - i3
    a = (dr + ui, di - ur)
    b = (dr - ui, di + ur)
    if inverse:
        a, b = b, a
    return [(sr + tr, si + ti), a, (sr - tr, si - ti), b]


def _strassen_lhs(a11, a12, a21, a22):
    return [a11 + a22, a21 + a22, a11, a22, a11 + a12, a21 - a11, a12 - a22]


STRASSEN_RHS_NEEDS = ((0, 3), (0,), (1, 3), (0, 2), (3,), (0, 1), (2, 3))


def _strassen_rhs(b11, b12, b21, b22):
    return [b11 + b22, b11, b12 - b22, b21 - b11, b22, b11 + b12, b21 + b22]


STRASSEN_USES = ({0: 1, 3: 1}, {2: 1, 3: -1}, {1: 1, 3: 1}, {0: 1, 2: 1}, {0: -1, 1: 1}, {3: 1}, {0: 1})


def _pieces(x):
    return [x[r:r + 16] for r in range(0, x.shape[0], 16)]


def _strassen_product(product, order, blocks, complete):
    blocks = list(blocks)
    for n, q in enumerate(order):
        m = _pieces((yield from product(q)))
        for b, sign in STRASSEN_USES[q].items():
            if blocks[b] is None:
                blocks[b] = m if sign > 0 else [-x for x in m]
            else:
                blocks[b] = [x + y if sign > 0 else x - y for x, y in zip(blocks[b], m)]
            if not any(b in STRASSEN_USES[later] for later in order[n + 1:]):
                complete(b, blocks[b])


def _gelu2(x):
    t = jnp.tanh(x * (x * x * GELU_C1 + GELU_C0))
    return x * t + x


def _layernorm_rows(x):
    d = x - jnp.sum(x, axis=-1, keepdims=True) * (1.0 / D)
    var = jnp.sum(d * d, axis=-1, keepdims=True) * (1.0 / D)
    return d * lax.rsqrt(var + EPS)


def _kernel(q_hbm, k_hbm, v_hbm, shift_hbm, ssm_hbm, ssmd_hbm, wi_hbm, wsp_hbm, bsp_hbm,
            wo_hbm, c_hbm, wmod_hbm, out_hbm,
            q_v, k_v, v_v, shift_v, ssm_v, ssmd_v, wi_v, wsp_v, bsp_v, wo_v, c_v, wmod_v,
            fwd_v, inv_v, out_v,
            mark_s, chan_s, bsp_s, mod_s, fstage, ktile, utile, kraw, khat, uhat, g_s, y_s, x1_s, xn_s, hq_s, hr_s, wq_s,
            a_s, z1_s, z2_s, wb_s, m_s, wot_s, wor_s, woq_s, pq_s, pr_s, o_s, sems, out_sem):
    copies = {}

    def queue(name, src, dst):
        group = copies.setdefault(name, [])
        group.append(pltpu.make_async_copy(src, dst, sems.at[list(copies).index(name)]))
        group[-1].start()

    def wait(*names):
        for name in names:
            for copy in copies[name]:
                copy.wait()

    def rows(ref, r0, n):
        return ref.at[pl.ds(r0, n), :]

    def queue_pairs(name, src, dst, r0, n):
        queue(name, rows(src, r0, n), rows(dst, r0 // 2, n // 2).bitcast(BF16))

    def queue_wmod(name, i0, i1):
        queue(name, wmod_hbm.at[:, i0 * D:i1 * D], wmod_v.at[:, i0 * D:i1 * D].bitcast(BF16))

    queue_pairs("small", ssm_hbm, ssm_v, 0, L)
    for src, dst in ((ssmd_hbm, ssmd_v), (shift_hbm, shift_v), (c_hbm, c_v), (bsp_hbm, bsp_v)):
        queue("small", src, dst)
    n = C
    for c in range(NCT):
        for h in range(NCH):
            for src, dst, pad in ((k_hbm, k_v, 8), (v_hbm, v_v, 0)):
                queue(f"tile{c}", src.at[pl.ds(h * n, n), pl.ds(c * L, L)],
                      dst.at[c, pl.ds(pad + h * n // 2, n // 2), :].bitcast(BF16))
        if c + 1 < NCT:
            queue_pairs(f"tile{c}", ssm_hbm, ssm_v, (c + 1) * L, L)
    queue_pairs(f"tile{NCT - 1}", q_hbm, q_v, 0, C)
    queue_wmod("first", 0, 3)
    queue_wmod("second", 3, 5)
    wi_groups = {FH: MB, FH + MB: FQ - MB, 0: FQ}
    for r0, n in wi_groups.items():
        for o in (0, FQ):
            queue_pairs(f"wi{r0}", wi_hbm, wi_v, r0 + o, n)
    for i in range(NCH):
        cols = pl.ds(i * C, C)
        queue(f"chunk{i}", wsp_hbm.at[:, cols], wsp_v.at[:, cols].bitcast(BF16))
        if i + 1 < NCH:
            queue_pairs(f"chunk{i}", q_hbm, q_v, (i + 1) * C, C)
        if i == 1:
            queue("chunk1", wo_hbm, wo_v)
    queue_wmod(f"chunk{NCH - 1}", 5, 6)

    def wait_step(i, names_of, steps):
        for n in steps:
            @pl.when(i == n)
            def _():
                wait(*names_of(n))

    def span(start, size):
        return pl.ds(start if isinstance(start, int) else pl.multiple_of(start, size), size)

    latest = [None]

    def paced(x):
        if latest[0] is None:
            return x
        n = x.shape[1] // L
        if x.shape[0] > 8:
            return jnp.concatenate([paced(x[:8]), x[8:]], axis=0)
        never = jnp.tile(mark_s[...], (1, n)) == NEVER
        return jnp.where(never, lax.bitcast_convert_type(jnp.tile(latest[0], (1, n)), x.dtype), x)

    def ticks(m):
        for r in range(0, m.shape[0], TICK):
            latest[0] = m[r:r + 8, 0:L]
            yield
        return m

    def load_group(ref, k2, g):
        return ref[k2 + zero, 16 * g:16 * g + 8, :], ref[k2 + zero, 16 * g + 8:16 * g + 16, :]

    def store_group(ref, k2, g, val):
        ref[k2, 16 * g:16 * g + 8, :] = val[0]
        ref[k2, 16 * g + 8:16 * g + 16, :] = val[1]

    def spectrum_groups(tiles, adjust=lambda g, pair: pair):
        e = [_dot(_bf16(_get(fwd_v, (), p, 1)), _bf16(_get(tiles, (), p + zero, 1)))
             for p in range(4)]
        for g in range(NPOS):
            latest[0] = e[0][16 * g:16 * g + 8]
            pairs = [(x[16 * g:16 * g + 8], x[16 * g + 8:16 * g + 16]) for x in e]
            yield _radix4([adjust(g, pairs[0])] + pairs[1:], False)

    def dft_matrices():
        sub = lax.broadcasted_iota(jnp.int32, (8, L), 0)
        lane = lax.broadcasted_iota(jnp.int32, (8, L), 1)

        def unit(turns):
            angle = (((turns + 2 * C) & (4 * C - 1)) - 2 * C).astype(F32) * (np.pi / (2 * C))
            return jnp.cos(angle), -jnp.sin(angle)

        def times(a, b):
            return a[0] * b[0] - a[1] * b[1], a[0] * b[1] + a[1] * b[0]

        for p in range(4):
            for inverse in (False, True):
                n1 = lane if inverse else 8 * (lane >> 4) + (lane & 7) + 8 * (lane & 8)
                n = 4 * n1 + p
                even, one, sixteen = unit((4 * sub + 1) * n), unit(2 * n), unit(32 * n)
                for parity in range(2):
                    w, parts = times(even, one) if parity else even, []
                    for _ in range(NPOS // 2):
                        parts += w
                        w = times(w, sixteen)
                    half = jnp.concatenate(parts, axis=0)
                    if inverse:
                        _put(inv_v, (p,), parity, slice(None), (half * (1.0 / C)).T)
                    else:
                        _put(fwd_v, (), p, slice(parity * L, (parity + 1) * L), half)

    def filter_tiles(c, m):
        fstage[m][0:CH, :] = pltpu.bitcast(
            _bf16(ssm_v[span(c * (L // 2), L // 2), m * C:(m + 1) * C]).T, U32)
        for u in range(L // 16):
            for s in range(2):
                a = paced(fstage[m][pl.ds(16 * u + s, 8, stride=2), :])
                b = fstage[m][pl.ds(L + 16 * u + s, 8, stride=2), :]
                for o, half in enumerate((_lo, _hi)):
                    _put(ktile[m], (), 2 * s + o, slice(16 * u, 16 * u + 16),
                         jnp.concatenate([half(a), half(b)], axis=0))
            yield

    def signal_tiles(c, j):
        w1, w2, w3 = [chan_s[c, t] for t in range(1, KS)]
        for u in range(L // 16):
            halves = []
            for h in range(2):
                w0 = paced(chan_s[c, 0])
                r0 = j * CH + h * L + 16 * u
                kw = [k_v[c, pl.ds(8 + r0 + o, 8, stride=2), :] for o in range(-2, 2)]
                vw = [v_v[c, pl.ds(r0 + o, 8, stride=2), :] for o in range(2)]
                ks = [_hi(kw[0])] + [f(x) for x in kw[1:] for f in (_lo, _hi)]
                vs = [f(x) for x in vw for f in (_lo, _hi)]
                halves.append([((w0 * ks[p + 3] + w1 * ks[p + 2]) + (w2 * ks[p + 1] + w3 * ks[p]))
                               * vs[p] for p in range(4)])
                if h == 1:
                    for p in range(4):
                        _put(utile[j], (), p, slice(16 * u, 16 * u + 16),
                             jnp.concatenate([halves[0][p], halves[1][p]], axis=0))
                yield

    def filter_spectrum(c, m):
        def skip(g, pair):
            re, im = pair
            d = chan_s[c, KS]
            if m % 2 == 0:
                return (re - d if m else re + d), im
            return re, (im - d if (m == 1) == (g < NPOS // 2) else im + d)

        before = None if m == 0 else khat[0].at[c % 2] if m == 1 else kraw[m % 2]
        for g, kk in enumerate(spectrum_groups(ktile[m], skip)):
            for k2 in range(4):
                re, im = kk[k2]
                if 0 < m < NCH - 1:
                    store_group(kraw[(m + 1) % 2], k2, g, kk[k2])
                if m > 0:
                    pre, pim = load_group(before, k2, g)
                    re, im = (re - pim, im + pre) if g < NPOS // 2 else (re + pim, im - pre)
                store_group(khat[m].at[c % 2], k2, g, (re, im))
            yield

    def signal_spectrum(c, j):
        for g, uu in enumerate(spectrum_groups(utile[j])):
            for k2 in range(4):
                store_group(uhat[j], k2, g, uu[k2])
            yield

    def chunk_product(c, i):
        for g in range(NPOS):
            ys = []
            for k2 in range(4):
                yr = yi = None
                for j in range(i + 1):
                    kr, ki = load_group(khat[i - j].at[c % 2], k2, g)
                    ur, ui = load_group(uhat[j], k2, g)
                    if j == 0 and k2 == 0:
                        kr = paced(kr)
                    pr, pi = kr * ur - ki * ui, kr * ui + ki * ur
                    yr, yi = (pr, pi) if yr is None else (yr + pr, yi + pi)
                ys.append((yr, yi))
                if k2 == 3:
                    for p, pair in enumerate(_radix4(ys, True)):
                        _put(g_s[i], (), p, slice(16 * g, 16 * g + 16), jnp.concatenate(pair, axis=0))
                yield

    def inverse_dft(c, i):
        y = None
        for n in range(2):
            part = [_dot(_bf16(_get(inv_v, (p,), n, 1)),
                         _bf16(_get(g_s[i], (), p + zero, 1, slice(n * L // 2, (n + 1) * L // 2))))
                    for p in range(4)]
            for r in range(0, L, 16):
                latest[0] = part[0][r:r + 8]
                if y is not None:
                    for o in (r, r + 8):
                        for p in range(4):
                            y_s[c, pl.ds(i * C + 4 * o + p, 8, stride=4), :] = (
                                y[p][o:o + 8] + part[p][o:o + 8])
                yield
            y = part

    dft_matrices()
    mark_s[...] = _get(fwd_v, (), 0, 1, slice(0, 8))
    g_s[NCH - 1][...] = jnp.zeros(g_s[NCH - 1].shape, BF16)
    k_v[:, 0:8, :] = jnp.zeros((NCT, 8, L), U32)
    wait("small")
    probe = lax.bitcast_convert_type(mark_s[...], jnp.int32)[0, 0]
    zero = (probe == NEVER).astype(jnp.int32)
    n_blocks = itertools.count()

    def block(name, *streams):
        latest[0] = None

        @pl.when(probe != NEVER + next(n_blocks))
        def _():
            with _scope(name):
                _interleave(*streams)

        latest[0] = None

    dvec = ssmd_v[...].astype(F32)
    taps = shift_v[...].astype(F32)
    for i in range(NCT):
        chan_s[i, KS] = jnp.broadcast_to(dvec[i:i + 1], (8, L))
        for t in range(KS):
            chan_s[i, t] = jnp.broadcast_to(taps[t:t + 1, i * L:(i + 1) * L], (8, L))

    stages = dict(T=filter_tiles, A=signal_tiles, K=filter_spectrum, B=signal_spectrum,
                  C=chunk_product, D=inverse_dft)

    def conv_stages(c, plan):
        def stage(x):
            tile = c + 1 if x in CONV_AHEAD else jnp.maximum(c - 1, 0) if x == "D3" else c
            return stages[x[0]](tile, int(x[1]))

        streams = {x: stage(x) for x in plan[0].split() + plan[1].split()}
        latest[0] = None
        for x in _conv_schedule(*plan):
            next(streams[x])
        latest[0] = None
        yield

    def conv_step(c, carry):
        wait_step(c, lambda n: [f"tile{n}"], range(NCT - 1))
        _interleave((conv_stages(c, CONV_STEP), 1))
        return carry

    block("fill", (itertools.chain(*[stages[x[0]](0, int(x[1])) for x in CONV_AHEAD]), 1))
    with _scope("conv"):
        lax.fori_loop(0, NCT - 1, conv_step, 0)

    def gated_residual(i, r, x, y0, normed=None):
        y = jnp.concatenate([y0] + [y_s[c, span(i * C + r, 16), :] for c in range(1, NCT)], axis=1)
        x1 = []
        for rows8 in (slice(0, 8), slice(8, 16)):
            xn = _layernorm_rows(x[rows8]) if normed is None else normed[rows8]
            x1.append(x[rows8] + (xn * mod_s[0] + mod_s[1]) * y[rows8])
        _put(x1_s, (i,), 0, slice(r, r + 16), jnp.concatenate(x1, axis=0))
        return [_layernorm_rows(x) for x in x1]

    def store_modulated(r, h):
        ops = [_strassen_rhs(h[0][s][:, :DM], h[1][s][:, :DM],
                             h[0][s][:, DM:2 * DM], h[1][s][:, DM:2 * DM]) for s in range(2)]
        for q in range(7):
            _put(hq_s, (q,), 0, slice(r, r + 16), jnp.concatenate([ops[0][q], ops[1][q]], axis=0))
        for a in range(2):
            _put(hr_s, (), 0, slice(a * CH + r, a * CH + r + 16),
                 jnp.concatenate(h[a], axis=0)[:, 2 * DM:])

    def paced_rows(words):
        words = jnp.concatenate([paced(words[:, :L]), words[:, L:]], axis=1)
        return _f32(words)

    def residual_stage(i):
        for r in range(0, CH, 16):
            normed = []
            for a in range(2):
                row = a * CH + r
                x = paced_rows(q_v[span(i * CH + row // 2, 8), :])
                normed.append([xn * mod_s[2] + mod_s[3] for xn in gated_residual(
                    i, row, x, y_s[0, span(i * C + row, 16), :])])
                if a == 1:
                    store_modulated(r, normed)
                yield

    cv = c_v[...].astype(F32)
    act = jnp.broadcast_to(cv * jax.nn.sigmoid(cv), (16, D)).astype(BF16)

    def modulation(i):
        return _dot(act, _bf16(wmod_v[:, i * D:(i + 1) * D]))[:8]

    def first_gate():
        sa, ca, ga = [modulation(i) for i in range(3)]
        mod_s[0] = (1.0 + ca) * ga
        mod_s[1] = sa * ga
        latest[0] = ga[:, :L]
        yield

    def first_norm():
        for r in range(0, C, 16):
            xn_s[r:r + 16, :] = _layernorm_rows(paced_rows(q_v[r // 2:r // 2 + 8, :]))
            yield

    def first_residual():
        done = []
        for r in range(0, C, 16):
            latest[0] = done[-DEPTH] if len(done) >= DEPTH else None
            xn = gated_residual(0, r, _f32(q_v[r // 2:r // 2 + 8, :]), paced(y_s[0, r:r + 16, :]),
                                xn_s[r:r + 16, :])
            xn_s[r:r + 16, :] = jnp.concatenate(xn, axis=0)
            done.append(xn[1][:, :L])
            yield

    def first_modulate():
        wait("second")
        shift, scale = modulation(3), 1.0 + modulation(4)
        mod_s[2] = scale
        mod_s[3] = shift
        for r in range(0, CH, 16):
            store_modulated(r, [[xn_s[pl.ds(a * CH + r + 8 * s, 8), :] * scale + shift
                                 for s in range(2)] for a in range(2)])
        yield

    wait(f"tile{NCT - 1}")
    block("conv_last", (conv_stages(NCT - 1, CONV_LAST), 1))
    wait("first")
    block("norm0", (itertools.chain(inverse_dft(NCT - 1, 3), first_gate()), 2 * NPOS),
          _spread(first_norm(), CH // 8, 0.0, 0.788))
    block("res0", (first_residual(), 1))
    block("mod", (first_modulate(), 1))

    def hidden_stage(i, first=False):
        def weight_sums(r0):
            for r in range(r0 // 2, (r0 + MB) // 2, 8):
                top, bot = slice(r, r + 8), slice(r + FQ // 2, r + FQ // 2 + 8)
                w = [paced(wi_v[top, :DM]), wi_v[top, DM:2 * DM],
                     wi_v[bot, :DM], paced(wi_v[bot, DM:2 * DM])]
                ops = _strassen_lhs(*[_f32(x) for x in w])
                for slot, q in enumerate(SUMMED_LHS):
                    _put(wq_s, (slot,), 0, slice(2 * r, 2 * r + 16), ops[q])
                yield

        def preact(r0, complete):
            top = slice(r0 // 2, (r0 + MB) // 2)
            bot = slice((r0 + FQ) // 2, (r0 + FQ + MB) // 2)
            following = 0 if r0 + MB == FH + FQ else r0 + MB
            sums = weight_sums(r0) if first else iter(())

            def product(q):
                if first and q == WAIT_AT and following in wi_groups:
                    wait(f"wi{following}")
                w = (wi_v[top, :DM] if q == 2 else wi_v[bot, DM:2 * DM] if q == 3
                     else _get(wq_s, (SUMMED_LHS.index(q),), 0, DM // L, top))
                m = _dot_nt(_bf16(w), _bf16(_get(hq_s, (q,), 0, DM // L)))
                for _ in ticks(m):
                    next(sums, None)
                    yield
                return m

            rest = []
            for part in (top, bot):
                rest.append(_dot_nt(_bf16(wi_v[part, 2 * DM:]), _bf16(_get(hr_s, (), 0, 1))))
                for _ in ticks(rest[-1]):
                    next(sums, None)
                    yield
            yield from _strassen_product(
                product, (2, 3, 4, 1, 0, 6, 5),
                [_pieces(rest[b // 2][:, (b % 2) * CH:(b % 2 + 1) * CH]) for b in range(4)], complete)

        def column_mean(acc):
            return jnp.broadcast_to(jnp.sum(acc, axis=0, keepdims=True) * (1.0 / FH), (8, C))

        total = [jnp.zeros((8, CH), F32)] * 2

        def activate():
            for r0 in range(0, FQ, MB):
                def complete(b, z):
                    for n, x in enumerate(z):
                        a = _gelu2(x)
                        f = (b // 2) * FQ + r0 + 16 * n
                        a_s[f:f + 16, (b % 2) * CH:(b % 2 + 1) * CH] = a
                        total[b % 2] = total[b % 2] + (a[:8] + a[8:])

                yield from preact(FH + r0, complete)

        def layernorm():
            mean = column_mean(jnp.concatenate(total, axis=1))
            acc = jnp.zeros((8, C), F32)
            for r in range(0, FH, 32):
                d = _tiles(a_s[r:r + 32, :]) - paced(mean)
                acc = acc + (d * d).sum(axis=0)
                yield
            rstd = lax.rsqrt(column_mean(acc) + 4.0 * EPS)
            means = [mean[:, c0:c0 + L] for c0 in range(0, C, L)]
            for r in range(0, FQ, 16):
                for c0 in range(0, CH, L):
                    blocks = []
                    for o in (0, FQ):
                        for cols in (slice(c0, c0 + L), slice(CH + c0, CH + c0 + L)):
                            m = means[cols.start // L]
                            if (o == 0) == (cols.start == c0):
                                m = paced(m)
                            d = (_tiles(a_s[o + r:o + r + 16, cols]) - m) * rstd[:, cols]
                            blocks.append(d.reshape(16, L))
                    for q, op in enumerate(_strassen_lhs(*blocks)):
                        _put(z2_s, (q,), c0 // L, slice(r, r + 16), op)
                    yield

        def gate():
            for r0 in range(0, FQ, MB):
                def complete(b, z):
                    for n, x in enumerate(z):
                        f = (b // 2) * FQ + r0 + 16 * n
                        _put(z1_s, (i,), 2 * (b % 2), slice(f, f + 16), _gelu2(x))

                yield from preact(r0, complete)

        return ((itertools.chain(activate(), gate()), 18 * FQ // TICK),
                _spread(layernorm(), FH // 32 + FQ // 8, 0.506, 0.979))

    def mixer_sums(i, n):
        left, right = span(i * C, CH), span(i * C + CH, CH)
        for r in range(0, L, 8):
            top, bot = span(n * CH + r, 8), span(n * CH + L + r, 8)
            w = [paced(wsp_v[top, left]), wsp_v[bot, left],
                 wsp_v[top, right], paced(wsp_v[bot, right])]
            ops = _strassen_rhs(*[_f32(x) for x in w])
            for slot, q in enumerate(SUMMED):
                _put(wb_s, (slot, n), 0, slice(2 * r, 2 * r + 16), ops[q])
            yield

    def mixer_operand(i, q, n):
        if q in SUMMED:
            return _get(wb_s, (SUMMED.index(q), n), 0, 2)
        o = 0 if q == 1 else 1
        return wsp_v[span(n * CH + o * L, L), span(i * C + o * CH, CH)]

    def mixer_partial(i):
        for products in ((1, 4), SUMMED):
            for n in range(0, NCH, 2):
                for q in products:
                    w = jnp.concatenate([mixer_operand(i, q, n + o) for o in range(2)], axis=0)
                    for r0 in range(0, FQ, MP):
                        z = _get(z2_s, (q,), 0, 2, slice(r0 // 2, (r0 + MP) // 2))
                        m = _dot_nt(_bf16(z), _bf16(w))
                        for r in range(0, MP, 8):
                            at = (q, slice(r0 + r, r0 + r + 8), slice(n * CH, (n + 2) * CH))
                            m_s[at] = jnp.where(i > 0, m_s[at], 0.0) + m[r:r + 8]
                        yield from ticks(m)

    def output_operands(i):
        for a in range(2):
            f = pl.multiple_of(a * FQ + i * L, 16)
            wot_s[a] = wo_v[pl.ds(f, L), :].T
        for r in range(0, DH, 16):
            w = [_get(wot_s, (), b % 2, 1, pl.ds((r + (b // 2) * DH) // 2, 8)) for b in range(4)]
            w[0], w[3] = paced(w[0]), paced(w[3])
            for q, op in enumerate(_strassen_lhs(*[_f32(x) for x in w])):
                _put(woq_s, (q,), i, slice(r, r + 16), op)
            yield

    wait(f"wi{FH}")
    block("hidden0", *hidden_stage(0, first=True))

    wait("chunk0")

    def chunk_step(i, carry):
        block("partial", (mixer_partial(i), 14 * FQ // TICK),
              _spread(itertools.chain(*[mixer_sums(i, n) for n in range(NCH)]),
                      NCH * L // 8, 0.0, SUMS_END),
              _spread(residual_stage(i + 1), CH // 8, RES_START, RES_END))
        wait_step(i, lambda n: [f"chunk{n + 1}"], range(NCH - 1))
        block("hidden", *hidden_stage(i + 1), _spread(output_operands(i), DH // 16, 0.121, 0.39))
        return carry

    lax.fori_loop(0, NCH - 1, chunk_step, 0)

    def gated_product(n):
        for r0, r1 in GATE_ROWS:
            def product(q):
                m = yield from ticks(_dot_nt(_bf16(_get(z2_s, (q,), 0, 2, slice(r0 // 2, r1 // 2))),
                                             _bf16(mixer_operand(NCH - 1, q, n))))
                return m_s[q, r0:r1, span(n * CH, CH)] + m

            p = {}

            def complete(b, g):
                t = span(n * C + (b % 2) * CH, CH)
                p[b] = []
                for k, x in enumerate(g):
                    r = r0 + 16 * k
                    f = ((b // 2) * FQ + r) // 2
                    z1 = _f32(_get(z1_s, (n,), 2 * (b % 2), 2, slice(f, f + 8)))
                    p[b].append(z1 * (_tiles(x) + bsp_s[:, t]).reshape(16, CH))
                    if r >= FM:
                        f = (b // 2) * (FQ - FM) + r - FM
                        _put(pr_s, (), 2 * (b % 2), slice(f, f + 16), p[b][k])
                        continue
                    ops = _strassen_rhs(*[p[a][k] if a in p else x for a in range(4)])
                    for q, needs in enumerate(STRASSEN_RHS_NEEDS):
                        if b in needs and all(a in p for a in needs):
                            _put(pq_s, (q,), 0, slice(r, r + 16), ops[q])

            yield from _strassen_product(product, GATE_ORDER, [None] * 4, complete)

    def project():
        rest = yield from ticks(_dot(wor_s[...], _bf16(_get(pr_s, (), 0, C // L))))

        def complete(b, o):
            for k, x in enumerate(o):
                d = (b // 2) * DH + 16 * k
                o_s[b % 2, d:d + 16, :] = x

        def product(q):
            return ticks(_dot(_bf16(_get(woq_s, (q,), 0, FM // L)), _bf16(_get(pq_s, (q,), 0, 2))))

        yield from _strassen_product(
            product, (1, 3, 4, 0, 6, 2, 5),
            [_pieces(rest[(b // 2) * DH:(b // 2 + 1) * DH, (b % 2) * CH:(b % 2 + 1) * CH])
             for b in range(4)], complete)

    def out_copy(row, n, c0=0, c1=NCT):
        at = (span(row, n), slice(c0 * L, c1 * L))
        return pltpu.make_async_copy(out_v.at[at], out_hbm.at[at], out_sem.at[0])

    def finish(n, h, c0=0, c1=NCT):
        for c in reversed(range(c0, c1)):
            for t0 in range(0, CH, L):
                cols = slice(c * L, (c + 1) * L)
                o = o_s[h, cols, t0:t0 + L].T
                x1 = _f32(_get(x1_s, (n,), c, 1, pl.ds((h * CH + t0) // 2, L // 2)))
                res = _tiles(x1) + mod_s[4, :, cols] * _tiles(o)
                out_v[span(n * C + h * CH + t0, L), cols] = res.reshape(L, L).astype(BF16)
                yield

    bvec = bsp_v[...].astype(F32)
    for i in range(S // L):
        bsp_s[:, i * L:(i + 1) * L] = jnp.broadcast_to(bvec[i:i + 1], (8, L))
    wor_s[...] = jnp.concatenate([wo_v[FM:FQ, :], wo_v[FQ + FM:FH, :]], axis=0).T
    gate_ticks = 7 * sum(-(-(b - a) // TICK) for a, b in GATE_ROWS)
    _interleave((gated_product(0), gate_ticks), (mixer_sums(NCH - 1, 0), 10 * L // 8 + 8))
    mod_s[4] = 0.5 * modulation(5)

    def output_step(n, carry):
        @pl.when(n > 0)
        def _():
            out_copy((n - 1) * C, C).start()

        latest[0] = None
        _interleave((project(), -(-D // TICK) + 7 * -(-DH // TICK)),
                    _spread(mixer_sums(NCH - 1, n + 1), L // 8, 0.032, 0.574))
        _interleave((gated_product(n + 1), gate_ticks),
                    _spread(itertools.chain(finish(n, 0), finish(n, 1)),
                            4 * NCT, 0.081, 0.835))
        return carry

    with _scope("output"):
        lax.fori_loop(0, NCH - 1, output_step, 0)
    out_copy((NCH - 2) * C, C).start()
    _interleave((project(), 1))
    latest[0] = None
    last_parts = ((0, 0, NCT), (1, 0, DH // L), (1, DH // L, NCT))
    for h, c0, c1 in last_parts:
        _interleave((finish(NCH - 1, h, c0, c1), 1))
        out_copy((NCH - 1) * C + h * CH, CH, c0, c1).start()
    for n in range(NCH - 1):
        out_copy(n * C, C).wait()
    for h, c0, c1 in last_parts:
        out_copy((NCH - 1) * C + h * CH, CH, c0, c1).wait()


@jax.jit
def pallas_adaLN_cond__ssm_conv_h3__mixer_gmlp__prompt_kernel(
    A_q: jax.Array,
    A_k: jax.Array,
    A_v: jax.Array,
    A_shift_k: jax.Array,
    A_ssm_k: jax.Array,
    A_ssm_D: jax.Array,
    B_x: jax.Array,
    B_w_in: jax.Array,
    B_w_sp: jax.Array,
    B_b_sp: jax.Array,
    B_w_out: jax.Array,
    c: jax.Array,
    w_mod: jax.Array,
):
    del B_x
    operands = (
        A_q.reshape(S, D), A_k.reshape(S, D), A_v.reshape(S, D), A_shift_k.T, A_ssm_k,
        A_ssm_D.reshape(NCT, L), B_w_in.T, B_w_sp, B_b_sp.reshape(S // L, L), B_w_out, c, w_mod,
    )
    def planes(*shape):
        return pltpu.VMEM((*shape, L), BF16)

    spectrum = pltpu.VMEM((4, 2 * L, L), F32)
    scratch = [
        pltpu.VMEM((S // 2, D), U32),
        pltpu.VMEM((NCT, 16 + S // 2, L), U32),
        pltpu.VMEM((NCT, 8 + S // 2, L), U32),
        pltpu.VMEM((KS, D), BF16),
        pltpu.VMEM((DH, S), U32),
        pltpu.VMEM((NCT, L), BF16),
        pltpu.VMEM((FH, D), U32),
        pltpu.VMEM((S // 2, S), U32),
        pltpu.VMEM((S // L, L), BF16),
        pltpu.VMEM((FH, D), BF16),
        pltpu.VMEM((1, D), BF16),
        pltpu.VMEM((DH, 6 * D), U32),
        planes(4, 2 * L),
        planes(4, 2, L),
        pltpu.VMEM((S, D), BF16),
        pltpu.VMEM((8, L), U32),
        pltpu.VMEM((NCT, KS + 1, 8, L), F32),
        pltpu.VMEM((8, S), F32),
        pltpu.VMEM((5, 8, D), F32),
        [pltpu.VMEM((CH + 8, L), U32)] * NCH,
        [planes(4, L)] * NCH,
        [planes(4, L)] * NCH,
        [spectrum] * 2,
        [pltpu.VMEM((2, 4, 2 * L, L), F32)] * NCH,
        [spectrum] * NCH,
        [planes(4, 2 * L)] * NCH,
        pltpu.VMEM((NCT, S + 8, L), F32),
        planes(NCH, NCT, C),
        pltpu.VMEM((C, D), F32),
        planes(7, DM // L, CH),
        planes(1, C),
        planes(5, DM // L, 2 * FH),
        pltpu.VMEM((FH, C), F32),
        planes(NCH, C // L, FH),
        planes(7, 2, FQ),
        planes(5, NCH, 2, CH),
        pltpu.VMEM((7, FQ, S // 2), F32),
        planes(2, D),
        pltpu.VMEM((D, FH - 2 * FM), BF16),
        planes(7, FM // L, DH),
        planes(7, 2, FM),
        planes(C // L, FH - 2 * FM),
        pltpu.VMEM((2, D, CH), F32),
        pltpu.SemaphoreType.DMA((15,)),
        pltpu.SemaphoreType.DMA((1,)),
    ]
    out = pl.pallas_call(
        _kernel,
        out_shape=jax.ShapeDtypeStruct((S, D), BF16),
        in_specs=[pl.BlockSpec(memory_space=pltpu.HBM)] * len(operands),
        out_specs=pl.BlockSpec(memory_space=pltpu.HBM),
        scratch_shapes=scratch,
        compiler_params=pltpu.CompilerParams(
            vmem_limit_bytes=120 * 1024 * 1024,
            flags={"XLA_TPU_EVENLY_DISTRIBUTE_CRITICAL_NODES": True}),
    )(*operands)
    return out.reshape(1, S, D)
```

```python
import contextlib
import itertools

import numpy as np

import jax
import jax.numpy as jnp
from jax import lax
import jax.experimental.pallas as pl
import jax.experimental.pallas.tpu as pltpu

S = 2048
D = 640
DH = D // 2
FH = 864
FQ = FH // 2
KS = 4
L = 128
NCT = D // L
C = 512
CH = C // 2
NCH = S // C
NPOS = 16
DM = 256
FM = 384
SUMMED_LHS = (0, 1, 4, 5, 6)
SUMMED_RHS = (0, 2, 3, 5, 6)
MB = 144
GATE_ROWS = ((0, 176), (176, 320), (320, FQ))
TICK = 24
DEPTH = 11
NEVER = 0x7F7F7F7F
CONV_STEP = ("K3 D3 B0 B1 D0 B2 D1 B3 D2 K0 K1 K2", "A0 A1 T3 T2 A3 C0 A2 C1 T0 C2 T1 C3", 71)
CONV_LAST = ("K3 D3 B0 B1 D0 B2 D1 B3 D2", "A0 A1 A2 C0 A3 C1 C2 C3", 71)
CONV_AHEAD = "T0 T1 T2 T3 K0 K1 K2".split()
CONV_LEAD = 4
EPS = 1e-5
GELU_C0 = float(np.sqrt(2.0 / np.pi))
GELU_C1 = GELU_C0 * 0.044715

F32 = jnp.float32
BF16 = jnp.bfloat16
U32 = jnp.uint32
NT_DIMS = (((1,), (1,)), ((), ()))

TRACE_SCOPES = [False]


def _scope(name):
    return jax.named_scope("ph_" + name) if TRACE_SCOPES[0] else contextlib.nullcontext()


def _lo(w):
    return lax.bitcast_convert_type(w << 16, F32)


def _hi(w):
    return lax.bitcast_convert_type(w & np.uint32(0xFFFF0000), F32)


def _bf16(words):
    return pltpu.bitcast(words, BF16)


def _f32(words):
    return _bf16(words).astype(F32)


def _put(ref, lead, first, rows, x):
    for n in range(x.shape[1] // L):
        ref[(*lead, first + n, rows)] = x[:, n * L:(n + 1) * L].astype(BF16)


def _get(ref, lead, first, count, word_rows=slice(None)):
    return jnp.concatenate(
        [ref.bitcast(U32)[(*lead, first + n, word_rows)] for n in range(count)], axis=1)


def _dot(a, b):
    return jnp.dot(a, b, preferred_element_type=F32)


def _dot_nt(a, b):
    return lax.dot_general(a, b, NT_DIMS, preferred_element_type=F32)


def _tiles(x):
    return x.reshape(x.shape[0] // 8, 8, x.shape[1])


def _interleave(*streams):
    steps = sorted(((k + 0.5) / n, i) for i, (_, n) in enumerate(streams) for k in range(n))
    for _, i in steps:
        next(streams[i][0], None)
    for stream, _ in streams:
        for _ in stream:
            pass


def _spread(stream, n, start, end):
    per_unit = n / (end - start)
    return itertools.chain(range(round(start * per_unit)), stream), round(per_unit)


def _conv_schedule(matmuls, vector, per_step):
    steps = dict(T=8, A=16, C=4 * NPOS)
    cost = dict(T=(24,) * 4, A=(46,) * 4, C=(12, 20, 28, 36), K=(17, 25, 25, 25),
                B=(16,) * 4, D=(6,) * 4)
    vector = [(x, k) for x in vector.split() for k in range(steps[x[0]])]
    matmul = [(x, k) for x in matmuls.split() for k in range(NPOS)]
    order, done, budget = [], set(), 0
    for n, (x, k) in enumerate(matmul):
        for ahead, _ in matmul[n:n + CONV_LEAD + 1]:
            need = dict(K="T", B="A", D="C")[ahead[0]] + ahead[1]
            while ahead not in ("K3", "D3") and any(v == need for v, _ in vector):
                order.append(vector.pop(0)[0])
                budget -= cost[order[-1][0]][int(order[-1][1])]
        order.append(x)
        done.add((x, k))
        budget = min(budget + per_step - cost[x[0]][int(x[1])], per_step)
        while vector and budget > 0:
            v, j = vector[0]
            if v[0] == "C" and ("B" + v[1], j // 4) not in done:
                break
            order.append(vector.pop(0)[0])
            budget -= cost[v[0]][int(v[1])]
    return order + [v for v, _ in vector]


def _radix4(e, inverse):
    (r0, i0), (r1, i1), (r2, i2), (r3, i3) = e
    sr, si, dr, di = r0 + r2, i0 + i2, r0 - r2, i0 - i2
    tr, ti, ur, ui = r1 + r3, i1 + i3, r1 - r3, i1 - i3
    a = (dr + ui, di - ur)
    b = (dr - ui, di + ur)
    if inverse:
        a, b = b, a
    return [(sr + tr, si + ti), a, (sr - tr, si - ti), b]


def _strassen_lhs(a11, a12, a21, a22):
    return [a11 + a22, a21 + a22, a11, a22, a11 + a12, a21 - a11, a12 - a22]


STRASSEN_RHS_NEEDS = ((0, 3), (0,), (1, 3), (0, 2), (3,), (0, 1), (2, 3))


def _strassen_rhs(b11, b12, b21, b22):
    return [b11 + b22, b11, b12 - b22, b21 - b11, b22, b11 + b12, b21 + b22]


STRASSEN_USES = ({0: 1, 3: 1}, {2: 1, 3: -1}, {1: 1, 3: 1}, {0: 1, 2: 1}, {0: -1, 1: 1}, {3: 1}, {0: 1})


def _pieces(x):
    return [x[r:r + 16] for r in range(0, x.shape[0], 16)]


def _strassen_product(product, order, blocks, complete):
    blocks = list(blocks)
    for n, q in enumerate(order):
        m = _pieces((yield from product(q)))
        for b, sign in STRASSEN_USES[q].items():
            if blocks[b] is None:
                blocks[b] = m if sign > 0 else [-x for x in m]
            else:
                blocks[b] = [x + y if sign > 0 else x - y for x, y in zip(blocks[b], m)]
            if not any(b in STRASSEN_USES[later] for later in order[n + 1:]):
                complete(b, blocks[b])


def _gelu2(x):
    t = jnp.tanh(x * (x * x * GELU_C1 + GELU_C0))
    return x * t + x


def _layernorm_rows(x):
    d = x - jnp.sum(x, axis=-1, keepdims=True) * (1.0 / D)
    var = jnp.sum(d * d, axis=-1, keepdims=True) * (1.0 / D)
    return d * lax.rsqrt(var + EPS)


def _kernel(q_hbm, k_hbm, v_hbm, shift_hbm, ssm_hbm, ssmd_hbm, wi_hbm, wsp_hbm, bsp_hbm,
            wo_hbm, c_hbm, wmod_hbm, out_hbm,
            q_v, k_v, v_v, shift_v, ssm_v, ssmd_v, wi_v, wsp_v, bsp_v, wo_v, c_v, wmod_v,
            fwd_v, inv_v, out_v,
            mark_s, chan_s, bsp_s, mod_s, fstage, ktile, utile, kraw, khat, uhat, g_s, y_s,
            x1_s, xn_s, hq_s, hr_s, wq_s, a_s, z1_s, z2_s, wb_s, m_s, wot_s, wor_s, woq_s,
            pq_s, pr_s, o_s, sems, out_sem):
    copies = {}

    def queue(name, src, dst):
        group = copies.setdefault(name, [])
        group.append(pltpu.make_async_copy(src, dst, sems.at[list(copies).index(name)]))
        group[-1].start()

    def wait(*names):
        for name in names:
            for copy in copies[name]:
                copy.wait()

    def rows(ref, r0, n):
        return ref.at[pl.ds(r0, n), :]

    def queue_pairs(name, src, dst, r0, n):
        queue(name, rows(src, r0, n), rows(dst, r0 // 2, n // 2).bitcast(BF16))

    def queue_wmod(name, i0, i1):
        queue(name, wmod_hbm.at[:, i0 * D:i1 * D], wmod_v.at[:, i0 * D:i1 * D].bitcast(BF16))

    queue_pairs("small", ssm_hbm, ssm_v, 0, L)
    for src, dst in ((ssmd_hbm, ssmd_v), (shift_hbm, shift_v), (c_hbm, c_v), (bsp_hbm, bsp_v)):
        queue("small", src, dst)
    for c in range(NCT):
        for n in range(NCH):
            for src, dst, pad, j in ((k_hbm, k_v, 8, n), (v_hbm, v_v, 0, (n + 2) % NCH)):
                queue(f"tile{c}", src.at[pl.ds(j * C, C), pl.ds(c * L, L)],
                      dst.at[c, pl.ds(pad + j * CH, CH), :].bitcast(BF16))
        if c + 1 < NCT:
            queue_pairs(f"tile{c}", ssm_hbm, ssm_v, (c + 1) * L, L)
    queue_pairs(f"tile{NCT - 1}", q_hbm, q_v, 0, C)
    queue_wmod("first", 0, 3)
    queue_wmod("second", 3, 5)
    wi_groups = {FH: MB, FH + MB: FQ - MB, 0: FQ}
    for r0, n in wi_groups.items():
        for o in (0, FQ):
            queue_pairs(f"wi{r0}", wi_hbm, wi_v, r0 + o, n)
    for i in range(NCH):
        cols = pl.ds(i * C, C)
        queue(f"chunk{i}", wsp_hbm.at[:, cols], wsp_v.at[:, cols].bitcast(BF16))
        if i + 1 < NCH:
            queue_pairs(f"chunk{i}", q_hbm, q_v, (i + 1) * C, C)
        if i == 1:
            queue("chunk1", wo_hbm, wo_v)
    queue_wmod(f"chunk{NCH - 1}", 5, 6)

    def wait_step(i, names_of, steps):
        for n in steps:
            @pl.when(i == n)
            def _():
                wait(*names_of(n))

    def span(start, size):
        return pl.ds(start if isinstance(start, int) else pl.multiple_of(start, size), size)

    latest = [None]

    def paced(x):
        if latest[0] is None:
            return x
        if x.shape[0] > 8:
            return jnp.concatenate([paced(x[:8]), x[8:]], axis=0)
        n = x.shape[1] // L
        never = jnp.tile(mark_s[...], (1, n)) == NEVER
        return jnp.where(never, lax.bitcast_convert_type(jnp.tile(latest[0], (1, n)), x.dtype), x)

    def ticks(m):
        for r in range(0, m.shape[0], TICK):
            latest[0] = m[r:r + 8, 0:L]
            yield
        return m

    def load_group(ref, k2, g):
        return ref[k2 + zero, 16 * g:16 * g + 8, :], ref[k2 + zero, 16 * g + 8:16 * g + 16, :]

    def store_group(ref, k2, g, val):
        ref[k2, 16 * g:16 * g + 8, :] = val[0]
        ref[k2, 16 * g + 8:16 * g + 16, :] = val[1]

    def spectrum_groups(tiles, adjust=lambda g, pair: pair):
        e = [_dot(_bf16(_get(fwd_v, (), p, 1)), _bf16(_get(tiles, (), p + zero, 1)))
             for p in range(4)]
        for g in range(NPOS):
            latest[0] = e[0][16 * g:16 * g + 8]
            pairs = [(x[16 * g:16 * g + 8], x[16 * g + 8:16 * g + 16]) for x in e]
            yield _radix4([adjust(g, pairs[0])] + pairs[1:], False)

    def dft_matrices():
        sub = lax.broadcasted_iota(jnp.int32, (8, L), 0)
        lane = lax.broadcasted_iota(jnp.int32, (8, L), 1)

        def unit(turns):
            angle = (((turns + 2 * C) & (4 * C - 1)) - 2 * C).astype(F32) * (np.pi / (2 * C))
            return jnp.cos(angle), -jnp.sin(angle)

        def times(a, b):
            return a[0] * b[0] - a[1] * b[1], a[0] * b[1] + a[1] * b[0]

        for p in range(4):
            for inverse in (False, True):
                n1 = lane if inverse else 8 * (lane >> 4) + (lane & 7) + 8 * (lane & 8)
                n = 4 * n1 + p
                even, one, sixteen = unit((4 * sub + 1) * n), unit(2 * n), unit(32 * n)
                for parity in range(2):
                    w, parts = times(even, one) if parity else even, []
                    for _ in range(NPOS // 2):
                        parts += w
                        w = times(w, sixteen)
                    half = jnp.concatenate(parts, axis=0)
                    if inverse:
                        _put(inv_v, (p,), parity, slice(None), (half * (1.0 / C)).T)
                    else:
                        _put(fwd_v, (), p, slice(parity * L, (parity + 1) * L), half)

    def filter_tiles(c, m):
        fstage[m][0:CH, :] = pltpu.bitcast(
            _bf16(ssm_v[span(c * (L // 2), L // 2), m * C:(m + 1) * C]).T, U32)
        for u in range(L // 16):
            for s in range(2):
                a = paced(fstage[m][pl.ds(16 * u + s, 8, stride=2), :])
                b = fstage[m][pl.ds(L + 16 * u + s, 8, stride=2), :]
                for o, half in enumerate((_lo, _hi)):
                    _put(ktile[m], (), 2 * s + o, slice(16 * u, 16 * u + 16),
                         jnp.concatenate([half(a), half(b)], axis=0))
            yield

    def signal_tiles(c, j):
        w1, w2, w3 = [chan_s[c, t] for t in range(1, KS)]
        for u in range(L // 16):
            halves = []
            for h in range(2):
                w0 = paced(chan_s[c, 0])
                r0 = j * CH + h * L + 16 * u
                kw = [k_v[c, pl.ds(8 + r0 + o, 8, stride=2), :] for o in range(-2, 2)]
                vw = [v_v[c, pl.ds(r0 + o, 8, stride=2), :] for o in range(2)]
                ks = [_hi(kw[0])] + [f(x) for x in kw[1:] for f in (_lo, _hi)]
                vs = [f(x) for x in vw for f in (_lo, _hi)]
                halves.append([((w0 * ks[p + 3] + w1 * ks[p + 2]) + (w2 * ks[p + 1] + w3 * ks[p]))
                               * vs[p] for p in range(4)])
                if h == 1:
                    for p in range(4):
                        _put(utile[j], (), p, slice(16 * u, 16 * u + 16),
                             jnp.concatenate([halves[0][p], halves[1][p]], axis=0))
                yield

    def filter_spectrum(c, m):
        def skip(g, pair):
            re, im = pair
            d = chan_s[c, KS]
            if m % 2 == 0:
                return (re - d if m else re + d), im
            return re, (im - d if (m == 1) == (g < NPOS // 2) else im + d)

        before = None if m == 0 else khat[0].at[c % 2] if m == 1 else kraw[m % 2]
        for g, kk in enumerate(spectrum_groups(ktile[m], skip)):
            for k2 in range(4):
                re, im = kk[k2]
                if 0 < m < NCH - 1:
                    store_group(kraw[(m + 1) % 2], k2, g, kk[k2])
                if m > 0:
                    pre, pim = load_group(before, k2, g)
                    re, im = (re - pim, im + pre) if g < NPOS // 2 else (re + pim, im - pre)
                store_group(khat[m].at[c % 2], k2, g, (re, im))
            yield

    def signal_spectrum(c, j):
        for g, uu in enumerate(spectrum_groups(utile[j])):
            for k2 in range(4):
                store_group(uhat[j], k2, g, uu[k2])
            yield

    def chunk_product(c, i):
        for g in range(NPOS):
            ys = []
            for k2 in range(4):
                yr = yi = None
                for j in range(i + 1):
                    kr, ki = load_group(khat[i - j].at[c % 2], k2, g)
                    ur, ui = load_group(uhat[j], k2, g)
                    if j == 0 and k2 == 0:
                        kr = paced(kr)
                    pr, pi = kr * ur - ki * ui, kr * ui + ki * ur
                    yr, yi = (pr, pi) if yr is None else (yr + pr, yi + pi)
                ys.append((yr, yi))
                if k2 == 3:
                    for p, pair in enumerate(_radix4(ys, True)):
                        _put(g_s[i], (), p, slice(16 * g, 16 * g + 16), jnp.concatenate(pair, axis=0))
                yield

    def inverse_dft(c, i):
        y = None
        for n in range(2):
            part = [_dot(_bf16(_get(inv_v, (p,), n, 1)),
                         _bf16(_get(g_s[i], (), p + zero, 1, slice(n * L // 2, (n + 1) * L // 2))))
                    for p in range(4)]
            for r in range(0, L, 16):
                latest[0] = part[0][r:r + 8]
                if y is not None:
                    for o in (r, r + 8):
                        for p in range(4):
                            y_s[c, pl.ds(i * C + 4 * o + p, 8, stride=4), :] = (
                                y[p][o:o + 8] + part[p][o:o + 8])
                yield
            y = part

    dft_matrices()
    mark_s[...] = _get(fwd_v, (), 0, 1, slice(0, 8))
    g_s[NCH - 1][...] = jnp.zeros(g_s[NCH - 1].shape, BF16)
    k_v[:, 0:8, :] = jnp.zeros((NCT, 8, L), U32)
    wait("small")
    probe = lax.bitcast_convert_type(mark_s[...], jnp.int32)[0, 0]
    zero = (probe == NEVER).astype(jnp.int32)
    n_blocks = itertools.count()

    def block(name, *streams):
        latest[0] = None

        @pl.when(probe != NEVER + next(n_blocks))
        def _():
            with _scope(name):
                _interleave(*streams)

        latest[0] = None

    bvec = bsp_v[...].astype(F32)
    for i in range(S // L):
        bsp_s[:, i * L:(i + 1) * L] = jnp.broadcast_to(bvec[i:i + 1], (8, L))
    dvec = ssmd_v[...].astype(F32)
    taps = shift_v[...].astype(F32)
    for i in range(NCT):
        chan_s[i, KS] = jnp.broadcast_to(dvec[i:i + 1], (8, L))
        for t in range(KS):
            chan_s[i, t] = jnp.broadcast_to(taps[t:t + 1, i * L:(i + 1) * L], (8, L))

    stages = dict(T=filter_tiles, A=signal_tiles, K=filter_spectrum, B=signal_spectrum,
                  C=chunk_product, D=inverse_dft)

    def conv_stages(c, plan):
        def stage(x):
            tile = c + 1 if x in CONV_AHEAD else jnp.maximum(c - 1, 0) if x == "D3" else c
            return stages[x[0]](tile, int(x[1]))

        streams = {x: stage(x) for x in plan[0].split() + plan[1].split()}
        latest[0] = None
        for x in _conv_schedule(*plan):
            next(streams[x])
        latest[0] = None
        yield

    def conv_step(c, carry):
        wait_step(c, lambda n: [f"tile{n}"], range(NCT - 1))
        _interleave((conv_stages(c, CONV_STEP), 1))
        return carry

    block("fill", (itertools.chain(*[stages[x[0]](0, int(x[1])) for x in CONV_AHEAD]), 1))
    with _scope("conv"):
        lax.fori_loop(0, NCT - 1, conv_step, 0)

    def gated_residual(i, r, x, y0, normed=None):
        y = jnp.concatenate([y0] + [y_s[c, span(i * C + r, 16), :] for c in range(1, NCT)], axis=1)
        x1 = []
        for rows8 in (slice(0, 8), slice(8, 16)):
            xn = _layernorm_rows(x[rows8]) if normed is None else normed[rows8]
            x1.append(x[rows8] + (xn * mod_s[0] + mod_s[1]) * y[rows8])
        _put(x1_s, (i,), 0, slice(r, r + 16), jnp.concatenate(x1, axis=0))
        return [_layernorm_rows(x) for x in x1]

    def store_modulated(r, h):
        ops = [_strassen_rhs(h[0][s][:, :DM], h[1][s][:, :DM],
                             h[0][s][:, DM:2 * DM], h[1][s][:, DM:2 * DM]) for s in range(2)]
        for q in range(7):
            _put(hq_s, (q,), 0, slice(r, r + 16), jnp.concatenate([ops[0][q], ops[1][q]], axis=0))
        for a in range(2):
            _put(hr_s, (), 0, slice(a * CH + r, a * CH + r + 16),
                 jnp.concatenate(h[a], axis=0)[:, 2 * DM:])

    def paced_rows(words):
        words = jnp.concatenate([paced(words[:, :L]), words[:, L:]], axis=1)
        return _f32(words)

    def residual_stage(i):
        for r in range(0, CH, 16):
            normed = []
            for a in range(2):
                row = a * CH + r
                x = paced_rows(q_v[span(i * CH + row // 2, 8), :])
                normed.append([xn * mod_s[2] + mod_s[3] for xn in gated_residual(
                    i, row, x, y_s[0, span(i * C + row, 16), :])])
                if a == 1:
                    store_modulated(r, normed)
                yield

    cv = c_v[...].astype(F32)
    act = jnp.broadcast_to(cv * jax.nn.sigmoid(cv), (16, D)).astype(BF16)

    def modulation(i):
        return _dot(act, _bf16(wmod_v[:, i * D:(i + 1) * D]))[:8]

    def first_gate():
        sa, ca, ga = [modulation(i) for i in range(3)]
        mod_s[0] = (1.0 + ca) * ga
        mod_s[1] = sa * ga
        latest[0] = ga[:, :L]
        yield

    def first_norm():
        for r in range(0, C, 16):
            xn_s[r:r + 16, :] = _layernorm_rows(paced_rows(q_v[r // 2:r // 2 + 8, :]))
            yield

    def first_residual():
        done = []
        for r in range(0, C, 16):
            latest[0] = done[-DEPTH] if len(done) >= DEPTH else None
            xn = gated_residual(0, r, _f32(q_v[r // 2:r // 2 + 8, :]), paced(y_s[0, r:r + 16, :]),
                                xn_s[r:r + 16, :])
            xn_s[r:r + 16, :] = jnp.concatenate(xn, axis=0)
            done.append(xn[1][:, :L])
            yield

    def first_modulate():
        wait("second")
        shift, scale = modulation(3), 1.0 + modulation(4)
        mod_s[2] = scale
        mod_s[3] = shift
        for r in range(0, CH, 16):
            store_modulated(r, [[xn_s[pl.ds(a * CH + r + 8 * s, 8), :] * scale + shift
                                 for s in range(2)] for a in range(2)])
        yield

    wait(f"tile{NCT - 1}")
    block("conv_last", (conv_stages(NCT - 1, CONV_LAST), 1))
    wait("first")
    block("norm0", (itertools.chain(inverse_dft(NCT - 1, 3), first_gate()), 2 * NPOS),
          _spread(first_norm(), CH // 8, 0.0, 0.788))
    block("res0", (first_residual(), 1))
    block("mod", (first_modulate(), 1))

    def hidden_stage(i, first=False):
        def weight_sums(r0):
            for r in range(r0 // 2, (r0 + MB) // 2, 8):
                top, bot = slice(r, r + 8), slice(r + FQ // 2, r + FQ // 2 + 8)
                w = [paced(wi_v[top, :DM]), wi_v[top, DM:2 * DM],
                     wi_v[bot, :DM], paced(wi_v[bot, DM:2 * DM])]
                ops = _strassen_lhs(*[_f32(x) for x in w])
                for slot, q in enumerate(SUMMED_LHS):
                    _put(wq_s, (slot,), 0, slice(2 * r, 2 * r + 16), ops[q])
                yield

        def preact(r0, complete):
            top = slice(r0 // 2, (r0 + MB) // 2)
            bot = slice((r0 + FQ) // 2, (r0 + FQ + MB) // 2)
            following = 0 if r0 + MB == FH + FQ else r0 + MB
            sums = weight_sums(r0) if first else iter(())

            def product(q):
                if first and q == 6 and following in wi_groups:
                    wait(f"wi{following}")
                w = (wi_v[top, :DM] if q == 2 else wi_v[bot, DM:2 * DM] if q == 3
                     else _get(wq_s, (SUMMED_LHS.index(q),), 0, DM // L, top))
                m = _dot_nt(_bf16(w), _bf16(_get(hq_s, (q,), 0, DM // L)))
                for _ in ticks(m):
                    next(sums, None)
                    yield
                return m

            rest = []
            for part in (top, bot):
                rest.append(_dot_nt(_bf16(wi_v[part, 2 * DM:]), _bf16(_get(hr_s, (), 0, 1))))
                for _ in ticks(rest[-1]):
                    next(sums, None)
                    yield
            yield from _strassen_product(
                product, (2, 3, 4, 1, 0, 6, 5),
                [_pieces(rest[b // 2][:, (b % 2) * CH:(b % 2 + 1) * CH]) for b in range(4)], complete)

        def column_mean(acc):
            return jnp.broadcast_to(jnp.sum(acc, axis=0, keepdims=True) * (1.0 / FH), (8, C))

        total = [jnp.zeros((8, CH), F32)] * 2

        def activate():
            for r0 in range(0, FQ, MB):
                def complete(b, z):
                    for n, x in enumerate(z):
                        a = _gelu2(x)
                        f = (b // 2) * FQ + r0 + 16 * n
                        a_s[f:f + 16, (b % 2) * CH:(b % 2 + 1) * CH] = a
                        total[b % 2] = total[b % 2] + (a[:8] + a[8:])

                yield from preact(FH + r0, complete)

        def layernorm():
            mean = column_mean(jnp.concatenate(total, axis=1))
            acc = jnp.zeros((8, C), F32)
            for r in range(0, FH, 32):
                d = _tiles(a_s[r:r + 32, :]) - paced(mean)
                acc = acc + (d * d).sum(axis=0)
                yield
            rstd = lax.rsqrt(column_mean(acc) + 4.0 * EPS)
            means = [mean[:, c0:c0 + L] for c0 in range(0, C, L)]
            for r in range(0, FQ, 16):
                for c0 in range(0, CH, L):
                    blocks = []
                    for o in (0, FQ):
                        for cols in (slice(c0, c0 + L), slice(CH + c0, CH + c0 + L)):
                            m = means[cols.start // L]
                            if (o == 0) == (cols.start == c0):
                                m = paced(m)
                            d = (_tiles(a_s[o + r:o + r + 16, cols]) - m) * rstd[:, cols]
                            blocks.append(d.reshape(16, L))
                    for q, op in enumerate(_strassen_lhs(*blocks)):
                        _put(z2_s, (q,), c0 // L, slice(r, r + 16), op)
                    yield

        def gate():
            for r0 in range(0, FQ, MB):
                def complete(b, z):
                    for n, x in enumerate(z):
                        f = (b // 2) * FQ + r0 + 16 * n
                        _put(z1_s, (i,), 2 * (b % 2), slice(f, f + 16), _gelu2(x))

                yield from preact(r0, complete)

        return ((itertools.chain(activate(), gate()), 18 * FQ // TICK),
                _spread(layernorm(), FH // 32 + FQ // 8, 0.506, 0.979))

    def mixer_sums(i, n):
        left, right = span(i * C, CH), span(i * C + CH, CH)
        for r in range(0, L, 8):
            top, bot = span(n * CH + r, 8), span(n * CH + L + r, 8)
            w = [paced(wsp_v[top, left]), wsp_v[bot, left],
                 wsp_v[top, right], paced(wsp_v[bot, right])]
            ops = _strassen_rhs(*[_f32(x) for x in w])
            for slot, q in enumerate(SUMMED_RHS):
                _put(wb_s, (slot, n), 0, slice(2 * r, 2 * r + 16), ops[q])
            yield

    def mixer_operand(i, q, n):
        if q in SUMMED_RHS:
            return _get(wb_s, (SUMMED_RHS.index(q), n), 0, 2)
        o = 0 if q == 1 else 1
        return wsp_v[span(n * CH + o * L, L), span(i * C + o * CH, CH)]

    def mixer_partial(i):
        for products in ((1, 4), SUMMED_RHS):
            for n in range(0, NCH, 2):
                for q in products:
                    w = jnp.concatenate([mixer_operand(i, q, n + o) for o in range(2)], axis=0)
                    m = _dot_nt(_bf16(_get(z2_s, (q,), 0, 2)), _bf16(w))
                    for r in range(0, FQ, 8):
                        at = (q, slice(r, r + 8), slice(n * CH, (n + 2) * CH))
                        m_s[at] = jnp.where(i > 0, m_s[at], 0.0) + m[r:r + 8]
                    yield from ticks(m)

    def output_operands(i):
        wor_s[...] = jnp.concatenate([wo_v[FM:FQ, :], wo_v[FQ + FM:FH, :]], axis=0).T
        for a in range(2):
            f = pl.multiple_of(a * FQ + i * L, 16)
            wot_s[a] = wo_v[pl.ds(f, L), :].T
        for r in range(0, DH, 16):
            w = [_get(wot_s, (), b % 2, 1, pl.ds((r + (b // 2) * DH) // 2, 8)) for b in range(4)]
            w[0], w[3] = paced(w[0]), paced(w[3])
            for q, op in enumerate(_strassen_lhs(*[_f32(x) for x in w])):
                _put(woq_s, (q,), i, slice(r, r + 16), op)
            yield

    wait(f"wi{FH}")
    block("hidden0", *hidden_stage(0, first=True))

    wait("chunk0")

    def chunk_step(i, carry):
        block("partial", (mixer_partial(i), 14 * FQ // TICK),
              _spread(itertools.chain(*[mixer_sums(i, n) for n in range(NCH)]),
                      NCH * L // 8, 0.0, 0.269),
              _spread(residual_stage(i + 1), CH // 8, 0.352, 0.882))
        wait_step(i, lambda n: [f"chunk{n + 1}"], range(NCH - 1))
        block("hidden", *hidden_stage(i + 1), _spread(output_operands(i), DH // 16, 0.121, 0.39))
        return carry

    lax.fori_loop(0, NCH - 1, chunk_step, 0)

    def gated_product(n):
        for r0, r1 in GATE_ROWS:
            def product(q):
                m = yield from ticks(_dot_nt(_bf16(_get(z2_s, (q,), 0, 2, slice(r0 // 2, r1 // 2))),
                                             _bf16(mixer_operand(NCH - 1, q, n))))
                return m_s[q, r0:r1, span(n * CH, CH)] + m

            p = {}

            def complete(b, g):
                t = span(n * C + (b % 2) * CH, CH)
                p[b] = []
                for k, x in enumerate(g):
                    r = r0 + 16 * k
                    f = ((b // 2) * FQ + r) // 2
                    z1 = _f32(_get(z1_s, (n,), 2 * (b % 2), 2, slice(f, f + 8)))
                    p[b].append(z1 * (_tiles(x) + bsp_s[:, t]).reshape(16, CH))
                    if r >= FM:
                        f = (b // 2) * (FQ - FM) + r - FM
                        _put(pr_s, (), 2 * (b % 2), slice(f, f + 16), p[b][k])
                        continue
                    ops = _strassen_rhs(*[p[a][k] if a in p else x for a in range(4)])
                    for q, needs in enumerate(STRASSEN_RHS_NEEDS):
                        if b in needs and all(a in p for a in needs):
                            _put(pq_s, (q,), 0, slice(r, r + 16), ops[q])

            yield from _strassen_product(product, (1, 4, 2, 0, 5, 3, 6), [None] * 4, complete)

    def project():
        rest = yield from ticks(_dot(wor_s[...], _bf16(_get(pr_s, (), 0, C // L))))

        def complete(b, o):
            for k, x in enumerate(o):
                d = (b // 2) * DH + 16 * k
                o_s[b % 2, d:d + 16, :] = x

        def product(q):
            return ticks(_dot(_bf16(_get(woq_s, (q,), 0, FM // L)), _bf16(_get(pq_s, (q,), 0, 2))))

        yield from _strassen_product(
            product, (1, 3, 4, 0, 6, 2, 5),
            [_pieces(rest[(b // 2) * DH:(b // 2 + 1) * DH, (b % 2) * CH:(b % 2 + 1) * CH])
             for b in range(4)], complete)

    def out_copy(row, n, c0=0, c1=NCT):
        at = (span(row, n), slice(c0 * L, c1 * L))
        return pltpu.make_async_copy(out_v.at[at], out_hbm.at[at], out_sem.at[0])

    def finish(n, h, c0=0, c1=NCT):
        for c in reversed(range(c0, c1)):
            for t0 in range(0, CH, L):
                cols = slice(c * L, (c + 1) * L)
                o = o_s[h, cols, t0:t0 + L].T
                x1 = _f32(_get(x1_s, (n,), c, 1, pl.ds((h * CH + t0) // 2, L // 2)))
                res = _tiles(x1) + mod_s[4, :, cols] * _tiles(o)
                out_v[span(n * C + h * CH + t0, L), cols] = res.reshape(L, L).astype(BF16)
                yield

    gate_ticks = 7 * sum(-(-(b - a) // TICK) for a, b in GATE_ROWS)
    _interleave((gated_product(0), gate_ticks), (mixer_sums(NCH - 1, 0), 10 * L // 8 + 8))
    mod_s[4] = 0.5 * modulation(5)

    def output_step(n, carry):
        @pl.when(n > 0)
        def _():
            out_copy((n - 1) * C, C).start()

        latest[0] = None
        _interleave((project(), -(-D // TICK) + 7 * -(-DH // TICK)),
                    _spread(mixer_sums(NCH - 1, n + 1), L // 8, 0.032, 0.574))
        _interleave((gated_product(n + 1), gate_ticks),
                    _spread(itertools.chain(finish(n, 0), finish(n, 1)),
                            4 * NCT, 0.081, 0.835))
        return carry

    with _scope("output"):
        lax.fori_loop(0, NCH - 1, output_step, 0)
    out_copy((NCH - 2) * C, C).start()
    _interleave((project(), 1))
    latest[0] = None
    last_parts = ((0, 0, NCT), (1, 0, DH // L), (1, DH // L, NCT))
    for h, c0, c1 in last_parts:
        _interleave((finish(NCH - 1, h, c0, c1), 1))
        out_copy((NCH - 1) * C + h * CH, CH, c0, c1).start()
    for n in range(NCH - 1):
        out_copy(n * C, C).wait()
    for h, c0, c1 in last_parts:
        out_copy((NCH - 1) * C + h * CH, CH, c0, c1).wait()


@jax.jit
def pallas_adaLN_cond__ssm_conv_h3__mixer_gmlp__prompt_kernel(
    A_q: jax.Array,
    A_k: jax.Array,
    A_v: jax.Array,
    A_shift_k: jax.Array,
    A_ssm_k: jax.Array,
    A_ssm_D: jax.Array,
    B_x: jax.Array,
    B_w_in: jax.Array,
    B_w_sp: jax.Array,
    B_b_sp: jax.Array,
    B_w_out: jax.Array,
    c: jax.Array,
    w_mod: jax.Array,
):
    del B_x
    operands = (
        A_q.reshape(S, D), A_k.reshape(S, D), A_v.reshape(S, D), A_shift_k.T, A_ssm_k,
        A_ssm_D.reshape(NCT, L), B_w_in.T, B_w_sp, B_b_sp.reshape(S // L, L), B_w_out, c, w_mod,
    )
    def planes(*shape):
        return pltpu.VMEM((*shape, L), BF16)

    spectrum = pltpu.VMEM((4, 2 * L, L), F32)
    scratch = [
        pltpu.VMEM((S // 2, D), U32),
        pltpu.VMEM((NCT, 16 + S // 2, L), U32),
        pltpu.VMEM((NCT, 8 + S // 2, L), U32),
        pltpu.VMEM((KS, D), BF16),
        pltpu.VMEM((DH, S), U32),
        pltpu.VMEM((NCT, L), BF16),
        pltpu.VMEM((FH, D), U32),
        pltpu.VMEM((S // 2, S), U32),
        pltpu.VMEM((S // L, L), BF16),
        pltpu.VMEM((FH, D), BF16),
        pltpu.VMEM((1, D), BF16),
        pltpu.VMEM((DH, 6 * D), U32),
        planes(4, 2 * L),
        planes(4, 2, L),
        pltpu.VMEM((S, D), BF16),
        pltpu.VMEM((8, L), U32),
        pltpu.VMEM((NCT, KS + 1, 8, L), F32),
        pltpu.VMEM((8, S), F32),
        pltpu.VMEM((5, 8, D), F32),
        [pltpu.VMEM((CH + 8, L), U32)] * NCH,
        [planes(4, L)] * NCH,
        [planes(4, L)] * NCH,
        [spectrum] * 2,
        [pltpu.VMEM((2, 4, 2 * L, L), F32)] * NCH,
        [spectrum] * NCH,
        [planes(4, 2 * L)] * NCH,
        pltpu.VMEM((NCT, S + 8, L), F32),
        planes(NCH, NCT, C),
        pltpu.VMEM((C, D), F32),
        planes(7, DM // L, CH),
        planes(1, C),
        planes(5, DM // L, 2 * FH),
        pltpu.VMEM((FH, C), F32),
        planes(NCH, C // L, FH),
        planes(7, 2, FQ),
        planes(5, NCH, 2, CH),
        pltpu.VMEM((7, FQ, S // 2), F32),
        planes(2, D),
        pltpu.VMEM((D, FH - 2 * FM), BF16),
        planes(7, FM // L, DH),
        planes(7, 2, FM),
        planes(C // L, FH - 2 * FM),
        pltpu.VMEM((2, D, CH), F32),
        pltpu.SemaphoreType.DMA((15,)),
        pltpu.SemaphoreType.DMA((1,)),
    ]
    out = pl.pallas_call(
        _kernel,
        out_shape=jax.ShapeDtypeStruct((S, D), BF16),
        in_specs=[pl.BlockSpec(memory_space=pltpu.HBM)] * len(operands),
        out_specs=pl.BlockSpec(memory_space=pltpu.HBM),
        scratch_shapes=scratch,
        compiler_params=pltpu.CompilerParams(
            vmem_limit_bytes=120 * 1024 * 1024,
            flags={"XLA_TPU_EVENLY_DISTRIBUTE_CRITICAL_NODES": True}),
    )(*operands)
    return out.reshape(1, S, D)
```

```python
import itertools

import numpy as np

import jax
import jax.numpy as jnp
from jax import lax
import jax.experimental.pallas as pl
import jax.experimental.pallas.tpu as pltpu

S = 2048
D = 640
DH = D // 2
FH = 864
FQ = FH // 2
KS = 4
L = 128
NCT = D // L
C = 512
CH = C // 2
NCH = S // C
NPOS = 16
DM = 256
FM = 384
SUMMED_LHS = (0, 1, 4, 5, 6)
SUMMED_RHS = (0, 2, 3, 5, 6)
MB = 144
GATE_ROWS = ((0, 176), (176, 320), (320, FQ))
TICK = 24
DEPTH = 11
NEVER = 0x7F7F7F7F
CONV_STEP = ("K3 D3 B0 B1 D0 B2 D1 B3 D2 K0 K1 K2", "A0 A1 T3 T2 A3 C0 A2 C1 T0 C2 T1 C3", 71)
CONV_LAST = ("K3 D3 B0 B1 D0 B2 D1 B3 D2", "A0 A1 A2 C0 A3 C1 C2 C3", 71)
CONV_AHEAD = "T0 T1 T2 T3 K0 K1 K2".split()
CONV_LEAD = 4
EPS = 1e-5
GELU_C0 = float(np.sqrt(2.0 / np.pi))
GELU_C1 = GELU_C0 * 0.044715

F32 = jnp.float32
BF16 = jnp.bfloat16
U32 = jnp.uint32
NT_DIMS = (((1,), (1,)), ((), ()))


def _lo(w):
    return lax.bitcast_convert_type(w << 16, F32)


def _hi(w):
    return lax.bitcast_convert_type(w & np.uint32(0xFFFF0000), F32)


def _bf16(words):
    return pltpu.bitcast(words, BF16)


def _f32(words):
    return _bf16(words).astype(F32)


def _put(ref, lead, first, rows, x):
    for n in range(x.shape[1] // L):
        ref[(*lead, first + n, rows)] = x[:, n * L:(n + 1) * L].astype(BF16)


def _get(ref, lead, first, count, word_rows=slice(None)):
    return jnp.concatenate(
        [ref.bitcast(U32)[(*lead, first + n, word_rows)] for n in range(count)], axis=1)


def _dot(a, b):
    return jnp.dot(a, b, preferred_element_type=F32)


def _dot_nt(a, b):
    return lax.dot_general(a, b, NT_DIMS, preferred_element_type=F32)


def _tiles(x):
    return x.reshape(x.shape[0] // 8, 8, x.shape[1])


def _interleave(*streams):
    steps = sorted(((k + 0.5) / n, i) for i, (_, n) in enumerate(streams) for k in range(n))
    for _, i in steps:
        next(streams[i][0], None)
    for stream, _ in streams:
        for _ in stream:
            pass


def _spread(stream, n, start, end):
    per_unit = n / (end - start)
    return itertools.chain(range(round(start * per_unit)), stream), round(per_unit)


def _conv_schedule(matmuls, vector, per_step):
    steps = dict(T=8, A=16, C=4 * NPOS)
    cost = dict(T=(24,) * 4, A=(46,) * 4, C=(12, 20, 28, 36), K=(17, 25, 25, 25),
                B=(16,) * 4, D=(6,) * 4)
    vector = [(x, k) for x in vector.split() for k in range(steps[x[0]])]
    matmul = [(x, k) for x in matmuls.split() for k in range(NPOS)]
    order, done, budget = [], set(), 0
    for n, (x, k) in enumerate(matmul):
        for ahead, _ in matmul[n:n + CONV_LEAD + 1]:
            need = dict(K="T", B="A", D="C")[ahead[0]] + ahead[1]
            while ahead not in ("K3", "D3") and any(v == need for v, _ in vector):
                order.append(vector.pop(0)[0])
                budget -= cost[order[-1][0]][int(order[-1][1])]
        order.append(x)
        done.add((x, k))
        budget = min(budget + per_step - cost[x[0]][int(x[1])], per_step)
        while vector and budget > 0:
            v, j = vector[0]
            if v[0] == "C" and ("B" + v[1], j // 4) not in done:
                break
            order.append(vector.pop(0)[0])
            budget -= cost[v[0]][int(v[1])]
    return order + [v for v, _ in vector]


def _radix4(e, inverse):
    (r0, i0), (r1, i1), (r2, i2), (r3, i3) = e
    sr, si, dr, di = r0 + r2, i0 + i2, r0 - r2, i0 - i2
    tr, ti, ur, ui = r1 + r3, i1 + i3, r1 - r3, i1 - i3
    a = (dr + ui, di - ur)
    b = (dr - ui, di + ur)
    if inverse:
        a, b = b, a
    return [(sr + tr, si + ti), a, (sr - tr, si - ti), b]


def _strassen_lhs(a11, a12, a21, a22):
    return [a11 + a22, a21 + a22, a11, a22, a11 + a12, a21 - a11, a12 - a22]


STRASSEN_RHS_NEEDS = ((0, 3), (0,), (1, 3), (0, 2), (3,), (0, 1), (2, 3))


def _strassen_rhs(b11, b12, b21, b22):
    return [b11 + b22, b11, b12 - b22, b21 - b11, b22, b11 + b12, b21 + b22]


STRASSEN_USES = ({0: 1, 3: 1}, {2: 1, 3: -1}, {1: 1, 3: 1}, {0: 1, 2: 1}, {0: -1, 1: 1},
                 {3: 1}, {0: 1})


def _pieces(x):
    return [x[r:r + 16] for r in range(0, x.shape[0], 16)]


def _strassen_product(product, order, blocks, complete):
    blocks = list(blocks)
    for n, q in enumerate(order):
        m = _pieces((yield from product(q)))
        for b, sign in STRASSEN_USES[q].items():
            if blocks[b] is None:
                blocks[b] = m if sign > 0 else [-x for x in m]
            else:
                blocks[b] = [x + y if sign > 0 else x - y for x, y in zip(blocks[b], m)]
            if not any(b in STRASSEN_USES[later] for later in order[n + 1:]):
                complete(b, blocks[b])


def _gelu2(x):
    t = jnp.tanh(x * (x * x * GELU_C1 + GELU_C0))
    return x * t + x


def _layernorm_rows(x):
    d = x - jnp.sum(x, axis=-1, keepdims=True) * (1.0 / D)
    var = jnp.sum(d * d, axis=-1, keepdims=True) * (1.0 / D)
    return d * lax.rsqrt(var + EPS)


def _kernel(q_hbm, k_hbm, v_hbm, shift_hbm, ssm_hbm, ssmd_hbm, wi_hbm, wsp_hbm, bsp_hbm,
            wo_hbm, c_hbm, wmod_hbm, out_hbm,
            q_v, k_v, v_v, shift_v, ssm_v, ssmd_v, wi_v, wsp_v, bsp_v, wo_v, c_v, wmod_v,
            fwd_v, inv_v, out_v,
            mark_s, chan_s, bsp_s, mod_s, fstage, ktile, utile, kraw, khat, uhat, g_s, y_s,
            x1_s, xn_s, hq_s, hr_s, wq_s, a_s, z1_s, z2_s, wb_s, m_s, wot_s, wor_s, woq_s,
            pq_s, pr_s, o_s, sems, out_sem):
    copies = {}

    def queue(name, src, dst):
        group = copies.setdefault(name, [])
        group.append(pltpu.make_async_copy(src, dst, sems.at[list(copies).index(name)]))
        group[-1].start()

    def wait(*names):
        for name in names:
            for copy in copies[name]:
                copy.wait()

    def rows(ref, r0, n):
        return ref.at[pl.ds(r0, n), :]

    def queue_pairs(name, src, dst, r0, n):
        queue(name, rows(src, r0, n), rows(dst, r0 // 2, n // 2).bitcast(BF16))

    def queue_wmod(name, i0, i1):
        queue(name, wmod_hbm.at[:, i0 * D:i1 * D], wmod_v.at[:, i0 * D:i1 * D].bitcast(BF16))

    queue_pairs("small", ssm_hbm, ssm_v, 0, L)
    for src, dst in ((ssmd_hbm, ssmd_v), (shift_hbm, shift_v), (c_hbm, c_v), (bsp_hbm, bsp_v)):
        queue("small", src, dst)
    for c in range(NCT):
        for n in range(NCH):
            for src, dst, pad, j in ((k_hbm, k_v, 8, n), (v_hbm, v_v, 0, (n + 2) % NCH)):
                queue(f"tile{c}", src.at[pl.ds(j * C, C), pl.ds(c * L, L)],
                      dst.at[c, pl.ds(pad + j * CH, CH), :].bitcast(BF16))
        if c + 1 < NCT:
            queue_pairs(f"tile{c}", ssm_hbm, ssm_v, (c + 1) * L, L)
    queue_pairs(f"tile{NCT - 1}", q_hbm, q_v, 0, C)
    queue_wmod("first", 0, 3)
    queue_wmod("second", 3, 5)
    wi_groups = {FH: MB, FH + MB: FQ - MB, 0: FQ}
    for r0, n in wi_groups.items():
        for o in (0, FQ):
            queue_pairs(f"wi{r0}", wi_hbm, wi_v, r0 + o, n)
    for i in range(NCH):
        cols = pl.ds(i * C, C)
        queue(f"chunk{i}", wsp_hbm.at[:, cols], wsp_v.at[:, cols].bitcast(BF16))
        if i + 1 < NCH:
            queue_pairs(f"chunk{i}", q_hbm, q_v, (i + 1) * C, C)
        if i == 1:
            queue("chunk1", wo_hbm, wo_v)
    queue_wmod(f"chunk{NCH - 1}", 5, 6)

    def wait_step(i, names_of, steps):
        for n in steps:
            @pl.when(i == n)
            def _():
                wait(*names_of(n))

    def span(start, size):
        return pl.ds(start if isinstance(start, int) else pl.multiple_of(start, size), size)

    latest = [None]

    def paced(x):
        if latest[0] is None:
            return x
        if x.shape[0] > 8:
            return jnp.concatenate([paced(x[:8]), x[8:]], axis=0)
        n = x.shape[1] // L
        never = jnp.tile(mark_s[...], (1, n)) == NEVER
        return jnp.where(never, lax.bitcast_convert_type(jnp.tile(latest[0], (1, n)), x.dtype), x)

    def ticks(m):
        for r in range(0, m.shape[0], TICK):
            latest[0] = m[r:r + 8, 0:L]
            yield
        return m

    def load_group(ref, k2, g):
        return ref[k2 + zero, 16 * g:16 * g + 8, :], ref[k2 + zero, 16 * g + 8:16 * g + 16, :]

    def store_group(ref, k2, g, val):
        ref[k2, 16 * g:16 * g + 8, :] = val[0]
        ref[k2, 16 * g + 8:16 * g + 16, :] = val[1]

    def spectrum_groups(tiles, adjust=lambda g, pair: pair):
        e = [_dot(_bf16(_get(fwd_v, (), p, 1)), _bf16(_get(tiles, (), p + zero, 1)))
             for p in range(4)]
        for g in range(NPOS):
            latest[0] = e[0][16 * g:16 * g + 8]
            pairs = [(x[16 * g:16 * g + 8], x[16 * g + 8:16 * g + 16]) for x in e]
            yield _radix4([adjust(g, pairs[0])] + pairs[1:], False)

    def dft_matrices():
        sub = lax.broadcasted_iota(jnp.int32, (8, L), 0)
        lane = lax.broadcasted_iota(jnp.int32, (8, L), 1)

        def unit(turns):
            angle = (((turns + 2 * C) & (4 * C - 1)) - 2 * C).astype(F32) * (np.pi / (2 * C))
            return jnp.cos(angle), -jnp.sin(angle)

        def times(a, b):
            return a[0] * b[0] - a[1] * b[1], a[0] * b[1] + a[1] * b[0]

        for p in range(4):
            for inverse in (False, True):
                n1 = lane if inverse else 8 * (lane >> 4) + (lane & 7) + 8 * (lane & 8)
                n = 4 * n1 + p
                even, one, sixteen = unit((4 * sub + 1) * n), unit(2 * n), unit(32 * n)
                for parity in range(2):
                    w, parts = times(even, one) if parity else even, []
                    for _ in range(NPOS // 2):
                        parts += w
                        w = times(w, sixteen)
                    half = jnp.concatenate(parts, axis=0)
                    if inverse:
                        _put(inv_v, (p,), parity, slice(None), (half * (1.0 / C)).T)
                    else:
                        _put(fwd_v, (), p, slice(parity * L, (parity + 1) * L), half)

    def filter_tiles(c, m):
        fstage[m][0:CH, :] = pltpu.bitcast(
            _bf16(ssm_v[span(c * (L // 2), L // 2), m * C:(m + 1) * C]).T, U32)
        for u in range(L // 16):
            for s in range(2):
                a = paced(fstage[m][pl.ds(16 * u + s, 8, stride=2), :])
                b = fstage[m][pl.ds(L + 16 * u + s, 8, stride=2), :]
                for o, half in enumerate((_lo, _hi)):
                    _put(ktile[m], (), 2 * s + o, slice(16 * u, 16 * u + 16),
                         jnp.concatenate([half(a), half(b)], axis=0))
            yield

    def signal_tiles(c, j):
        w1, w2, w3 = [chan_s[c, t] for t in range(1, KS)]
        for u in range(L // 16):
            halves = []
            for h in range(2):
                w0 = paced(chan_s[c, 0])
                r0 = j * CH + h * L + 16 * u
                kw = [k_v[c, pl.ds(8 + r0 + o, 8, stride=2), :] for o in range(-2, 2)]
                vw = [v_v[c, pl.ds(r0 + o, 8, stride=2), :] for o in range(2)]
                ks = [_hi(kw[0])] + [f(x) for x in kw[1:] for f in (_lo, _hi)]
                vs = [f(x) for x in vw for f in (_lo, _hi)]
                halves.append([((w0 * ks[p + 3] + w1 * ks[p + 2]) + (w2 * ks[p + 1] + w3 * ks[p]))
                               * vs[p] for p in range(4)])
                if h == 1:
                    for p in range(4):
                        _put(utile[j], (), p, slice(16 * u, 16 * u + 16),
                             jnp.concatenate([halves[0][p], halves[1][p]], axis=0))
                yield

    def filter_spectrum(c, m):
        def skip(g, pair):
            re, im = pair
            d = chan_s[c, KS]
            if m % 2 == 0:
                return (re - d if m else re + d), im
            return re, (im - d if (m == 1) == (g < NPOS // 2) else im + d)

        before = None if m == 0 else khat[0].at[c % 2] if m == 1 else kraw[m % 2]
        for g, kk in enumerate(spectrum_groups(ktile[m], skip)):
            for k2 in range(4):
                re, im = kk[k2]
                if 0 < m < NCH - 1:
                    store_group(kraw[(m + 1) % 2], k2, g, kk[k2])
                if m > 0:
                    pre, pim = load_group(before, k2, g)
                    re, im = (re - pim, im + pre) if g < NPOS // 2 else (re + pim, im - pre)
                store_group(khat[m].at[c % 2], k2, g, (re, im))
            yield

    def signal_spectrum(c, j):
        for g, uu in enumerate(spectrum_groups(utile[j])):
            for k2 in range(4):
                store_group(uhat[j], k2, g, uu[k2])
            yield

    def chunk_product(c, i):
        for g in range(NPOS):
            ys = []
            for k2 in range(4):
                yr = yi = None
                for j in range(i + 1):
                    kr, ki = load_group(khat[i - j].at[c % 2], k2, g)
                    ur, ui = load_group(uhat[j], k2, g)
                    if j == 0 and k2 == 0:
                        kr = paced(kr)
                    pr, pi = kr * ur - ki * ui, kr * ui + ki * ur
                    yr, yi = (pr, pi) if yr is None else (yr + pr, yi + pi)
                ys.append((yr, yi))
                if k2 == 3:
                    for p, pair in enumerate(_radix4(ys, True)):
                        _put(g_s[i], (), p, slice(16 * g, 16 * g + 16), jnp.concatenate(pair, axis=0))
                yield

    def inverse_dft(c, i):
        y = None
        for n in range(2):
            part = [_dot(_bf16(_get(inv_v, (p,), n, 1)),
                         _bf16(_get(g_s[i], (), p + zero, 1, slice(n * L // 2, (n + 1) * L // 2))))
                    for p in range(4)]
            for r in range(0, L, 16):
                latest[0] = part[0][r:r + 8]
                if y is not None:
                    for o in (r, r + 8):
                        for p in range(4):
                            y_s[c, pl.ds(i * C + 4 * o + p, 8, stride=4), :] = (
                                y[p][o:o + 8] + part[p][o:o + 8])
                yield
            y = part

    dft_matrices()
    mark_s[...] = _get(fwd_v, (), 0, 1, slice(0, 8))
    g_s[NCH - 1][...] = jnp.zeros(g_s[NCH - 1].shape, BF16)
    k_v[:, 0:8, :] = jnp.zeros((NCT, 8, L), U32)
    wait("small")
    probe = lax.bitcast_convert_type(mark_s[...], jnp.int32)[0, 0]
    zero = (probe == NEVER).astype(jnp.int32)
    n_blocks = itertools.count()

    def block(*streams):
        latest[0] = None

        @pl.when(probe != NEVER + next(n_blocks))
        def _():
            _interleave(*streams)

        latest[0] = None

    bvec = bsp_v[...].astype(F32)
    for i in range(S // L):
        bsp_s[:, i * L:(i + 1) * L] = jnp.broadcast_to(bvec[i:i + 1], (8, L))
    dvec = ssmd_v[...].astype(F32)
    taps = shift_v[...].astype(F32)
    for i in range(NCT):
        chan_s[i, KS] = jnp.broadcast_to(dvec[i:i + 1], (8, L))
        for t in range(KS):
            chan_s[i, t] = jnp.broadcast_to(taps[t:t + 1, i * L:(i + 1) * L], (8, L))

    stages = dict(T=filter_tiles, A=signal_tiles, K=filter_spectrum, B=signal_spectrum,
                  C=chunk_product, D=inverse_dft)

    def conv_stages(c, plan):
        def stage(x):
            tile = c + 1 if x in CONV_AHEAD else jnp.maximum(c - 1, 0) if x == "D3" else c
            return stages[x[0]](tile, int(x[1]))

        streams = {x: stage(x) for x in plan[0].split() + plan[1].split()}
        latest[0] = None
        for x in _conv_schedule(*plan):
            next(streams[x])
        latest[0] = None
        yield

    def conv_step(c, carry):
        wait_step(c, lambda n: [f"tile{n}"], range(NCT - 1))
        _interleave((conv_stages(c, CONV_STEP), 1))
        return carry

    block((itertools.chain(*[stages[x[0]](0, int(x[1])) for x in CONV_AHEAD]), 1))
    lax.fori_loop(0, NCT - 1, conv_step, 0)

    def gated_residual(i, r, x, y0, normed=None):
        y = jnp.concatenate([y0] + [y_s[c, span(i * C + r, 16), :] for c in range(1, NCT)], axis=1)
        x1 = []
        for rows8 in (slice(0, 8), slice(8, 16)):
            xn = _layernorm_rows(x[rows8]) if normed is None else normed[rows8]
            x1.append(x[rows8] + (xn * mod_s[0] + mod_s[1]) * y[rows8])
        _put(x1_s, (i,), 0, slice(r, r + 16), jnp.concatenate(x1, axis=0))
        return [_layernorm_rows(x) for x in x1]

    def store_modulated(r, h):
        ops = [_strassen_rhs(h[0][s][:, :DM], h[1][s][:, :DM],
                             h[0][s][:, DM:2 * DM], h[1][s][:, DM:2 * DM]) for s in range(2)]
        for q in range(7):
            _put(hq_s, (q,), 0, slice(r, r + 16), jnp.concatenate([ops[0][q], ops[1][q]], axis=0))
        for a in range(2):
            _put(hr_s, (), 0, slice(a * CH + r, a * CH + r + 16),
                 jnp.concatenate(h[a], axis=0)[:, 2 * DM:])

    def paced_rows(words):
        words = jnp.concatenate([paced(words[:, :L]), words[:, L:]], axis=1)
        return _f32(words)

    def residual_stage(i):
        for r in range(0, CH, 16):
            normed = []
            for a in range(2):
                row = a * CH + r
                x = paced_rows(q_v[span(i * CH + row // 2, 8), :])
                normed.append([xn * mod_s[2] + mod_s[3] for xn in gated_residual(
                    i, row, x, y_s[0, span(i * C + row, 16), :])])
                if a == 1:
                    store_modulated(r, normed)
                yield

    cv = c_v[...].astype(F32)
    act = jnp.broadcast_to(cv * jax.nn.sigmoid(cv), (16, D)).astype(BF16)

    def modulation(i):
        return _dot(act, _bf16(wmod_v[:, i * D:(i + 1) * D]))[:8]

    def first_gate():
        sa, ca, ga = [modulation(i) for i in range(3)]
        mod_s[0] = (1.0 + ca) * ga
        mod_s[1] = sa * ga
        latest[0] = ga[:, :L]
        yield

    def first_norm():
        for r in range(0, C, 16):
            xn_s[r:r + 16, :] = _layernorm_rows(paced_rows(q_v[r // 2:r // 2 + 8, :]))
            yield

    def first_residual():
        done = []
        for r in range(0, C, 16):
            latest[0] = done[-DEPTH] if len(done) >= DEPTH else None
            xn = gated_residual(0, r, _f32(q_v[r // 2:r // 2 + 8, :]), paced(y_s[0, r:r + 16, :]),
                                xn_s[r:r + 16, :])
            xn_s[r:r + 16, :] = jnp.concatenate(xn, axis=0)
            done.append(xn[1][:, :L])
            yield

    def first_modulate():
        wait("second")
        shift, scale = modulation(3), 1.0 + modulation(4)
        mod_s[2] = scale
        mod_s[3] = shift
        for r in range(0, CH, 16):
            store_modulated(r, [[xn_s[pl.ds(a * CH + r + 8 * s, 8), :] * scale + shift
                                 for s in range(2)] for a in range(2)])
        yield

    wait(f"tile{NCT - 1}")
    block((conv_stages(NCT - 1, CONV_LAST), 1))
    wait("first")
    block((itertools.chain(inverse_dft(NCT - 1, 3), first_gate()), 2 * NPOS),
          _spread(first_norm(), CH // 8, 0.0, 0.788))
    block((first_residual(), 1))
    block((first_modulate(), 1))

    def hidden_stage(i, first=False):
        def weight_sums(r0):
            for r in range(r0 // 2, (r0 + MB) // 2, 8):
                top, bot = slice(r, r + 8), slice(r + FQ // 2, r + FQ // 2 + 8)
                w = [paced(wi_v[top, :DM]), wi_v[top, DM:2 * DM],
                     wi_v[bot, :DM], paced(wi_v[bot, DM:2 * DM])]
                ops = _strassen_lhs(*[_f32(x) for x in w])
                for slot, q in enumerate(SUMMED_LHS):
                    _put(wq_s, (slot,), 0, slice(2 * r, 2 * r + 16), ops[q])
                yield

        def preact(r0, complete):
            top = slice(r0 // 2, (r0 + MB) // 2)
            bot = slice((r0 + FQ) // 2, (r0 + FQ + MB) // 2)
            following = 0 if r0 + MB == FH + FQ else r0 + MB
            sums = weight_sums(r0) if first else iter(())

            def product(q):
                if first and q == 6 and following in wi_groups:
                    wait(f"wi{following}")
                w = (wi_v[top, :DM] if q == 2 else wi_v[bot, DM:2 * DM] if q == 3
                     else _get(wq_s, (SUMMED_LHS.index(q),), 0, DM // L, top))
                m = _dot_nt(_bf16(w), _bf16(_get(hq_s, (q,), 0, DM // L)))
                for _ in ticks(m):
                    next(sums, None)
                    yield
                return m

            rest = []
            for part in (top, bot):
                rest.append(_dot_nt(_bf16(wi_v[part, 2 * DM:]), _bf16(_get(hr_s, (), 0, 1))))
                for _ in ticks(rest[-1]):
                    next(sums, None)
                    yield
            yield from _strassen_product(
                product, (2, 3, 4, 1, 0, 6, 5),
                [_pieces(rest[b // 2][:, (b % 2) * CH:(b % 2 + 1) * CH]) for b in range(4)],
                complete)

        def column_mean(acc):
            return jnp.broadcast_to(jnp.sum(acc, axis=0, keepdims=True) * (1.0 / FH), (8, C))

        total = [jnp.zeros((8, CH), F32)] * 2

        def activate():
            for r0 in range(0, FQ, MB):
                def complete(b, z):
                    for n, x in enumerate(z):
                        a = _gelu2(x)
                        f = (b // 2) * FQ + r0 + 16 * n
                        a_s[f:f + 16, (b % 2) * CH:(b % 2 + 1) * CH] = a
                        total[b % 2] = total[b % 2] + (a[:8] + a[8:])

                yield from preact(FH + r0, complete)

        def layernorm():
            mean = column_mean(jnp.concatenate(total, axis=1))
            acc = jnp.zeros((8, C), F32)
            for r in range(0, FH, 32):
                d = _tiles(a_s[r:r + 32, :]) - paced(mean)
                acc = acc + (d * d).sum(axis=0)
                yield
            rstd = lax.rsqrt(column_mean(acc) + 4.0 * EPS)
            means = [mean[:, c0:c0 + L] for c0 in range(0, C, L)]
            for r in range(0, FQ, 16):
                for c0 in range(0, CH, L):
                    blocks = []
                    for o in (0, FQ):
                        for cols in (slice(c0, c0 + L), slice(CH + c0, CH + c0 + L)):
                            m = means[cols.start // L]
                            if (o == 0) == (cols.start == c0):
                                m = paced(m)
                            d = (_tiles(a_s[o + r:o + r + 16, cols]) - m) * rstd[:, cols]
                            blocks.append(d.reshape(16, L))
                    for q, op in enumerate(_strassen_lhs(*blocks)):
                        _put(z2_s, (q,), c0 // L, slice(r, r + 16), op)
                    yield

        def gate():
            for r0 in range(0, FQ, MB):
                def complete(b, z):
                    for n, x in enumerate(z):
                        f = (b // 2) * FQ + r0 + 16 * n
                        _put(z1_s, (i,), 2 * (b % 2), slice(f, f + 16), _gelu2(x))

                yield from preact(r0, complete)

        return ((itertools.chain(activate(), gate()), 18 * FQ // TICK),
                _spread(layernorm(), FH // 32 + FQ // 8, 0.506, 0.979))

    def mixer_sums(i, n):
        left, right = span(i * C, CH), span(i * C + CH, CH)
        for r in range(0, L, 8):
            top, bot = span(n * CH + r, 8), span(n * CH + L + r, 8)
            w = [paced(wsp_v[top, left]), wsp_v[bot, left],
                 wsp_v[top, right], paced(wsp_v[bot, right])]
            ops = _strassen_rhs(*[_f32(x) for x in w])
            for slot, q in enumerate(SUMMED_RHS):
                _put(wb_s, (slot, n), 0, slice(2 * r, 2 * r + 16), ops[q])
            yield

    def mixer_operand(i, q, n):
        if q in SUMMED_RHS:
            return _get(wb_s, (SUMMED_RHS.index(q), n), 0, 2)
        o = 0 if q == 1 else 1
        return wsp_v[span(n * CH + o * L, L), span(i * C + o * CH, CH)]

    def mixer_partial(i):
        for products in ((1, 4), SUMMED_RHS):
            for n in range(0, NCH, 2):
                for q in products:
                    w = jnp.concatenate([mixer_operand(i, q, n + o) for o in range(2)], axis=0)
                    m = _dot_nt(_bf16(_get(z2_s, (q,), 0, 2)), _bf16(w))
                    for r in range(0, FQ, 8):
                        at = (q, slice(r, r + 8), slice(n * CH, (n + 2) * CH))
                        m_s[at] = jnp.where(i > 0, m_s[at], 0.0) + m[r:r + 8]
                    yield from ticks(m)

    def output_operands(i):
        wor_s[...] = jnp.concatenate([wo_v[FM:FQ, :], wo_v[FQ + FM:FH, :]], axis=0).T
        for a in range(2):
            f = pl.multiple_of(a * FQ + i * L, 16)
            wot_s[a] = wo_v[pl.ds(f, L), :].T
        for r in range(0, DH, 16):
            w = [_get(wot_s, (), b % 2, 1, pl.ds((r + (b // 2) * DH) // 2, 8)) for b in range(4)]
            w[0], w[3] = paced(w[0]), paced(w[3])
            for q, op in enumerate(_strassen_lhs(*[_f32(x) for x in w])):
                _put(woq_s, (q,), i, slice(r, r + 16), op)
            yield

    wait(f"wi{FH}")
    block(*hidden_stage(0, first=True))

    wait("chunk0")

    def chunk_step(i, carry):
        block((mixer_partial(i), 14 * FQ // TICK),
              _spread(itertools.chain(*[mixer_sums(i, n) for n in range(NCH)]),
                      NCH * L // 8, 0.0, 0.269),
              _spread(residual_stage(i + 1), CH // 8, 0.352, 0.882))
        wait_step(i, lambda n: [f"chunk{n + 1}"], range(NCH - 1))
        block(*hidden_stage(i + 1), _spread(output_operands(i), DH // 16, 0.121, 0.39))
        return carry

    lax.fori_loop(0, NCH - 1, chunk_step, 0)

    def gated_product(n):
        for r0, r1 in GATE_ROWS:
            def product(q):
                m = yield from ticks(_dot_nt(_bf16(_get(z2_s, (q,), 0, 2, slice(r0 // 2, r1 // 2))),
                                             _bf16(mixer_operand(NCH - 1, q, n))))
                return m_s[q, r0:r1, span(n * CH, CH)] + m

            p = {}

            def complete(b, g):
                t = span(n * C + (b % 2) * CH, CH)
                p[b] = []
                for k, x in enumerate(g):
                    r = r0 + 16 * k
                    f = ((b // 2) * FQ + r) // 2
                    z1 = _f32(_get(z1_s, (n,), 2 * (b % 2), 2, slice(f, f + 8)))
                    p[b].append(z1 * (_tiles(x) + bsp_s[:, t]).reshape(16, CH))
                    if r >= FM:
                        f = (b // 2) * (FQ - FM) + r - FM
                        _put(pr_s, (), 2 * (b % 2), slice(f, f + 16), p[b][k])
                        continue
                    ops = _strassen_rhs(*[p[a][k] if a in p else x for a in range(4)])
                    for q, needs in enumerate(STRASSEN_RHS_NEEDS):
                        if b in needs and all(a in p for a in needs):
                            _put(pq_s, (q,), 0, slice(r, r + 16), ops[q])

            yield from _strassen_product(product, (1, 4, 2, 0, 5, 3, 6), [None] * 4, complete)

    def project():
        rest = yield from ticks(_dot(wor_s[...], _bf16(_get(pr_s, (), 0, C // L))))

        def complete(b, o):
            for k, x in enumerate(o):
                d = (b // 2) * DH + 16 * k
                o_s[b % 2, d:d + 16, :] = x

        def product(q):
            return ticks(_dot(_bf16(_get(woq_s, (q,), 0, FM // L)), _bf16(_get(pq_s, (q,), 0, 2))))

        yield from _strassen_product(
            product, (1, 3, 4, 0, 6, 2, 5),
            [_pieces(rest[(b // 2) * DH:(b // 2 + 1) * DH, (b % 2) * CH:(b % 2 + 1) * CH])
             for b in range(4)], complete)

    def out_copy(row, n, c0=0, c1=NCT):
        at = (span(row, n), slice(c0 * L, c1 * L))
        return pltpu.make_async_copy(out_v.at[at], out_hbm.at[at], out_sem.at[0])

    def finish(n, h, c0=0, c1=NCT):
        for c in reversed(range(c0, c1)):
            for t0 in range(0, CH, L):
                cols = slice(c * L, (c + 1) * L)
                o = o_s[h, cols, t0:t0 + L].T
                x1 = _f32(_get(x1_s, (n,), c, 1, pl.ds((h * CH + t0) // 2, L // 2)))
                res = _tiles(x1) + mod_s[4, :, cols] * _tiles(o)
                out_v[span(n * C + h * CH + t0, L), cols] = res.reshape(L, L).astype(BF16)
                yield

    gate_ticks = 7 * sum(-(-(b - a) // TICK) for a, b in GATE_ROWS)
    _interleave((gated_product(0), gate_ticks), (mixer_sums(NCH - 1, 0), 10 * L // 8 + 8))
    mod_s[4] = 0.5 * modulation(5)

    def output_step(n, carry):
        @pl.when(n > 0)
        def _():
            out_copy((n - 1) * C, C).start()

        latest[0] = None
        _interleave((project(), -(-D // TICK) + 7 * -(-DH // TICK)),
                    _spread(mixer_sums(NCH - 1, n + 1), L // 8, 0.032, 0.574))
        _interleave((gated_product(n + 1), gate_ticks),
                    _spread(itertools.chain(finish(n, 0), finish(n, 1)),
                            4 * NCT, 0.081, 0.835))
        return carry

    lax.fori_loop(0, NCH - 1, output_step, 0)
    out_copy((NCH - 2) * C, C).start()
    _interleave((project(), 1))
    latest[0] = None
    last_parts = ((0, 0, NCT), (1, 0, DH // L), (1, DH // L, NCT))
    for h, c0, c1 in last_parts:
        _interleave((finish(NCH - 1, h, c0, c1), 1))
        out_copy((NCH - 1) * C + h * CH, CH, c0, c1).start()
    for n in range(NCH - 1):
        out_copy(n * C, C).wait()
    for h, c0, c1 in last_parts:
        out_copy((NCH - 1) * C + h * CH, CH, c0, c1).wait()


@jax.jit
def pallas_adaLN_cond__ssm_conv_h3__mixer_gmlp__prompt_kernel(
    A_q: jax.Array,
    A_k: jax.Array,
    A_v: jax.Array,
    A_shift_k: jax.Array,
    A_ssm_k: jax.Array,
    A_ssm_D: jax.Array,
    B_x: jax.Array,
    B_w_in: jax.Array,
    B_w_sp: jax.Array,
    B_b_sp: jax.Array,
    B_w_out: jax.Array,
    c: jax.Array,
    w_mod: jax.Array,
):
    del B_x
    operands = (
        A_q.reshape(S, D), A_k.reshape(S, D), A_v.reshape(S, D), A_shift_k.T, A_ssm_k,
        A_ssm_D.reshape(NCT, L), B_w_in.T, B_w_sp, B_b_sp.reshape(S // L, L), B_w_out, c, w_mod,
    )
    def planes(*shape):
        return pltpu.VMEM((*shape, L), BF16)

    spectrum = pltpu.VMEM((4, 2 * L, L), F32)
    scratch = [
        pltpu.VMEM((S // 2, D), U32),
        pltpu.VMEM((NCT, 16 + S // 2, L), U32),
        pltpu.VMEM((NCT, 8 + S // 2, L), U32),
        pltpu.VMEM((KS, D), BF16),
        pltpu.VMEM((DH, S), U32),
        pltpu.VMEM((NCT, L), BF16),
        pltpu.VMEM((FH, D), U32),
        pltpu.VMEM((S // 2, S), U32),
        pltpu.VMEM((S // L, L), BF16),
        pltpu.VMEM((FH, D), BF16),
        pltpu.VMEM((1, D), BF16),
        pltpu.VMEM((DH, 6 * D), U32),
        planes(4, 2 * L),
        planes(4, 2, L),
        pltpu.VMEM((S, D), BF16),
        pltpu.VMEM((8, L), U32),
        pltpu.VMEM((NCT, KS + 1, 8, L), F32),
        pltpu.VMEM((8, S), F32),
        pltpu.VMEM((5, 8, D), F32),
        [pltpu.VMEM((CH + 8, L), U32)] * NCH,
        [planes(4, L)] * NCH,
        [planes(4, L)] * NCH,
        [spectrum] * 2,
        [pltpu.VMEM((2, 4, 2 * L, L), F32)] * NCH,
        [spectrum] * NCH,
        [planes(4, 2 * L)] * NCH,
        pltpu.VMEM((NCT, S + 8, L), F32),
        planes(NCH, NCT, C),
        pltpu.VMEM((C, D), F32),
        planes(7, DM // L, CH),
        planes(1, C),
        planes(5, DM // L, 2 * FH),
        pltpu.VMEM((FH, C), F32),
        planes(NCH, C // L, FH),
        planes(7, 2, FQ),
        planes(5, NCH, 2, CH),
        pltpu.VMEM((7, FQ, S // 2), F32),
        planes(2, D),
        pltpu.VMEM((D, FH - 2 * FM), BF16),
        planes(7, FM // L, DH),
        planes(7, 2, FM),
        planes(C // L, FH - 2 * FM),
        pltpu.VMEM((2, D, CH), F32),
        pltpu.SemaphoreType.DMA((15,)),
        pltpu.SemaphoreType.DMA((1,)),
    ]
    out = pl.pallas_call(
        _kernel,
        out_shape=jax.ShapeDtypeStruct((S, D), BF16),
        in_specs=[pl.BlockSpec(memory_space=pltpu.HBM)] * len(operands),
        out_specs=pl.BlockSpec(memory_space=pltpu.HBM),
        scratch_shapes=scratch,
        compiler_params=pltpu.CompilerParams(
            vmem_limit_bytes=120 * 1024 * 1024,
            flags={"XLA_TPU_EVENLY_DISTRIBUTE_CRITICAL_NODES": True}),
    )(*operands)
    return out.reshape(1, S, D)
```
